```python
import jax
import jax.numpy as jnp

def _softmax(x, axis=-1):
    return jax.nn.softmax(x, axis=axis)

def _gelu(x):
    return jax.nn.gelu(x, approximate=True)

def _silu(x):
    return jax.nn.silu(x)

def _sigmoid(x):
    return jax.nn.sigmoid(x)

def _layernorm(x, axis=-1, eps=1e-05):
    m = jnp.mean(x, axis=axis, keepdims=True)
    v = jnp.var(x, axis=axis, keepdims=True)
    return (x - m) / jnp.sqrt(v + eps)

def _scatter_add(tgt, idx, src, axis=0):
    return tgt.at[idx].add(src)

def _segment_sum(src, seg, n):
    return jax.ops.segment_sum(src, seg, n)

class _Rng:

    def __init__(self, key):
        self._k = key

    def _next(self):
        self._k, sub = jax.random.split(self._k)
        return sub

    def normal(self, shape):
        return jax.random.normal(self._next(), shape, dtype=jnp.bfloat16)

    def randint(self, lo, hi, shape):
        return jax.random.randint(self._next(), shape, lo, hi, dtype=jnp.int32)

    def uniform(self, shape, lo=0.0, hi=1.0):
        return jax.random.uniform(self._next(), shape, jnp.bfloat16, lo, hi)

    def permutation(self, n):
        return jax.random.permutation(self._next(), n)
kernel_name = 'interleave_layers__memory_aug_recurrent_mem_tr__linear_kernel_hedgehog__prompt'

def setup_inputs():
    _rng = _Rng(jax.random.key(int.from_bytes(__import__("os").urandom(4), "little")))
    _w = lambda a: (lambda t: t.astype(jnp.bfloat16) if jnp.issubdtype(t.dtype, jnp.floating) else t)(jnp.asarray(a))

    def _A_setup():
        B, S, Dm = (1, 2048, 640)
        H, Dh = (32, 192)
        M, seg = (8, 32)
        seg = min(seg, S)
        S = S // seg * seg
        return {'x': _w((lambda *s: _rng.normal(s) * 0.05)(B, S, Dm)), 'mem0': _w((lambda *s: _rng.normal(s) * 0.05)(B, M, Dm)), 'Wq': _w((lambda *s: _rng.normal(s) * 0.05)(Dm, H, Dh) * Dm ** (-0.5)), 'Wk': _w((lambda *s: _rng.normal(s) * 0.05)(Dm, H, Dh) * Dm ** (-0.5)), 'Wv': _w((lambda *s: _rng.normal(s) * 0.05)(Dm, H, Dh) * Dm ** (-0.5)), 'Wo': _w((lambda *s: _rng.normal(s) * 0.05)(H, Dh, Dm) * (H * Dh) ** (-0.5)), 'seg_len': seg}
    _A_in = _A_setup()

    def _B_setup():
        B, S, D, H = (1, 2048, 640, 32)
        Dh = D // H
        return {'x': _w((lambda *s: _rng.normal(s) * 0.05)(B, S, D)), 'wqkv': _w((lambda *s: _rng.normal(s) * 0.05)(D, 3 * D)), 'w_phi': _w((lambda *s: _rng.normal(s) * 0.05)(H, Dh, Dh) * Dh ** (-0.5)), 'wo': _w((lambda *s: _rng.normal(s) * 0.05)(D, D))}
    _B_in = _B_setup()
    return {'A_x': _A_in['x'], 'A_mem0': _A_in['mem0'], 'A_Wq': _A_in['Wq'], 'A_Wk': _A_in['Wk'], 'A_Wv': _A_in['Wv'], 'A_Wo': _A_in['Wo'], 'A_seg_len': _A_in['seg_len'], 'B_x': _B_in['x'], 'B_wqkv': _B_in['wqkv'], 'B_w_phi': _B_in['w_phi'], 'B_wo': _B_in['wo']}

def reference(A_x, A_mem0, A_Wq, A_Wk, A_Wv, A_Wo, A_seg_len, B_x, B_wqkv, B_w_phi, B_wo):

    def _A_ref(x, mem0, Wq, Wk, Wv, Wo, seg_len):
        B, S, Dm = x.shape
        H, Dh = (Wq.shape[1], Wq.shape[2])
        M = mem0.shape[1]
        scale = Dh ** (-0.5)
        n_seg = S // seg_len
        L = M + seg_len
        idx = jnp.arange(L)
        mask = (idx[:, None] < M) | (idx[:, None] >= idx[None, :])
        mem = mem0
        outs = []
        for s in range(n_seg):
            xs = x[:, s * seg_len:(s + 1) * seg_len, :].copy()
            h = jnp.concatenate([mem, xs], axis=1)
            q = jnp.einsum('btd,dhe->bhte', h, Wq)
            k = jnp.einsum('btd,dhe->bhte', h, Wk)
            v = jnp.einsum('btd,dhe->bhte', h, Wv)
            scores = jnp.einsum('bhqe,bhke->bhqk', q, k) * scale
            scores = jnp.where(mask[None, None], scores, -1000000000.0)
            p = _softmax(scores, axis=-1)
            o = jnp.einsum('bhqk,bhke->bhqe', p, v)
            o = jnp.einsum('bhte,hed->btd', o, Wo)
            mem = o[:, :M, :].copy()
            outs.append(o[:, M:, :])
        return jnp.concatenate(outs, axis=1)

    def _B_ref(x, wqkv, w_phi, wo):
        B, S, D = x.shape
        H = 32
        Dh = D // H
        qkv = (lambda x, *d: x.transpose(*d))((x @ wqkv).reshape(B, S, 3, H, Dh), 2, 0, 3, 1, 4)
        q, k, v = (qkv[0], qkv[1], qkv[2])
        pq = jnp.einsum('bhsd,hdf->bhsf', q, w_phi)
        pk = jnp.einsum('bhsd,hdf->bhsf', k, w_phi)
        phi_q = jnp.concatenate([_softmax(pq, axis=-1), _softmax(-pq, axis=-1)], axis=-1)
        phi_k = jnp.concatenate([_softmax(pk, axis=-1), _softmax(-pk, axis=-1)], axis=-1)
        kv = jnp.einsum('bhsf,bhsd->bhfd', phi_k, v)
        z = jnp.einsum('bhsf->bhf', phi_k)
        num = jnp.einsum('bhqf,bhfd->bhqd', phi_q, kv)
        den = jnp.einsum('bhqf,bhf->bhq', phi_q, z)[..., None] + 1e-06
        o = num / den
        return (lambda x, *d: x.transpose(*d))(o, 0, 2, 1, 3).reshape(B, S, D) @ wo
    x = A_x
    x = x + _A_ref(_layernorm(x, axis=-1), A_mem0, A_Wq, A_Wk, A_Wv, A_Wo, A_seg_len)
    x = x + _B_ref(_layernorm(x, axis=-1), B_wqkv, B_w_phi, B_wo)
    x = x + _A_ref(_layernorm(x, axis=-1), A_mem0, A_Wq, A_Wk, A_Wv, A_Wo, A_seg_len)
    x = x + _B_ref(_layernorm(x, axis=-1), B_wqkv, B_w_phi, B_wo)
    return x
```

```python
import functools
import math

import jax
import jax.numpy as jnp
from jax import lax
import jax.experimental.pallas as pl
import jax.experimental.pallas.tpu as pltpu

F32 = jnp.float32
BF16 = jnp.bfloat16
NT = (((1,), (1,)), ((), ()))
TN = (((0,), (0,)), ((), ()))
LOG2E = math.log2(math.e)

LAG_S = 2
LAG_PV = 2
O_PAIRS = 4
TB = 256
GB = 4
W_AHEAD = 3


def _iota(shape, axis):
    return lax.broadcasted_iota(jnp.int32, shape, axis)


def _div(v, d):
    return (v * ((1 << 18) // d + 1)) >> 18


def _layernorm(x):
    m = jnp.mean(x, axis=-1, keepdims=True)
    c = x - m
    v = jnp.mean(c * c, axis=-1, keepdims=True)
    return c / jnp.sqrt(v + 1e-5)


def _round_bf16(x):
    return x.astype(BF16).astype(F32)


def _a_step(s, mem, *, seg, dh, xn_ref, x_ref, w_ref, wo_ref, o_ref):
    n_mem = mem.shape[0]
    rows = n_mem + seg
    pw = 2 * dh
    n_pairs = w_ref.shape[0]
    scale = dh ** -0.5
    r0 = pl.multiple_of(s * seg, seg)
    h = jnp.concatenate([mem, xn_ref[pl.ds(r0, seg), :]], axis=0)

    first = _iota((rows, 128), 1) < (dh - 128)
    col = _iota((rows, 2 * rows), 1)
    row = _iota((rows, 2 * rows), 0)
    is_a = col < rows
    visible = (row < n_mem) | (row >= jnp.where(is_a, col, col - rows))
    zero = jnp.zeros((rows, 128), F32)

    def block_diag(t):
        t0, t1, t2 = t[:, 0:128], t[:, 128:256], t[:, 256:384]
        top = jnp.concatenate([t0, jnp.where(first, t1, 0.0), zero], axis=1)
        bot = jnp.concatenate([zero, jnp.where(first, 0.0, t1), t2], axis=1)
        return jnp.concatenate([top, bot], axis=0).astype(BF16)

    qkv, probs = {}, {}

    def scores(p):
        t = qkv[p]
        sc = lax.dot_general(t[:, 0:pw], block_diag(t[:, pw:2 * pw]), NT,
                             preferred_element_type=F32)
        sc = jnp.where(visible, sc * scale, -1e9)
        max_a = jnp.max(jnp.where(is_a, sc, -jnp.inf), axis=1, keepdims=True)
        max_b = jnp.max(jnp.where(is_a, -jnp.inf, sc), axis=1, keepdims=True)
        e = jnp.exp(sc - jnp.where(is_a, max_a, max_b))
        sum_a = jnp.sum(jnp.where(is_a, e, 0.0), axis=1, keepdims=True)
        sum_b = jnp.sum(jnp.where(is_a, 0.0, e), axis=1, keepdims=True)
        probs[p] = e / jnp.where(is_a, sum_a, sum_b)

    def values(p):
        o_ref[:, p * pw:(p + 1) * pw] = jnp.dot(
            probs[p], block_diag(qkv[p][:, 2 * pw:3 * pw]), preferred_element_type=F32)

    out = None
    n_out = n_pairs // O_PAIRS
    done = 0

    def project(c, acc):
        lo, hi = c * O_PAIRS * pw, (c + 1) * O_PAIRS * pw
        r = jnp.dot(o_ref[:, lo:hi], wo_ref[lo:hi, :], preferred_element_type=F32)
        return r if acc is None else acc + r

    for t in range(n_pairs + LAG_S + LAG_PV):
        if t < n_pairs:
            qkv[t] = jnp.dot(h, w_ref[t], preferred_element_type=F32)
        elif done < n_out - 1:
            out = project(done, out)
            done += 1
        if 0 <= t - LAG_S < n_pairs:
            scores(t - LAG_S)
        if 0 <= t - LAG_S - LAG_PV < n_pairs:
            values(t - LAG_S - LAG_PV)
    while done < n_out:
        out = project(done, out)
        done += 1

    x_ref[pl.ds(r0, seg), :] += out[n_mem:, :]
    return out[:n_mem, :]


def _pair_reduce(t, op):
    r = t[0:8]
    for i in range(8, t.shape[0], 8):
        r = op(r, t[i:i + 8])
    r = op(r, pltpu.roll(r, 4, 0))
    return op(r, pltpu.roll(r, 2, 0))


def _tile_rows(r, n):
    return jnp.concatenate([r] * (n // 8), axis=0)


def _feature_map(p):
    n = p.shape[0]
    e_pos = jnp.exp2(p - _tile_rows(_pair_reduce(p, jnp.maximum), n))
    e_neg = jnp.exp2(_tile_rows(_pair_reduce(p, jnp.minimum), n) - p)
    inv_pos = 1.0 / _pair_reduce(e_pos, jnp.add)
    inv_neg = 1.0 / _pair_reduce(e_neg, jnp.add)
    return jnp.concatenate(
        [e_pos * _tile_rows(inv_pos, n), e_neg * _tile_rows(inv_neg, n)], axis=0).astype(BF16)


def _b_weights(wqkv_ref, wphi_ref, wob_ref, bq_ref, bkv_ref, bo_ref):
    d = wob_ref.shape[0]
    dh, _, heads = wphi_ref.shape
    gr = 2 * dh
    c = _iota((dh, d), 1)
    c_feat = c - _div(c, dh) * dh
    spread = (_div(_iota((heads, d), 1), dh) == _iota((heads, d), 0)).astype(BF16)
    by_feat = jnp.zeros((dh, d), F32)
    for e in range(dh):
        t = jnp.dot(wphi_ref[e], spread, preferred_element_type=F32)
        by_feat = jnp.where(c_feat == e, t, by_feat)
    by_feat = by_feat.astype(BF16)

    blk = GB * gr
    for b in range(d // blk):
        lo = b * blk // 128 * 128
        hi = -(-(b + 1) * blk // 128) * 128
        r = _iota((blk, hi - lo), 0)
        g = _div(r, gr)
        head = 2 * (g + b * GB) + (r & 1)
        feat = (r - g * gr) >> 1
        cc = _iota((blk, hi - lo), 1) + lo
        perm = (cc == head * dh + feat).astype(BF16)
        rs = _iota((blk, dh), 0)
        sel = (((rs - _div(rs, gr) * gr) >> 1) == _iota((blk, dh), 1)).astype(BF16)
        phi = jnp.dot(sel, by_feat[:, lo:hi], preferred_element_type=F32)
        phi = jnp.where(_div(cc, dh) == head, phi, 0.0).astype(BF16)
        wq = lax.dot_general(phi, wqkv_ref[:, lo:hi], NT, preferred_element_type=F32)
        wk = lax.dot_general(phi, wqkv_ref[:, d + lo:d + hi], NT, preferred_element_type=F32)
        wv = lax.dot_general(perm, wqkv_ref[:, 2 * d + lo:2 * d + hi], NT,
                             preferred_element_type=F32)
        bq_ref[b] = (wq * LOG2E).astype(BF16)
        bkv_ref[b, 0:blk, :] = (wk * LOG2E).astype(BF16)
        bkv_ref[b, blk:2 * blk, :] = wv.astype(BF16)
        bo_ref[b * blk:(b + 1) * blk, :] = jnp.dot(
            perm, wob_ref[lo:hi, :], preferred_element_type=F32).astype(BF16)


def _b_keys(c, carry, *, x_ref, xb_ref, bkv_ref, kv_ref):
    r0 = pl.multiple_of(c * TB, TB)
    xb = _layernorm(x_ref[pl.ds(r0, TB), :]).astype(BF16)
    xb_ref[pl.ds(r0, TB), :] = xb
    n_blk = bkv_ref.shape[0]
    blk = bkv_ref.shape[1] // 2
    gr = blk // GB
    ones = jnp.ones((8, TB), F32)
    for b in range(n_blk):
        t = lax.dot_general(bkv_ref[b], xb, NT, preferred_element_type=F32)
        for i in range(GB):
            phi = _feature_map(t[i * gr:(i + 1) * gr])
            v = jnp.concatenate([t[blk + i * gr:blk + (i + 1) * gr], ones], axis=0)
            kv_ref[b * GB + i] += lax.dot_general(
                v.astype(BF16), phi, NT, preferred_element_type=F32)
    return carry


def _b_queries(c, carry, *, x_ref, xb_ref, xn_ref, y_ref, bq_ref, bo_ref, kvm_ref, ot_ref):
    r0 = pl.multiple_of(c * TB, TB)
    xb = xb_ref[pl.ds(r0, TB), :]
    n_blk, blk, _ = bq_ref.shape
    gr = blk // GB
    for b in range(n_blk):
        t = lax.dot_general(bq_ref[b], xb, NT, preferred_element_type=F32)
        for i in range(GB):
            g = b * GB + i
            phi = _feature_map(t[i * gr:(i + 1) * gr])
            r = jnp.dot(kvm_ref[g], phi, preferred_element_type=F32)
            inv = 1.0 / (r[gr:gr + 8] + 1e-6)
            ot_ref[g * gr:(g + 1) * gr, :] = r[0:gr] * _tile_rows(inv, gr)
    y = lax.dot_general(ot_ref[...].astype(BF16), bo_ref[...], TN, preferred_element_type=F32)
    x = x_ref[pl.ds(r0, TB), :] + y
    x_ref[pl.ds(r0, TB), :] = x
    y_ref[pl.ds(r0, TB), :] = x.astype(BF16)
    xn_ref[pl.ds(r0, TB), :] = _round_bf16(_layernorm(x))
    return carry


def _kernel(x_hbm, mem0_ref, wq_hbm, wk_hbm, wv_hbm, wo_hbm, wqkvb_hbm, wphi_ref, wob_hbm,
            out_hbm,
            x_ref, xn_ref, xb_ref, y_ref, stage_ref, w_ref, wo_ref, o_ref,
            wqkvb_ref, wob_ref, bq_ref, bkv_ref, bo_ref, kv_ref, kvm_ref, ot_ref,
            w_sem, wo_sem, in_sem, out_sem, *, seg, dh):
    s_len = x_ref.shape[0]
    n_pairs = w_ref.shape[0]
    pw = 2 * dh
    n_chunks = s_len // TB

    def w_copy(p, j):
        src = (wq_hbm, wk_hbm, wv_hbm)[j]
        return pltpu.make_async_copy(
            src.at[pl.ds(pl.multiple_of(p * pw, pw), pw), :], stage_ref.at[p, j], w_sem.at[p, j])

    def out_copy(c):
        rows = pl.ds(pl.multiple_of(c * TB, TB), TB)
        return pltpu.make_async_copy(y_ref.at[rows, :], out_hbm.at[rows, :], out_sem.at[c])

    x_copy = pltpu.make_async_copy(x_hbm, y_ref, in_sem.at[0])
    wqkvb_copy = pltpu.make_async_copy(wqkvb_hbm, wqkvb_ref, in_sem.at[1])
    wob_copy = pltpu.make_async_copy(wob_hbm, wob_ref, in_sem.at[2])
    wo_copy = pltpu.make_async_copy(wo_hbm, wo_ref, wo_sem.at[0])

    x_copy.start()
    for p in range(W_AHEAD):
        for j in range(3):
            w_copy(p, j).start()
    x_copy.wait()

    def first_norm(c, carry):
        rows = pl.ds(pl.multiple_of(c * TB, TB), TB)
        x = y_ref[rows, :].astype(F32)
        x_ref[rows, :] = x
        xn_ref[rows, :] = _round_bf16(_layernorm(x))
        return carry

    lax.fori_loop(0, n_chunks, first_norm, 0)

    def load_pair(p, carry):
        @pl.when(p + W_AHEAD < n_pairs)
        def _():
            for j in range(3):
                w_copy(p + W_AHEAD, j).start()

        @pl.when(p + W_AHEAD == n_pairs)
        def _():
            wo_copy.start()

        for j in range(3):
            w_copy(p, j).wait()
        for j in range(3):
            w_ref[p, :, j * pw:(j + 1) * pw] = stage_ref[p, j].T
        return carry

    lax.fori_loop(0, n_pairs, load_pair, 0)
    wo_copy.wait()
    wqkvb_copy.start()
    wob_copy.start()

    a_step = functools.partial(_a_step, seg=seg, dh=dh, xn_ref=xn_ref, x_ref=x_ref,
                               w_ref=w_ref, wo_ref=wo_ref, o_ref=o_ref)
    b_keys = functools.partial(_b_keys, x_ref=x_ref, xb_ref=xb_ref, bkv_ref=bkv_ref,
                               kv_ref=kv_ref)
    b_queries = functools.partial(_b_queries, x_ref=x_ref, xb_ref=xb_ref, xn_ref=xn_ref,
                                  y_ref=y_ref, bq_ref=bq_ref, bo_ref=bo_ref, kvm_ref=kvm_ref,
                                  ot_ref=ot_ref)

    def layer_pair(layer, carry):
        lax.fori_loop(0, s_len // seg, a_step, mem0_ref[...].astype(F32))

        @pl.when(layer == 0)
        def _():
            wqkvb_copy.wait()
            wob_copy.wait()
            _b_weights(wqkvb_ref, wphi_ref, wob_ref, bq_ref, bkv_ref, bo_ref)

        kv_ref[...] = jnp.zeros(kv_ref.shape, F32)
        lax.fori_loop(0, n_chunks, b_keys, 0)
        same_head = ((_iota(kv_ref.shape, 1) ^ _iota(kv_ref.shape, 2)) & 1) == 0
        kvm_ref[...] = jnp.where(same_head, kv_ref[...], 0.0).astype(BF16)

        def queries(c, carry):
            b_queries(c, carry)

            @pl.when(layer == 1)
            def _():
                out_copy(c).start()

            return carry

        lax.fori_loop(0, n_chunks, queries, 0)
        return carry

    lax.fori_loop(0, 2, layer_pair, 0)
    for c in range(n_chunks):
        out_copy(c).wait()


@functools.partial(jax.jit, static_argnames=("A_seg_len",))
def pallas_interleave_layers__memory_aug_recurrent_mem_tr__linear_kernel_hedgehog__prompt_kernel(
    A_x, A_mem0, A_Wq, A_Wk, A_Wv, A_Wo, A_seg_len, B_x, B_wqkv, B_w_phi, B_wo,
):
    del B_x
    batch, s_len, d = A_x.shape
    _, heads, dh = A_Wq.shape
    n_mem = A_mem0.shape[1]
    seg = int(A_seg_len)
    b_heads, b_dh, _ = B_w_phi.shape
    rows = n_mem + seg
    n_pairs = heads // 2
    gr = 2 * b_dh
    blk = GB * gr
    assert batch == 1 and dh == 192 and heads % (2 * O_PAIRS) == 0
    assert n_mem % 8 == 0 and seg % 8 == 0 and 2 * rows <= 128
    assert s_len % seg == 0 and s_len % TB == 0
    assert b_heads * b_dh == d and gr % 8 == 0 and d % blk == 0

    def head_major(w):
        return w.transpose(1, 2, 0).reshape(heads * dh, d)

    hbm = pl.BlockSpec(memory_space=pltpu.HBM)
    vmem = pl.BlockSpec(memory_space=pltpu.VMEM)
    out = pl.pallas_call(
        functools.partial(_kernel, seg=seg, dh=dh),
        out_shape=jax.ShapeDtypeStruct((s_len, d), A_x.dtype),
        in_specs=[hbm, vmem, hbm, hbm, hbm, hbm, hbm, vmem, hbm],
        out_specs=hbm,
        scratch_shapes=[
            pltpu.VMEM((s_len, d), F32),
            pltpu.VMEM((s_len, d), F32),
            pltpu.VMEM((s_len, d), BF16),
            pltpu.VMEM((s_len, d), BF16),
            pltpu.VMEM((n_pairs, 3, 2 * dh, d), BF16),
            pltpu.VMEM((n_pairs, d, 6 * dh), BF16),
            pltpu.VMEM((heads * dh, d), BF16),
            pltpu.VMEM((rows, heads * dh), F32),
            pltpu.VMEM(B_wqkv.shape, BF16),
            pltpu.VMEM(B_wo.shape, BF16),
            pltpu.VMEM((d // blk, blk, d), BF16),
            pltpu.VMEM((d // blk, 2 * blk, d), BF16),
            pltpu.VMEM((d, d), BF16),
            pltpu.VMEM((b_heads // 2, gr + 8, 2 * gr), F32),
            pltpu.VMEM((b_heads // 2, gr + 8, 2 * gr), BF16),
            pltpu.VMEM((d, TB), F32),
            pltpu.SemaphoreType.DMA((n_pairs, 3)),
            pltpu.SemaphoreType.DMA((1,)),
            pltpu.SemaphoreType.DMA((3,)),
            pltpu.SemaphoreType.DMA((s_len // TB,)),
        ],
        compiler_params=pltpu.CompilerParams(vmem_limit_bytes=110 * 1024 * 1024),
    )(
        A_x.reshape(s_len, d), A_mem0.reshape(n_mem, d),
        head_major(A_Wq), head_major(A_Wk), head_major(A_Wv), A_Wo.reshape(heads * dh, d),
        B_wqkv, B_w_phi.transpose(1, 2, 0), B_wo,
    )
    return out.reshape(batch, s_len, d)
```

```python
import functools
import math

import jax
import jax.numpy as jnp
from jax import lax
import jax.experimental.pallas as pl
import jax.experimental.pallas.tpu as pltpu

F32 = jnp.float32
BF16 = jnp.bfloat16
NT = (((1,), (1,)), ((), ()))
TN = (((0,), (0,)), ((), ()))
LOG2E = math.log2(math.e)

LAG_S = 2
LAG_PV = 2
O_PAIRS = 4
A_UNROLL = (2, 2)
K_SPLIT = 512
PRE = 8
P_UNROLL = 1
TB = 256
B_UNROLL = 2
GB = 4


def _iota(shape, axis):
    return lax.broadcasted_iota(jnp.int32, shape, axis)


def _div(v, d):
    return (v * ((1 << 18) // d + 1)) >> 18


def _layernorm(x):
    m = jnp.mean(x, axis=-1, keepdims=True)
    c = x - m
    v = jnp.mean(c * c, axis=-1, keepdims=True)
    return c * lax.rsqrt(v + 1e-5)


def _a_step(s, carry, *, dh, x_in, x_ref, xb_ref, w_ref, wo_ref, pre_ref, o_ref):
    mem, xn = carry
    n_mem, seg = mem.shape[0], xn.shape[0]
    rows = n_mem + seg
    pw = 2 * dh
    n_pairs = w_ref.shape[0]
    scale = dh ** -0.5

    nxt = jnp.minimum(s + 1, x_ref.shape[0] - 1)
    prv = jnp.maximum(s - 1, 0)
    xn_next = _layernorm(x_in[nxt].astype(F32))
    xb_ref[prv] = _layernorm(x_ref[prv]).astype(BF16)

    h = jnp.concatenate([mem, xn], axis=0)
    h_short = h[:rows - PRE].astype(BF16)

    first = _iota((rows, 128), 1) < (dh - 128)
    col = _iota((rows, 2 * rows), 1)
    row = _iota((rows, 2 * rows), 0)
    is_a = col < rows
    visible = (row < n_mem) | (row >= jnp.where(is_a, col, col - rows))
    zero = jnp.zeros((rows, 128), F32)

    def block_diag(t):
        t0, t1, t2 = t[:, 0:128], t[:, 128:256], t[:, 256:384]
        top = jnp.concatenate([t0, jnp.where(first, t1, 0.0), zero], axis=1)
        bot = jnp.concatenate([zero, jnp.where(first, 0.0, t1), t2], axis=1)
        return jnp.concatenate([top, bot], axis=0).astype(BF16)

    qkv, probs = {}, {}

    def times_w(lhs, p, lo, hi):
        def part(k0, k1):
            w = pltpu.bitcast(w_ref[p, k0 // 2:k1 // 2, lo:hi], BF16)
            return jnp.dot(lhs[:, k0:k1], w, preferred_element_type=F32)

        if p == 0 and lo == 0 and K_SPLIT:
            return part(0, K_SPLIT) + part(K_SPLIT, lhs.shape[1])
        return part(0, lhs.shape[1])

    def project_in(p):
        if pre_ref is None:
            qkv[p] = times_w(h, p, 0, 3 * pw)
        else:
            q = times_w(h, p, 0, pw)
            kv = jnp.concatenate(
                [times_w(h_short, p, pw, 3 * pw),
                 pre_ref[p, pl.ds(pl.multiple_of(s * PRE, PRE), PRE), :]], axis=0)
            qkv[p] = jnp.concatenate([q, kv], axis=1)

    def scores(p):
        t = qkv[p]
        sc = lax.dot_general(t[:, 0:pw], block_diag(t[:, pw:2 * pw]), NT,
                             preferred_element_type=F32)
        sc = jnp.where(visible, sc * scale, -1e9)
        max_a = jnp.max(jnp.where(is_a, sc, -jnp.inf), axis=1, keepdims=True)
        max_b = jnp.max(jnp.where(is_a, -jnp.inf, sc), axis=1, keepdims=True)
        e = jnp.exp(sc - jnp.where(is_a, max_a, max_b))
        sum_a = jnp.sum(jnp.where(is_a, e, 0.0), axis=1, keepdims=True)
        sum_b = jnp.sum(jnp.where(is_a, 0.0, e), axis=1, keepdims=True)
        probs[p] = e / jnp.where(is_a, sum_a, sum_b)

    def values(p):
        o_ref[:, p * pw:(p + 1) * pw] = jnp.dot(
            probs[p], block_diag(qkv[p][:, 2 * pw:3 * pw]), preferred_element_type=F32)

    def project_out(c, acc):
        lo, hi = c * O_PAIRS * pw, (c + 1) * O_PAIRS * pw

        def part(c0, c1):
            return jnp.dot(o_ref[:, lo:hi], wo_ref[lo:hi, c0:c1], preferred_element_type=F32)

        d = wo_ref.shape[1]
        if hi == wo_ref.shape[0] and K_SPLIT:
            r = jnp.concatenate([part(0, K_SPLIT), part(K_SPLIT, d)], axis=1)
        else:
            r = part(0, d)
        return r if acc is None else acc + r

    out = None
    n_out = n_pairs // O_PAIRS
    done = 0
    for t in range(n_pairs + LAG_S + LAG_PV):
        if t < n_pairs:
            project_in(t)
        elif done < n_out - 1:
            out = project_out(done, out)
            done += 1
        if 0 <= t - LAG_S < n_pairs:
            scores(t - LAG_S)
        if 0 <= t - LAG_S - LAG_PV < n_pairs:
            values(t - LAG_S - LAG_PV)
    while done < n_out:
        out = project_out(done, out)
        done += 1

    x_ref[s] = x_in[s].astype(F32) + out[n_mem:, :]
    return out[:n_mem, :], xn_next


def _pair_reduce(t, op):
    r = t[0:8]
    for i in range(8, t.shape[0], 8):
        r = op(r, t[i:i + 8])
    r = op(r, pltpu.roll(r, 4, 0))
    return op(r, pltpu.roll(r, 2, 0))


def _tile_rows(r, n):
    return jnp.concatenate([r] * (n // 8), axis=0)


def _feature_map(p):
    n = p.shape[0]
    e_pos = jnp.exp2(p - _tile_rows(_pair_reduce(p, jnp.maximum), n))
    e_neg = jnp.exp2(_tile_rows(_pair_reduce(p, jnp.minimum), n) - p)
    inv_pos = 1.0 / _pair_reduce(e_pos, jnp.add)
    inv_neg = 1.0 / _pair_reduce(e_neg, jnp.add)
    return jnp.concatenate(
        [e_pos * _tile_rows(inv_pos, n), e_neg * _tile_rows(inv_neg, n)], axis=0).astype(BF16)


def _b_weights(wqkv_ref, wphi_ref, bq_ref, bkv_ref):
    d = wqkv_ref.shape[0]
    dh, _, heads = wphi_ref.shape
    gr = 2 * dh
    c = _iota((dh, d), 1)
    c_feat = c - _div(c, dh) * dh
    spread = (_div(_iota((heads, d), 1), dh) == _iota((heads, d), 0)).astype(BF16)
    by_feat = jnp.zeros((dh, d), F32)
    for e in range(dh):
        t = jnp.dot(wphi_ref[e], spread, preferred_element_type=F32)
        by_feat = jnp.where(c_feat == e, t, by_feat)
    by_feat = by_feat.astype(BF16)

    blk = GB * gr
    r = _iota((blk, dh), 0)
    sel = (((r - _div(r, gr) * gr) >> 1) == _iota((blk, dh), 1)).astype(BF16)
    wv = wqkv_ref[:, 2 * d:3 * d].T
    for b in range(d // blk):
        lo = b * blk // 128 * 128
        hi = -(-(b + 1) * blk // 128) * 128
        r = _iota((blk, hi - lo), 0)
        head = 2 * (_div(r, gr) + b * GB) + (r & 1)
        phi = jnp.dot(sel, by_feat[:, lo:hi], preferred_element_type=F32)
        phi = jnp.where(_div(_iota((1, hi - lo), 1) + lo, dh) == head, phi, 0.0).astype(BF16)
        wq = lax.dot_general(phi, wqkv_ref[:, lo:hi], NT, preferred_element_type=F32)
        wk = lax.dot_general(phi, wqkv_ref[:, d + lo:d + hi], NT, preferred_element_type=F32)
        bq_ref[b] = (wq * LOG2E).astype(BF16)
        bkv_ref[b, 0:blk, :] = (wk * LOG2E).astype(BF16)
        bkv_ref[b, blk:2 * blk, :] = wv[b * blk:(b + 1) * blk]


def _rows(ref, start, n):
    k = n // ref.shape[1]
    return ref[pl.ds(start * k, k)].reshape(n, ref.shape[2])


def _b_keys(it, carry, *, xb_ref, bkv_ref, kv_ref):
    n_blk = bkv_ref.shape[0]
    blk = bkv_ref.shape[1] // 2
    gr = blk // GB
    ones = jnp.ones((8, TB), F32)

    def project(j, b):
        return lax.dot_general(bkv_ref[b], _rows(xb_ref, it * B_UNROLL + j, TB), NT,
                               preferred_element_type=F32)

    def accumulate(b, t):
        for i in range(GB):
            phi = _feature_map(t[i * gr:(i + 1) * gr])
            v = jnp.concatenate([t[blk + i * gr:blk + (i + 1) * gr], ones], axis=0)
            kv_ref[b * GB + i] += lax.dot_general(
                v.astype(BF16), phi, NT, preferred_element_type=F32)

    pending = None
    for j in range(B_UNROLL):
        for b in range(n_blk):
            t = project(j, b)
            if pending is not None:
                accumulate(*pending)
            pending = (b, t)
    accumulate(*pending)
    return carry


def _b_queries(it, *, x_ref, xb_ref, y_ref, bq_ref, bo_ref, kvm_ref, ot_ref):
    n_blk, blk, _ = bq_ref.shape
    gr = blk // GB
    upper = _iota((8, TB), 0) < 4

    def project(j, b):
        return lax.dot_general(bq_ref[b], _rows(xb_ref, it * B_UNROLL + j, TB), NT,
                               preferred_element_type=F32)

    def attend(j, b, t):
        for i in range(GB):
            g = b * GB + i
            phi = _feature_map(t[i * gr:(i + 1) * gr])
            r = jnp.dot(kvm_ref[g], phi, preferred_element_type=F32)
            inv = 1.0 / (r[gr:gr + 8] + 1e-6)
            swapped = pltpu.roll(inv, 4, 0)
            n = (gr - 8) // 16
            inv = jnp.concatenate([jnp.where(upper, inv, swapped)] * n + [inv]
                                  + [jnp.where(upper, swapped, inv)] * n, axis=0)
            ot_ref[j, g * gr:(g + 1) * gr, :] = r[0:gr] * inv

    def finish(j, half):
        at = (it * B_UNROLL + j) * (TB // 128) + half
        o = ot_ref[j, :, half * 128:(half + 1) * 128].astype(BF16)
        x = _rows(x_ref, at, 128) + lax.dot_general(o, bo_ref[...], TN,
                                                    preferred_element_type=F32)
        k = 128 // x_ref.shape[1]
        x = x.reshape((k,) + x_ref.shape[1:])
        x_ref[pl.ds(at * k, k)] = x
        y_ref[pl.ds(at * k, k)] = x.astype(BF16)

    tails = [(j, half) for j in range(B_UNROLL) for half in range(TB // 128)]
    pending = None
    for j in range(B_UNROLL):
        for b in range(n_blk):
            t = project(j, b)
            if pending is not None:
                attend(*pending)
            pending = (j, b, t)
    if B_UNROLL > 1:
        finish(*tails.pop(0))
    attend(*pending)
    for tail in tails:
        finish(*tail)


def _kernel(x_hbm, mem0_ref, wq_hbm, wk_hbm, wv_hbm, wo_hbm, wqkvb_hbm, wphi_ref, wob_hbm,
            out_hbm,
            x_ref, xb_ref, y_ref, xt_ref, xp_ref, stage_ref, pre_ref, w_ref, wo_ref, o_ref,
            wqkvb_ref, bo_ref, bq_ref, bkv_ref, kv_ref, kvm_ref, ot_ref,
            w_sem, in_sem, out_sem, *, dh):
    n_seg, seg, d = x_ref.shape
    n_pairs = w_ref.shape[0]
    pw = 2 * dh
    n_iter = n_seg * seg // (TB * B_UNROLL)

    def pair_rows(p):
        return pl.ds(pl.multiple_of(p * pw, pw), pw)

    def w_copy(p, j):
        return pltpu.make_async_copy(
            (wq_hbm, wk_hbm, wv_hbm)[j].at[pair_rows(p), :],
            stage_ref.at[p, j * pw:(j + 1) * pw, :], w_sem.at[p, j])

    def out_copy(i):
        part = pl.ds(i * (n_seg // n_iter), n_seg // n_iter)
        return pltpu.make_async_copy(y_ref.at[part], out_hbm.at[part], out_sem.at[i])

    xt_copy = pltpu.make_async_copy(x_hbm.at[:, seg - PRE:seg, :], xt_ref, in_sem.at[0])
    wqkvb_copy = pltpu.make_async_copy(wqkvb_hbm, wqkvb_ref, in_sem.at[1])
    wob_copy = pltpu.make_async_copy(wob_hbm, bo_ref, in_sem.at[2])

    xt_copy.start()
    w_copy(0, 1).start()
    w_copy(0, 2).start()
    xt_copy.wait()

    w_copy(0, 0).start()
    for j in (1, 2, 0):
        w_copy(1, j).start()
    xp_ref[...] = _layernorm(xt_ref[...].astype(F32).reshape(n_seg * PRE, d)).astype(BF16)

    def pre_project(p, carry):
        @pl.when(p + 2 < n_pairs)
        def _():
            for j in range(3):
                w_copy(jnp.minimum(p + 2, n_pairs - 1), j).start()

        part = pl.ds(p * (n_seg // n_pairs), n_seg // n_pairs)
        pltpu.make_async_copy(x_hbm.at[part], y_ref.at[part], in_sem.at[3]).start()
        pltpu.make_async_copy(
            wo_hbm.at[pair_rows(p), :], wo_ref.at[pair_rows(p), :], in_sem.at[4]).start()
        for j in range(3):
            w_copy(p, j).wait()
        pre_ref[p] = lax.dot_general(xp_ref[...], stage_ref[p, pw:3 * pw, :], NT,
                                     preferred_element_type=F32)
        for j in range(3):
            w_ref[p, :, j * pw:(j + 1) * pw] = pltpu.bitcast(
                stage_ref[p, j * pw:(j + 1) * pw, :].T, jnp.uint32)
        return carry

    lax.fori_loop(0, n_pairs, pre_project, 0, unroll=P_UNROLL)

    pltpu.make_async_copy(x_hbm, y_ref, in_sem.at[3]).wait()
    pltpu.make_async_copy(wo_hbm, wo_ref, in_sem.at[4]).wait()

    wqkvb_copy.start()
    wob_copy.start()
    x_ref[0] = y_ref[0].astype(F32)

    def layer_a(x_in, pre, unroll):
        step = functools.partial(_a_step, dh=dh, x_in=x_in, x_ref=x_ref, xb_ref=xb_ref,
                                 w_ref=w_ref, wo_ref=wo_ref, pre_ref=pre, o_ref=o_ref)
        lax.fori_loop(0, n_seg, step, (mem0_ref[...].astype(F32), _layernorm(x_ref[0])),
                      unroll=unroll)

    b_keys = functools.partial(_b_keys, xb_ref=xb_ref, bkv_ref=bkv_ref, kv_ref=kv_ref)
    b_queries = functools.partial(_b_queries, x_ref=x_ref, xb_ref=xb_ref, y_ref=y_ref,
                                  bq_ref=bq_ref, bo_ref=bo_ref, kvm_ref=kvm_ref, ot_ref=ot_ref)

    def layer_pair(layer, carry):
        @pl.when(layer == 0)
        def _():
            layer_a(y_ref, pre_ref, A_UNROLL[0])

        @pl.when(layer == 0)
        def _():
            wqkvb_copy.wait()
            wob_copy.wait()
            _b_weights(wqkvb_ref, wphi_ref, bq_ref, bkv_ref)

        @pl.when(layer == 1)
        def _():
            layer_a(x_ref, None, A_UNROLL[1])

        xb_ref[n_seg - 1] = _layernorm(x_ref[n_seg - 1]).astype(BF16)
        kv_ref[...] = jnp.zeros(kv_ref.shape, F32)
        lax.fori_loop(0, n_iter, b_keys, 0)

        gr = kv_ref.shape[1] - 8
        r = _iota(kv_ref.shape, 1)
        second = ((r >= gr // 2) & (r < gr)) | (r >= gr + 4)
        same_head = second == ((_iota(kv_ref.shape, 2) & 1) == 1)
        kvm_ref[...] = jnp.where(same_head, kv_ref[...], 0.0).astype(BF16)

        def queries(it, carry):
            b_queries(it)

            @pl.when(layer == 1)
            def _():
                out_copy(it).start()

            return carry

        lax.fori_loop(0, n_iter, queries, 0)

        return carry

    lax.fori_loop(0, 2, layer_pair, 0)
    for i in range(n_iter):
        out_copy(i).wait()


@functools.partial(jax.jit, static_argnames=("A_seg_len",))
def pallas_interleave_layers__memory_aug_recurrent_mem_tr__linear_kernel_hedgehog__prompt_kernel(
    A_x, A_mem0, A_Wq, A_Wk, A_Wv, A_Wo, A_seg_len, B_x, B_wqkv, B_w_phi, B_wo,
):
    del B_x
    batch, s_len, d = A_x.shape
    _, heads, dh = A_Wq.shape
    n_mem = A_mem0.shape[1]
    seg = int(A_seg_len)
    b_heads, b_dh, _ = B_w_phi.shape
    rows = n_mem + seg
    n_pairs = heads // 2
    gr = 2 * b_dh
    blk = GB * gr
    n_seg = s_len // seg
    assert batch == 1 and dh == 192 and heads % (2 * O_PAIRS) == 0
    assert n_mem % 8 == 0 and seg % 16 == 0 and 128 % seg == 0 and 2 * rows <= 128
    assert s_len % (TB * B_UNROLL) == 0 and n_seg % n_pairs == 0
    assert b_heads * b_dh == d and b_dh % 8 == 4 and d % blk == 0

    def head_major(w):
        return w.transpose(1, 2, 0).reshape(heads * dh, d)

    hbm = pl.BlockSpec(memory_space=pltpu.HBM)
    vmem = pl.BlockSpec(memory_space=pltpu.VMEM)
    out = pl.pallas_call(
        functools.partial(_kernel, dh=dh),
        out_shape=jax.ShapeDtypeStruct((n_seg, seg, d), A_x.dtype),
        in_specs=[hbm, vmem, hbm, hbm, hbm, hbm, hbm, vmem, hbm],
        out_specs=hbm,
        scratch_shapes=[
            pltpu.VMEM((n_seg, seg, d), F32),
            pltpu.VMEM((n_seg, seg, d), BF16),
            pltpu.VMEM((n_seg, seg, d), BF16),
            pltpu.VMEM((n_seg, PRE, d), BF16),
            pltpu.VMEM((n_seg * PRE, d), BF16),
            pltpu.VMEM((n_pairs, 6 * dh, d), BF16),
            pltpu.VMEM((n_pairs, n_seg * PRE, 4 * dh), F32),
            pltpu.VMEM((n_pairs, d // 2, 6 * dh), jnp.uint32),
            pltpu.VMEM((heads * dh, d), BF16),
            pltpu.VMEM((rows, heads * dh), F32),
            pltpu.VMEM(B_wqkv.shape, BF16),
            pltpu.VMEM(B_wo.shape, BF16),
            pltpu.VMEM((d // blk, blk, d), BF16),
            pltpu.VMEM((d // blk, 2 * blk, d), BF16),
            pltpu.VMEM((b_heads // 2, gr + 8, 2 * gr), F32),
            pltpu.VMEM((b_heads // 2, gr + 8, 2 * gr), BF16),
            pltpu.VMEM((B_UNROLL, d, TB), F32),
            pltpu.SemaphoreType.DMA((n_pairs, 3)),
            pltpu.SemaphoreType.DMA((5,)),
            pltpu.SemaphoreType.DMA((s_len // (TB * B_UNROLL),)),
        ],
        compiler_params=pltpu.CompilerParams(vmem_limit_bytes=120 * 1024 * 1024),
    )(
        A_x.reshape(n_seg, seg, d), A_mem0.reshape(n_mem, d),
        head_major(A_Wq), head_major(A_Wk), head_major(A_Wv), A_Wo.reshape(heads * dh, d),
        B_wqkv, B_w_phi.transpose(1, 2, 0), B_wo,
    )
    return out.reshape(batch, s_len, d)
```

```python
import functools
import math

import jax
import jax.numpy as jnp
from jax import lax
import jax.experimental.pallas as pl
import jax.experimental.pallas.tpu as pltpu

F32 = jnp.float32
BF16 = jnp.bfloat16
NT = (((1,), (1,)), ((), ()))
TN = (((0,), (0,)), ((), ()))
LOG2E = math.log2(math.e)

LAG_S = 2
LAG_PV = 2
O_PAIRS = 4
A_UNROLL = (2, 2)
K_SPLIT = 512
NORM_AT = (4, 8)
PRE = 8
P_UNROLL = 1
TB = 256
B_UNROLL = 2
GB = 4


def _iota(shape, axis):
    return lax.broadcasted_iota(jnp.int32, shape, axis)


def _div(v, d):
    return (v * ((1 << 18) // d + 1)) >> 18


def _layernorm(x):
    m = jnp.mean(x, axis=-1, keepdims=True)
    c = x - m
    v = jnp.mean(c * c, axis=-1, keepdims=True)
    return c * lax.rsqrt(v + 1e-5)


def _a_step(s, carry, *, dh, x_in, x_ref, xb_ref, w_ref, wo_ref, pre_ref, o_ref):
    mem, xn = carry
    n_mem, seg = mem.shape[0], xn.shape[0]
    rows = n_mem + seg
    pw = 2 * dh
    n_pairs = w_ref.shape[0]
    scale = dh ** -0.5

    nxt = jnp.minimum(s + 1, x_ref.shape[0] - 1)
    prv = jnp.maximum(s - 1, 0)
    xn_next = _layernorm(x_in[nxt].astype(F32))
    xb_prev = _layernorm(x_ref[prv])
    xb_ref[prv] = xb_prev.astype(BF16)

    def schedule_before(value, early):
        t = functools.reduce(jnp.maximum, [early[i:i + 8, j:j + 128]
                                           for i in range(0, early.shape[0], 8)
                                           for j in range(0, early.shape[1], 128)])
        head = jnp.where(s < 0, t[:, :value.shape[1]], value[0:8])
        return jnp.concatenate([head, value[8:]], axis=0)

    h = jnp.concatenate([mem, xn], axis=0)
    h_short = h[:rows - PRE].astype(BF16)

    first = _iota((rows, 128), 1) < (dh - 128)
    col = _iota((rows, 2 * rows), 1)
    row = _iota((rows, 2 * rows), 0)
    is_a = col < rows
    visible = (row < n_mem) | (row >= jnp.where(is_a, col, col - rows))
    zero = jnp.zeros((rows, 128), F32)

    def block_diag(t):
        t0, t1, t2 = t[:, 0:128], t[:, 128:256], t[:, 256:384]
        top = jnp.concatenate([t0, jnp.where(first, t1, 0.0), zero], axis=1)
        bot = jnp.concatenate([zero, jnp.where(first, 0.0, t1), t2], axis=1)
        return jnp.concatenate([top, bot], axis=0).astype(BF16)

    qkv, probs = {}, {}

    def times_w(lhs, p, lo, hi):
        def part(k0, k1):
            w = pltpu.bitcast(w_ref[p, k0 // 2:k1 // 2, lo:hi], BF16)
            return jnp.dot(lhs[:, k0:k1], w, preferred_element_type=F32)

        if p == 0 and lo == 0 and K_SPLIT:
            return part(K_SPLIT, lhs.shape[1]) + part(0, K_SPLIT)
        return part(0, lhs.shape[1])

    def project_in(p):
        if pre_ref is None:
            qkv[p] = times_w(h, p, 0, 3 * pw)
        else:
            q = times_w(h, p, 0, pw)
            kv = jnp.concatenate(
                [times_w(h_short, p, pw, 3 * pw),
                 pre_ref[p, pl.ds(pl.multiple_of(s * PRE, PRE), PRE), :]], axis=0)
            qkv[p] = jnp.concatenate([q, kv], axis=1)

    def scores(p):
        t = qkv[p]
        sc = lax.dot_general(t[:, 0:pw], block_diag(t[:, pw:2 * pw]), NT,
                             preferred_element_type=F32)
        sc = jnp.where(visible, sc * scale, -1e9)
        max_a = jnp.max(jnp.where(is_a, sc, -jnp.inf), axis=1, keepdims=True)
        max_b = jnp.max(jnp.where(is_a, -jnp.inf, sc), axis=1, keepdims=True)
        e = jnp.exp(sc - jnp.where(is_a, max_a, max_b))
        sum_a = jnp.sum(jnp.where(is_a, e, 0.0), axis=1, keepdims=True)
        sum_b = jnp.sum(jnp.where(is_a, 0.0, e), axis=1, keepdims=True)
        probs[p] = e / jnp.where(is_a, sum_a, sum_b)
        if p == NORM_AT[0]:
            probs[p] = schedule_before(probs[p], xn_next)
        if p == NORM_AT[1]:
            probs[p] = schedule_before(probs[p], xb_prev)

    def values(p):
        o_ref[:, p * pw:(p + 1) * pw] = jnp.dot(
            probs[p], block_diag(qkv[p][:, 2 * pw:3 * pw]), preferred_element_type=F32)

    def project_out(c, acc):
        lo, hi = c * O_PAIRS * pw, (c + 1) * O_PAIRS * pw

        def part(c0, c1):
            return jnp.dot(o_ref[:, lo:hi], wo_ref[lo:hi, c0:c1], preferred_element_type=F32)

        d = wo_ref.shape[1]
        if hi == wo_ref.shape[0] and K_SPLIT:
            r = jnp.concatenate([part(0, K_SPLIT), part(K_SPLIT, d)], axis=1)
        else:
            r = part(0, d)
        return r if acc is None else acc + r

    out = None
    n_out = n_pairs // O_PAIRS
    done = 0
    for t in range(n_pairs + LAG_S + LAG_PV):
        if t < n_pairs:
            project_in(t)
        elif done < n_out - 1:
            out = project_out(done, out)
            done += 1
        if 0 <= t - LAG_S < n_pairs:
            scores(t - LAG_S)
        if 0 <= t - LAG_S - LAG_PV < n_pairs:
            values(t - LAG_S - LAG_PV)
    while done < n_out:
        out = project_out(done, out)
        done += 1

    x_ref[s] = x_in[s].astype(F32) + out[n_mem:, :]
    return out[:n_mem, :], xn_next


def _pair_reduce(t, op):
    r = t[0:8]
    for i in range(8, t.shape[0], 8):
        r = op(r, t[i:i + 8])
    r = op(r, pltpu.roll(r, 4, 0))
    return op(r, pltpu.roll(r, 2, 0))


def _tile_rows(r, n):
    return jnp.concatenate([r] * (n // 8), axis=0)


def _feature_map(p):
    n = p.shape[0]
    e_pos = jnp.exp2(p - _tile_rows(_pair_reduce(p, jnp.maximum), n))
    e_neg = jnp.exp2(_tile_rows(_pair_reduce(p, jnp.minimum), n) - p)
    inv_pos = 1.0 / _pair_reduce(e_pos, jnp.add)
    inv_neg = 1.0 / _pair_reduce(e_neg, jnp.add)
    return jnp.concatenate(
        [e_pos * _tile_rows(inv_pos, n), e_neg * _tile_rows(inv_neg, n)], axis=0).astype(BF16)


def _b_weights(wqkv_ref, wphi_ref, bq_ref, bkv_ref):
    d = wqkv_ref.shape[0]
    dh, _, heads = wphi_ref.shape
    gr = 2 * dh
    c = _iota((dh, d), 1)
    c_feat = c - _div(c, dh) * dh
    spread = (_div(_iota((heads, d), 1), dh) == _iota((heads, d), 0)).astype(BF16)
    by_feat = jnp.zeros((dh, d), F32)
    for e in range(dh):
        t = jnp.dot(wphi_ref[e], spread, preferred_element_type=F32)
        by_feat = jnp.where(c_feat == e, t, by_feat)
    by_feat = by_feat.astype(BF16)

    blk = GB * gr
    r = _iota((blk, dh), 0)
    sel = (((r - _div(r, gr) * gr) >> 1) == _iota((blk, dh), 1)).astype(BF16)
    wv = wqkv_ref[:, 2 * d:3 * d].T
    for b in range(d // blk):
        lo = b * blk // 128 * 128
        hi = -(-(b + 1) * blk // 128) * 128
        r = _iota((blk, hi - lo), 0)
        head = 2 * (_div(r, gr) + b * GB) + (r & 1)
        phi = jnp.dot(sel, by_feat[:, lo:hi], preferred_element_type=F32)
        phi = jnp.where(_div(_iota((1, hi - lo), 1) + lo, dh) == head, phi, 0.0).astype(BF16)
        wq = lax.dot_general(phi, wqkv_ref[:, lo:hi], NT, preferred_element_type=F32)
        wk = lax.dot_general(phi, wqkv_ref[:, d + lo:d + hi], NT, preferred_element_type=F32)
        bq_ref[b] = (wq * LOG2E).astype(BF16)
        bkv_ref[b, 0:blk, :] = (wk * LOG2E).astype(BF16)
        bkv_ref[b, blk:2 * blk, :] = wv[b * blk:(b + 1) * blk]


def _rows(ref, start, n):
    k = n // ref.shape[1]
    return ref[pl.ds(start * k, k)].reshape(n, ref.shape[2])


def _b_keys(it, carry, *, xb_ref, bkv_ref, kv_ref):
    n_blk = bkv_ref.shape[0]
    blk = bkv_ref.shape[1] // 2
    gr = blk // GB
    ones = jnp.ones((8, TB), F32)

    def project(j, b):
        return lax.dot_general(bkv_ref[b], _rows(xb_ref, it * B_UNROLL + j, TB), NT,
                               preferred_element_type=F32)

    def accumulate(b, t):
        for i in range(GB):
            phi = _feature_map(t[i * gr:(i + 1) * gr])
            v = jnp.concatenate([t[blk + i * gr:blk + (i + 1) * gr], ones], axis=0)
            kv_ref[b * GB + i] += lax.dot_general(
                v.astype(BF16), phi, NT, preferred_element_type=F32)

    pending = None
    for j in range(B_UNROLL):
        for b in range(n_blk):
            t = project(j, b)
            if pending is not None:
                accumulate(*pending)
            pending = (b, t)
    accumulate(*pending)
    return carry


def _b_queries(it, *, x_ref, xb_ref, y_ref, bq_ref, bo_ref, kvm_ref, ot_ref):
    n_blk, blk, _ = bq_ref.shape
    gr = blk // GB
    upper = _iota((8, TB), 0) < 4

    def project(j, b):
        return lax.dot_general(bq_ref[b], _rows(xb_ref, it * B_UNROLL + j, TB), NT,
                               preferred_element_type=F32)

    def attend(j, b, t):
        for i in range(GB):
            g = b * GB + i
            phi = _feature_map(t[i * gr:(i + 1) * gr])
            r = jnp.dot(kvm_ref[g], phi, preferred_element_type=F32)
            inv = 1.0 / (r[gr:gr + 8] + 1e-6)
            swapped = pltpu.roll(inv, 4, 0)
            n = (gr - 8) // 16
            inv = jnp.concatenate([jnp.where(upper, inv, swapped)] * n + [inv]
                                  + [jnp.where(upper, swapped, inv)] * n, axis=0)
            ot_ref[j, g * gr:(g + 1) * gr, :] = r[0:gr] * inv

    def finish(j, half):
        at = (it * B_UNROLL + j) * (TB // 128) + half
        o = ot_ref[j, :, half * 128:(half + 1) * 128].astype(BF16)
        x = _rows(x_ref, at, 128) + lax.dot_general(o, bo_ref[...], TN,
                                                    preferred_element_type=F32)
        k = 128 // x_ref.shape[1]
        x = x.reshape((k,) + x_ref.shape[1:])
        x_ref[pl.ds(at * k, k)] = x
        y_ref[pl.ds(at * k, k)] = x.astype(BF16)

    tails = [(j, half) for j in range(B_UNROLL) for half in range(TB // 128)]
    pending = None
    for j in range(B_UNROLL):
        for b in range(n_blk):
            t = project(j, b)
            if pending is not None:
                attend(*pending)
            pending = (j, b, t)
    if B_UNROLL > 1:
        finish(*tails.pop(0))
    attend(*pending)
    for tail in tails:
        finish(*tail)


def _kernel(x_hbm, mem0_ref, wq_hbm, wk_hbm, wv_hbm, wo_hbm, wqkvb_hbm, wphi_ref, wob_hbm,
            out_hbm,
            x_ref, xb_ref, y_ref, xt_ref, xp_ref, stage_ref, pre_ref, w_ref, wo_ref, o_ref,
            wqkvb_ref, bo_ref, bq_ref, bkv_ref, kv_ref, kvm_ref, ot_ref,
            w_sem, in_sem, out_sem, *, dh):
    n_seg, seg, d = x_ref.shape
    n_pairs = w_ref.shape[0]
    pw = 2 * dh
    n_iter = n_seg * seg // (TB * B_UNROLL)

    def pair_rows(p):
        return pl.ds(pl.multiple_of(p * pw, pw), pw)

    def w_copy(p, j):
        return pltpu.make_async_copy(
            (wq_hbm, wk_hbm, wv_hbm)[j].at[pair_rows(p), :],
            stage_ref.at[p, j * pw:(j + 1) * pw, :], w_sem.at[p, j])

    def out_copy(i):
        part = pl.ds(i * (n_seg // n_iter), n_seg // n_iter)
        return pltpu.make_async_copy(y_ref.at[part], out_hbm.at[part], out_sem.at[i])

    xt_copy = pltpu.make_async_copy(x_hbm.at[:, seg - PRE:seg, :], xt_ref, in_sem.at[0])
    wqkvb_copy = pltpu.make_async_copy(wqkvb_hbm, wqkvb_ref, in_sem.at[1])
    wob_copy = pltpu.make_async_copy(wob_hbm, bo_ref, in_sem.at[2])

    xt_copy.start()
    w_copy(0, 1).start()
    w_copy(0, 2).start()
    xt_copy.wait()

    w_copy(0, 0).start()
    for j in (1, 2, 0):
        w_copy(1, j).start()
    xp_ref[...] = _layernorm(xt_ref[...].astype(F32).reshape(n_seg * PRE, d)).astype(BF16)

    def pre_project(p, carry):
        @pl.when(p + 2 < n_pairs)
        def _():
            for j in range(3):
                w_copy(jnp.minimum(p + 2, n_pairs - 1), j).start()

        part = pl.ds(p * (n_seg // n_pairs), n_seg // n_pairs)
        pltpu.make_async_copy(x_hbm.at[part], y_ref.at[part], in_sem.at[3]).start()
        pltpu.make_async_copy(
            wo_hbm.at[pair_rows(p), :], wo_ref.at[pair_rows(p), :], in_sem.at[4]).start()
        for j in range(3):
            w_copy(p, j).wait()
        pre_ref[p] = lax.dot_general(xp_ref[...], stage_ref[p, pw:3 * pw, :], NT,
                                     preferred_element_type=F32)
        for j in range(3):
            w_ref[p, :, j * pw:(j + 1) * pw] = pltpu.bitcast(
                stage_ref[p, j * pw:(j + 1) * pw, :].T, jnp.uint32)
        return carry

    lax.fori_loop(0, n_pairs, pre_project, 0, unroll=P_UNROLL)

    pltpu.make_async_copy(x_hbm, y_ref, in_sem.at[3]).wait()
    pltpu.make_async_copy(wo_hbm, wo_ref, in_sem.at[4]).wait()

    wqkvb_copy.start()
    wob_copy.start()
    x_ref[0] = y_ref[0].astype(F32)

    def layer_a(x_in, pre, unroll):
        step = functools.partial(_a_step, dh=dh, x_in=x_in, x_ref=x_ref, xb_ref=xb_ref,
                                 w_ref=w_ref, wo_ref=wo_ref, pre_ref=pre, o_ref=o_ref)
        lax.fori_loop(0, n_seg, step, (mem0_ref[...].astype(F32), _layernorm(x_ref[0])),
                      unroll=unroll)

    b_keys = functools.partial(_b_keys, xb_ref=xb_ref, bkv_ref=bkv_ref, kv_ref=kv_ref)
    b_queries = functools.partial(_b_queries, x_ref=x_ref, xb_ref=xb_ref, y_ref=y_ref,
                                  bq_ref=bq_ref, bo_ref=bo_ref, kvm_ref=kvm_ref, ot_ref=ot_ref)

    def layer_pair(layer, carry):
        @pl.when(layer == 0)
        def _():
            layer_a(y_ref, pre_ref, A_UNROLL[0])

        @pl.when(layer == 0)
        def _():
            wqkvb_copy.wait()
            wob_copy.wait()
            _b_weights(wqkvb_ref, wphi_ref, bq_ref, bkv_ref)

        @pl.when(layer == 1)
        def _():
            layer_a(x_ref, None, A_UNROLL[1])

        xb_ref[n_seg - 1] = _layernorm(x_ref[n_seg - 1]).astype(BF16)
        kv_ref[...] = jnp.zeros(kv_ref.shape, F32)
        lax.fori_loop(0, n_iter, b_keys, 0)

        gr = kv_ref.shape[1] - 8
        r = _iota(kv_ref.shape, 1)
        second = ((r >= gr // 2) & (r < gr)) | (r >= gr + 4)
        same_head = second == ((_iota(kv_ref.shape, 2) & 1) == 1)
        kvm_ref[...] = jnp.where(same_head, kv_ref[...], 0.0).astype(BF16)

        def queries(it, carry):
            b_queries(it)

            @pl.when(layer == 1)
            def _():
                out_copy(it).start()

            return carry

        lax.fori_loop(0, n_iter, queries, 0)

        return carry

    lax.fori_loop(0, 2, layer_pair, 0)
    for i in range(n_iter):
        out_copy(i).wait()


@functools.partial(jax.jit, static_argnames=("A_seg_len",))
def pallas_interleave_layers__memory_aug_recurrent_mem_tr__linear_kernel_hedgehog__prompt_kernel(
    A_x, A_mem0, A_Wq, A_Wk, A_Wv, A_Wo, A_seg_len, B_x, B_wqkv, B_w_phi, B_wo,
):
    del B_x
    batch, s_len, d = A_x.shape
    _, heads, dh = A_Wq.shape
    n_mem = A_mem0.shape[1]
    seg = int(A_seg_len)
    b_heads, b_dh, _ = B_w_phi.shape
    rows = n_mem + seg
    n_pairs = heads // 2
    gr = 2 * b_dh
    blk = GB * gr
    n_seg = s_len // seg
    assert batch == 1 and dh == 192 and heads % (2 * O_PAIRS) == 0
    assert n_mem % 8 == 0 and seg % 16 == 0 and 128 % seg == 0 and 2 * rows <= 128
    assert s_len % (TB * B_UNROLL) == 0 and n_seg % n_pairs == 0
    assert b_heads * b_dh == d and b_dh % 8 == 4 and d % blk == 0

    def head_major(w):
        return w.transpose(1, 2, 0).reshape(heads * dh, d)

    hbm = pl.BlockSpec(memory_space=pltpu.HBM)
    vmem = pl.BlockSpec(memory_space=pltpu.VMEM)
    out = pl.pallas_call(
        functools.partial(_kernel, dh=dh),
        out_shape=jax.ShapeDtypeStruct((n_seg, seg, d), A_x.dtype),
        in_specs=[hbm, vmem, hbm, hbm, hbm, hbm, hbm, vmem, hbm],
        out_specs=hbm,
        scratch_shapes=[
            pltpu.VMEM((n_seg, seg, d), F32),
            pltpu.VMEM((n_seg, seg, d), BF16),
            pltpu.VMEM((n_seg, seg, d), BF16),
            pltpu.VMEM((n_seg, PRE, d), BF16),
            pltpu.VMEM((n_seg * PRE, d), BF16),
            pltpu.VMEM((n_pairs, 6 * dh, d), BF16),
            pltpu.VMEM((n_pairs, n_seg * PRE, 4 * dh), F32),
            pltpu.VMEM((n_pairs, d // 2, 6 * dh), jnp.uint32),
            pltpu.VMEM((heads * dh, d), BF16),
            pltpu.VMEM((rows, heads * dh), F32),
            pltpu.VMEM(B_wqkv.shape, BF16),
            pltpu.VMEM(B_wo.shape, BF16),
            pltpu.VMEM((d // blk, blk, d), BF16),
            pltpu.VMEM((d // blk, 2 * blk, d), BF16),
            pltpu.VMEM((b_heads // 2, gr + 8, 2 * gr), F32),
            pltpu.VMEM((b_heads // 2, gr + 8, 2 * gr), BF16),
            pltpu.VMEM((B_UNROLL, d, TB), F32),
            pltpu.SemaphoreType.DMA((n_pairs, 3)),
            pltpu.SemaphoreType.DMA((5,)),
            pltpu.SemaphoreType.DMA((s_len // (TB * B_UNROLL),)),
        ],
        compiler_params=pltpu.CompilerParams(vmem_limit_bytes=120 * 1024 * 1024),
    )(
        A_x.reshape(n_seg, seg, d), A_mem0.reshape(n_mem, d),
        head_major(A_Wq), head_major(A_Wk), head_major(A_Wv), A_Wo.reshape(heads * dh, d),
        B_wqkv, B_w_phi.transpose(1, 2, 0), B_wo,
    )
    return out.reshape(batch, s_len, d)
```

```python
import functools
import math

import jax
import jax.numpy as jnp
from jax import lax
import jax.experimental.pallas as pl
import jax.experimental.pallas.tpu as pltpu

F32 = jnp.float32
BF16 = jnp.bfloat16
NT = (((1,), (1,)), ((), ()))
LOG2E = math.log2(math.e)

LAG_S = 2
LAG_PV = 2
O_PAIRS = 4
A_UNROLL = (2, 2)
K_SPLIT = 512
NORM_AT = (4, 8)
PRE = 8
P_UNROLL = 1
TB = 512
K_PAIRS = 8
Q_PAIRS = 8
Q_LAG = 1
F_PAIRS = 2
O_ROWS = (128, 128, 128, 128)


def _iota(shape, axis):
    return lax.broadcasted_iota(jnp.int32, shape, axis)


def _div(v, d):
    return (v * ((1 << 18) // d + 1)) >> 18


def _pack(x):
    return pltpu.bitcast(x.astype(BF16), jnp.uint32)


def _unpack(x):
    return pltpu.bitcast(x, BF16)


def _recip(x):
    r = pl.reciprocal(x, approx=True)
    return r * (2.0 - x * r)


def _layernorm(x):
    m = jnp.mean(x, axis=-1, keepdims=True)
    c = x - m
    v = jnp.mean(c * c, axis=-1, keepdims=True)
    return c * lax.rsqrt(v + 1e-5)


def _a_step(s, carry, *, dh, x_in, x_ref, xb_ref, w_ref, wo_ref, pre_ref, o_ref):
    mem, xn = carry
    n_mem, seg = mem.shape[0], xn.shape[0]
    rows = n_mem + seg
    pw = 2 * dh
    n_pairs = w_ref.shape[0]
    scale = dh ** -0.5

    nxt = jnp.minimum(s + 1, x_ref.shape[0] - 1)
    prv = jnp.maximum(s - 1, 0)
    xn_next = _layernorm(x_in[nxt].astype(F32))
    xb_prev = _layernorm(x_ref[prv])
    xb_ref[prv] = xb_prev.astype(BF16)

    def schedule_before(value, early):
        t = functools.reduce(jnp.maximum, [early[i:i + 8, j:j + 128]
                                           for i in range(0, early.shape[0], 8)
                                           for j in range(0, early.shape[1], 128)])
        head = jnp.where(s < 0, t[:, :value.shape[1]], value[0:8])
        return jnp.concatenate([head, value[8:]], axis=0)

    h = jnp.concatenate([mem, xn], axis=0)
    h_short = h[:rows - PRE].astype(BF16)

    first = _iota((rows, 128), 1) < (dh - 128)
    col = _iota((rows, 2 * rows), 1)
    row = _iota((rows, 2 * rows), 0)
    is_a = col < rows
    visible = (row < n_mem) | (row >= jnp.where(is_a, col, col - rows))
    zero = jnp.zeros((rows, 128), F32)

    def block_diag(t):
        t0, t1, t2 = t[:, 0:128], t[:, 128:256], t[:, 256:384]
        top = jnp.concatenate([t0, jnp.where(first, t1, 0.0), zero], axis=1)
        bot = jnp.concatenate([zero, jnp.where(first, 0.0, t1), t2], axis=1)
        return jnp.concatenate([top, bot], axis=0).astype(BF16)

    qkv, probs = {}, {}

    def times_w(lhs, p, lo, hi):
        def part(k0, k1):
            w = _unpack(w_ref[p, k0 // 2:k1 // 2, lo:hi])
            return jnp.dot(lhs[:, k0:k1], w, preferred_element_type=F32)

        if p == 0 and lo == 0 and K_SPLIT:
            return part(K_SPLIT, lhs.shape[1]) + part(0, K_SPLIT)
        return part(0, lhs.shape[1])

    def project_in(p):
        if pre_ref is None:
            qkv[p] = times_w(h, p, 0, 3 * pw)
        else:
            q = times_w(h, p, 0, pw)
            kv = jnp.concatenate(
                [times_w(h_short, p, pw, 3 * pw),
                 pre_ref[p, pl.ds(pl.multiple_of(s * PRE, PRE), PRE), :]], axis=0)
            qkv[p] = jnp.concatenate([q, kv], axis=1)

    def scores(p):
        t = qkv[p]
        sc = lax.dot_general(t[:, 0:pw], block_diag(t[:, pw:2 * pw]), NT,
                             preferred_element_type=F32)
        sc = jnp.where(visible, sc * scale, -1e9)
        max_a = jnp.max(jnp.where(is_a, sc, -jnp.inf), axis=1, keepdims=True)
        max_b = jnp.max(jnp.where(is_a, -jnp.inf, sc), axis=1, keepdims=True)
        e = jnp.exp(sc - jnp.where(is_a, max_a, max_b))
        sum_a = jnp.sum(jnp.where(is_a, e, 0.0), axis=1, keepdims=True)
        sum_b = jnp.sum(jnp.where(is_a, 0.0, e), axis=1, keepdims=True)
        probs[p] = e * _recip(jnp.where(is_a, sum_a, sum_b))
        if p == NORM_AT[0]:
            probs[p] = schedule_before(probs[p], xn_next)
        if p == NORM_AT[1]:
            probs[p] = schedule_before(probs[p], xb_prev)

    def values(p):
        o_ref[:, p * pw:(p + 1) * pw] = jnp.dot(
            probs[p], block_diag(qkv[p][:, 2 * pw:3 * pw]), preferred_element_type=F32)

    def project_out(c, acc):
        lo, hi = c * O_PAIRS * pw, (c + 1) * O_PAIRS * pw

        def part(c0, c1):
            return jnp.dot(o_ref[:, lo:hi], wo_ref[lo:hi, c0:c1], preferred_element_type=F32)

        d = wo_ref.shape[1]
        if hi == wo_ref.shape[0] and K_SPLIT:
            r = jnp.concatenate([part(0, K_SPLIT), part(K_SPLIT, d)], axis=1)
        else:
            r = part(0, d)
        return r if acc is None else acc + r

    out = None
    n_out = n_pairs // O_PAIRS
    done = 0
    for t in range(n_pairs + LAG_S + LAG_PV):
        if t < n_pairs:
            project_in(t)
        elif done < n_out - 1:
            out = project_out(done, out)
            done += 1
        if 0 <= t - LAG_S < n_pairs:
            scores(t - LAG_S)
        if 0 <= t - LAG_S - LAG_PV < n_pairs:
            values(t - LAG_S - LAG_PV)
    while done < n_out:
        out = project_out(done, out)
        done += 1

    x_ref[s] = x_in[s].astype(F32) + out[n_mem:, :]
    return out[:n_mem, :], xn_next


def _pair_reduce(t, op):
    r = t[0:8]
    for i in range(8, t.shape[0], 8):
        r = op(r, t[i:i + 8])
    r = op(r, pltpu.roll(r, 4, 0))
    return op(r, pltpu.roll(r, 2, 0))


def _tile_rows(r, n):
    return jnp.concatenate([r] * (n // 8), axis=0)


def _feature_map(p):
    n = p.shape[0]
    e_pos = jnp.exp2(p - _tile_rows(_pair_reduce(p, jnp.maximum), n))
    e_neg = jnp.exp2(_tile_rows(_pair_reduce(p, jnp.minimum), n) - p)
    inv_pos = _recip(_pair_reduce(e_pos, jnp.add))
    inv_neg = _recip(_pair_reduce(e_neg, jnp.add))
    return jnp.concatenate(
        [e_pos * _tile_rows(inv_pos, n), e_neg * _tile_rows(inv_neg, n)], axis=0)


def _b_weights(wqkv_ref, wphi_ref, wob_ref, bq_ref, bkv_ref, bo_ref):
    d = wqkv_ref.shape[0]
    dh, _, heads = wphi_ref.shape
    gr = 2 * dh
    c = _iota((dh, d), 1)
    c_feat = c - _div(c, dh) * dh
    spread = (_div(_iota((heads, d), 1), dh) == _iota((heads, d), 0)).astype(BF16)
    by_feat = jnp.zeros((dh, d), F32)
    for e in range(dh):
        t = jnp.dot(wphi_ref[e], spread, preferred_element_type=F32)
        by_feat = jnp.where(c_feat == e, t, by_feat)
    by_feat = by_feat.astype(BF16)

    blk = F_PAIRS * gr
    r = _iota((blk, dh), 0)
    sel = (((r - _div(r, gr) * gr) >> 1) == _iota((blk, dh), 1)).astype(BF16)
    half = bkv_ref.shape[1]
    bo_ref[...] = _pack(wob_ref[...])
    wv = wqkv_ref[:, 2 * d:3 * d].T
    for b in range(d // half):
        bkv_ref[b, half // 2:half, :] = _pack(wv[b * half:(b + 1) * half])
    phis = []
    for b in range(d // blk):
        lo = b * blk // 128 * 128
        hi = -(-(b + 1) * blk // 128) * 128
        r = _iota((blk, hi - lo), 0)
        head = 2 * (_div(r, gr) + b * F_PAIRS) + (r & 1)
        phi = jnp.dot(sel, by_feat[:, lo:hi], preferred_element_type=F32)
        phi = jnp.where(_div(_iota((1, hi - lo), 1) + lo, dh) == head, phi, 0.0)
        phis.append((phi.astype(BF16), lo, hi))
    for b, (phi, lo, hi) in enumerate(phis):
        wq = lax.dot_general(phi, wqkv_ref[:, lo:hi], NT, preferred_element_type=F32)
        wk = lax.dot_general(phi, wqkv_ref[:, d + lo:d + hi], NT, preferred_element_type=F32)
        bq_ref[b * blk // 2:(b + 1) * blk // 2, :] = _pack(wq * LOG2E)
        at = b * blk % half // 2
        bkv_ref[b * blk // half, at:at + blk // 2, :] = _pack(wk * LOG2E)


def _chunk_rows(ref, it, r0, n):
    seg = ref.shape[1]
    return pl.ds(it * (TB // seg) + r0 // seg, n // seg)


def _b_keys(it, carry, *, xb_ref, bkv_ref, kv_ref, z_ref):
    n_blk, half, _ = bkv_ref.shape
    gr = half // K_PAIRS
    xb = xb_ref[_chunk_rows(xb_ref, it, 0, TB)].reshape(TB, -1)

    def accumulate(b, t):
        for i in range(K_PAIRS):
            g = b * K_PAIRS + i
            phi = _feature_map(t[i * gr:(i + 1) * gr])
            z_ref[g] += sum(phi[:, j:j + 128] for j in range(0, TB, 128))
            kv_ref[g] += lax.dot_general(t[half + i * gr:half + (i + 1) * gr], phi.astype(BF16),
                                         NT, preferred_element_type=F32)

    pending = None
    for b in range(n_blk):
        t = lax.dot_general(_unpack(bkv_ref[b]), xb, NT, preferred_element_type=F32)
        if pending is not None:
            accumulate(*pending)
        pending = (b, t)
    accumulate(*pending)
    return carry


def _b_queries(it, *, x_ref, xb_ref, y_ref, bq_ref, bo_ref, kv_ref, z_ref, ot_ref, on_ref):
    n_groups, gr, _ = kv_ref.shape
    blk = Q_PAIRS * gr
    sub = _iota((8, TB), 0)
    xb = xb_ref[_chunk_rows(xb_ref, it, 0, TB)].reshape(TB, -1)

    def attend(b, t):
        outs = []
        for i in range(Q_PAIRS):
            g = b * Q_PAIRS + i
            phi = _feature_map(t[i * gr:(i + 1) * gr])
            num = jnp.dot(kv_ref[g], phi.astype(BF16), preferred_element_type=F32)
            z = jnp.concatenate([z_ref[g]] * (TB // 128), axis=1)
            inv = _recip(_pair_reduce(phi * z, jnp.add) + 1e-6)
            other = pltpu.roll(inv, 1, 0)
            inv_a = jnp.where((sub & 1) == 0, inv, other)
            inv_b = jnp.where((sub & 1) == 0, other, inv)
            n = (gr - 8) // 16
            inv = jnp.concatenate(
                [inv_a] * n + [jnp.where(sub < 4, inv_a, inv_b)] + [inv_b] * n, axis=0)
            outs.append(num * inv)
        ot_ref[b * blk // 2:(b + 1) * blk // 2, :] = _pack(jnp.concatenate(outs, axis=0))

    n_blk = n_groups // Q_PAIRS
    proj = {}
    for b in range(n_blk + Q_LAG):
        if b < n_blk:
            proj[b] = lax.dot_general(_unpack(bq_ref[b * blk // 2:(b + 1) * blk // 2, :]), xb,
                                      NT, preferred_element_type=F32)
        if b >= Q_LAG:
            attend(b - Q_LAG, proj[b - Q_LAG])
    on_ref[...] = _pack(_unpack(ot_ref[...]).T)
    r0 = 0
    for n in O_ROWS:
        at = _chunk_rows(x_ref, it, r0, n)
        y = jnp.dot(_unpack(on_ref[r0 // 2:(r0 + n) // 2, :]), _unpack(bo_ref[...]),
                    preferred_element_type=F32)
        x = x_ref[at] + y.reshape((-1,) + x_ref.shape[1:])
        x_ref[at] = x
        y_ref[at] = x.astype(BF16)
        r0 += n


def _kernel(x_hbm, mem0_hbm, wq_hbm, wk_hbm, wv_hbm, wo_hbm, wqkvb_hbm, wphi_hbm, wob_hbm,
            out_hbm,
            x_ref, xb_ref, y_ref, xt_ref, xp_ref, stage_ref, pre_ref, w_ref, wo_ref, o_ref,
            mem0_ref, wphi_ref, wqkvb_ref, wob_ref, bo_ref, bq_ref, bkv_ref, kv_ref, z_ref, ot_ref, on_ref,
            w_sem, in_sem, out_sem, *, dh):
    n_seg, seg, d = x_ref.shape
    n_pairs = w_ref.shape[0]
    pw = 2 * dh
    n_iter = n_seg * seg // TB

    def pair_rows(p):
        return pl.ds(pl.multiple_of(p * pw, pw), pw)

    def w_copy(p, j):
        return pltpu.make_async_copy(
            (wq_hbm, wk_hbm, wv_hbm)[j].at[pair_rows(p), :],
            stage_ref.at[p, j * pw:(j + 1) * pw, :], w_sem.at[p, j])

    def out_copy(i):
        part = pl.ds(i * (n_seg // n_iter), n_seg // n_iter)
        return pltpu.make_async_copy(y_ref.at[part], out_hbm.at[part], out_sem.at[i])

    xt_copy = pltpu.make_async_copy(x_hbm.at[:, seg - PRE:seg, :], xt_ref, in_sem.at[0])
    wqkvb_copy = pltpu.make_async_copy(wqkvb_hbm, wqkvb_ref, in_sem.at[1])
    wphi_copy = pltpu.make_async_copy(wphi_hbm, wphi_ref, in_sem.at[5])
    mem0_copy = pltpu.make_async_copy(mem0_hbm, mem0_ref, in_sem.at[6])
    wob_copy = pltpu.make_async_copy(wob_hbm, wob_ref, in_sem.at[2])

    xt_copy.start()
    w_copy(0, 1).start()
    w_copy(0, 2).start()
    xt_copy.wait()

    w_copy(0, 0).start()
    mem0_copy.start()
    for j in (1, 2, 0):
        w_copy(1, j).start()
    xp_ref[...] = _layernorm(xt_ref[...].astype(F32).reshape(n_seg * PRE, d)).astype(BF16)

    def pre_project(p, carry):
        @pl.when(p + 2 < n_pairs)
        def _():
            for j in range(3):
                w_copy(jnp.minimum(p + 2, n_pairs - 1), j).start()

        part = pl.ds(p * (n_seg // n_pairs), n_seg // n_pairs)
        pltpu.make_async_copy(x_hbm.at[part], y_ref.at[part], in_sem.at[3]).start()
        pltpu.make_async_copy(
            wo_hbm.at[pair_rows(p), :], wo_ref.at[pair_rows(p), :], in_sem.at[4]).start()
        for j in range(3):
            w_copy(p, j).wait()
        pre_ref[p] = lax.dot_general(xp_ref[...], stage_ref[p, pw:3 * pw, :], NT,
                                     preferred_element_type=F32)
        for j in range(3):
            w_ref[p, :, j * pw:(j + 1) * pw] = _pack(stage_ref[p, j * pw:(j + 1) * pw, :].T)
        return carry

    lax.fori_loop(0, n_pairs, pre_project, 0, unroll=P_UNROLL)

    pltpu.make_async_copy(x_hbm, y_ref, in_sem.at[3]).wait()
    pltpu.make_async_copy(wo_hbm, wo_ref, in_sem.at[4]).wait()

    wqkvb_copy.start()
    wob_copy.start()
    wphi_copy.start()
    mem0_copy.wait()
    x_ref[0] = y_ref[0].astype(F32)

    def layer_a(x_in, pre, unroll):
        step = functools.partial(_a_step, dh=dh, x_in=x_in, x_ref=x_ref, xb_ref=xb_ref,
                                 w_ref=w_ref, wo_ref=wo_ref, pre_ref=pre, o_ref=o_ref)
        lax.fori_loop(0, n_seg, step, (mem0_ref[...].astype(F32), _layernorm(x_ref[0])),
                      unroll=unroll)

    b_keys = functools.partial(_b_keys, xb_ref=xb_ref, bkv_ref=bkv_ref, kv_ref=kv_ref,
                               z_ref=z_ref)
    b_queries = functools.partial(_b_queries, x_ref=x_ref, xb_ref=xb_ref, y_ref=y_ref,
                                  bq_ref=bq_ref, bo_ref=bo_ref, kv_ref=kv_ref, z_ref=z_ref,
                                  ot_ref=ot_ref, on_ref=on_ref)

    def layer_pair(layer, carry):
        @pl.when(layer == 0)
        def _():
            layer_a(y_ref, pre_ref, A_UNROLL[0])

        @pl.when(layer == 0)
        def _():
            wqkvb_copy.wait()
            wob_copy.wait()
            wphi_copy.wait()
            _b_weights(wqkvb_ref, wphi_ref, wob_ref, bq_ref, bkv_ref, bo_ref)

        @pl.when(layer == 1)
        def _():
            layer_a(x_ref, None, A_UNROLL[1])

        xb_ref[n_seg - 1] = _layernorm(x_ref[n_seg - 1]).astype(BF16)
        kv_ref[...] = jnp.zeros(kv_ref.shape, F32)
        z_ref[...] = jnp.zeros(z_ref.shape, F32)
        lax.fori_loop(0, n_iter, b_keys, 0)

        same_head = ((_iota(kv_ref.shape, 1) >= kv_ref.shape[1] // 2)
                     == ((_iota(kv_ref.shape, 2) & 1) == 1))
        kv_ref[...] = jnp.where(same_head, kv_ref[...], 0.0)
        z_ref[...] = jnp.broadcast_to(jnp.sum(z_ref[...], axis=-1, keepdims=True), z_ref.shape)

        def queries(it, carry):
            b_queries(it)

            @pl.when(layer == 1)
            def _():
                out_copy(it).start()

            return carry

        lax.fori_loop(0, n_iter, queries, 0)

        return carry

    lax.fori_loop(0, 2, layer_pair, 0)
    for i in range(n_iter):
        out_copy(i).wait()


@functools.partial(jax.jit, static_argnames=("A_seg_len",))
def pallas_interleave_layers__memory_aug_recurrent_mem_tr__linear_kernel_hedgehog__prompt_kernel(
    A_x, A_mem0, A_Wq, A_Wk, A_Wv, A_Wo, A_seg_len, B_x, B_wqkv, B_w_phi, B_wo,
):
    del B_x
    batch, s_len, d = A_x.shape
    _, heads, dh = A_Wq.shape
    n_mem = A_mem0.shape[1]
    seg = int(A_seg_len)
    b_heads, b_dh, _ = B_w_phi.shape
    rows = n_mem + seg
    n_pairs = heads // 2
    gr = 2 * b_dh
    half = K_PAIRS * gr
    n_seg = s_len // seg
    assert batch == 1 and dh == 192 and heads % (2 * O_PAIRS) == 0
    assert n_mem % 8 == 0 and seg % 16 == 0 and 128 % seg == 0 and 2 * rows <= 128
    assert s_len % TB == 0 and sum(O_ROWS) == TB and n_seg % n_pairs == 0
    assert b_heads * b_dh == d and b_dh % 8 == 4 and d % half == 0

    def head_major(w):
        return w.transpose(1, 2, 0).reshape(heads * dh, d)

    hbm = pl.BlockSpec(memory_space=pltpu.HBM)
    out = pl.pallas_call(
        functools.partial(_kernel, dh=dh),
        out_shape=jax.ShapeDtypeStruct((n_seg, seg, d), A_x.dtype),
        in_specs=[hbm] * 9,
        out_specs=hbm,
        scratch_shapes=[
            pltpu.VMEM((n_seg, seg, d), F32),
            pltpu.VMEM((n_seg, seg, d), BF16),
            pltpu.VMEM((n_seg, seg, d), BF16),
            pltpu.VMEM((n_seg, PRE, d), BF16),
            pltpu.VMEM((n_seg * PRE, d), BF16),
            pltpu.VMEM((n_pairs, 6 * dh, d), BF16),
            pltpu.VMEM((n_pairs, n_seg * PRE, 4 * dh), F32),
            pltpu.VMEM((n_pairs, d // 2, 6 * dh), jnp.uint32),
            pltpu.VMEM((heads * dh, d), BF16),
            pltpu.VMEM((rows, heads * dh), F32),
            pltpu.VMEM((n_mem, d), BF16),
            pltpu.VMEM((b_dh, b_dh, b_heads), BF16),
            pltpu.VMEM(B_wqkv.shape, BF16),
            pltpu.VMEM(B_wo.shape, BF16),
            pltpu.VMEM((d // 2, d), jnp.uint32),
            pltpu.VMEM((d // 2, d), jnp.uint32),
            pltpu.VMEM((d // half, half, d), jnp.uint32),
            pltpu.VMEM((b_heads // 2, gr, 2 * gr), F32),
            pltpu.VMEM((b_heads // 2, 2 * gr, 128), F32),
            pltpu.VMEM((d // 2, TB), jnp.uint32),
            pltpu.VMEM((TB // 2, d), jnp.uint32),
            pltpu.SemaphoreType.DMA((n_pairs, 3)),
            pltpu.SemaphoreType.DMA((7,)),
            pltpu.SemaphoreType.DMA((s_len // TB,)),
        ],
        compiler_params=pltpu.CompilerParams(vmem_limit_bytes=120 * 1024 * 1024),
    )(
        A_x.reshape(n_seg, seg, d), A_mem0.reshape(n_mem, d),
        head_major(A_Wq), head_major(A_Wk), head_major(A_Wv), A_Wo.reshape(heads * dh, d),
        B_wqkv, B_w_phi.transpose(1, 2, 0), B_wo,
    )
    return out.reshape(batch, s_len, d)
```

```python
import functools
import math

import jax
import jax.numpy as jnp
from jax import lax
import jax.experimental.pallas as pl
import jax.experimental.pallas.tpu as pltpu

F32 = jnp.float32
BF16 = jnp.bfloat16
NT = (((1,), (1,)), ((), ()))
LOG2E = math.log2(math.e)

LAG_S = 2
LAG_PV = 2
O_PAIRS = 4
A_UNROLL = (2, 2)
K_SPLIT = 512
NORM_AT = (4, 8)
PRE = 8
P_UNROLL = 1
TB = 512
K_PAIRS = 8
Q_PAIRS = 8
Q_LAG = 1
F_PAIRS = 2
O_ROWS = (128, 128, 128, 128)


def _iota(shape, axis):
    return lax.broadcasted_iota(jnp.int32, shape, axis)


def _div(v, d):
    return (v * ((1 << 18) // d + 1)) >> 18


def _pack(x):
    return pltpu.bitcast(x.astype(BF16), jnp.uint32)


def _unpack(x):
    return pltpu.bitcast(x, BF16)


def _recip(x):
    r = pl.reciprocal(x, approx=True)
    return r * (2.0 - x * r)


def _layernorm(x):
    m = jnp.mean(x, axis=-1, keepdims=True)
    c = x - m
    v = jnp.mean(c * c, axis=-1, keepdims=True)
    return c * lax.rsqrt(v + 1e-5)


def _a_step(s, carry, *, dh, x_in, x_ref, xb_ref, w_ref, wo_ref, pre_ref, o_ref):
    mem, xn = carry
    n_mem, seg = mem.shape[0], xn.shape[0]
    rows = n_mem + seg
    pw = 2 * dh
    n_pairs = w_ref.shape[0]
    scale = dh ** -0.5

    nxt = jnp.minimum(s + 1, x_ref.shape[0] - 1)
    prv = jnp.maximum(s - 1, 0)
    xn_next = _layernorm(x_in[nxt].astype(F32))
    xb_prev = _layernorm(x_ref[prv])
    xb_ref[prv] = xb_prev.astype(BF16)

    def schedule_before(value, early):
        t = functools.reduce(jnp.maximum, [early[i:i + 8, j:j + 128]
                                           for i in range(0, early.shape[0], 8)
                                           for j in range(0, early.shape[1], 128)])
        head = jnp.where(s < 0, t[:, :value.shape[1]], value[0:8])
        return jnp.concatenate([head, value[8:]], axis=0)

    h = jnp.concatenate([mem, xn], axis=0)
    h_short = h[:rows - PRE].astype(BF16)

    first = _iota((rows, 128), 1) < (dh - 128)
    col = _iota((rows, 2 * rows), 1)
    row = _iota((rows, 2 * rows), 0)
    is_a = col < rows
    visible = (row < n_mem) | (row >= jnp.where(is_a, col, col - rows))
    zero = jnp.zeros((rows, 128), F32)

    def block_diag(t):
        t0, t1, t2 = t[:, 0:128], t[:, 128:256], t[:, 256:384]
        top = jnp.concatenate([t0, jnp.where(first, t1, 0.0), zero], axis=1)
        bot = jnp.concatenate([zero, jnp.where(first, 0.0, t1), t2], axis=1)
        return jnp.concatenate([top, bot], axis=0).astype(BF16)

    qkv, probs = {}, {}

    def times_w(lhs, p, lo, hi):
        def part(k0, k1):
            w = _unpack(w_ref[p, k0 // 2:k1 // 2, lo:hi])
            return jnp.dot(lhs[:, k0:k1], w, preferred_element_type=F32)

        if p == 0 and lo == 0 and K_SPLIT:
            return part(K_SPLIT, lhs.shape[1]) + part(0, K_SPLIT)
        return part(0, lhs.shape[1])

    def project_in(p):
        if pre_ref is None:
            qkv[p] = times_w(h, p, 0, 3 * pw)
        else:
            q = times_w(h, p, 0, pw)
            kv = jnp.concatenate(
                [times_w(h_short, p, pw, 3 * pw),
                 pre_ref[p, pl.ds(pl.multiple_of(s * PRE, PRE), PRE), :]], axis=0)
            qkv[p] = jnp.concatenate([q, kv], axis=1)

    def scores(p):
        t = qkv[p]
        sc = lax.dot_general(t[:, 0:pw], block_diag(t[:, pw:2 * pw]), NT,
                             preferred_element_type=F32)
        sc = jnp.where(visible, sc * scale, -1e9)
        max_a = jnp.max(jnp.where(is_a, sc, -jnp.inf), axis=1, keepdims=True)
        max_b = jnp.max(jnp.where(is_a, -jnp.inf, sc), axis=1, keepdims=True)
        e = jnp.exp(sc - jnp.where(is_a, max_a, max_b))
        sum_a = jnp.sum(jnp.where(is_a, e, 0.0), axis=1, keepdims=True)
        sum_b = jnp.sum(jnp.where(is_a, 0.0, e), axis=1, keepdims=True)
        probs[p] = e * _recip(jnp.where(is_a, sum_a, sum_b))
        if p == NORM_AT[0]:
            probs[p] = schedule_before(probs[p], xn_next)
        if p == NORM_AT[1]:
            probs[p] = schedule_before(probs[p], xb_prev)

    def values(p):
        o_ref[:, p * pw:(p + 1) * pw] = jnp.dot(
            probs[p], block_diag(qkv[p][:, 2 * pw:3 * pw]), preferred_element_type=F32)

    def project_out(c, acc):
        lo, hi = c * O_PAIRS * pw, (c + 1) * O_PAIRS * pw

        def part(c0, c1):
            return jnp.dot(o_ref[:, lo:hi], wo_ref[lo:hi, c0:c1], preferred_element_type=F32)

        d = wo_ref.shape[1]
        if hi == wo_ref.shape[0] and K_SPLIT:
            r = jnp.concatenate([part(0, K_SPLIT), part(K_SPLIT, d)], axis=1)
        else:
            r = part(0, d)
        return r if acc is None else acc + r

    out = None
    n_out = n_pairs // O_PAIRS
    done = 0
    for t in range(n_pairs + LAG_S + LAG_PV):
        if t < n_pairs:
            project_in(t)
        elif done < n_out - 1:
            out = project_out(done, out)
            done += 1
        if 0 <= t - LAG_S < n_pairs:
            scores(t - LAG_S)
        if 0 <= t - LAG_S - LAG_PV < n_pairs:
            values(t - LAG_S - LAG_PV)
    while done < n_out:
        out = project_out(done, out)
        done += 1

    x_ref[s] = x_in[s].astype(F32) + out[n_mem:, :]
    return out[:n_mem, :], xn_next


def _pair_reduce(t, op):
    r = t[0:8]
    for i in range(8, t.shape[0], 8):
        r = op(r, t[i:i + 8])
    r = op(r, pltpu.roll(r, 4, 0))
    return op(r, pltpu.roll(r, 2, 0))


def _tile_rows(r, n):
    return jnp.concatenate([r] * (n // 8), axis=0)


def _feature_map(p):
    n = p.shape[0]
    e_pos = jnp.exp2(p - _tile_rows(_pair_reduce(p, jnp.maximum), n))
    e_neg = jnp.exp2(_tile_rows(_pair_reduce(p, jnp.minimum), n) - p)
    inv_pos = _recip(_pair_reduce(e_pos, jnp.add))
    inv_neg = _recip(_pair_reduce(e_neg, jnp.add))
    return jnp.concatenate(
        [e_pos * _tile_rows(inv_pos, n), e_neg * _tile_rows(inv_neg, n)], axis=0)


def _b_weights(wqkv_ref, wphi_ref, wob_ref, bq_ref, bkv_ref, bo_ref):
    d = wqkv_ref.shape[0]
    dh, _, heads = wphi_ref.shape
    gr = 2 * dh
    c = _iota((dh, d), 1)
    c_feat = c - _div(c, dh) * dh
    spread = (_div(_iota((heads, d), 1), dh) == _iota((heads, d), 0)).astype(BF16)
    by_feat = jnp.zeros((dh, d), F32)
    for e in range(dh):
        t = jnp.dot(wphi_ref[e], spread, preferred_element_type=F32)
        by_feat = jnp.where(c_feat == e, t, by_feat)
    by_feat = by_feat.astype(BF16)

    blk = F_PAIRS * gr
    r = _iota((blk, dh), 0)
    sel = (((r - _div(r, gr) * gr) >> 1) == _iota((blk, dh), 1)).astype(BF16)
    half = bkv_ref.shape[1]
    bo_ref[...] = _pack(wob_ref[...])
    wv = wqkv_ref[:, 2 * d:3 * d].T
    for b in range(d // half):
        bkv_ref[b, half // 2:half, :] = _pack(wv[b * half:(b + 1) * half])
    phis = []
    for b in range(d // blk):
        lo = b * blk // 128 * 128
        hi = -(-(b + 1) * blk // 128) * 128
        r = _iota((blk, hi - lo), 0)
        head = 2 * (_div(r, gr) + b * F_PAIRS) + (r & 1)
        phi = jnp.dot(sel, by_feat[:, lo:hi], preferred_element_type=F32)
        phi = jnp.where(_div(_iota((1, hi - lo), 1) + lo, dh) == head, phi, 0.0)
        phis.append((phi.astype(BF16), lo, hi))
    for b, (phi, lo, hi) in enumerate(phis):
        wq = lax.dot_general(phi, wqkv_ref[:, lo:hi], NT, preferred_element_type=F32)
        wk = lax.dot_general(phi, wqkv_ref[:, d + lo:d + hi], NT, preferred_element_type=F32)
        bq_ref[b * blk // 2:(b + 1) * blk // 2, :] = _pack(wq * LOG2E)
        at = b * blk % half // 2
        bkv_ref[b * blk // half, at:at + blk // 2, :] = _pack(wk * LOG2E)


def _chunk_rows(ref, it, r0, n):
    seg = ref.shape[1]
    return pl.ds(it * (TB // seg) + r0 // seg, n // seg)


def _b_keys(it, carry, *, x_ref, xb_ref, bkv_ref, kv_ref, z_ref):
    n_blk, half, _ = bkv_ref.shape
    gr = half // K_PAIRS
    xb = xb_ref[_chunk_rows(xb_ref, it, 0, TB)].reshape(TB, -1)
    last = x_ref.shape[0] - 1
    xb_ref[last] = _layernorm(x_ref[last]).astype(BF16)
    same_head = (_iota((gr, 2 * gr), 0) >= gr // 2) == ((_iota((gr, 2 * gr), 1) & 1) == 1)

    def accumulate(b, t):
        for i in range(K_PAIRS):
            g = b * K_PAIRS + i
            phi = _feature_map(t[i * gr:(i + 1) * gr])
            z_ref[g] += jnp.broadcast_to(jnp.sum(phi, axis=1, keepdims=True), z_ref.shape[1:])
            kv = lax.dot_general(t[half + i * gr:half + (i + 1) * gr], phi.astype(BF16), NT,
                                 preferred_element_type=F32)
            kv_ref[g] += jnp.where(same_head, kv, 0.0)

    pending = None
    for b in range(n_blk):
        t = lax.dot_general(_unpack(bkv_ref[b]), xb, NT, preferred_element_type=F32)
        if pending is not None:
            accumulate(*pending)
        pending = (b, t)
    accumulate(*pending)
    return carry


def _b_queries(it, send, *, x_ref, xb_ref, y_ref, bq_ref, bo_ref, kv_ref, z_ref, ot_ref, on_ref):
    n_groups, gr, _ = kv_ref.shape
    blk = Q_PAIRS * gr
    sub = _iota((8, TB), 0)
    xb = xb_ref[_chunk_rows(xb_ref, it, 0, TB)].reshape(TB, -1)

    def attend(b, t):
        outs = []
        for i in range(Q_PAIRS):
            g = b * Q_PAIRS + i
            phi = _feature_map(t[i * gr:(i + 1) * gr])
            num = jnp.dot(kv_ref[g], phi.astype(BF16), preferred_element_type=F32)
            z = jnp.concatenate([z_ref[g]] * (TB // 128), axis=1)
            inv = _recip(_pair_reduce(phi * z, jnp.add) + 1e-6)
            other = pltpu.roll(inv, 1, 0)
            inv_a = jnp.where((sub & 1) == 0, inv, other)
            inv_b = jnp.where((sub & 1) == 0, other, inv)
            n = (gr - 8) // 16
            inv = jnp.concatenate(
                [inv_a] * n + [jnp.where(sub < 4, inv_a, inv_b)] + [inv_b] * n, axis=0)
            outs.append(num * inv)
        ot_ref[b * blk // 2:(b + 1) * blk // 2, :] = _pack(jnp.concatenate(outs, axis=0))

    n_blk = n_groups // Q_PAIRS
    proj = {}
    for b in range(n_blk + Q_LAG):
        if b < n_blk:
            proj[b] = lax.dot_general(_unpack(bq_ref[b * blk // 2:(b + 1) * blk // 2, :]), xb,
                                      NT, preferred_element_type=F32)
        if b >= Q_LAG:
            attend(b - Q_LAG, proj[b - Q_LAG])
    on_ref[...] = _pack(_unpack(ot_ref[...]).T)
    r0 = 0
    for i, n in enumerate(O_ROWS):
        at = _chunk_rows(x_ref, it, r0, n)
        y = jnp.dot(_unpack(on_ref[r0 // 2:(r0 + n) // 2, :]), _unpack(bo_ref[...]),
                    preferred_element_type=F32)
        x = x_ref[at] + y.reshape((-1,) + x_ref.shape[1:])
        x_ref[at] = x
        y_ref[at] = x.astype(BF16)
        send(i)
        r0 += n


def _kernel(x_hbm, mem0_hbm, wq_hbm, wk_hbm, wv_hbm, wo_hbm, wqkvb_hbm, wphi_hbm, wob_hbm,
            out_hbm,
            x_ref, xb_ref, y_ref, xt_ref, xp_ref, stage_ref, pre_ref, w_ref, wo_ref, o_ref,
            mem0_ref, wphi_ref, wqkvb_ref, wob_ref, bo_ref, bq_ref, bkv_ref, kv_ref, z_ref, ot_ref, on_ref,
            w_sem, in_sem, out_sem, *, dh):
    n_seg, seg, d = x_ref.shape
    n_pairs = w_ref.shape[0]
    pw = 2 * dh
    n_iter = n_seg * seg // TB

    def pair_rows(p):
        return pl.ds(pl.multiple_of(p * pw, pw), pw)

    def w_copy(p, j):
        return pltpu.make_async_copy(
            (wq_hbm, wk_hbm, wv_hbm)[j].at[pair_rows(p), :],
            stage_ref.at[p, j * pw:(j + 1) * pw, :], w_sem.at[p, j])

    def out_copy(it, i):
        part = _chunk_rows(y_ref, it, sum(O_ROWS[:i]), O_ROWS[i])
        return pltpu.make_async_copy(y_ref.at[part], out_hbm.at[part], out_sem.at[0])

    xt_copy = pltpu.make_async_copy(x_hbm.at[:, seg - PRE:seg, :], xt_ref, in_sem.at[0])
    wqkvb_copy = pltpu.make_async_copy(wqkvb_hbm, wqkvb_ref, in_sem.at[1])
    wphi_copy = pltpu.make_async_copy(wphi_hbm, wphi_ref, in_sem.at[5])
    mem0_copy = pltpu.make_async_copy(mem0_hbm, mem0_ref, in_sem.at[6])
    wob_copy = pltpu.make_async_copy(wob_hbm, wob_ref, in_sem.at[2])

    xt_copy.start()
    w_copy(0, 1).start()
    w_copy(0, 2).start()
    xt_copy.wait()

    w_copy(0, 0).start()
    mem0_copy.start()
    for j in (1, 2, 0):
        w_copy(1, j).start()
    xp_ref[...] = _layernorm(xt_ref[...].astype(F32).reshape(n_seg * PRE, d)).astype(BF16)

    def pre_project(p, carry):
        @pl.when(p + 2 < n_pairs)
        def _():
            for j in range(3):
                w_copy(jnp.minimum(p + 2, n_pairs - 1), j).start()

        part = pl.ds(p * (n_seg // n_pairs), n_seg // n_pairs)
        pltpu.make_async_copy(x_hbm.at[part], y_ref.at[part], in_sem.at[3]).start()
        pltpu.make_async_copy(
            wo_hbm.at[pair_rows(p), :], wo_ref.at[pair_rows(p), :], in_sem.at[4]).start()
        for j in range(3):
            w_copy(p, j).wait()
        pre_ref[p] = lax.dot_general(xp_ref[...], stage_ref[p, pw:3 * pw, :], NT,
                                     preferred_element_type=F32)
        for j in range(3):
            w_ref[p, :, j * pw:(j + 1) * pw] = _pack(stage_ref[p, j * pw:(j + 1) * pw, :].T)
        return carry

    lax.fori_loop(0, n_pairs, pre_project, 0, unroll=P_UNROLL)

    pltpu.make_async_copy(x_hbm, y_ref, in_sem.at[3]).wait()
    pltpu.make_async_copy(wo_hbm, wo_ref, in_sem.at[4]).wait()

    wqkvb_copy.start()
    wob_copy.start()
    wphi_copy.start()
    mem0_copy.wait()
    x_ref[0] = y_ref[0].astype(F32)

    def layer_a(x_in, pre, unroll):
        step = functools.partial(_a_step, dh=dh, x_in=x_in, x_ref=x_ref, xb_ref=xb_ref,
                                 w_ref=w_ref, wo_ref=wo_ref, pre_ref=pre, o_ref=o_ref)
        lax.fori_loop(0, n_seg, step, (mem0_ref[...].astype(F32), _layernorm(x_ref[0])),
                      unroll=unroll)

    b_keys = functools.partial(_b_keys, x_ref=x_ref, xb_ref=xb_ref, bkv_ref=bkv_ref,
                               kv_ref=kv_ref, z_ref=z_ref)
    b_queries = functools.partial(_b_queries, x_ref=x_ref, xb_ref=xb_ref, y_ref=y_ref,
                                  bq_ref=bq_ref, bo_ref=bo_ref, kv_ref=kv_ref, z_ref=z_ref,
                                  ot_ref=ot_ref, on_ref=on_ref)

    def layer_pair(layer, carry):
        @pl.when(layer == 0)
        def _():
            layer_a(y_ref, pre_ref, A_UNROLL[0])

        @pl.when(layer == 0)
        def _():
            wqkvb_copy.wait()
            wob_copy.wait()
            wphi_copy.wait()
            _b_weights(wqkvb_ref, wphi_ref, wob_ref, bq_ref, bkv_ref, bo_ref)

        @pl.when(layer == 1)
        def _():
            layer_a(x_ref, None, A_UNROLL[1])

        kv_ref[...] = jnp.zeros(kv_ref.shape, F32)
        z_ref[...] = jnp.zeros(z_ref.shape, F32)
        lax.fori_loop(0, n_iter, b_keys, 0)

        def queries(it, carry):
            def send(i):
                @pl.when(layer == 1)
                def _():
                    out_copy(it, i).start()

            b_queries(it, send)
            return carry

        lax.fori_loop(0, n_iter, queries, 0)

        return carry

    lax.fori_loop(0, 2, layer_pair, 0)
    pltpu.make_async_copy(y_ref, out_hbm, out_sem.at[0]).wait()


@functools.partial(jax.jit, static_argnames=("A_seg_len",))
def pallas_interleave_layers__memory_aug_recurrent_mem_tr__linear_kernel_hedgehog__prompt_kernel(
    A_x, A_mem0, A_Wq, A_Wk, A_Wv, A_Wo, A_seg_len, B_x, B_wqkv, B_w_phi, B_wo,
):
    del B_x
    batch, s_len, d = A_x.shape
    _, heads, dh = A_Wq.shape
    n_mem = A_mem0.shape[1]
    seg = int(A_seg_len)
    b_heads, b_dh, _ = B_w_phi.shape
    rows = n_mem + seg
    n_pairs = heads // 2
    gr = 2 * b_dh
    half = K_PAIRS * gr
    n_seg = s_len // seg
    assert batch == 1 and dh == 192 and heads % (2 * O_PAIRS) == 0
    assert n_mem % 8 == 0 and seg % 16 == 0 and 128 % seg == 0 and 2 * rows <= 128
    assert s_len % TB == 0 and s_len > TB == sum(O_ROWS) and n_seg % n_pairs == 0
    assert b_heads * b_dh == d and b_dh % 8 == 4 and d % half == 0

    def head_major(w):
        return w.transpose(1, 2, 0).reshape(heads * dh, d)

    hbm = pl.BlockSpec(memory_space=pltpu.HBM)
    out = pl.pallas_call(
        functools.partial(_kernel, dh=dh),
        out_shape=jax.ShapeDtypeStruct((n_seg, seg, d), A_x.dtype),
        in_specs=[hbm] * 9,
        out_specs=hbm,
        scratch_shapes=[
            pltpu.VMEM((n_seg, seg, d), F32),
            pltpu.VMEM((n_seg, seg, d), BF16),
            pltpu.VMEM((n_seg, seg, d), BF16),
            pltpu.VMEM((n_seg, PRE, d), BF16),
            pltpu.VMEM((n_seg * PRE, d), BF16),
            pltpu.VMEM((n_pairs, 6 * dh, d), BF16),
            pltpu.VMEM((n_pairs, n_seg * PRE, 4 * dh), F32),
            pltpu.VMEM((n_pairs, d // 2, 6 * dh), jnp.uint32),
            pltpu.VMEM((heads * dh, d), BF16),
            pltpu.VMEM((rows, heads * dh), F32),
            pltpu.VMEM((n_mem, d), BF16),
            pltpu.VMEM((b_dh, b_dh, b_heads), BF16),
            pltpu.VMEM(B_wqkv.shape, BF16),
            pltpu.VMEM(B_wo.shape, BF16),
            pltpu.VMEM((d // 2, d), jnp.uint32),
            pltpu.VMEM((d // 2, d), jnp.uint32),
            pltpu.VMEM((d // half, half, d), jnp.uint32),
            pltpu.VMEM((b_heads // 2, gr, 2 * gr), F32),
            pltpu.VMEM((b_heads // 2, 2 * gr, 128), F32),
            pltpu.VMEM((d // 2, TB), jnp.uint32),
            pltpu.VMEM((TB // 2, d), jnp.uint32),
            pltpu.SemaphoreType.DMA((n_pairs, 3)),
            pltpu.SemaphoreType.DMA((7,)),
            pltpu.SemaphoreType.DMA((1,)),
        ],
        compiler_params=pltpu.CompilerParams(vmem_limit_bytes=120 * 1024 * 1024),
    )(
        A_x.reshape(n_seg, seg, d), A_mem0.reshape(n_mem, d),
        head_major(A_Wq), head_major(A_Wk), head_major(A_Wv), A_Wo.reshape(heads * dh, d),
        B_wqkv, B_w_phi.transpose(1, 2, 0), B_wo,
    )
    return out.reshape(batch, s_len, d)
```

```python
import functools
import math

import jax
import jax.numpy as jnp
from jax import lax
import jax.experimental.pallas as pl
import jax.experimental.pallas.tpu as pltpu

F32 = jnp.float32
BF16 = jnp.bfloat16
NT = (((1,), (1,)), ((), ()))
LOG2E = math.log2(math.e)

LAG_S = 2
LAG_PV = 2
O_SPLITS = (0, 2, 4, 6, 8, 16)
A_UNROLL = (2, 2)
K_SPLIT = 512
NORM_AT = (4, 8)
PRE = 8
TB = 512
K_PAIRS = 8
Q_PAIRS = 8
Q_LAG = 1
F_PAIRS = 2
O_ROWS = (128, 128, 128, 128)


def _iota(shape, axis):
    return lax.broadcasted_iota(jnp.int32, shape, axis)


def _div(v, d):
    return (v * ((1 << 18) // d + 1)) >> 18


def _pack(x):
    return pltpu.bitcast(x.astype(BF16), jnp.uint32)


def _unpack(x):
    return pltpu.bitcast(x, BF16)


def _recip(x):
    r = pl.reciprocal(x, approx=True)
    return r * (2.0 - x * r)


def _layernorm(x):
    m = jnp.mean(x, axis=-1, keepdims=True)
    c = x - m
    v = jnp.mean(c * c, axis=-1, keepdims=True)
    return c * lax.rsqrt(v + 1e-5)


def _a_step(s, carry, opens, closes, *, dh, x_in, x_ref, xb_ref, w_ref, wo_ref, pre_ref, o_ref):
    mem, xn = carry
    n_mem, seg = mem.shape[0], xn.shape[0]
    rows = n_mem + seg
    pw = 2 * dh
    n_pairs = w_ref.shape[0]
    scale = dh ** -0.5

    nxt = jnp.minimum(s + 1, x_ref.shape[0] - 1)
    prv = jnp.maximum(s - 1, 0)
    xn_next = _layernorm(x_in[nxt].astype(F32))
    xb_prev = _layernorm(x_ref[prv])
    xb_ref[prv] = xb_prev.astype(BF16)

    def schedule_before(value, early):
        t = functools.reduce(jnp.maximum, [early[i:i + 8, j:j + 128]
                                           for i in range(0, early.shape[0], 8)
                                           for j in range(0, early.shape[1], 128)])
        head = jnp.where(s < 0, t[:, :value.shape[1]], value[0:8])
        return jnp.concatenate([head, value[8:]], axis=0)

    h = jnp.concatenate([mem, xn], axis=0)
    h_short = h[:rows - PRE].astype(BF16)

    first = _iota((rows, 128), 1) < (dh - 128)
    col = _iota((rows, 2 * rows), 1)
    row = _iota((rows, 2 * rows), 0)
    is_a = col < rows
    visible = (row < n_mem) | (row >= jnp.where(is_a, col, col - rows))
    zero = jnp.zeros((rows, 128), F32)

    def block_diag(t):
        t0, t1, t2 = t[:, 0:128], t[:, 128:256], t[:, 256:384]
        top = jnp.concatenate([t0, jnp.where(first, t1, 0.0), zero], axis=1)
        bot = jnp.concatenate([zero, jnp.where(first, 0.0, t1), t2], axis=1)
        return jnp.concatenate([top, bot], axis=0).astype(BF16)

    q, k, v, probs = {}, {}, {}, {}

    def times_w(lhs, p, lo, hi):
        def part(k0, k1):
            w = _unpack(w_ref[p, k0 // 2:k1 // 2, lo:hi])
            return jnp.dot(lhs[:, k0:k1], w, preferred_element_type=F32)

        if p == 0 and lo == 0 and not opens:
            return part(K_SPLIT, lhs.shape[1]) + part(0, K_SPLIT)
        return part(0, lhs.shape[1])

    def project_short(p, j):
        done = pre_ref[p, pl.ds(pl.multiple_of(s * PRE, PRE), PRE), (j - 1) * pw:j * pw]
        return jnp.concatenate([times_w(h_short, p, j * pw, (j + 1) * pw), done], axis=0)

    def scores(p):
        sc = lax.dot_general(q[p], block_diag(k[p]), NT, preferred_element_type=F32)
        sc = jnp.where(visible, sc * scale, -1e9)
        max_a = jnp.max(jnp.where(is_a, sc, -jnp.inf), axis=1, keepdims=True)
        max_b = jnp.max(jnp.where(is_a, -jnp.inf, sc), axis=1, keepdims=True)
        e = jnp.exp(sc - jnp.where(is_a, max_a, max_b))
        sum_a = jnp.sum(jnp.where(is_a, e, 0.0), axis=1, keepdims=True)
        sum_b = jnp.sum(jnp.where(is_a, 0.0, e), axis=1, keepdims=True)
        probs[p] = e * _recip(jnp.where(is_a, sum_a, sum_b))
        if p == NORM_AT[0]:
            probs[p] = schedule_before(probs[p], xn_next)
        if p == NORM_AT[1]:
            probs[p] = schedule_before(probs[p], xb_prev)

    def values(p):
        o_ref[:, p * pw:(p + 1) * pw] = jnp.dot(
            probs[p], block_diag(v[p]), preferred_element_type=F32)

    def project_out(p0, p1, acc):
        lo, hi = p0 * pw, p1 * pw

        def part(k0, k1, c0, c1):
            return jnp.dot(o_ref[:, k0:k1], wo_ref[k0:k1, c0:c1], preferred_element_type=F32)

        d = wo_ref.shape[1]
        if p1 < n_pairs:
            r = part(lo, hi, 0, d)
        elif closes:
            return part(hi - 128, hi, 0, d) + (part(lo, hi - 128, 0, d) + acc)
        else:
            r = jnp.concatenate([part(lo, hi, 0, K_SPLIT), part(lo, hi, K_SPLIT, d)], axis=1)
        return r if acc is None else r + acc

    out = None
    todo = list(zip(O_SPLITS[:-1], O_SPLITS[1:]))
    for t in range(n_pairs + LAG_S + LAG_PV):
        if t >= n_pairs:
            out = project_out(*todo.pop(0), out)
        elif pre_ref is None:
            r = times_w(h, t, 0, 3 * pw)
            q[t], k[t], v[t] = r[:, 0:pw], r[:, pw:2 * pw], r[:, 2 * pw:3 * pw]
        else:
            q[t] = times_w(h, t, 0, pw)
            k[t] = project_short(t, 1)
        if 0 <= t - LAG_S < n_pairs:
            scores(t - LAG_S)
        if 0 <= t - LAG_S - LAG_PV < n_pairs:
            values(t - LAG_S - LAG_PV)
        if t < n_pairs and pre_ref is not None:
            v[t] = project_short(t, 2)
    for part in todo:
        out = project_out(*part, out)

    x_ref[s] = x_in[s].astype(F32) + out[n_mem:, :]
    return out[:n_mem, :], xn_next


def _pair_reduce(t, op):
    r = t[0:8]
    for i in range(8, t.shape[0], 8):
        r = op(r, t[i:i + 8])
    r = op(r, pltpu.roll(r, 4, 0))
    return op(r, pltpu.roll(r, 2, 0))


def _tile_rows(r, n):
    return jnp.concatenate([r] * (n // 8), axis=0)


def _feature_map(p):
    n = p.shape[0]
    e_pos = jnp.exp2(p - _tile_rows(_pair_reduce(p, jnp.maximum), n))
    e_neg = jnp.exp2(_tile_rows(_pair_reduce(p, jnp.minimum), n) - p)
    inv_pos = _recip(_pair_reduce(e_pos, jnp.add))
    inv_neg = _recip(_pair_reduce(e_neg, jnp.add))
    return jnp.concatenate(
        [e_pos * _tile_rows(inv_pos, n), e_neg * _tile_rows(inv_neg, n)], axis=0)


def _b_weights(wqkv_ref, wphi_ref, wob_ref, bq_ref, bkv_ref, bo_ref):
    d = wqkv_ref.shape[0]
    dh, _, heads = wphi_ref.shape
    gr = 2 * dh
    c = _iota((dh, d), 1)
    c_feat = c - _div(c, dh) * dh
    spread = (_div(_iota((heads, d), 1), dh) == _iota((heads, d), 0)).astype(BF16)
    by_feat = jnp.zeros((dh, d), F32)
    for e in range(dh):
        t = jnp.dot(wphi_ref[e], spread, preferred_element_type=F32)
        by_feat = jnp.where(c_feat == e, t, by_feat)
    by_feat = by_feat.astype(BF16)

    blk = F_PAIRS * gr
    r = _iota((blk, dh), 0)
    sel = (((r - _div(r, gr) * gr) >> 1) == _iota((blk, dh), 1)).astype(BF16)
    half = bkv_ref.shape[1]
    bo_ref[...] = _pack(wob_ref[...])
    wv = wqkv_ref[:, 2 * d:3 * d].T
    for b in range(d // half):
        bkv_ref[b, half // 2:half, :] = _pack(wv[b * half:(b + 1) * half])
    phis = []
    for b in range(d // blk):
        lo = b * blk // 128 * 128
        hi = -(-(b + 1) * blk // 128) * 128
        r = _iota((blk, hi - lo), 0)
        head = 2 * (_div(r, gr) + b * F_PAIRS) + (r & 1)
        phi = jnp.dot(sel, by_feat[:, lo:hi], preferred_element_type=F32)
        phi = jnp.where(_div(_iota((1, hi - lo), 1) + lo, dh) == head, phi, 0.0)
        phis.append((phi.astype(BF16), lo, hi))
    for b, (phi, lo, hi) in enumerate(phis):
        wq = lax.dot_general(phi, wqkv_ref[:, lo:hi], NT, preferred_element_type=F32)
        wk = lax.dot_general(phi, wqkv_ref[:, d + lo:d + hi], NT, preferred_element_type=F32)
        bq_ref[b * blk // 2:(b + 1) * blk // 2, :] = _pack(wq * LOG2E)
        at = b * blk % half // 2
        bkv_ref[b * blk // half, at:at + blk // 2, :] = _pack(wk * LOG2E)


def _chunk_rows(ref, it, r0, n):
    seg = ref.shape[1]
    return pl.ds(it * (TB // seg) + r0 // seg, n // seg)


def _b_keys(it, carry, *, x_ref, xb_ref, bkv_ref, kv_ref, z_ref):
    n_blk, half, _ = bkv_ref.shape
    gr = half // K_PAIRS
    xb = xb_ref[_chunk_rows(xb_ref, it, 0, TB)].reshape(TB, -1)
    last = x_ref.shape[0] - 1
    xb_ref[last] = _layernorm(x_ref[last]).astype(BF16)
    same_head = (_iota((gr, 2 * gr), 0) >= gr // 2) == ((_iota((gr, 2 * gr), 1) & 1) == 1)

    def accumulate(b, t):
        for i in range(K_PAIRS):
            g = b * K_PAIRS + i
            phi = _feature_map(t[i * gr:(i + 1) * gr])
            z_ref[g] += jnp.broadcast_to(jnp.sum(phi, axis=1, keepdims=True), z_ref.shape[1:])
            kv = lax.dot_general(t[half + i * gr:half + (i + 1) * gr], phi.astype(BF16), NT,
                                 preferred_element_type=F32)
            kv_ref[g] += jnp.where(same_head, kv, 0.0)

    pending = None
    for b in range(n_blk):
        t = lax.dot_general(_unpack(bkv_ref[b]), xb, NT, preferred_element_type=F32)
        if pending is not None:
            accumulate(*pending)
        pending = (b, t)
    accumulate(*pending)
    return carry


def _b_queries(it, send, *, x_ref, xb_ref, y_ref, bq_ref, bo_ref, kv_ref, z_ref, ot_ref, on_ref):
    n_groups, gr, _ = kv_ref.shape
    blk = Q_PAIRS * gr
    sub = _iota((8, TB), 0)
    xb = xb_ref[_chunk_rows(xb_ref, it, 0, TB)].reshape(TB, -1)

    def attend(b, t):
        outs = []
        for i in range(Q_PAIRS):
            g = b * Q_PAIRS + i
            phi = _feature_map(t[i * gr:(i + 1) * gr])
            num = jnp.dot(kv_ref[g], phi.astype(BF16), preferred_element_type=F32)
            z = jnp.concatenate([z_ref[g]] * (TB // 128), axis=1)
            inv = _recip(_pair_reduce(phi * z, jnp.add) + 1e-6)
            other = pltpu.roll(inv, 1, 0)
            inv_a = jnp.where((sub & 1) == 0, inv, other)
            inv_b = jnp.where((sub & 1) == 0, other, inv)
            n = (gr - 8) // 16
            inv = jnp.concatenate(
                [inv_a] * n + [jnp.where(sub < 4, inv_a, inv_b)] + [inv_b] * n, axis=0)
            outs.append(num * inv)
        ot_ref[b * blk // 2:(b + 1) * blk // 2, :] = _pack(jnp.concatenate(outs, axis=0))

    n_blk = n_groups // Q_PAIRS
    proj = {}
    for b in range(n_blk + Q_LAG):
        if b < n_blk:
            proj[b] = lax.dot_general(_unpack(bq_ref[b * blk // 2:(b + 1) * blk // 2, :]), xb,
                                      NT, preferred_element_type=F32)
        if b >= Q_LAG:
            attend(b - Q_LAG, proj[b - Q_LAG])
    on_ref[...] = _pack(_unpack(ot_ref[...]).T)
    r0 = 0
    for i, n in enumerate(O_ROWS):
        at = _chunk_rows(x_ref, it, r0, n)
        y = jnp.dot(_unpack(on_ref[r0 // 2:(r0 + n) // 2, :]), _unpack(bo_ref[...]),
                    preferred_element_type=F32)
        x = x_ref[at] + y.reshape((-1,) + x_ref.shape[1:])
        x_ref[at] = x
        y_ref[at] = x.astype(BF16)
        send(i)
        r0 += n


def _kernel(x_hbm, mem0_hbm, wq_hbm, wk_hbm, wv_hbm, wo_hbm, wqkvb_hbm, wphi_hbm, wob_hbm,
            out_hbm,
            x_ref, xb_ref, y_ref, xt_ref, xp_ref, stage_ref, pre_ref, w_ref, wo_ref, o_ref,
            mem0_ref, wphi_ref, wqkvb_ref, wob_ref, bo_ref, bq_ref, bkv_ref, kv_ref, z_ref, ot_ref, on_ref,
            w_sem, in_sem, out_sem, *, dh):
    n_seg, seg, d = x_ref.shape
    n_pairs = w_ref.shape[0]
    pw = 2 * dh
    n_iter = n_seg * seg // TB

    def pair_rows(p):
        return pl.ds(pl.multiple_of(p * pw, pw), pw)

    def w_copy(p, j):
        return pltpu.make_async_copy(
            (wq_hbm, wk_hbm, wv_hbm)[j].at[pair_rows(p), :],
            stage_ref.at[p, j * pw:(j + 1) * pw, :], w_sem.at[p, j])

    def out_copy(it, i):
        part = _chunk_rows(y_ref, it, sum(O_ROWS[:i]), O_ROWS[i])
        return pltpu.make_async_copy(y_ref.at[part], out_hbm.at[part], out_sem.at[0])

    xt_copy = pltpu.make_async_copy(x_hbm.at[:, seg - PRE:seg, :], xt_ref, in_sem.at[0])
    wqkvb_copy = pltpu.make_async_copy(wqkvb_hbm, wqkvb_ref, in_sem.at[1])
    wphi_copy = pltpu.make_async_copy(wphi_hbm, wphi_ref, in_sem.at[5])
    mem0_copy = pltpu.make_async_copy(mem0_hbm, mem0_ref, in_sem.at[6])
    wob_copy = pltpu.make_async_copy(wob_hbm, wob_ref, in_sem.at[2])

    xt_copy.start()
    w_copy(0, 1).start()
    xt_copy.wait()

    w_copy(0, 2).start()
    w_copy(0, 0).start()
    xp_ref[...] = _layernorm(xt_ref[...].astype(F32).reshape(n_seg * PRE, d)).astype(BF16)

    mem0_copy.start()
    for j in (1, 2, 0):
        w_copy(1, j).start()

    def pre_project(p, carry):
        @pl.when(p + 2 < n_pairs)
        def _():
            for j in range(3):
                w_copy(jnp.minimum(p + 2, n_pairs - 1), j).start()

        part = pl.ds(p * (n_seg // n_pairs), n_seg // n_pairs)
        pltpu.make_async_copy(x_hbm.at[part], y_ref.at[part], in_sem.at[3]).start()
        pltpu.make_async_copy(
            wo_hbm.at[pair_rows(p), :], wo_ref.at[pair_rows(p), :], in_sem.at[4]).start()
        for j in range(3):
            w_copy(p, j).wait()
        pre_ref[p] = lax.dot_general(xp_ref[...], stage_ref[p, pw:3 * pw, :], NT,
                                     preferred_element_type=F32)
        for j in range(3):
            w_ref[p, :, j * pw:(j + 1) * pw] = _pack(stage_ref[p, j * pw:(j + 1) * pw, :].T)
        return carry

    lax.fori_loop(0, n_pairs, pre_project, 0)

    pltpu.make_async_copy(x_hbm, y_ref, in_sem.at[3]).wait()
    pltpu.make_async_copy(wo_hbm, wo_ref, in_sem.at[4]).wait()

    wqkvb_copy.start()
    wob_copy.start()
    wphi_copy.start()
    mem0_copy.wait()
    x_ref[0] = y_ref[0].astype(F32)

    def layer_a(x_in, pre, unroll):
        step = functools.partial(_a_step, dh=dh, x_in=x_in, x_ref=x_ref, xb_ref=xb_ref,
                                 w_ref=w_ref, wo_ref=wo_ref, pre_ref=pre, o_ref=o_ref)

        def steps(it, carry):
            for i in range(unroll):
                carry = step(it * unroll + i, carry, i == 0, i == unroll - 1)
            return carry

        lax.fori_loop(0, n_seg // unroll, steps,
                      (mem0_ref[...].astype(F32), _layernorm(x_ref[0])))

    b_keys = functools.partial(_b_keys, x_ref=x_ref, xb_ref=xb_ref, bkv_ref=bkv_ref,
                               kv_ref=kv_ref, z_ref=z_ref)
    b_queries = functools.partial(_b_queries, x_ref=x_ref, xb_ref=xb_ref, y_ref=y_ref,
                                  bq_ref=bq_ref, bo_ref=bo_ref, kv_ref=kv_ref, z_ref=z_ref,
                                  ot_ref=ot_ref, on_ref=on_ref)

    def layer_pair(layer, carry):
        @pl.when(layer == 0)
        def _():
            layer_a(y_ref, pre_ref, A_UNROLL[0])

        @pl.when(layer == 0)
        def _():
            wqkvb_copy.wait()
            wob_copy.wait()
            wphi_copy.wait()
            _b_weights(wqkvb_ref, wphi_ref, wob_ref, bq_ref, bkv_ref, bo_ref)

        @pl.when(layer == 1)
        def _():
            layer_a(x_ref, None, A_UNROLL[1])

        kv_ref[...] = jnp.zeros(kv_ref.shape, F32)
        z_ref[...] = jnp.zeros(z_ref.shape, F32)
        lax.fori_loop(0, n_iter, b_keys, 0)

        def queries(it, carry):
            def send(i):
                @pl.when(layer == 1)
                def _():
                    out_copy(it, i).start()

            b_queries(it, send)
            return carry

        lax.fori_loop(0, n_iter, queries, 0)

        return carry

    lax.fori_loop(0, 2, layer_pair, 0)
    pltpu.make_async_copy(y_ref, out_hbm, out_sem.at[0]).wait()


@functools.partial(jax.jit, static_argnames=("A_seg_len",))
def pallas_interleave_layers__memory_aug_recurrent_mem_tr__linear_kernel_hedgehog__prompt_kernel(
    A_x, A_mem0, A_Wq, A_Wk, A_Wv, A_Wo, A_seg_len, B_x, B_wqkv, B_w_phi, B_wo,
):
    del B_x
    batch, s_len, d = A_x.shape
    _, heads, dh = A_Wq.shape
    n_mem = A_mem0.shape[1]
    seg = int(A_seg_len)
    b_heads, b_dh, _ = B_w_phi.shape
    rows = n_mem + seg
    n_pairs = heads // 2
    gr = 2 * b_dh
    half = K_PAIRS * gr
    n_seg = s_len // seg
    assert batch == 1 and dh == 192 and heads == 2 * O_SPLITS[-1]
    assert n_mem % 8 == 0 and seg % 16 == 0 and 128 % seg == 0 and 2 * rows <= 128
    assert s_len % TB == 0 and s_len > TB == sum(O_ROWS) and n_seg % n_pairs == 0
    assert b_heads * b_dh == d and b_dh % 8 == 4 and d % half == 0

    def head_major(w):
        return w.transpose(1, 2, 0).reshape(heads * dh, d)

    hbm = pl.BlockSpec(memory_space=pltpu.HBM)
    out = pl.pallas_call(
        functools.partial(_kernel, dh=dh),
        out_shape=jax.ShapeDtypeStruct((n_seg, seg, d), A_x.dtype),
        in_specs=[hbm] * 9,
        out_specs=hbm,
        scratch_shapes=[
            pltpu.VMEM((n_seg, seg, d), F32),
            pltpu.VMEM((n_seg, seg, d), BF16),
            pltpu.VMEM((n_seg, seg, d), BF16),
            pltpu.VMEM((n_seg, PRE, d), BF16),
            pltpu.VMEM((n_seg * PRE, d), BF16),
            pltpu.VMEM((n_pairs, 6 * dh, d), BF16),
            pltpu.VMEM((n_pairs, n_seg * PRE, 4 * dh), F32),
            pltpu.VMEM((n_pairs, d // 2, 6 * dh), jnp.uint32),
            pltpu.VMEM((heads * dh, d), BF16),
            pltpu.VMEM((rows, heads * dh), F32),
            pltpu.VMEM((n_mem, d), BF16),
            pltpu.VMEM((b_dh, b_dh, b_heads), BF16),
            pltpu.VMEM(B_wqkv.shape, BF16),
            pltpu.VMEM(B_wo.shape, BF16),
            pltpu.VMEM((d // 2, d), jnp.uint32),
            pltpu.VMEM((d // 2, d), jnp.uint32),
            pltpu.VMEM((d // half, half, d), jnp.uint32),
            pltpu.VMEM((b_heads // 2, gr, 2 * gr), F32),
            pltpu.VMEM((b_heads // 2, 2 * gr, 128), F32),
            pltpu.VMEM((d // 2, TB), jnp.uint32),
            pltpu.VMEM((TB // 2, d), jnp.uint32),
            pltpu.SemaphoreType.DMA((n_pairs, 3)),
            pltpu.SemaphoreType.DMA((7,)),
            pltpu.SemaphoreType.DMA((1,)),
        ],
        compiler_params=pltpu.CompilerParams(vmem_limit_bytes=120 * 1024 * 1024),
    )(
        A_x.reshape(n_seg, seg, d), A_mem0.reshape(n_mem, d),
        head_major(A_Wq), head_major(A_Wk), head_major(A_Wv), A_Wo.reshape(heads * dh, d),
        B_wqkv, B_w_phi.transpose(1, 2, 0), B_wo,
    )
    return out.reshape(batch, s_len, d)
```

```python
import functools
import math

import jax
import jax.numpy as jnp
from jax import lax
import jax.experimental.pallas as pl
import jax.experimental.pallas.tpu as pltpu

F32 = jnp.float32
BF16 = jnp.bfloat16
NT = (((1,), (1,)), ((), ()))
LOG2E = math.log2(math.e)

LAG_S = 2
LAG_PV = 2
O_SPLITS = (0, 2, 4, 6, 8, 16)
A_UNROLL = (2, 2)
K_SPLIT = 512
NORM_AT = (4, 8)
PRE = 8
TB = 512
K_PAIRS = 8
Q_PAIRS = 8
Q_LAG = 1
F_PAIRS = 2
O_ROWS = (128, 128, 128, 128)


def _iota(shape, axis):
    return lax.broadcasted_iota(jnp.int32, shape, axis)


def _div(v, d):
    return (v * ((1 << 18) // d + 1)) >> 18


def _pack(x):
    return pltpu.bitcast(x.astype(BF16), jnp.uint32)


def _unpack(x):
    return pltpu.bitcast(x, BF16)


def _recip(x):
    r = pl.reciprocal(x, approx=True)
    return r * (2.0 - x * r)


def _layernorm(x):
    m = jnp.mean(x, axis=-1, keepdims=True)
    c = x - m
    v = jnp.mean(c * c, axis=-1, keepdims=True)
    return c * lax.rsqrt(v + 1e-5)


def _a_step(s, carry, opens, closes, *, dh, x_in, x_ref, xb_ref, w_ref, wo_ref, pre_ref, o_ref):
    mem, xn = carry
    n_mem, seg = mem.shape[0], xn.shape[0]
    rows = n_mem + seg
    pw = 2 * dh
    n_pairs = w_ref.shape[0]
    scale = dh ** -0.5

    nxt = jnp.minimum(s + 1, x_ref.shape[0] - 1)
    prv = jnp.maximum(s - 1, 0)
    xn_next = _layernorm(x_in[nxt].astype(F32))
    xb_prev = _layernorm(x_ref[prv])
    xb_ref[prv] = xb_prev.astype(BF16)

    def schedule_before(value, early):
        t = functools.reduce(jnp.maximum, [early[i:i + 8, j:j + 128]
                                           for i in range(0, early.shape[0], 8)
                                           for j in range(0, early.shape[1], 128)])
        head = jnp.where(s < 0, t[:, :value.shape[1]], value[0:8])
        return jnp.concatenate([head, value[8:]], axis=0)

    h = jnp.concatenate([mem, xn], axis=0)
    h_short = h[:rows - PRE].astype(BF16)

    first = _iota((rows, 128), 1) < (dh - 128)
    col = _iota((rows, 2 * rows), 1)
    row = _iota((rows, 2 * rows), 0)
    is_a = col < rows
    visible = (row < n_mem) | (row >= jnp.where(is_a, col, col - rows))
    zero = jnp.zeros((rows, 128), F32)

    def block_diag(t):
        t0, t1, t2 = t[:, 0:128], t[:, 128:256], t[:, 256:384]
        top = jnp.concatenate([t0, jnp.where(first, t1, 0.0), zero], axis=1)
        bot = jnp.concatenate([zero, jnp.where(first, 0.0, t1), t2], axis=1)
        return jnp.concatenate([top, bot], axis=0).astype(BF16)

    q, k, v, probs = {}, {}, {}, {}

    def times_w(lhs, p, lo, hi):
        def part(k0, k1):
            w = _unpack(w_ref[p, k0 // 2:k1 // 2, lo:hi])
            return jnp.dot(lhs[:, k0:k1], w, preferred_element_type=F32)

        if p == 0 and lo == 0 and not opens:
            return part(K_SPLIT, lhs.shape[1]) + part(0, K_SPLIT)
        return part(0, lhs.shape[1])

    def project_short(p, j):
        done = pre_ref[p, pl.ds(pl.multiple_of(s * PRE, PRE), PRE), (j - 1) * pw:j * pw]
        return jnp.concatenate([times_w(h_short, p, j * pw, (j + 1) * pw), done], axis=0)

    def scores(p):
        sc = lax.dot_general(q[p], block_diag(k[p]), NT, preferred_element_type=F32)
        sc = jnp.where(visible, sc * scale, -1e9)
        max_a = jnp.max(jnp.where(is_a, sc, -jnp.inf), axis=1, keepdims=True)
        max_b = jnp.max(jnp.where(is_a, -jnp.inf, sc), axis=1, keepdims=True)
        e = jnp.exp(sc - jnp.where(is_a, max_a, max_b))
        sum_a = jnp.sum(jnp.where(is_a, e, 0.0), axis=1, keepdims=True)
        sum_b = jnp.sum(jnp.where(is_a, 0.0, e), axis=1, keepdims=True)
        probs[p] = e * _recip(jnp.where(is_a, sum_a, sum_b))
        if p == NORM_AT[0]:
            probs[p] = schedule_before(probs[p], xn_next)
        if p == NORM_AT[1]:
            probs[p] = schedule_before(probs[p], xb_prev)

    def values(p):
        o_ref[:, p * pw:(p + 1) * pw] = jnp.dot(
            probs[p], block_diag(v[p]), preferred_element_type=F32)

    def project_out(p0, p1, acc):
        lo, hi = p0 * pw, p1 * pw

        def part(k0, k1, c0, c1):
            return jnp.dot(o_ref[:, k0:k1], wo_ref[k0:k1, c0:c1], preferred_element_type=F32)

        d = wo_ref.shape[1]
        if p1 < n_pairs:
            r = part(lo, hi, 0, d)
        elif closes:
            return part(hi - 128, hi, 0, d) + (part(lo, hi - 128, 0, d) + acc)
        else:
            r = jnp.concatenate([part(lo, hi, 0, K_SPLIT), part(lo, hi, K_SPLIT, d)], axis=1)
        return r if acc is None else r + acc

    out = None
    todo = list(zip(O_SPLITS[:-1], O_SPLITS[1:]))
    for t in range(n_pairs + LAG_S + LAG_PV):
        if t >= n_pairs:
            out = project_out(*todo.pop(0), out)
        elif pre_ref is None:
            r = times_w(h, t, 0, 3 * pw)
            q[t], k[t], v[t] = r[:, 0:pw], r[:, pw:2 * pw], r[:, 2 * pw:3 * pw]
        else:
            q[t] = times_w(h, t, 0, pw)
            k[t] = project_short(t, 1)
        if 0 <= t - LAG_S < n_pairs:
            scores(t - LAG_S)
        if 0 <= t - LAG_S - LAG_PV < n_pairs:
            values(t - LAG_S - LAG_PV)
        if t < n_pairs and pre_ref is not None:
            v[t] = project_short(t, 2)
    for part in todo:
        out = project_out(*part, out)

    x_ref[s] = x_in[s].astype(F32) + out[n_mem:, :]
    return out[:n_mem, :], xn_next


def _pair_reduce(t, op):
    r = t[0:8]
    for i in range(8, t.shape[0], 8):
        r = op(r, t[i:i + 8])
    r = op(r, pltpu.roll(r, 4, 0))
    return op(r, pltpu.roll(r, 2, 0))


def _tile_rows(r, n):
    return jnp.concatenate([r] * (n // 8), axis=0)


def _feature_map(p):
    n = p.shape[0]
    e_pos = jnp.exp2(p - _tile_rows(_pair_reduce(p, jnp.maximum), n))
    e_neg = jnp.exp2(_tile_rows(_pair_reduce(p, jnp.minimum), n) - p)
    inv_pos = _recip(_pair_reduce(e_pos, jnp.add))
    inv_neg = _recip(_pair_reduce(e_neg, jnp.add))
    return jnp.concatenate(
        [e_pos * _tile_rows(inv_pos, n), e_neg * _tile_rows(inv_neg, n)], axis=0)


def _b_weights(wqkv_ref, wphi_ref, wob_ref, bq_ref, bkv_ref, bo_ref):
    d = wqkv_ref.shape[0]
    dh, _, heads = wphi_ref.shape
    gr = 2 * dh
    c = _iota((dh, d), 1)
    c_feat = c - _div(c, dh) * dh
    spread = (_div(_iota((heads, d), 1), dh) == _iota((heads, d), 0)).astype(BF16)
    by_feat = jnp.zeros((dh, d), F32)
    for e in range(dh):
        t = jnp.dot(wphi_ref[e], spread, preferred_element_type=F32)
        by_feat = jnp.where(c_feat == e, t, by_feat)
    by_feat = by_feat.astype(BF16)

    blk = F_PAIRS * gr
    r = _iota((blk, dh), 0)
    sel = (((r - _div(r, gr) * gr) >> 1) == _iota((blk, dh), 1)).astype(BF16)
    half = bkv_ref.shape[1]
    bo_ref[...] = _pack(wob_ref[...])
    wv = wqkv_ref[:, 2 * d:3 * d].T
    for b in range(d // half):
        bkv_ref[b, half // 2:half, :] = _pack(wv[b * half:(b + 1) * half])
    phis = []
    for b in range(d // blk):
        lo = b * blk // 128 * 128
        hi = -(-(b + 1) * blk // 128) * 128
        r = _iota((blk, hi - lo), 0)
        head = 2 * (_div(r, gr) + b * F_PAIRS) + (r & 1)
        phi = jnp.dot(sel, by_feat[:, lo:hi], preferred_element_type=F32)
        phi = jnp.where(_div(_iota((1, hi - lo), 1) + lo, dh) == head, phi, 0.0)
        phis.append((phi.astype(BF16), lo, hi))
    for b, (phi, lo, hi) in enumerate(phis):
        wq = lax.dot_general(phi, wqkv_ref[:, lo:hi], NT, preferred_element_type=F32)
        wk = lax.dot_general(phi, wqkv_ref[:, d + lo:d + hi], NT, preferred_element_type=F32)
        bq_ref[b * blk // 2:(b + 1) * blk // 2, :] = _pack(wq * LOG2E)
        at = b * blk % half // 2
        bkv_ref[b * blk // half, at:at + blk // 2, :] = _pack(wk * LOG2E)


def _chunk_rows(ref, it, r0, n):
    seg = ref.shape[1]
    return pl.ds(it * (TB // seg) + r0 // seg, n // seg)


def _b_keys(it, carry, *, x_ref, xb_ref, bkv_ref, kv_ref, z_ref):
    n_blk, half, _ = bkv_ref.shape
    gr = half // K_PAIRS
    xb = xb_ref[_chunk_rows(xb_ref, it, 0, TB)].reshape(TB, -1)
    last = x_ref.shape[0] - 1
    xb_ref[last] = _layernorm(x_ref[last]).astype(BF16)
    same_head = (_iota((gr, 2 * gr), 0) >= gr // 2) == ((_iota((gr, 2 * gr), 1) & 1) == 1)

    def accumulate(b, t):
        for i in range(K_PAIRS):
            g = b * K_PAIRS + i
            phi = _feature_map(t[i * gr:(i + 1) * gr])
            z_ref[g] += jnp.broadcast_to(jnp.sum(phi, axis=1, keepdims=True), z_ref.shape[1:])
            kv = lax.dot_general(t[half + i * gr:half + (i + 1) * gr], phi.astype(BF16), NT,
                                 preferred_element_type=F32)
            kv_ref[g] += jnp.where(same_head, kv, 0.0)

    pending = None
    for b in range(n_blk):
        t = lax.dot_general(_unpack(bkv_ref[b]), xb, NT, preferred_element_type=F32)
        if pending is not None:
            accumulate(*pending)
        pending = (b, t)
    accumulate(*pending)
    return carry


def _b_queries(it, send, *, x_ref, xb_ref, y_ref, bq_ref, bo_ref, kv_ref, z_ref, ot_ref, on_ref):
    n_groups, gr, _ = kv_ref.shape
    blk = Q_PAIRS * gr
    sub = _iota((8, TB), 0)
    xb = xb_ref[_chunk_rows(xb_ref, it, 0, TB)].reshape(TB, -1)

    def attend(b, t):
        outs = []
        for i in range(Q_PAIRS):
            g = b * Q_PAIRS + i
            phi = _feature_map(t[i * gr:(i + 1) * gr])
            num = jnp.dot(kv_ref[g], phi.astype(BF16), preferred_element_type=F32)
            z = jnp.concatenate([z_ref[g]] * (TB // 128), axis=1)
            inv = _recip(_pair_reduce(phi * z, jnp.add) + 1e-6)
            other = pltpu.roll(inv, 1, 0)
            inv_a = jnp.where((sub & 1) == 0, inv, other)
            inv_b = jnp.where((sub & 1) == 0, other, inv)
            n = (gr - 8) // 16
            inv = jnp.concatenate(
                [inv_a] * n + [jnp.where(sub < 4, inv_a, inv_b)] + [inv_b] * n, axis=0)
            outs.append(num * inv)
        ot_ref[b * blk // 2:(b + 1) * blk // 2, :] = _pack(jnp.concatenate(outs, axis=0))

    n_blk = n_groups // Q_PAIRS
    proj = {}
    for b in range(n_blk + Q_LAG):
        if b < n_blk:
            proj[b] = lax.dot_general(_unpack(bq_ref[b * blk // 2:(b + 1) * blk // 2, :]), xb,
                                      NT, preferred_element_type=F32)
        if b >= Q_LAG:
            attend(b - Q_LAG, proj[b - Q_LAG])
    on_ref[...] = _pack(_unpack(ot_ref[...]).T)
    r0 = 0
    for i, n in enumerate(O_ROWS):
        at = _chunk_rows(x_ref, it, r0, n)
        y = jnp.dot(_unpack(on_ref[r0 // 2:(r0 + n) // 2, :]), _unpack(bo_ref[...]),
                    preferred_element_type=F32)
        x = x_ref[at] + y.reshape((-1,) + x_ref.shape[1:])
        x_ref[at] = x
        y_ref[at] = x.astype(BF16)
        send(i)
        r0 += n


def _kernel(x_hbm, mem0_hbm, wq_hbm, wk_hbm, wv_hbm, wo_hbm, wqkvb_hbm, wphi_hbm, wob_hbm,
            out_hbm,
            x_ref, xb_ref, y_ref, xp_ref, stage_ref, pre_ref, w_ref, wo_ref, o_ref,
            mem0_ref, wphi_ref, wqkvb_ref, wob_ref, bo_ref, bq_ref, bkv_ref, kv_ref, z_ref, ot_ref, on_ref,
            w_sem, in_sem, out_sem, *, dh):
    n_seg, seg, d = x_ref.shape
    n_pairs = w_ref.shape[0]
    pw = 2 * dh
    n_iter = n_seg * seg // TB

    def pair_rows(p):
        return pl.ds(pl.multiple_of(p * pw, pw), pw)

    def w_copy(p, j):
        return pltpu.make_async_copy(
            (wq_hbm, wk_hbm, wv_hbm)[j].at[pair_rows(p), :],
            stage_ref.at[p, j * pw:(j + 1) * pw, :], w_sem.at[p, j])

    def out_copy(it, i):
        part = _chunk_rows(y_ref, it, sum(O_ROWS[:i]), O_ROWS[i])
        return pltpu.make_async_copy(y_ref.at[part], out_hbm.at[part], out_sem.at[0])

    def x_copy(part, rows, sem):
        return pltpu.make_async_copy(x_hbm.at[part, rows, :], y_ref.at[part, rows, :], sem)

    head, tail = slice(0, seg - PRE), slice(seg - PRE, seg)
    xt_copy = x_copy(slice(None), tail, in_sem.at[0])
    wqkvb_copy = pltpu.make_async_copy(wqkvb_hbm, wqkvb_ref, in_sem.at[1])
    wphi_copy = pltpu.make_async_copy(wphi_hbm, wphi_ref, in_sem.at[5])
    mem0_copy = pltpu.make_async_copy(mem0_hbm, mem0_ref, in_sem.at[6])
    wob_copy = pltpu.make_async_copy(wob_hbm, wob_ref, in_sem.at[2])

    xt_copy.start()
    w_copy(0, 1).start()
    xt_copy.wait()

    w_copy(0, 2).start()
    xp_ref[...] = _layernorm(y_ref[:, tail, :].astype(F32).reshape(n_seg * PRE, d)).astype(BF16)

    mem0_copy.start()
    w_copy(0, 0).start()
    for j in (1, 2, 0):
        w_copy(1, j).start()

    def pre_project(p, carry):
        @pl.when(p + 2 < n_pairs)
        def _():
            for j in range(3):
                w_copy(jnp.minimum(p + 2, n_pairs - 1), j).start()

        part = pl.ds(p * (n_seg // n_pairs), n_seg // n_pairs)
        x_copy(part, head, in_sem.at[3]).start()
        pltpu.make_async_copy(
            wo_hbm.at[pair_rows(p), :], wo_ref.at[pair_rows(p), :], in_sem.at[4]).start()
        before = jnp.maximum(p - 1, 0)

        @pl.when(p > 0)
        def _():
            w_copy(before, 0).wait()

        w_copy(p, 1).wait()
        w_copy(p, 2).wait()
        pre_ref[p] = lax.dot_general(xp_ref[...], stage_ref[p, pw:3 * pw, :], NT,
                                     preferred_element_type=F32)
        w_ref[before, :, 0:pw] = _pack(stage_ref[before, pair_rows(jnp.where(p > 0, 0, 1)), :].T)
        for j in (1, 2):
            w_ref[p, :, j * pw:(j + 1) * pw] = _pack(stage_ref[p, j * pw:(j + 1) * pw, :].T)
        return carry

    lax.fori_loop(0, n_pairs, pre_project, 0)

    w_copy(n_pairs - 1, 0).wait()
    w_ref[n_pairs - 1, :, 0:pw] = _pack(stage_ref[n_pairs - 1, 0:pw, :].T)
    x_copy(slice(None), head, in_sem.at[3]).wait()
    pltpu.make_async_copy(wo_hbm, wo_ref, in_sem.at[4]).wait()

    wqkvb_copy.start()
    wob_copy.start()
    wphi_copy.start()
    mem0_copy.wait()
    x_ref[0] = y_ref[0].astype(F32)

    def layer_a(x_in, pre, unroll):
        step = functools.partial(_a_step, dh=dh, x_in=x_in, x_ref=x_ref, xb_ref=xb_ref,
                                 w_ref=w_ref, wo_ref=wo_ref, pre_ref=pre, o_ref=o_ref)

        def steps(it, carry):
            for i in range(unroll):
                carry = step(it * unroll + i, carry, i == 0, i == unroll - 1)
            return carry

        lax.fori_loop(0, n_seg // unroll, steps,
                      (mem0_ref[...].astype(F32), _layernorm(x_ref[0])))

    b_keys = functools.partial(_b_keys, x_ref=x_ref, xb_ref=xb_ref, bkv_ref=bkv_ref,
                               kv_ref=kv_ref, z_ref=z_ref)
    b_queries = functools.partial(_b_queries, x_ref=x_ref, xb_ref=xb_ref, y_ref=y_ref,
                                  bq_ref=bq_ref, bo_ref=bo_ref, kv_ref=kv_ref, z_ref=z_ref,
                                  ot_ref=ot_ref, on_ref=on_ref)

    def layer_pair(layer, carry):
        @pl.when(layer == 0)
        def _():
            layer_a(y_ref, pre_ref, A_UNROLL[0])

        @pl.when(layer == 0)
        def _():
            wqkvb_copy.wait()
            wob_copy.wait()
            wphi_copy.wait()
            _b_weights(wqkvb_ref, wphi_ref, wob_ref, bq_ref, bkv_ref, bo_ref)

        @pl.when(layer == 1)
        def _():
            layer_a(x_ref, None, A_UNROLL[1])

        kv_ref[...] = jnp.zeros(kv_ref.shape, F32)
        z_ref[...] = jnp.zeros(z_ref.shape, F32)
        lax.fori_loop(0, n_iter, b_keys, 0)

        def queries(it, carry):
            def send(i):
                @pl.when(layer == 1)
                def _():
                    out_copy(it, i).start()

            b_queries(it, send)
            return carry

        lax.fori_loop(0, n_iter, queries, 0)

        return carry

    lax.fori_loop(0, 2, layer_pair, 0)
    pltpu.make_async_copy(y_ref, out_hbm, out_sem.at[0]).wait()


@functools.partial(jax.jit, static_argnames=("A_seg_len",))
def pallas_interleave_layers__memory_aug_recurrent_mem_tr__linear_kernel_hedgehog__prompt_kernel(
    A_x, A_mem0, A_Wq, A_Wk, A_Wv, A_Wo, A_seg_len, B_x, B_wqkv, B_w_phi, B_wo,
):
    del B_x
    batch, s_len, d = A_x.shape
    _, heads, dh = A_Wq.shape
    n_mem = A_mem0.shape[1]
    seg = int(A_seg_len)
    b_heads, b_dh, _ = B_w_phi.shape
    rows = n_mem + seg
    n_pairs = heads // 2
    gr = 2 * b_dh
    half = K_PAIRS * gr
    n_seg = s_len // seg
    assert batch == 1 and dh == 192 and heads == 2 * O_SPLITS[-1]
    assert n_mem % 8 == 0 and seg % 16 == 0 and 128 % seg == 0 and 2 * rows <= 128
    assert s_len % TB == 0 and s_len > TB == sum(O_ROWS) and n_seg % n_pairs == 0
    assert b_heads * b_dh == d and b_dh % 8 == 4 and d % half == 0

    def head_major(w):
        return w.transpose(1, 2, 0).reshape(heads * dh, d)

    hbm = pl.BlockSpec(memory_space=pltpu.HBM)
    out = pl.pallas_call(
        functools.partial(_kernel, dh=dh),
        out_shape=jax.ShapeDtypeStruct((n_seg, seg, d), A_x.dtype),
        in_specs=[hbm] * 9,
        out_specs=hbm,
        scratch_shapes=[
            pltpu.VMEM((n_seg, seg, d), F32),
            pltpu.VMEM((n_seg, seg, d), BF16),
            pltpu.VMEM((n_seg, seg, d), BF16),
            pltpu.VMEM((n_seg * PRE, d), BF16),
            pltpu.VMEM((n_pairs, 6 * dh, d), BF16),
            pltpu.VMEM((n_pairs, n_seg * PRE, 4 * dh), F32),
            pltpu.VMEM((n_pairs, d // 2, 6 * dh), jnp.uint32),
            pltpu.VMEM((heads * dh, d), BF16),
            pltpu.VMEM((rows, heads * dh), F32),
            pltpu.VMEM((n_mem, d), BF16),
            pltpu.VMEM((b_dh, b_dh, b_heads), BF16),
            pltpu.VMEM(B_wqkv.shape, BF16),
            pltpu.VMEM(B_wo.shape, BF16),
            pltpu.VMEM((d // 2, d), jnp.uint32),
            pltpu.VMEM((d // 2, d), jnp.uint32),
            pltpu.VMEM((d // half, half, d), jnp.uint32),
            pltpu.VMEM((b_heads // 2, gr, 2 * gr), F32),
            pltpu.VMEM((b_heads // 2, 2 * gr, 128), F32),
            pltpu.VMEM((d // 2, TB), jnp.uint32),
            pltpu.VMEM((TB // 2, d), jnp.uint32),
            pltpu.SemaphoreType.DMA((n_pairs, 3)),
            pltpu.SemaphoreType.DMA((7,)),
            pltpu.SemaphoreType.DMA((1,)),
        ],
        compiler_params=pltpu.CompilerParams(vmem_limit_bytes=120 * 1024 * 1024),
    )(
        A_x.reshape(n_seg, seg, d), A_mem0.reshape(n_mem, d),
        head_major(A_Wq), head_major(A_Wk), head_major(A_Wv), A_Wo.reshape(heads * dh, d),
        B_wqkv, B_w_phi.transpose(1, 2, 0), B_wo,
    )
    return out.reshape(batch, s_len, d)
```

```python
import functools
import math

import jax
import jax.numpy as jnp
from jax import lax
import jax.experimental.pallas as pl
import jax.experimental.pallas.tpu as pltpu

F32 = jnp.float32
BF16 = jnp.bfloat16
NT = (((1,), (1,)), ((), ()))
LOG2E = math.log2(math.e)

LAG_S = 2
LAG_PV = 2
O_SPLITS = (0, 2, 4, 6, 8, 16)
A_UNROLL = (2, 2)
K_SPLIT = 512
NORM_AT = (4, 8)
PRE = 8
TB = 512
K_PAIRS = 8
Q_PAIRS = 8
Q_LAG = 1
F_PAIRS = 2
O_ROWS = (128, 128, 128, 128)


def _iota(shape, axis):
    return lax.broadcasted_iota(jnp.int32, shape, axis)


def _div(v, d):
    return (v * ((1 << 18) // d + 1)) >> 18


def _pack(x):
    return pltpu.bitcast(x.astype(BF16), jnp.uint32)


def _unpack(x):
    return pltpu.bitcast(x, BF16)


def _recip(x):
    r = pl.reciprocal(x, approx=True)
    return r * (2.0 - x * r)


def _layernorm(x):
    m = jnp.mean(x, axis=-1, keepdims=True)
    c = x - m
    v = jnp.mean(c * c, axis=-1, keepdims=True)
    return c * lax.rsqrt(v + 1e-5)


def _a_step(s, carry, opens, closes, *, dh, x_in, x_ref, xb_ref, w_ref, wo_ref, pre_ref, o_ref):
    mem, xn = carry
    n_mem, seg = mem.shape[0], xn.shape[0]
    rows = n_mem + seg
    pw = 2 * dh
    n_pairs = w_ref.shape[0]
    scale = dh ** -0.5

    nxt = jnp.minimum(s + 1, x_ref.shape[0] - 1)
    prv = jnp.maximum(s - 1, 0)
    xn_next = _layernorm(x_in[nxt].astype(F32))
    xb_prev = _layernorm(x_ref[prv])
    xb_ref[prv] = xb_prev.astype(BF16)

    def schedule_before(value, early):
        t = functools.reduce(jnp.maximum, [early[i:i + 8, j:j + 128]
                                           for i in range(0, early.shape[0], 8)
                                           for j in range(0, early.shape[1], 128)])
        head = jnp.where(s < 0, t[:, :value.shape[1]], value[0:8])
        return jnp.concatenate([head, value[8:]], axis=0)

    h = jnp.concatenate([mem, xn], axis=0)
    h_short = h[:rows - PRE].astype(BF16)

    first = _iota((rows, 128), 1) < (dh - 128)
    col = _iota((rows, 2 * rows), 1)
    row = _iota((rows, 2 * rows), 0)
    is_a = col < rows
    visible = (row < n_mem) | (row >= jnp.where(is_a, col, col - rows))
    zero = jnp.zeros((rows, 128), F32)

    def block_diag(t):
        t0, t1, t2 = t[:, 0:128], t[:, 128:256], t[:, 256:384]
        top = jnp.concatenate([t0, jnp.where(first, t1, 0.0), zero], axis=1)
        bot = jnp.concatenate([zero, jnp.where(first, 0.0, t1), t2], axis=1)
        return jnp.concatenate([top, bot], axis=0).astype(BF16)

    q, k, v, probs = {}, {}, {}, {}

    def times_w(lhs, p, lo, hi):
        def part(k0, k1):
            w = _unpack(w_ref[p, k0 // 2:k1 // 2, lo:hi])
            return jnp.dot(lhs[:, k0:k1], w, preferred_element_type=F32)

        if p == 0 and lo == 0 and not opens:
            return part(K_SPLIT, lhs.shape[1]) + part(0, K_SPLIT)
        return part(0, lhs.shape[1])

    def project_short(p, j):
        done = pre_ref[p, pl.ds(pl.multiple_of(s * PRE, PRE), PRE), (j - 1) * pw:j * pw]
        return jnp.concatenate([times_w(h_short, p, j * pw, (j + 1) * pw), done], axis=0)

    def scores(p):
        sc = lax.dot_general(q[p], block_diag(k[p]), NT, preferred_element_type=F32)
        sc = jnp.where(visible, sc * scale, -1e9)
        max_a = jnp.max(jnp.where(is_a, sc, -jnp.inf), axis=1, keepdims=True)
        max_b = jnp.max(jnp.where(is_a, -jnp.inf, sc), axis=1, keepdims=True)
        e = jnp.exp(sc - jnp.where(is_a, max_a, max_b))
        sum_a = jnp.sum(jnp.where(is_a, e, 0.0), axis=1, keepdims=True)
        sum_b = jnp.sum(jnp.where(is_a, 0.0, e), axis=1, keepdims=True)
        probs[p] = e * _recip(jnp.where(is_a, sum_a, sum_b))
        if p == NORM_AT[0]:
            probs[p] = schedule_before(probs[p], xn_next)
        if p == NORM_AT[1]:
            probs[p] = schedule_before(probs[p], xb_prev)

    def values(p):
        o_ref[:, p * pw:(p + 1) * pw] = jnp.dot(
            probs[p], block_diag(v[p]), preferred_element_type=F32)

    def project_out(p0, p1, acc):
        lo, hi = p0 * pw, p1 * pw

        def part(k0, k1, c0, c1):
            return jnp.dot(o_ref[:, k0:k1], wo_ref[k0:k1, c0:c1], preferred_element_type=F32)

        d = wo_ref.shape[1]
        if p1 < n_pairs:
            r = part(lo, hi, 0, d)
        elif closes:
            return part(hi - 128, hi, 0, d) + (part(lo, hi - 128, 0, d) + acc)
        else:
            r = jnp.concatenate([part(lo, hi, 0, K_SPLIT), part(lo, hi, K_SPLIT, d)], axis=1)
        return r if acc is None else r + acc

    out = None
    todo = list(zip(O_SPLITS[:-1], O_SPLITS[1:]))
    for t in range(n_pairs + LAG_S + LAG_PV):
        if t >= n_pairs:
            out = project_out(*todo.pop(0), out)
        elif pre_ref is None:
            r = times_w(h, t, 0, 3 * pw)
            q[t], k[t], v[t] = r[:, 0:pw], r[:, pw:2 * pw], r[:, 2 * pw:3 * pw]
        else:
            q[t] = times_w(h, t, 0, pw)
            k[t] = project_short(t, 1)
        if 0 <= t - LAG_S < n_pairs:
            scores(t - LAG_S)
        if 0 <= t - LAG_S - LAG_PV < n_pairs:
            values(t - LAG_S - LAG_PV)
        if t < n_pairs and pre_ref is not None:
            v[t] = project_short(t, 2)
    for part in todo:
        out = project_out(*part, out)

    x_ref[s] = x_in[s].astype(F32) + out[n_mem:, :]
    return out[:n_mem, :], xn_next


def _pair_reduce(t, op):
    r = t[0:8]
    for i in range(8, t.shape[0], 8):
        r = op(r, t[i:i + 8])
    r = op(r, pltpu.roll(r, 4, 0))
    return op(r, pltpu.roll(r, 2, 0))


def _tile_rows(r, n):
    return jnp.concatenate([r] * (n // 8), axis=0)


def _feature_map(p):
    n = p.shape[0]
    e_pos = jnp.exp2(p - _tile_rows(_pair_reduce(p, jnp.maximum), n))
    e_neg = jnp.exp2(_tile_rows(_pair_reduce(p, jnp.minimum), n) - p)
    inv_pos = _recip(_pair_reduce(e_pos, jnp.add))
    inv_neg = _recip(_pair_reduce(e_neg, jnp.add))
    return jnp.concatenate(
        [e_pos * _tile_rows(inv_pos, n), e_neg * _tile_rows(inv_neg, n)], axis=0)


def _fold_span(b, blk):
    return b * blk // 128 * 128, -(-(b + 1) * blk // 128) * 128


def _expand_phi(wphi_ref, phi_ref):
    dh, _, heads = wphi_ref.shape
    d = dh * heads
    gr = 2 * dh
    c = _iota((dh, d), 1)
    c_feat = c - _div(c, dh) * dh
    spread = (_div(_iota((heads, d), 1), dh) == _iota((heads, d), 0)).astype(BF16)
    by_feat = jnp.zeros((dh, d), F32)
    for e in range(dh):
        t = jnp.dot(wphi_ref[e], spread, preferred_element_type=F32)
        by_feat = jnp.where(c_feat == e, t, by_feat)
    by_feat = by_feat.astype(BF16)
    blk = F_PAIRS * gr
    r = _iota((blk, dh), 0)
    sel = (((r - _div(r, gr) * gr) >> 1) == _iota((blk, dh), 1)).astype(BF16)
    for b in range(d // blk):
        lo, hi = _fold_span(b, blk)
        r = _iota((blk, hi - lo), 0)
        head = 2 * (_div(r, gr) + b * F_PAIRS) + (r & 1)
        phi = jnp.dot(sel, by_feat[:, lo:hi], preferred_element_type=F32)
        phi_ref[b, :, 0:hi - lo] = _pack(
            jnp.where(_div(_iota((1, hi - lo), 1) + lo, dh) == head, phi, 0.0))


def _b_weights(wqkv_ref, phi_ref, wob_ref, bq_ref, bkv_ref, bo_ref):
    d = wqkv_ref.shape[0]
    blk = 2 * phi_ref.shape[1]
    half = bkv_ref.shape[1]
    bo_ref[...] = _pack(wob_ref[...])
    wv = wqkv_ref[:, 2 * d:3 * d].T
    for b in range(d // half):
        bkv_ref[b, half // 2:half, :] = _pack(wv[b * half:(b + 1) * half])
    for b in range(d // blk):
        lo, hi = _fold_span(b, blk)
        phi = _unpack(phi_ref[b, :, 0:hi - lo])
        wq = lax.dot_general(phi, wqkv_ref[:, lo:hi], NT, preferred_element_type=F32)
        wk = lax.dot_general(phi, wqkv_ref[:, d + lo:d + hi], NT, preferred_element_type=F32)
        bq_ref[b * blk // 2:(b + 1) * blk // 2, :] = _pack(wq * LOG2E)
        at = b * blk % half // 2
        bkv_ref[b * blk // half, at:at + blk // 2, :] = _pack(wk * LOG2E)


def _chunk_rows(ref, it, r0, n):
    seg = ref.shape[1]
    return pl.ds(it * (TB // seg) + r0 // seg, n // seg)


def _b_keys(it, carry, *, x_ref, xb_ref, bkv_ref, kv_ref, z_ref):
    n_blk, half, _ = bkv_ref.shape
    gr = half // K_PAIRS
    xb = xb_ref[_chunk_rows(xb_ref, it, 0, TB)].reshape(TB, -1)
    last = x_ref.shape[0] - 1
    xb_ref[last] = _layernorm(x_ref[last]).astype(BF16)
    same_head = (_iota((gr, 2 * gr), 0) >= gr // 2) == ((_iota((gr, 2 * gr), 1) & 1) == 1)

    def accumulate(b, t):
        for i in range(K_PAIRS):
            g = b * K_PAIRS + i
            phi = _feature_map(t[i * gr:(i + 1) * gr])
            z_ref[g] = jnp.where(it > 0, z_ref[g], 0.0) + jnp.sum(phi, axis=1, keepdims=True)
            kv = lax.dot_general(t[half + i * gr:half + (i + 1) * gr], phi.astype(BF16), NT,
                                 preferred_element_type=F32)
            kv_ref[g] = jnp.where(it > 0, kv_ref[g], 0.0) + jnp.where(same_head, kv, 0.0)

    pending = None
    for b in range(n_blk):
        t = lax.dot_general(_unpack(bkv_ref[b]), xb, NT, preferred_element_type=F32)
        if pending is not None:
            accumulate(*pending)
        pending = (b, t)
    accumulate(*pending)
    return carry


def _b_queries(it, send, *, x_ref, xb_ref, y_ref, bq_ref, bo_ref, kv_ref, z_ref, ot_ref, on_ref):
    n_groups, gr, _ = kv_ref.shape
    blk = Q_PAIRS * gr
    sub = _iota((8, TB), 0)
    xb = xb_ref[_chunk_rows(xb_ref, it, 0, TB)].reshape(TB, -1)

    def attend(b, t):
        outs = []
        for i in range(Q_PAIRS):
            g = b * Q_PAIRS + i
            phi = _feature_map(t[i * gr:(i + 1) * gr])
            num = jnp.dot(kv_ref[g], phi.astype(BF16), preferred_element_type=F32)
            z = jnp.concatenate([z_ref[g]] * (TB // 128), axis=1)
            inv = _recip(_pair_reduce(phi * z, jnp.add) + 1e-6)
            other = pltpu.roll(inv, 1, 0)
            inv_a = jnp.where((sub & 1) == 0, inv, other)
            inv_b = jnp.where((sub & 1) == 0, other, inv)
            n = (gr - 8) // 16
            inv = jnp.concatenate(
                [inv_a] * n + [jnp.where(sub < 4, inv_a, inv_b)] + [inv_b] * n, axis=0)
            outs.append(num * inv)
        ot_ref[b * blk // 2:(b + 1) * blk // 2, :] = _pack(jnp.concatenate(outs, axis=0))

    n_blk = n_groups // Q_PAIRS
    proj = {}
    for b in range(n_blk + Q_LAG):
        if b < n_blk:
            proj[b] = lax.dot_general(_unpack(bq_ref[b * blk // 2:(b + 1) * blk // 2, :]), xb,
                                      NT, preferred_element_type=F32)
        if b >= Q_LAG:
            attend(b - Q_LAG, proj[b - Q_LAG])
    on_ref[...] = _pack(_unpack(ot_ref[...]).T)
    r0 = 0
    for i, n in enumerate(O_ROWS):
        at = _chunk_rows(x_ref, it, r0, n)
        y = jnp.dot(_unpack(on_ref[r0 // 2:(r0 + n) // 2, :]), _unpack(bo_ref[...]),
                    preferred_element_type=F32)
        x = x_ref[at] + y.reshape((-1,) + x_ref.shape[1:])
        x_ref[at] = x
        y_ref[at] = x.astype(BF16)
        send(i)
        r0 += n


def _kernel(x_hbm, mem0_hbm, wq_hbm, wk_hbm, wv_hbm, wo_hbm, wqkvb_hbm, wphi_hbm, wob_hbm,
            out_hbm,
            x_ref, xb_ref, y_ref, xp_ref, stage_ref, pre_ref, w_ref, wo_ref, o_ref,
            mem0_ref, wphi_ref, phi_ref, wqkvb_ref, wob_ref, bo_ref, bq_ref, bkv_ref, kv_ref, z_ref, ot_ref, on_ref,
            w_sem, in_sem, out_sem, *, dh):
    n_seg, seg, d = x_ref.shape
    n_pairs = w_ref.shape[0]
    pw = 2 * dh
    n_iter = n_seg * seg // TB

    def pair_rows(p):
        return pl.ds(pl.multiple_of(p * pw, pw), pw)

    def w_copy(p, j):
        return pltpu.make_async_copy(
            (wq_hbm, wk_hbm, wv_hbm)[j].at[pair_rows(p), :],
            stage_ref.at[p, j * pw:(j + 1) * pw, :], w_sem.at[p, j])

    def out_copy(it, i):
        part = _chunk_rows(y_ref, it, sum(O_ROWS[:i]), O_ROWS[i])
        return pltpu.make_async_copy(y_ref.at[part], out_hbm.at[part], out_sem.at[0])

    def x_copy(part, rows, sem):
        return pltpu.make_async_copy(x_hbm.at[part, rows, :], y_ref.at[part, rows, :], sem)

    head, tail = slice(0, seg - PRE), slice(seg - PRE, seg)
    xt_copy = x_copy(slice(None), tail, in_sem.at[0])
    wqkvb_copy = pltpu.make_async_copy(wqkvb_hbm, wqkvb_ref, in_sem.at[1])
    wphi_copy = pltpu.make_async_copy(wphi_hbm, wphi_ref, in_sem.at[5])
    mem0_copy = pltpu.make_async_copy(mem0_hbm, mem0_ref, in_sem.at[6])
    wob_copy = pltpu.make_async_copy(wob_hbm, wob_ref, in_sem.at[2])

    wphi_copy.start()
    xt_copy.start()
    w_copy(0, 1).start()
    w_copy(0, 2).start()
    wphi_copy.wait()
    _expand_phi(wphi_ref, phi_ref)
    xt_copy.wait()

    xp_ref[...] = _layernorm(y_ref[:, tail, :].astype(F32).reshape(n_seg * PRE, d)).astype(BF16)

    mem0_copy.start()
    w_copy(0, 0).start()
    for j in (1, 2, 0):
        w_copy(1, j).start()

    def pre_project(p, carry):
        @pl.when(p + 2 < n_pairs)
        def _():
            for j in range(3):
                w_copy(jnp.minimum(p + 2, n_pairs - 1), j).start()

        part = pl.ds(p * (n_seg // n_pairs), n_seg // n_pairs)
        x_copy(part, head, in_sem.at[3]).start()
        pltpu.make_async_copy(
            wo_hbm.at[pair_rows(p), :], wo_ref.at[pair_rows(p), :], in_sem.at[4]).start()
        before = jnp.maximum(p - 1, 0)

        @pl.when(p > 0)
        def _():
            w_copy(before, 0).wait()

        w_copy(p, 1).wait()
        w_copy(p, 2).wait()
        pre_ref[p] = lax.dot_general(xp_ref[...], stage_ref[p, pw:3 * pw, :], NT,
                                     preferred_element_type=F32)
        w_ref[before, :, 0:pw] = _pack(stage_ref[before, pair_rows(jnp.where(p > 0, 0, 1)), :].T)
        for j in (1, 2):
            w_ref[p, :, j * pw:(j + 1) * pw] = _pack(stage_ref[p, j * pw:(j + 1) * pw, :].T)
        return carry

    lax.fori_loop(0, n_pairs, pre_project, 0)

    w_copy(n_pairs - 1, 0).wait()
    w_ref[n_pairs - 1, :, 0:pw] = _pack(stage_ref[n_pairs - 1, 0:pw, :].T)
    x_copy(slice(None), head, in_sem.at[3]).wait()
    pltpu.make_async_copy(wo_hbm, wo_ref, in_sem.at[4]).wait()

    wqkvb_copy.start()
    wob_copy.start()
    mem0_copy.wait()
    x_ref[0] = y_ref[0].astype(F32)

    def layer_a(x_in, pre, unroll):
        step = functools.partial(_a_step, dh=dh, x_in=x_in, x_ref=x_ref, xb_ref=xb_ref,
                                 w_ref=w_ref, wo_ref=wo_ref, pre_ref=pre, o_ref=o_ref)

        def steps(it, carry):
            for i in range(unroll):
                carry = step(it * unroll + i, carry, i == 0, i == unroll - 1)
            return carry

        lax.fori_loop(0, n_seg // unroll, steps,
                      (mem0_ref[...].astype(F32), _layernorm(x_ref[0])))

    b_keys = functools.partial(_b_keys, x_ref=x_ref, xb_ref=xb_ref, bkv_ref=bkv_ref,
                               kv_ref=kv_ref, z_ref=z_ref)
    b_queries = functools.partial(_b_queries, x_ref=x_ref, xb_ref=xb_ref, y_ref=y_ref,
                                  bq_ref=bq_ref, bo_ref=bo_ref, kv_ref=kv_ref, z_ref=z_ref,
                                  ot_ref=ot_ref, on_ref=on_ref)

    def layer_pair(layer, carry):
        @pl.when(layer == 0)
        def _():
            layer_a(y_ref, pre_ref, A_UNROLL[0])

        @pl.when(layer == 0)
        def _():
            wqkvb_copy.wait()
            wob_copy.wait()
            _b_weights(wqkvb_ref, phi_ref, wob_ref, bq_ref, bkv_ref, bo_ref)

        @pl.when(layer == 1)
        def _():
            layer_a(x_ref, None, A_UNROLL[1])

        lax.fori_loop(0, n_iter, b_keys, 0)

        def queries(it, carry):
            def send(i):
                @pl.when(layer == 1)
                def _():
                    out_copy(it, i).start()

            b_queries(it, send)
            return carry

        lax.fori_loop(0, n_iter, queries, 0)

        return carry

    lax.fori_loop(0, 2, layer_pair, 0)
    pltpu.make_async_copy(y_ref, out_hbm, out_sem.at[0]).wait()


@functools.partial(jax.jit, static_argnames=("A_seg_len",))
def pallas_interleave_layers__memory_aug_recurrent_mem_tr__linear_kernel_hedgehog__prompt_kernel(
    A_x, A_mem0, A_Wq, A_Wk, A_Wv, A_Wo, A_seg_len, B_x, B_wqkv, B_w_phi, B_wo,
):
    del B_x
    batch, s_len, d = A_x.shape
    _, heads, dh = A_Wq.shape
    n_mem = A_mem0.shape[1]
    seg = int(A_seg_len)
    b_heads, b_dh, _ = B_w_phi.shape
    rows = n_mem + seg
    n_pairs = heads // 2
    gr = 2 * b_dh
    half = K_PAIRS * gr
    n_seg = s_len // seg
    assert batch == 1 and dh == 192 and heads == 2 * O_SPLITS[-1]
    assert n_mem % 8 == 0 and seg % 16 == 0 and 128 % seg == 0 and 2 * rows <= 128
    assert s_len % TB == 0 and s_len > TB == sum(O_ROWS) and n_seg % n_pairs == 0
    assert b_heads * b_dh == d and b_dh % 8 == 4 and d % half == 0

    def head_major(w):
        return w.transpose(1, 2, 0).reshape(heads * dh, d)

    hbm = pl.BlockSpec(memory_space=pltpu.HBM)
    out = pl.pallas_call(
        functools.partial(_kernel, dh=dh),
        out_shape=jax.ShapeDtypeStruct((n_seg, seg, d), A_x.dtype),
        in_specs=[hbm] * 9,
        out_specs=hbm,
        scratch_shapes=[
            pltpu.VMEM((n_seg, seg, d), F32),
            pltpu.VMEM((n_seg, seg, d), BF16),
            pltpu.VMEM((n_seg, seg, d), BF16),
            pltpu.VMEM((n_seg * PRE, d), BF16),
            pltpu.VMEM((n_pairs, 6 * dh, d), BF16),
            pltpu.VMEM((n_pairs, n_seg * PRE, 4 * dh), F32),
            pltpu.VMEM((n_pairs, d // 2, 6 * dh), jnp.uint32),
            pltpu.VMEM((heads * dh, d), BF16),
            pltpu.VMEM((rows, heads * dh), F32),
            pltpu.VMEM((n_mem, d), BF16),
            pltpu.VMEM((b_dh, b_dh, b_heads), BF16),
            pltpu.VMEM((d // (F_PAIRS * gr), F_PAIRS * gr // 2, 256), jnp.uint32),
            pltpu.VMEM(B_wqkv.shape, BF16),
            pltpu.VMEM(B_wo.shape, BF16),
            pltpu.VMEM((d // 2, d), jnp.uint32),
            pltpu.VMEM((d // 2, d), jnp.uint32),
            pltpu.VMEM((d // half, half, d), jnp.uint32),
            pltpu.VMEM((b_heads // 2, gr, 2 * gr), F32),
            pltpu.VMEM((b_heads // 2, 2 * gr, 128), F32),
            pltpu.VMEM((d // 2, TB), jnp.uint32),
            pltpu.VMEM((TB // 2, d), jnp.uint32),
            pltpu.SemaphoreType.DMA((n_pairs, 3)),
            pltpu.SemaphoreType.DMA((7,)),
            pltpu.SemaphoreType.DMA((1,)),
        ],
        compiler_params=pltpu.CompilerParams(vmem_limit_bytes=120 * 1024 * 1024),
    )(
        A_x.reshape(n_seg, seg, d), A_mem0.reshape(n_mem, d),
        head_major(A_Wq), head_major(A_Wk), head_major(A_Wv), A_Wo.reshape(heads * dh, d),
        B_wqkv, B_w_phi.transpose(1, 2, 0), B_wo,
    )
    return out.reshape(batch, s_len, d)
```

```python
import functools
import math

import jax
import jax.numpy as jnp
from jax import lax
import jax.experimental.pallas as pl
import jax.experimental.pallas.tpu as pltpu

F32 = jnp.float32
BF16 = jnp.bfloat16
NT = (((1,), (1,)), ((), ()))
LOG2E = math.log2(math.e)

LAG_S = (1, 2)
LAG_PV = (2, 2)
O_SPLITS = ((0, 2, 4, 6, 16), (0, 2, 4, 6, 8, 16))
A_UNROLL = (2, 2)
K_SPLIT = 512
NORM_AT = (4, 8)
PRE = 8
TB = 512
K_PAIRS = 8
Q_PAIRS = 8
Q_LAG = 1
F_PAIRS = 2
O_ROWS = (128, 128, 128, 128)


def _iota(shape, axis):
    return lax.broadcasted_iota(jnp.int32, shape, axis)


def _div(v, d):
    return (v * ((1 << 18) // d + 1)) >> 18


def _pack(x):
    return pltpu.bitcast(x.astype(BF16), jnp.uint32)


def _unpack(x):
    return pltpu.bitcast(x, BF16)


def _recip(x):
    r = pl.reciprocal(x, approx=True)
    return r * (2.0 - x * r)


def _layernorm(x):
    m = jnp.mean(x, axis=-1, keepdims=True)
    c = x - m
    v = jnp.mean(c * c, axis=-1, keepdims=True)
    return c * lax.rsqrt(v + 1e-5)


def _a_step(s, carry, opens, closes, *, layer, dh, x_in, x_ref, xb_ref, w_ref, wo_ref, pre_ref, o_ref):
    mem, xn = carry
    n_mem, seg = mem.shape[0], xn.shape[0]
    rows = n_mem + seg
    pw = 2 * dh
    n_pairs = w_ref.shape[0]
    scale = dh ** -0.5

    nxt = jnp.minimum(s + 1, x_ref.shape[0] - 1)
    prv = jnp.maximum(s - 1, 0)
    xn_next = _layernorm(x_in[nxt].astype(F32))
    xb_prev = _layernorm(x_ref[prv])
    xb_ref[prv] = xb_prev.astype(BF16)

    def schedule_before(value, early):
        t = functools.reduce(jnp.maximum, [early[i:i + 8, j:j + 128]
                                           for i in range(0, early.shape[0], 8)
                                           for j in range(0, early.shape[1], 128)])
        head = jnp.where(s < 0, t[:, :value.shape[1]], value[0:8])
        return jnp.concatenate([head, value[8:]], axis=0)

    h = jnp.concatenate([mem, xn], axis=0)
    h_short = h[:rows - PRE].astype(BF16)

    first = _iota((rows, 128), 1) < (dh - 128)
    col = _iota((rows, 2 * rows), 1)
    row = _iota((rows, 2 * rows), 0)
    is_a = col < rows
    visible = (row < n_mem) | (row >= jnp.where(is_a, col, col - rows))
    zero = jnp.zeros((rows, 128), F32)

    def block_diag(t):
        t0, t1, t2 = t[:, 0:128], t[:, 128:256], t[:, 256:384]
        top = jnp.concatenate([t0, jnp.where(first, t1, 0.0), zero], axis=1)
        bot = jnp.concatenate([zero, jnp.where(first, 0.0, t1), t2], axis=1)
        return jnp.concatenate([top, bot], axis=0).astype(BF16)

    q, k, v, probs = {}, {}, {}, {}

    def times_w(lhs, p, lo, hi):
        def part(k0, k1):
            w = _unpack(w_ref[p, k0 // 2:k1 // 2, lo:hi])
            return jnp.dot(lhs[:, k0:k1], w, preferred_element_type=F32)

        if p == 0 and lo == 0 and not opens:
            return part(K_SPLIT, lhs.shape[1]) + part(0, K_SPLIT)
        return part(0, lhs.shape[1])

    def project_short(p, j):
        done = pre_ref[p, pl.ds(pl.multiple_of(s * PRE, PRE), PRE), (j - 1) * pw:j * pw]
        return jnp.concatenate([times_w(h_short, p, j * pw, (j + 1) * pw), done], axis=0)

    def scores(p):
        sc = lax.dot_general(q[p], block_diag(k[p]), NT, preferred_element_type=F32)
        sc = jnp.where(visible, sc * scale, -1e9)
        max_a = jnp.max(jnp.where(is_a, sc, -jnp.inf), axis=1, keepdims=True)
        max_b = jnp.max(jnp.where(is_a, -jnp.inf, sc), axis=1, keepdims=True)
        e = jnp.exp(sc - jnp.where(is_a, max_a, max_b))
        sum_a = jnp.sum(jnp.where(is_a, e, 0.0), axis=1, keepdims=True)
        sum_b = jnp.sum(jnp.where(is_a, 0.0, e), axis=1, keepdims=True)
        probs[p] = e * _recip(jnp.where(is_a, sum_a, sum_b))
        if p == NORM_AT[0]:
            probs[p] = schedule_before(probs[p], xn_next)
        if p == NORM_AT[1]:
            probs[p] = schedule_before(probs[p], xb_prev)

    def values(p):
        o_ref[:, p * pw:(p + 1) * pw] = jnp.dot(
            probs[p], block_diag(v[p]), preferred_element_type=F32)

    def project_out(p0, p1, acc):
        lo, hi = p0 * pw, p1 * pw

        def part(k0, k1, c0, c1):
            return jnp.dot(o_ref[:, k0:k1], wo_ref[k0:k1, c0:c1], preferred_element_type=F32)

        d = wo_ref.shape[1]
        if p1 < n_pairs:
            r = part(lo, hi, 0, d)
        elif closes:
            return part(hi - 128, hi, 0, d) + (part(lo, hi - 128, 0, d) + acc)
        else:
            r = jnp.concatenate([part(lo, hi, 0, K_SPLIT), part(lo, hi, K_SPLIT, d)], axis=1)
        return r if acc is None else r + acc

    out = None
    lag_s, lag_v = LAG_S[layer], LAG_S[layer] + LAG_PV[layer]
    todo = list(zip(O_SPLITS[layer][:-1], O_SPLITS[layer][1:]))
    for t in range(n_pairs + lag_v):
        if t >= n_pairs:
            out = project_out(*todo.pop(0), out)
        elif pre_ref is None:
            r = times_w(h, t, 0, 3 * pw)
            q[t], k[t], v[t] = r[:, 0:pw], r[:, pw:2 * pw], r[:, 2 * pw:3 * pw]
        else:
            q[t] = times_w(h, t, 0, pw)
            k[t] = project_short(t, 1)
        if 0 <= t - lag_s < n_pairs:
            scores(t - lag_s)
        if 0 <= t - lag_v < n_pairs:
            values(t - lag_v)
        if t < n_pairs and pre_ref is not None:
            v[t] = project_short(t, 2)
    for part in todo:
        out = project_out(*part, out)

    x_ref[s] = x_in[s].astype(F32) + out[n_mem:, :]
    return out[:n_mem, :], xn_next


def _pair_reduce(t, op):
    r = t[0:8]
    for i in range(8, t.shape[0], 8):
        r = op(r, t[i:i + 8])
    r = op(r, pltpu.roll(r, 4, 0))
    return op(r, pltpu.roll(r, 2, 0))


def _tile_rows(r, n):
    return jnp.concatenate([r] * (n // 8), axis=0)


def _feature_map(p):
    n = p.shape[0]
    e_pos = jnp.exp2(p - _tile_rows(_pair_reduce(p, jnp.maximum), n))
    e_neg = jnp.exp2(_tile_rows(_pair_reduce(p, jnp.minimum), n) - p)
    inv_pos = _recip(_pair_reduce(e_pos, jnp.add))
    inv_neg = _recip(_pair_reduce(e_neg, jnp.add))
    return jnp.concatenate(
        [e_pos * _tile_rows(inv_pos, n), e_neg * _tile_rows(inv_neg, n)], axis=0)


def _fold_span(b, blk):
    return b * blk // 128 * 128, -(-(b + 1) * blk // 128) * 128


def _expand_phi(wphi_ref, phi_ref):
    dh, _, heads = wphi_ref.shape
    d = dh * heads
    gr = 2 * dh
    c = _iota((dh, d), 1)
    c_feat = c - _div(c, dh) * dh
    spread = (_div(_iota((heads, d), 1), dh) == _iota((heads, d), 0)).astype(BF16)
    by_feat = jnp.zeros((dh, d), F32)
    for e in range(dh):
        t = jnp.dot(wphi_ref[e], spread, preferred_element_type=F32)
        by_feat = jnp.where(c_feat == e, t, by_feat)
    by_feat = by_feat.astype(BF16)
    blk = F_PAIRS * gr
    r = _iota((blk, dh), 0)
    sel = (((r - _div(r, gr) * gr) >> 1) == _iota((blk, dh), 1)).astype(BF16)
    for b in range(d // blk):
        lo, hi = _fold_span(b, blk)
        r = _iota((blk, hi - lo), 0)
        head = 2 * (_div(r, gr) + b * F_PAIRS) + (r & 1)
        phi = jnp.dot(sel, by_feat[:, lo:hi], preferred_element_type=F32)
        phi_ref[b, :, 0:hi - lo] = _pack(
            jnp.where(_div(_iota((1, hi - lo), 1) + lo, dh) == head, phi, 0.0))


def _b_weights(wqkv_ref, phi_ref, wob_ref, bq_ref, bkv_ref, bo_ref):
    d = wqkv_ref.shape[0]
    blk = 2 * phi_ref.shape[1]
    half = bkv_ref.shape[1]
    bo_ref[...] = _pack(wob_ref[...])
    wv = wqkv_ref[:, 2 * d:3 * d].T
    for b in range(d // half):
        bkv_ref[b, half // 2:half, :] = _pack(wv[b * half:(b + 1) * half])
    for b in range(d // blk):
        lo, hi = _fold_span(b, blk)
        phi = _unpack(phi_ref[b, :, 0:hi - lo])
        wq = lax.dot_general(phi, wqkv_ref[:, lo:hi], NT, preferred_element_type=F32)
        wk = lax.dot_general(phi, wqkv_ref[:, d + lo:d + hi], NT, preferred_element_type=F32)
        bq_ref[b * blk // 2:(b + 1) * blk // 2, :] = _pack(wq * LOG2E)
        at = b * blk % half // 2
        bkv_ref[b * blk // half, at:at + blk // 2, :] = _pack(wk * LOG2E)


def _chunk_rows(ref, it, r0, n):
    seg = ref.shape[1]
    return pl.ds(it * (TB // seg) + r0 // seg, n // seg)


def _b_keys(it, carry, *, x_ref, xb_ref, bkv_ref, kv_ref, z_ref):
    n_blk, half, _ = bkv_ref.shape
    gr = half // K_PAIRS
    xb = xb_ref[_chunk_rows(xb_ref, it, 0, TB)].reshape(TB, -1)
    last = x_ref.shape[0] - 1
    xb_ref[last] = _layernorm(x_ref[last]).astype(BF16)
    same_head = (_iota((gr, 2 * gr), 0) >= gr // 2) == ((_iota((gr, 2 * gr), 1) & 1) == 1)

    def accumulate(b, t):
        for i in range(K_PAIRS):
            g = b * K_PAIRS + i
            phi = _feature_map(t[i * gr:(i + 1) * gr])
            z_ref[g] = jnp.where(it > 0, z_ref[g], 0.0) + jnp.sum(phi, axis=1, keepdims=True)
            kv = lax.dot_general(t[half + i * gr:half + (i + 1) * gr], phi.astype(BF16), NT,
                                 preferred_element_type=F32)
            kv_ref[g] = jnp.where(it > 0, kv_ref[g], 0.0) + jnp.where(same_head, kv, 0.0)

    pending = None
    for b in range(n_blk):
        t = lax.dot_general(_unpack(bkv_ref[b]), xb, NT, preferred_element_type=F32)
        if pending is not None:
            accumulate(*pending)
        pending = (b, t)
    accumulate(*pending)
    return carry


def _b_queries(it, send, *, x_ref, xb_ref, y_ref, bq_ref, bo_ref, kv_ref, z_ref, ot_ref, on_ref):
    n_groups, gr, _ = kv_ref.shape
    blk = Q_PAIRS * gr
    sub = _iota((8, TB), 0)
    xb = xb_ref[_chunk_rows(xb_ref, it, 0, TB)].reshape(TB, -1)

    def attend(b, t):
        outs = []
        for i in range(Q_PAIRS):
            g = b * Q_PAIRS + i
            phi = _feature_map(t[i * gr:(i + 1) * gr])
            num = jnp.dot(kv_ref[g], phi.astype(BF16), preferred_element_type=F32)
            z = jnp.concatenate([z_ref[g]] * (TB // 128), axis=1)
            inv = _recip(_pair_reduce(phi * z, jnp.add) + 1e-6)
            other = pltpu.roll(inv, 1, 0)
            inv_a = jnp.where((sub & 1) == 0, inv, other)
            inv_b = jnp.where((sub & 1) == 0, other, inv)
            n = (gr - 8) // 16
            inv = jnp.concatenate(
                [inv_a] * n + [jnp.where(sub < 4, inv_a, inv_b)] + [inv_b] * n, axis=0)
            outs.append(num * inv)
        ot_ref[b * blk // 2:(b + 1) * blk // 2, :] = _pack(jnp.concatenate(outs, axis=0))

    n_blk = n_groups // Q_PAIRS
    proj = {}
    for b in range(n_blk + Q_LAG):
        if b < n_blk:
            proj[b] = lax.dot_general(_unpack(bq_ref[b * blk // 2:(b + 1) * blk // 2, :]), xb,
                                      NT, preferred_element_type=F32)
        if b >= Q_LAG:
            attend(b - Q_LAG, proj[b - Q_LAG])
    on_ref[...] = _pack(_unpack(ot_ref[...]).T)
    r0 = 0
    for i, n in enumerate(O_ROWS):
        at = _chunk_rows(x_ref, it, r0, n)
        y = jnp.dot(_unpack(on_ref[r0 // 2:(r0 + n) // 2, :]), _unpack(bo_ref[...]),
                    preferred_element_type=F32)
        x = x_ref[at] + y.reshape((-1,) + x_ref.shape[1:])
        x_ref[at] = x
        y_ref[at] = x.astype(BF16)
        send(i)
        r0 += n


def _kernel(x_hbm, mem0_hbm, wq_hbm, wk_hbm, wv_hbm, wo_hbm, wqkvb_hbm, wphi_hbm, wob_hbm,
            out_hbm,
            x_ref, xb_ref, y_ref, xp_ref, stage_ref, pre_ref, w_ref, wo_ref, o_ref,
            mem0_ref, wphi_ref, phi_ref, wqkvb_ref, wob_ref, bo_ref, bq_ref, bkv_ref, kv_ref, z_ref, ot_ref, on_ref,
            w_sem, in_sem, out_sem, *, dh):
    n_seg, seg, d = x_ref.shape
    n_pairs = w_ref.shape[0]
    pw = 2 * dh
    n_iter = n_seg * seg // TB

    def pair_rows(p):
        return pl.ds(pl.multiple_of(p * pw, pw), pw)

    def w_copy(p, j):
        return pltpu.make_async_copy(
            (wq_hbm, wk_hbm, wv_hbm)[j].at[pair_rows(p), :],
            stage_ref.at[p, j * pw:(j + 1) * pw, :], w_sem.at[p, j])

    def out_copy(it, i):
        part = _chunk_rows(y_ref, it, sum(O_ROWS[:i]), O_ROWS[i])
        return pltpu.make_async_copy(y_ref.at[part], out_hbm.at[part], out_sem.at[0])

    def x_copy(part, rows, sem):
        return pltpu.make_async_copy(x_hbm.at[part, rows, :], y_ref.at[part, rows, :], sem)

    head, tail = slice(0, seg - PRE), slice(seg - PRE, seg)
    xt_copy = x_copy(slice(None), tail, in_sem.at[0])
    wqkvb_copy = pltpu.make_async_copy(wqkvb_hbm, wqkvb_ref, in_sem.at[1])
    wphi_copy = pltpu.make_async_copy(wphi_hbm, wphi_ref, in_sem.at[5])
    mem0_copy = pltpu.make_async_copy(mem0_hbm, mem0_ref, in_sem.at[6])
    wob_copy = pltpu.make_async_copy(wob_hbm, wob_ref, in_sem.at[2])

    wphi_copy.start()
    xt_copy.start()
    w_copy(0, 1).start()
    w_copy(0, 2).start()
    wphi_copy.wait()
    _expand_phi(wphi_ref, phi_ref)
    xt_copy.wait()

    xp_ref[...] = _layernorm(y_ref[:, tail, :].astype(F32).reshape(n_seg * PRE, d)).astype(BF16)

    mem0_copy.start()
    w_copy(0, 0).start()
    for j in (1, 2, 0):
        w_copy(1, j).start()

    def pre_project(p, carry):
        @pl.when(p + 2 < n_pairs)
        def _():
            for j in range(3):
                w_copy(jnp.minimum(p + 2, n_pairs - 1), j).start()

        part = pl.ds(p * (n_seg // n_pairs), n_seg // n_pairs)
        x_copy(part, head, in_sem.at[3]).start()
        pltpu.make_async_copy(
            wo_hbm.at[pair_rows(p), :], wo_ref.at[pair_rows(p), :], in_sem.at[4]).start()
        before = jnp.maximum(p - 1, 0)

        @pl.when(p > 0)
        def _():
            w_copy(before, 0).wait()

        w_copy(p, 1).wait()
        w_copy(p, 2).wait()
        pre_ref[p] = lax.dot_general(xp_ref[...], stage_ref[p, pw:3 * pw, :], NT,
                                     preferred_element_type=F32)
        w_ref[before, :, 0:pw] = _pack(stage_ref[before, pair_rows(jnp.where(p > 0, 0, 1)), :].T)
        for j in (1, 2):
            w_ref[p, :, j * pw:(j + 1) * pw] = _pack(stage_ref[p, j * pw:(j + 1) * pw, :].T)
        return carry

    lax.fori_loop(0, n_pairs, pre_project, 0)

    w_copy(n_pairs - 1, 0).wait()
    w_ref[n_pairs - 1, :, 0:pw] = _pack(stage_ref[n_pairs - 1, 0:pw, :].T)
    x_copy(slice(None), head, in_sem.at[3]).wait()
    pltpu.make_async_copy(wo_hbm, wo_ref, in_sem.at[4]).wait()

    wqkvb_copy.start()
    wob_copy.start()
    mem0_copy.wait()
    x_ref[0] = y_ref[0].astype(F32)

    def layer_a(layer, x_in, pre):
        unroll = A_UNROLL[layer]
        step = functools.partial(_a_step, layer=layer, dh=dh, x_in=x_in, x_ref=x_ref, xb_ref=xb_ref,
                                 w_ref=w_ref, wo_ref=wo_ref, pre_ref=pre, o_ref=o_ref)

        def steps(it, carry):
            for i in range(unroll):
                carry = step(it * unroll + i, carry, i == 0, i == unroll - 1)
            return carry

        lax.fori_loop(0, n_seg // unroll, steps,
                      (mem0_ref[...].astype(F32), _layernorm(x_ref[0])))

    b_keys = functools.partial(_b_keys, x_ref=x_ref, xb_ref=xb_ref, bkv_ref=bkv_ref,
                               kv_ref=kv_ref, z_ref=z_ref)
    b_queries = functools.partial(_b_queries, x_ref=x_ref, xb_ref=xb_ref, y_ref=y_ref,
                                  bq_ref=bq_ref, bo_ref=bo_ref, kv_ref=kv_ref, z_ref=z_ref,
                                  ot_ref=ot_ref, on_ref=on_ref)

    def layer_pair(layer, carry):
        @pl.when(layer == 0)
        def _():
            layer_a(0, y_ref, pre_ref)

        @pl.when(layer == 0)
        def _():
            wqkvb_copy.wait()
            wob_copy.wait()
            _b_weights(wqkvb_ref, phi_ref, wob_ref, bq_ref, bkv_ref, bo_ref)

        @pl.when(layer == 1)
        def _():
            layer_a(1, x_ref, None)

        lax.fori_loop(0, n_iter, b_keys, 0)

        def queries(it, carry):
            def send(i):
                @pl.when(layer == 1)
                def _():
                    out_copy(it, i).start()

            b_queries(it, send)
            return carry

        lax.fori_loop(0, n_iter, queries, 0)

        return carry

    lax.fori_loop(0, 2, layer_pair, 0)
    pltpu.make_async_copy(y_ref, out_hbm, out_sem.at[0]).wait()


@functools.partial(jax.jit, static_argnames=("A_seg_len",))
def pallas_interleave_layers__memory_aug_recurrent_mem_tr__linear_kernel_hedgehog__prompt_kernel(
    A_x, A_mem0, A_Wq, A_Wk, A_Wv, A_Wo, A_seg_len, B_x, B_wqkv, B_w_phi, B_wo,
):
    del B_x
    batch, s_len, d = A_x.shape
    _, heads, dh = A_Wq.shape
    n_mem = A_mem0.shape[1]
    seg = int(A_seg_len)
    b_heads, b_dh, _ = B_w_phi.shape
    rows = n_mem + seg
    n_pairs = heads // 2
    gr = 2 * b_dh
    half = K_PAIRS * gr
    n_seg = s_len // seg
    assert batch == 1 and dh == 192 and heads == 2 * O_SPLITS[0][-1]
    assert n_mem % 8 == 0 and seg % 16 == 0 and 128 % seg == 0 and 2 * rows <= 128
    assert s_len % TB == 0 and s_len > TB == sum(O_ROWS) and n_seg % n_pairs == 0
    assert b_heads * b_dh == d and b_dh % 8 == 4 and d % half == 0

    def head_major(w):
        return w.transpose(1, 2, 0).reshape(heads * dh, d)

    hbm = pl.BlockSpec(memory_space=pltpu.HBM)
    out = pl.pallas_call(
        functools.partial(_kernel, dh=dh),
        out_shape=jax.ShapeDtypeStruct((n_seg, seg, d), A_x.dtype),
        in_specs=[hbm] * 9,
        out_specs=hbm,
        scratch_shapes=[
            pltpu.VMEM((n_seg, seg, d), F32),
            pltpu.VMEM((n_seg, seg, d), BF16),
            pltpu.VMEM((n_seg, seg, d), BF16),
            pltpu.VMEM((n_seg * PRE, d), BF16),
            pltpu.VMEM((n_pairs, 6 * dh, d), BF16),
            pltpu.VMEM((n_pairs, n_seg * PRE, 4 * dh), F32),
            pltpu.VMEM((n_pairs, d // 2, 6 * dh), jnp.uint32),
            pltpu.VMEM((heads * dh, d), BF16),
            pltpu.VMEM((rows, heads * dh), F32),
            pltpu.VMEM((n_mem, d), BF16),
            pltpu.VMEM((b_dh, b_dh, b_heads), BF16),
            pltpu.VMEM((d // (F_PAIRS * gr), F_PAIRS * gr // 2, 256), jnp.uint32),
            pltpu.VMEM(B_wqkv.shape, BF16),
            pltpu.VMEM(B_wo.shape, BF16),
            pltpu.VMEM((d // 2, d), jnp.uint32),
            pltpu.VMEM((d // 2, d), jnp.uint32),
            pltpu.VMEM((d // half, half, d), jnp.uint32),
            pltpu.VMEM((b_heads // 2, gr, 2 * gr), F32),
            pltpu.VMEM((b_heads // 2, 2 * gr, 128), F32),
            pltpu.VMEM((d // 2, TB), jnp.uint32),
            pltpu.VMEM((TB // 2, d), jnp.uint32),
            pltpu.SemaphoreType.DMA((n_pairs, 3)),
            pltpu.SemaphoreType.DMA((7,)),
            pltpu.SemaphoreType.DMA((1,)),
        ],
        compiler_params=pltpu.CompilerParams(vmem_limit_bytes=120 * 1024 * 1024),
    )(
        A_x.reshape(n_seg, seg, d), A_mem0.reshape(n_mem, d),
        head_major(A_Wq), head_major(A_Wk), head_major(A_Wv), A_Wo.reshape(heads * dh, d),
        B_wqkv, B_w_phi.transpose(1, 2, 0), B_wo,
    )
    return out.reshape(batch, s_len, d)
```

```python
import functools
import math

import jax
import jax.numpy as jnp
from jax import lax
import jax.experimental.pallas as pl
import jax.experimental.pallas.tpu as pltpu

F32 = jnp.float32
BF16 = jnp.bfloat16
NT = (((1,), (1,)), ((), ()))
LOG2E = math.log2(math.e)

LAG_S = (1, 2)
LAG_PV = (2, 2)
O_SPLITS = ((0, 2, 4, 6, 16), (0, 2, 4, 6, 8, 16))
A_UNROLL = (2, 2)
K_SPLIT = 512
NORM_AT = (4, 8)
PRE = 8
TB = 512
K_PAIRS = 8
Q_PAIRS = 8
F_PAIRS = 2
O_ROWS = (128, 128, 128, 128)


def _iota(shape, axis):
    return lax.broadcasted_iota(jnp.int32, shape, axis)


def _div(v, d):
    return (v * ((1 << 18) // d + 1)) >> 18


def _pack(x):
    return pltpu.bitcast(x.astype(BF16), jnp.uint32)


def _unpack(x):
    return pltpu.bitcast(x, BF16)


def _recip(x):
    r = pl.reciprocal(x, approx=True)
    return r * (2.0 - x * r)


def _layernorm(x):
    m = jnp.mean(x, axis=-1, keepdims=True)
    c = x - m
    v = jnp.mean(c * c, axis=-1, keepdims=True)
    return c * lax.rsqrt(v + 1e-5)


def _a_step(s, carry, opens, closes, *, layer, dh, x_in, x_ref, xb_ref, w_ref, wo_ref, pre_ref,
            o_ref):
    mem, xn = carry
    n_mem, seg = mem.shape[0], xn.shape[0]
    rows = n_mem + seg
    pw = 2 * dh
    n_pairs = w_ref.shape[0]
    scale = dh ** -0.5

    nxt = jnp.minimum(s + 1, x_ref.shape[0] - 1)
    prv = jnp.maximum(s - 1, 0)
    xn_next = _layernorm(x_in[nxt].astype(F32))
    xb_prev = _layernorm(x_ref[prv])
    xb_ref[prv] = xb_prev.astype(BF16)

    def schedule_before(value, early):
        t = functools.reduce(jnp.maximum, [early[i:i + 8, j:j + 128]
                                           for i in range(0, early.shape[0], 8)
                                           for j in range(0, early.shape[1], 128)])
        head = jnp.where(s < 0, t[:, :value.shape[1]], value[0:8])
        return jnp.concatenate([head, value[8:]], axis=0)

    h = jnp.concatenate([mem, xn], axis=0)
    h_short = h[:rows - PRE].astype(BF16)

    first = _iota((rows, 128), 1) < (dh - 128)
    col = _iota((rows, 2 * rows), 1)
    row = _iota((rows, 2 * rows), 0)
    is_a = col < rows
    visible = (row < n_mem) | (row >= jnp.where(is_a, col, col - rows))
    zero = jnp.zeros((rows, 128), F32)

    def block_diag(t):
        t0, t1, t2 = t[:, 0:128], t[:, 128:256], t[:, 256:384]
        top = jnp.concatenate([t0, jnp.where(first, t1, 0.0), zero], axis=1)
        bot = jnp.concatenate([zero, jnp.where(first, 0.0, t1), t2], axis=1)
        return jnp.concatenate([top, bot], axis=0).astype(BF16)

    q, k, v, probs = {}, {}, {}, {}

    def times_w(lhs, p, lo, hi):
        def part(k0, k1):
            w = _unpack(w_ref[p, k0 // 2:k1 // 2, lo:hi])
            return jnp.dot(lhs[:, k0:k1], w, preferred_element_type=F32)

        if p == 0 and lo == 0 and not opens:
            return part(K_SPLIT, lhs.shape[1]) + part(0, K_SPLIT)
        return part(0, lhs.shape[1])

    def project_short(p, j):
        done = pre_ref[p, pl.ds(pl.multiple_of(s * PRE, PRE), PRE), (j - 1) * pw:j * pw]
        return jnp.concatenate([times_w(h_short, p, j * pw, (j + 1) * pw), done], axis=0)

    def scores(p):
        sc = lax.dot_general(q[p], block_diag(k[p]), NT, preferred_element_type=F32)
        sc = jnp.where(visible, sc * scale, -1e9)
        max_a = jnp.max(jnp.where(is_a, sc, -jnp.inf), axis=1, keepdims=True)
        max_b = jnp.max(jnp.where(is_a, -jnp.inf, sc), axis=1, keepdims=True)
        e = jnp.exp(sc - jnp.where(is_a, max_a, max_b))
        sum_a = jnp.sum(jnp.where(is_a, e, 0.0), axis=1, keepdims=True)
        sum_b = jnp.sum(jnp.where(is_a, 0.0, e), axis=1, keepdims=True)
        probs[p] = e * _recip(jnp.where(is_a, sum_a, sum_b))
        if p == NORM_AT[0]:
            probs[p] = schedule_before(probs[p], xn_next)
        if p == NORM_AT[1]:
            probs[p] = schedule_before(probs[p], xb_prev)

    def values(p):
        o_ref[:, p * pw:(p + 1) * pw] = jnp.dot(
            probs[p], block_diag(v[p]), preferred_element_type=F32)

    def project_out(p0, p1, acc):
        lo, hi = p0 * pw, p1 * pw

        def part(k0, k1, c0, c1):
            return jnp.dot(o_ref[:, k0:k1], wo_ref[k0:k1, c0:c1], preferred_element_type=F32)

        d = wo_ref.shape[1]
        if p1 < n_pairs:
            r = part(lo, hi, 0, d)
        elif closes:
            return part(hi - 128, hi, 0, d) + (part(lo, hi - 128, 0, d) + acc)
        else:
            r = jnp.concatenate([part(lo, hi, 0, K_SPLIT), part(lo, hi, K_SPLIT, d)], axis=1)
        return r if acc is None else r + acc

    out = None
    lag_s, lag_v = LAG_S[layer], LAG_S[layer] + LAG_PV[layer]
    todo = list(zip(O_SPLITS[layer][:-1], O_SPLITS[layer][1:]))
    for t in range(n_pairs + lag_v):
        if t >= n_pairs:
            out = project_out(*todo.pop(0), out)
        elif pre_ref is None:
            r = times_w(h, t, 0, 3 * pw)
            q[t], k[t], v[t] = r[:, 0:pw], r[:, pw:2 * pw], r[:, 2 * pw:3 * pw]
        else:
            q[t] = times_w(h, t, 0, pw)
            k[t] = project_short(t, 1)
        if 0 <= t - lag_s < n_pairs:
            scores(t - lag_s)
        if 0 <= t - lag_v < n_pairs:
            values(t - lag_v)
        if t < n_pairs and pre_ref is not None:
            v[t] = project_short(t, 2)
    for part in todo:
        out = project_out(*part, out)

    x_ref[s] = x_in[s].astype(F32) + out[n_mem:, :]
    return out[:n_mem, :], xn_next


def _pair_reduce(t, op):
    r = t[0:8]
    for i in range(8, t.shape[0], 8):
        r = op(r, t[i:i + 8])
    r = op(r, pltpu.roll(r, 4, 0))
    return op(r, pltpu.roll(r, 2, 0))


def _tile_rows(r, n):
    return jnp.concatenate([r] * (n // 8), axis=0)


def _feature_map(p):
    n = p.shape[0]
    e_pos = jnp.exp2(p - _tile_rows(_pair_reduce(p, jnp.maximum), n))
    e_neg = jnp.exp2(_tile_rows(_pair_reduce(p, jnp.minimum), n) - p)
    inv_pos = _recip(_pair_reduce(e_pos, jnp.add))
    inv_neg = _recip(_pair_reduce(e_neg, jnp.add))
    return jnp.concatenate(
        [e_pos * _tile_rows(inv_pos, n), e_neg * _tile_rows(inv_neg, n)], axis=0)


def _fold_span(b, blk):
    return b * blk // 128 * 128, -(-(b + 1) * blk // 128) * 128


def _expand_phi(wphi_ref, phi_ref):
    dh, _, heads = wphi_ref.shape
    d = dh * heads
    gr = 2 * dh
    c = _iota((dh, d), 1)
    c_feat = c - _div(c, dh) * dh
    spread = (_div(_iota((heads, d), 1), dh) == _iota((heads, d), 0)).astype(BF16)
    by_feat = jnp.zeros((dh, d), F32)
    for e in range(dh):
        t = jnp.dot(wphi_ref[e], spread, preferred_element_type=F32)
        by_feat = jnp.where(c_feat == e, t, by_feat)
    by_feat = by_feat.astype(BF16)
    blk = F_PAIRS * gr
    r = _iota((blk, dh), 0)
    sel = (((r - _div(r, gr) * gr) >> 1) == _iota((blk, dh), 1)).astype(BF16)
    for b in range(d // blk):
        lo, hi = _fold_span(b, blk)
        r = _iota((blk, hi - lo), 0)
        head = 2 * (_div(r, gr) + b * F_PAIRS) + (r & 1)
        phi = jnp.dot(sel, by_feat[:, lo:hi], preferred_element_type=F32)
        phi_ref[b, :, 0:hi - lo] = _pack(
            jnp.where(_div(_iota((1, hi - lo), 1) + lo, dh) == head, phi, 0.0))


def _b_weights(wqkv_ref, phi_ref, wob_ref, bq_ref, bkv_ref, bo_ref):
    d = wqkv_ref.shape[0]
    blk = 2 * phi_ref.shape[1]
    half = bkv_ref.shape[1]
    bo_ref[...] = _pack(wob_ref[...])
    wv = wqkv_ref[:, 2 * d:3 * d].T
    for b in range(d // half):
        bkv_ref[b, half // 2:half, :] = _pack(wv[b * half:(b + 1) * half])
    for b in range(d // blk):
        lo, hi = _fold_span(b, blk)
        phi = _unpack(phi_ref[b, :, 0:hi - lo])
        wq = lax.dot_general(phi, wqkv_ref[:, lo:hi], NT, preferred_element_type=F32)
        wk = lax.dot_general(phi, wqkv_ref[:, d + lo:d + hi], NT, preferred_element_type=F32)
        bq_ref[b * blk // 2:(b + 1) * blk // 2, :] = _pack(wq * LOG2E)
        at = b * blk % half // 2
        bkv_ref[b * blk // half, at:at + blk // 2, :] = _pack(wk * LOG2E)


def _chunk_rows(ref, it, r0, n):
    seg = ref.shape[1]
    return pl.ds(it * (TB // seg) + r0 // seg, n // seg)


def _b_keys(it, carry, *, x_ref, xb_ref, bkv_ref, kv_ref, z_ref):
    n_blk, half, _ = bkv_ref.shape
    gr = half // K_PAIRS
    xb = xb_ref[_chunk_rows(xb_ref, it, 0, TB)].reshape(TB, -1)
    last = x_ref.shape[0] - 1
    xb_ref[last] = _layernorm(x_ref[last]).astype(BF16)
    same_head = (_iota((gr, 2 * gr), 0) >= gr // 2) == ((_iota((gr, 2 * gr), 1) & 1) == 1)

    def accumulate(b, t):
        for i in range(K_PAIRS):
            g = b * K_PAIRS + i
            phi = _feature_map(t[i * gr:(i + 1) * gr])
            z_ref[g] = jnp.where(it > 0, z_ref[g], 0.0) + jnp.sum(phi, axis=1, keepdims=True)
            kv = lax.dot_general(t[half + i * gr:half + (i + 1) * gr], phi.astype(BF16), NT,
                                 preferred_element_type=F32)
            kv_ref[g] = jnp.where(it > 0, kv_ref[g], 0.0) + jnp.where(same_head, kv, 0.0)

    pending = None
    for b in range(n_blk):
        t = lax.dot_general(_unpack(bkv_ref[b]), xb, NT, preferred_element_type=F32)
        if pending is not None:
            accumulate(*pending)
        pending = (b, t)
    accumulate(*pending)
    return carry


def _b_queries(it, send, *, x_ref, xb_ref, y_ref, bq_ref, bo_ref, kv_ref, z_ref, ot_ref, on_ref):
    n_groups, gr, _ = kv_ref.shape
    blk = Q_PAIRS * gr
    sub = _iota((8, TB), 0)
    xb = xb_ref[_chunk_rows(xb_ref, it, 0, TB)].reshape(TB, -1)

    def attend(b, t):
        outs = []
        for i in range(Q_PAIRS):
            g = b * Q_PAIRS + i
            phi = _feature_map(t[i * gr:(i + 1) * gr])
            num = jnp.dot(kv_ref[g], phi.astype(BF16), preferred_element_type=F32)
            z = jnp.concatenate([z_ref[g]] * (TB // 128), axis=1)
            inv = _recip(_pair_reduce(phi * z, jnp.add) + 1e-6)
            other = pltpu.roll(inv, 1, 0)
            inv_a = jnp.where((sub & 1) == 0, inv, other)
            inv_b = jnp.where((sub & 1) == 0, other, inv)
            n = (gr - 8) // 16
            inv = jnp.concatenate(
                [inv_a] * n + [jnp.where(sub < 4, inv_a, inv_b)] + [inv_b] * n, axis=0)
            outs.append(num * inv)
        ot_ref[b * blk // 2:(b + 1) * blk // 2, :] = _pack(jnp.concatenate(outs, axis=0))

    n_blk = n_groups // Q_PAIRS
    proj = {}
    for b in range(n_blk + 1):
        if b < n_blk:
            proj[b] = lax.dot_general(_unpack(bq_ref[b * blk // 2:(b + 1) * blk // 2, :]), xb,
                                      NT, preferred_element_type=F32)
        if b > 0:
            attend(b - 1, proj[b - 1])
    on_ref[...] = _pack(_unpack(ot_ref[...]).T)
    r0 = 0
    for i, n in enumerate(O_ROWS):
        at = _chunk_rows(x_ref, it, r0, n)
        y = jnp.dot(_unpack(on_ref[r0 // 2:(r0 + n) // 2, :]), _unpack(bo_ref[...]),
                    preferred_element_type=F32)
        x = x_ref[at] + y.reshape((-1,) + x_ref.shape[1:])
        x_ref[at] = x
        y_ref[at] = x.astype(BF16)
        send(i)
        r0 += n


def _kernel(x_hbm, mem0_hbm, wq_hbm, wk_hbm, wv_hbm, wo_hbm, wqkvb_hbm, wphi_hbm, wob_hbm,
            out_hbm,
            x_ref, xb_ref, y_ref, xp_ref, stage_ref, pre_ref, w_ref, wo_ref, o_ref,
            mem0_ref, wphi_ref, phi_ref, wqkvb_ref, wob_ref, bo_ref, bq_ref, bkv_ref,
            kv_ref, z_ref, ot_ref, on_ref,
            w_sem, in_sem, out_sem, *, dh):
    n_seg, seg, d = x_ref.shape
    n_pairs = w_ref.shape[0]
    pw = 2 * dh
    n_iter = n_seg * seg // TB

    def pair_rows(p):
        return pl.ds(pl.multiple_of(p * pw, pw), pw)

    def w_copy(p, j):
        return pltpu.make_async_copy(
            (wq_hbm, wk_hbm, wv_hbm)[j].at[pair_rows(p), :],
            stage_ref.at[p, j * pw:(j + 1) * pw, :], w_sem.at[p, j])

    def out_copy(it, i):
        part = _chunk_rows(y_ref, it, sum(O_ROWS[:i]), O_ROWS[i])
        return pltpu.make_async_copy(y_ref.at[part], out_hbm.at[part], out_sem.at[0])

    def x_copy(part, rows, sem):
        return pltpu.make_async_copy(x_hbm.at[part, rows, :], y_ref.at[part, rows, :], sem)

    head, tail = slice(0, seg - PRE), slice(seg - PRE, seg)
    xt_copy = x_copy(slice(None), tail, in_sem.at[0])
    wqkvb_copy = pltpu.make_async_copy(wqkvb_hbm, wqkvb_ref, in_sem.at[1])
    wphi_copy = pltpu.make_async_copy(wphi_hbm, wphi_ref, in_sem.at[5])
    mem0_copy = pltpu.make_async_copy(mem0_hbm, mem0_ref, in_sem.at[6])
    wob_copy = pltpu.make_async_copy(wob_hbm, wob_ref, in_sem.at[2])

    wphi_copy.start()
    xt_copy.start()
    w_copy(0, 1).start()
    w_copy(0, 2).start()
    wphi_copy.wait()
    _expand_phi(wphi_ref, phi_ref)
    xt_copy.wait()

    xp_ref[...] = _layernorm(y_ref[:, tail, :].astype(F32).reshape(n_seg * PRE, d)).astype(BF16)

    mem0_copy.start()
    w_copy(0, 0).start()
    for j in (1, 2, 0):
        w_copy(1, j).start()

    def pre_project(p, carry):
        @pl.when(p + 2 < n_pairs)
        def _():
            for j in range(3):
                w_copy(jnp.minimum(p + 2, n_pairs - 1), j).start()

        part = pl.ds(p * (n_seg // n_pairs), n_seg // n_pairs)
        x_copy(part, head, in_sem.at[3]).start()
        pltpu.make_async_copy(
            wo_hbm.at[pair_rows(p), :], wo_ref.at[pair_rows(p), :], in_sem.at[4]).start()
        before = jnp.maximum(p - 1, 0)

        @pl.when(p > 0)
        def _():
            w_copy(before, 0).wait()

        w_copy(p, 1).wait()
        w_copy(p, 2).wait()
        pre_ref[p] = lax.dot_general(xp_ref[...], stage_ref[p, pw:3 * pw, :], NT,
                                     preferred_element_type=F32)
        w_ref[before, :, 0:pw] = _pack(stage_ref[before, pair_rows(jnp.where(p > 0, 0, 1)), :].T)
        for j in (1, 2):
            w_ref[p, :, j * pw:(j + 1) * pw] = _pack(stage_ref[p, j * pw:(j + 1) * pw, :].T)
        return carry

    lax.fori_loop(0, n_pairs, pre_project, 0)

    w_copy(n_pairs - 1, 0).wait()
    w_ref[n_pairs - 1, :, 0:pw] = _pack(stage_ref[n_pairs - 1, 0:pw, :].T)
    x_copy(slice(None), head, in_sem.at[3]).wait()
    pltpu.make_async_copy(wo_hbm, wo_ref, in_sem.at[4]).wait()

    wqkvb_copy.start()
    wob_copy.start()
    mem0_copy.wait()
    x_ref[0] = y_ref[0].astype(F32)

    def layer_a(layer, x_in, pre):
        unroll = A_UNROLL[layer]
        step = functools.partial(_a_step, layer=layer, dh=dh, x_in=x_in, x_ref=x_ref, xb_ref=xb_ref,
                                 w_ref=w_ref, wo_ref=wo_ref, pre_ref=pre, o_ref=o_ref)

        def steps(it, carry):
            for i in range(unroll):
                carry = step(it * unroll + i, carry, i == 0, i == unroll - 1)
            return carry

        lax.fori_loop(0, n_seg // unroll, steps,
                      (mem0_ref[...].astype(F32), _layernorm(x_ref[0])))

    b_keys = functools.partial(_b_keys, x_ref=x_ref, xb_ref=xb_ref, bkv_ref=bkv_ref,
                               kv_ref=kv_ref, z_ref=z_ref)
    b_queries = functools.partial(_b_queries, x_ref=x_ref, xb_ref=xb_ref, y_ref=y_ref,
                                  bq_ref=bq_ref, bo_ref=bo_ref, kv_ref=kv_ref, z_ref=z_ref,
                                  ot_ref=ot_ref, on_ref=on_ref)

    def layer_pair(layer, carry):
        @pl.when(layer == 0)
        def _():
            layer_a(0, y_ref, pre_ref)

        @pl.when(layer == 0)
        def _():
            wqkvb_copy.wait()
            wob_copy.wait()
            _b_weights(wqkvb_ref, phi_ref, wob_ref, bq_ref, bkv_ref, bo_ref)

        @pl.when(layer == 1)
        def _():
            layer_a(1, x_ref, None)

        lax.fori_loop(0, n_iter, b_keys, 0)

        def queries(it, carry):
            def send(i):
                @pl.when(layer == 1)
                def _():
                    out_copy(it, i).start()

            b_queries(it, send)
            return carry

        lax.fori_loop(0, n_iter, queries, 0)

        return carry

    lax.fori_loop(0, 2, layer_pair, 0)
    pltpu.make_async_copy(y_ref, out_hbm, out_sem.at[0]).wait()


@functools.partial(jax.jit, static_argnames=("A_seg_len",))
def pallas_interleave_layers__memory_aug_recurrent_mem_tr__linear_kernel_hedgehog__prompt_kernel(
    A_x, A_mem0, A_Wq, A_Wk, A_Wv, A_Wo, A_seg_len, B_x, B_wqkv, B_w_phi, B_wo,
):
    del B_x
    batch, s_len, d = A_x.shape
    _, heads, dh = A_Wq.shape
    n_mem = A_mem0.shape[1]
    seg = int(A_seg_len)
    b_heads, b_dh, _ = B_w_phi.shape
    rows = n_mem + seg
    n_pairs = heads // 2
    gr = 2 * b_dh
    half = K_PAIRS * gr
    n_seg = s_len // seg
    assert batch == 1 and dh == 192 and heads == 2 * O_SPLITS[0][-1]
    assert n_mem % 8 == 0 and seg % 16 == 0 and 128 % seg == 0 and 2 * rows <= 128
    assert s_len % TB == 0 and s_len > TB == sum(O_ROWS) and n_seg % n_pairs == 0
    assert b_heads * b_dh == d and b_dh % 8 == 4 and d % half == 0

    def head_major(w):
        return w.transpose(1, 2, 0).reshape(heads * dh, d)

    hbm = pl.BlockSpec(memory_space=pltpu.HBM)
    out = pl.pallas_call(
        functools.partial(_kernel, dh=dh),
        out_shape=jax.ShapeDtypeStruct((n_seg, seg, d), A_x.dtype),
        in_specs=[hbm] * 9,
        out_specs=hbm,
        scratch_shapes=[
            pltpu.VMEM((n_seg, seg, d), F32),
            pltpu.VMEM((n_seg, seg, d), BF16),
            pltpu.VMEM((n_seg, seg, d), BF16),
            pltpu.VMEM((n_seg * PRE, d), BF16),
            pltpu.VMEM((n_pairs, 6 * dh, d), BF16),
            pltpu.VMEM((n_pairs, n_seg * PRE, 4 * dh), F32),
            pltpu.VMEM((n_pairs, d // 2, 6 * dh), jnp.uint32),
            pltpu.VMEM((heads * dh, d), BF16),
            pltpu.VMEM((rows, heads * dh), F32),
            pltpu.VMEM((n_mem, d), BF16),
            pltpu.VMEM((b_dh, b_dh, b_heads), BF16),
            pltpu.VMEM((d // (F_PAIRS * gr), F_PAIRS * gr // 2, 256), jnp.uint32),
            pltpu.VMEM(B_wqkv.shape, BF16),
            pltpu.VMEM(B_wo.shape, BF16),
            pltpu.VMEM((d // 2, d), jnp.uint32),
            pltpu.VMEM((d // 2, d), jnp.uint32),
            pltpu.VMEM((d // half, half, d), jnp.uint32),
            pltpu.VMEM((b_heads // 2, gr, 2 * gr), F32),
            pltpu.VMEM((b_heads // 2, 2 * gr, 128), F32),
            pltpu.VMEM((d // 2, TB), jnp.uint32),
            pltpu.VMEM((TB // 2, d), jnp.uint32),
            pltpu.SemaphoreType.DMA((n_pairs, 3)),
            pltpu.SemaphoreType.DMA((7,)),
            pltpu.SemaphoreType.DMA((1,)),
        ],
        compiler_params=pltpu.CompilerParams(vmem_limit_bytes=120 * 1024 * 1024),
    )(
        A_x.reshape(n_seg, seg, d), A_mem0.reshape(n_mem, d),
        head_major(A_Wq), head_major(A_Wk), head_major(A_Wv), A_Wo.reshape(heads * dh, d),
        B_wqkv, B_w_phi.transpose(1, 2, 0), B_wo,
    )
    return out.reshape(batch, s_len, d)
```

```python
import functools
import math

import jax
import jax.numpy as jnp
from jax import lax
import jax.experimental.pallas as pl
import jax.experimental.pallas.tpu as pltpu

F32 = jnp.float32
BF16 = jnp.bfloat16
NT = (((1,), (1,)), ((), ()))
LOG2E = math.log2(math.e)
MASKED = -1e9

LAG_S = (2, 2)
LAG_PV = (2, 2)
O_SPLITS = ((0, 2, 4, 6, 8, 13, 16), (0, 2, 4, 6, 8, 13, 16))
VPU_ROWS = ((range(15), ()), (range(15), ()))
VPU_DUE = (0, 0)
EXP_AHEAD = 2
A_UNROLL = (2, 2)
K_SPLIT = 512
NORM_AT = (4, 8)
PRE = 8
TB = 512
K_PAIRS = 8
Q_PAIRS = 8
F_PAIRS = 2
O_ROWS = (128, 128, 128, 128)


def _iota(shape, axis):
    return lax.broadcasted_iota(jnp.int32, shape, axis)


def _div(v, d):
    return (v * ((1 << 18) // d + 1)) >> 18


def _pack(x):
    return pltpu.bitcast(x.astype(BF16), jnp.uint32)


def _unpack(x):
    return pltpu.bitcast(x, BF16)


def _recip(x):
    r = pl.reciprocal(x, approx=True)
    return r * (2.0 - x * r)


def _layernorm(x):
    m = jnp.mean(x, axis=-1, keepdims=True)
    c = x - m
    v = jnp.mean(c * c, axis=-1, keepdims=True)
    return c * lax.rsqrt(v + 1e-5)


def _a_step(s, carry, opens, closes, *, layer, dh, x_in, x_ref, xb_ref, w_ref, wo_ref, pre_ref,
            o_ref, near_ref):
    mem, xn = carry
    n_mem, seg = mem.shape[0], xn.shape[0]
    rows = n_mem + seg
    pw = 2 * dh
    n_pairs = w_ref.shape[0]
    scale = dh ** -0.5

    nxt = jnp.minimum(s + 1, x_ref.shape[0] - 1)
    prv = jnp.maximum(s - 1, 0)
    xn_next = _layernorm(x_in[nxt].astype(F32))
    xb_prev = _layernorm(x_ref[prv])
    xb_ref[prv] = xb_prev.astype(BF16)

    def after(early, value):
        return value if early is None else jnp.where(s < 0, early[:, :value.shape[1]], value)

    def after_all(early, value):
        t = functools.reduce(jnp.maximum, [early[i:i + 8, j:j + 128]
                                           for i in range(0, early.shape[0], 8)
                                           for j in range(0, early.shape[1], 128)])
        return jnp.concatenate([after(t, value[0:8]), value[8:]], axis=0)

    h = jnp.concatenate([mem, xn], axis=0)
    h_short = h[:rows - PRE].astype(BF16)

    first = _iota((rows, 128), 1) < 64
    zero = jnp.zeros((rows, 128), F32)

    def key_blocks(t):
        t0, t1, t2 = t[:, 0:128], t[:, 128:256], t[:, 256:384]
        top = jnp.concatenate([t0, jnp.where(first, t1, 0.0), zero], axis=1)
        bot = jnp.concatenate([zero, jnp.where(first, 0.0, t1), t2], axis=1)
        return jnp.concatenate([top, bot], axis=0).astype(BF16)

    def value_blocks(t):
        mine = jnp.concatenate([first] * 3, axis=1)
        return jnp.concatenate(
            [jnp.where(mine, t, 0.0), jnp.where(mine, 0.0, t)], axis=0).astype(BF16)

    def vpu_rows(p):
        return [n_mem + 8 * i for i, pairs in enumerate(VPU_ROWS[layer]) if p in pairs]

    def mxu_rows(p):
        return [r for r in range(0, rows, 8) if r not in vpu_rows(p)]

    def pick(t, starts):
        return jnp.concatenate([t[r:r + 8] for r in starts], axis=0)

    q, k, v, probs, near_done = {}, {}, {}, {}, {}

    def times_w(lhs, p, lo, hi):
        def part(k0, k1):
            w = _unpack(w_ref[p, k0 // 2:k1 // 2, lo:hi])
            return jnp.dot(lhs[:, k0:k1], w, preferred_element_type=F32)

        if p == 0 and lo == 0 and not opens:
            return part(K_SPLIT, lhs.shape[1]) + part(0, K_SPLIT)
        return part(0, lhs.shape[1])

    def project_short(p, j):
        done = pre_ref[p, pl.ds(pl.multiple_of(s * PRE, PRE), PRE), (j - 1) * pw:j * pw]
        return jnp.concatenate([times_w(h_short, p, j * pw, (j + 1) * pw), done], axis=0)

    def scores(p):
        col = pick(_iota((rows, 2 * rows), 1), mxu_rows(p))
        row = pick(_iota((rows, 2 * rows), 0), mxu_rows(p))
        is_a = col < rows
        visible = (row < n_mem) | (row >= jnp.where(is_a, col, col - rows))
        sc = lax.dot_general(pick(q[p], mxu_rows(p)), key_blocks(k[p]), NT,
                             preferred_element_type=F32)
        sc = jnp.where(visible, sc * scale, MASKED)
        max_a = jnp.max(jnp.where(is_a, sc, -jnp.inf), axis=1, keepdims=True)
        max_b = jnp.max(jnp.where(is_a, -jnp.inf, sc), axis=1, keepdims=True)
        e = jnp.exp(sc - jnp.where(is_a, max_a, max_b))
        sum_a = jnp.sum(jnp.where(is_a, e, 0.0), axis=1, keepdims=True)
        sum_b = jnp.sum(jnp.where(is_a, 0.0, e), axis=1, keepdims=True)
        probs[p] = e * _recip(jnp.where(is_a, sum_a, sum_b))
        if p == NORM_AT[0]:
            probs[p] = after_all(xn_next, probs[p])
        if p == NORM_AT[1]:
            probs[p] = after_all(xb_prev, probs[p])
        if VPU_DUE[layer] and p - VPU_DUE[layer] in near_done:
            probs[p] = after_all(near_done[p - VPU_DUE[layer]], probs[p])

    def values(p):
        o = jnp.dot(probs[p], value_blocks(v[p]), preferred_element_type=F32)
        for i, r in enumerate(mxu_rows(p)):
            o_ref[r:r + 8, p * pw:(p + 1) * pw] = o[8 * i:8 * i + 8]

    chain = [None, None]

    def attend_on_vpu(p, r):
        def key_row(j, i):
            return jnp.broadcast_to(near_ref[p, j:j + 1, 128 * i:128 * (i + 1)], (8, 128))

        half, sub = first[0:8], _iota((8, 128), 0)
        t = q[p][r:r + 8] * (scale * LOG2E)
        q0, q2 = t[:, 0:128], t[:, 256:384]
        q1a, q1b = jnp.where(half, t[:, 128:256], 0.0), jnp.where(half, 0.0, t[:, 128:256])
        sc = []
        for j in range(r + 8):
            k1 = after(chain[0], key_row(j, 1))
            dot_a = q0 * after(chain[0], key_row(j, 0)) + q1a * k1
            chain[0] = q2 * after(dot_a, key_row(j, 2)) + q1b * k1
            t = jnp.where(half, jnp.sum(dot_a, axis=1, keepdims=True),
                          jnp.sum(chain[0], axis=1, keepdims=True))
            sc.append(t if j <= r else jnp.where(sub >= j - r, t, MASKED * LOG2E))
        top = functools.reduce(jnp.maximum, sc)
        seen = []
        for j in range(r + 8):
            e = jnp.exp2(sc[j] - after(seen[j - EXP_AHEAD] if j >= EXP_AHEAD else None, top))
            weight = after(chain[1], e)
            terms = [weight * key_row(j, 3 + i) for i in range(3)]
            total = e if j == 0 else total + e
            acc = terms if j == 0 else [a + b for a, b in zip(acc, terms)]
            chain[1] = acc[2]
            seen.append(acc[2])
        inv = _recip(total)
        o_ref[r:r + 8, p * pw:(p + 1) * pw] = jnp.concatenate([a * inv for a in acc], axis=1)
        near_done[p] = acc[2]

    def attend_early_rows(p):
        if vpu_rows(p):
            n = vpu_rows(p)[-1] + 8
            near_ref[p, 0:n, 0:pw] = k[p][0:n]
            near_ref[p, 0:n, pw:2 * pw] = v[p][0:n]
        for r in vpu_rows(p):
            attend_on_vpu(p, r)

    def project_out(p0, p1, acc):
        lo, hi = 3 * p0, 3 * p1

        def part(k0, k1, c0, c1):
            w = wo_ref[k0:k1, :, :, c0:c1].reshape((k1 - k0) * 128, c1 - c0)
            return jnp.dot(o_ref[:, k0 * 128:k1 * 128], w, preferred_element_type=F32)

        d = wo_ref.shape[-1]
        if p1 < n_pairs:
            r = part(lo, hi, 0, d)
        elif closes:
            return part(hi - 1, hi, 0, d) + (part(lo, hi - 1, 0, d) + acc)
        else:
            r = jnp.concatenate([part(lo, hi, 0, K_SPLIT), part(lo, hi, K_SPLIT, d)], axis=1)
        return r if acc is None else r + acc

    out = None
    lag_s, lag_v = LAG_S[layer], LAG_S[layer] + LAG_PV[layer]
    todo = list(zip(O_SPLITS[layer][:-1], O_SPLITS[layer][1:]))
    for t in range(n_pairs + lag_v):
        if t >= n_pairs:
            out = project_out(*todo.pop(0), out)
        elif pre_ref is None:
            r = times_w(h, t, 0, 3 * pw)
            q[t], k[t], v[t] = r[:, 0:pw], r[:, pw:2 * pw], r[:, 2 * pw:3 * pw]
        else:
            q[t] = times_w(h, t, 0, pw)
            k[t] = project_short(t, 1)
        if 0 <= t - lag_s < n_pairs:
            scores(t - lag_s)
        if 0 <= t - lag_v < n_pairs:
            values(t - lag_v)
        if t < n_pairs and pre_ref is not None:
            v[t] = project_short(t, 2)
        if t < n_pairs:
            attend_early_rows(t)
    for part in todo:
        out = project_out(*part, out)

    x_ref[s] = x_in[s].astype(F32) + out[n_mem:, :]
    return out[:n_mem, :], xn_next


def _pair_reduce(t, op):
    r = t[0:8]
    for i in range(8, t.shape[0], 8):
        r = op(r, t[i:i + 8])
    r = op(r, pltpu.roll(r, 4, 0))
    return op(r, pltpu.roll(r, 2, 0))


def _tile_rows(r, n):
    return jnp.concatenate([r] * (n // 8), axis=0)


def _feature_map(p):
    n = p.shape[0]
    e_pos = jnp.exp2(p - _tile_rows(_pair_reduce(p, jnp.maximum), n))
    e_neg = jnp.exp2(_tile_rows(_pair_reduce(p, jnp.minimum), n) - p)
    inv_pos = _recip(_pair_reduce(e_pos, jnp.add))
    inv_neg = _recip(_pair_reduce(e_neg, jnp.add))
    return jnp.concatenate(
        [e_pos * _tile_rows(inv_pos, n), e_neg * _tile_rows(inv_neg, n)], axis=0)


def _fold_span(b, blk):
    return b * blk // 128 * 128, -(-(b + 1) * blk // 128) * 128


def _expand_phi(wphi_ref, phi_ref):
    dh, _, heads = wphi_ref.shape
    d = dh * heads
    gr = 2 * dh
    c = _iota((dh, d), 1)
    c_feat = c - _div(c, dh) * dh
    spread = (_div(_iota((heads, d), 1), dh) == _iota((heads, d), 0)).astype(BF16)
    by_feat = jnp.zeros((dh, d), F32)
    for e in range(dh):
        t = jnp.dot(wphi_ref[e], spread, preferred_element_type=F32)
        by_feat = jnp.where(c_feat == e, t, by_feat)
    by_feat = by_feat.astype(BF16)
    blk = F_PAIRS * gr
    r = _iota((blk, dh), 0)
    sel = (((r - _div(r, gr) * gr) >> 1) == _iota((blk, dh), 1)).astype(BF16)
    for b in range(d // blk):
        lo, hi = _fold_span(b, blk)
        r = _iota((blk, hi - lo), 0)
        head = 2 * (_div(r, gr) + b * F_PAIRS) + (r & 1)
        phi = jnp.dot(sel, by_feat[:, lo:hi], preferred_element_type=F32)
        phi_ref[b, :, 0:hi - lo] = _pack(
            jnp.where(_div(_iota((1, hi - lo), 1) + lo, dh) == head, phi, 0.0))


def _b_weights(wqkv_ref, phi_ref, wob_ref, bq_ref, bkv_ref, bo_ref):
    d = wqkv_ref.shape[0]
    blk = 2 * phi_ref.shape[1]
    half = bkv_ref.shape[1]
    bo_ref[...] = _pack(wob_ref[...])
    wv = wqkv_ref[:, 2 * d:3 * d].T
    for b in range(d // half):
        bkv_ref[b, half // 2:half, :] = _pack(wv[b * half:(b + 1) * half])
    for b in range(d // blk):
        lo, hi = _fold_span(b, blk)
        phi = _unpack(phi_ref[b, :, 0:hi - lo])
        wq = lax.dot_general(phi, wqkv_ref[:, lo:hi], NT, preferred_element_type=F32)
        wk = lax.dot_general(phi, wqkv_ref[:, d + lo:d + hi], NT, preferred_element_type=F32)
        bq_ref[b * blk // 2:(b + 1) * blk // 2, :] = _pack(wq * LOG2E)
        at = b * blk % half // 2
        bkv_ref[b * blk // half, at:at + blk // 2, :] = _pack(wk * LOG2E)


def _chunk_rows(ref, it, r0, n):
    seg = ref.shape[1]
    return pl.ds(it * (TB // seg) + r0 // seg, n // seg)


def _b_keys(it, carry, *, x_ref, xb_ref, bkv_ref, kv_ref, z_ref):
    n_blk, half, _ = bkv_ref.shape
    gr = half // K_PAIRS
    xb = xb_ref[_chunk_rows(xb_ref, it, 0, TB)].reshape(TB, -1)
    last = x_ref.shape[0] - 1
    xb_ref[last] = _layernorm(x_ref[last]).astype(BF16)
    same_head = (_iota((gr, 2 * gr), 0) >= gr // 2) == ((_iota((gr, 2 * gr), 1) & 1) == 1)

    def accumulate(b, t):
        for i in range(K_PAIRS):
            g = b * K_PAIRS + i
            phi = _feature_map(t[i * gr:(i + 1) * gr])
            z_ref[g] = jnp.where(it > 0, z_ref[g], 0.0) + jnp.sum(phi, axis=1, keepdims=True)
            kv = lax.dot_general(t[half + i * gr:half + (i + 1) * gr], phi.astype(BF16), NT,
                                 preferred_element_type=F32)
            kv_ref[g] = jnp.where(it > 0, kv_ref[g], 0.0) + jnp.where(same_head, kv, 0.0)

    pending = None
    for b in range(n_blk):
        t = lax.dot_general(_unpack(bkv_ref[b]), xb, NT, preferred_element_type=F32)
        if pending is not None:
            accumulate(*pending)
        pending = (b, t)
    accumulate(*pending)
    return carry


def _b_queries(it, send, *, x_ref, xb_ref, y_ref, bq_ref, bo_ref, kv_ref, z_ref, ot_ref, on_ref):
    n_groups, gr, _ = kv_ref.shape
    blk = Q_PAIRS * gr
    sub = _iota((8, TB), 0)
    xb = xb_ref[_chunk_rows(xb_ref, it, 0, TB)].reshape(TB, -1)

    def attend(b, t):
        outs = []
        for i in range(Q_PAIRS):
            g = b * Q_PAIRS + i
            phi = _feature_map(t[i * gr:(i + 1) * gr])
            num = jnp.dot(kv_ref[g], phi.astype(BF16), preferred_element_type=F32)
            z = jnp.concatenate([z_ref[g]] * (TB // 128), axis=1)
            inv = _recip(_pair_reduce(phi * z, jnp.add) + 1e-6)
            other = pltpu.roll(inv, 1, 0)
            inv_a = jnp.where((sub & 1) == 0, inv, other)
            inv_b = jnp.where((sub & 1) == 0, other, inv)
            n = (gr - 8) // 16
            inv = jnp.concatenate(
                [inv_a] * n + [jnp.where(sub < 4, inv_a, inv_b)] + [inv_b] * n, axis=0)
            outs.append(num * inv)
        ot_ref[b * blk // 2:(b + 1) * blk // 2, :] = _pack(jnp.concatenate(outs, axis=0))

    n_blk = n_groups // Q_PAIRS
    proj = {}
    for b in range(n_blk + 1):
        if b < n_blk:
            proj[b] = lax.dot_general(_unpack(bq_ref[b * blk // 2:(b + 1) * blk // 2, :]), xb,
                                      NT, preferred_element_type=F32)
        if b > 0:
            attend(b - 1, proj[b - 1])
    on_ref[...] = _pack(_unpack(ot_ref[...]).T)
    r0 = 0
    for i, n in enumerate(O_ROWS):
        at = _chunk_rows(x_ref, it, r0, n)
        y = jnp.dot(_unpack(on_ref[r0 // 2:(r0 + n) // 2, :]), _unpack(bo_ref[...]),
                    preferred_element_type=F32)
        x = x_ref[at] + y.reshape((-1,) + x_ref.shape[1:])
        x_ref[at] = x
        y_ref[at] = x.astype(BF16)
        send(i)
        r0 += n


def _kernel(x_hbm, mem0_hbm, wq_hbm, wk_hbm, wv_hbm, wo_hbm, wqkvb_hbm, wphi_hbm, wob_hbm,
            out_hbm,
            x_ref, xb_ref, y_ref, xp_ref, stage_ref, pre_ref, w_ref, wo_ref, o_ref, near_ref,
            mem0_ref, wphi_ref, phi_ref, wqkvb_ref, wob_ref, bo_ref, bq_ref, bkv_ref,
            kv_ref, z_ref, ot_ref, on_ref,
            w_sem, in_sem, out_sem, *, dh):
    n_seg, seg, d = x_ref.shape
    n_pairs = w_ref.shape[0]
    pw = 2 * dh
    n_iter = n_seg * seg // TB

    def w_copies(p, j):
        if j < 2:
            return [pltpu.make_async_copy((wq_hbm, wk_hbm)[j].at[p],
                                          stage_ref.at[p, 3 * j:3 * j + 3], w_sem.at[p, j])]
        return [pltpu.make_async_copy(wv_hbm.at[p, i], stage_ref.at[p, 6:9, i], w_sem.at[p, 2 + i])
                for i in range(2)]

    def start_w(p, *slots):
        for j in slots:
            for copy in w_copies(p, j):
                copy.start()

    def wait_w(p, *slots):
        for j in slots:
            for copy in w_copies(p, j):
                copy.wait()

    def staged(p, tiles):
        return stage_ref[p, tiles].reshape(-1, d)

    def out_copy(it, i):
        part = _chunk_rows(y_ref, it, sum(O_ROWS[:i]), O_ROWS[i])
        return pltpu.make_async_copy(y_ref.at[part], out_hbm.at[part], out_sem.at[0])

    def x_copy(part, rows, sem):
        return pltpu.make_async_copy(x_hbm.at[part, rows, :], y_ref.at[part, rows, :], sem)

    head, tail = slice(0, seg - PRE), slice(seg - PRE, seg)
    xt_copy = x_copy(slice(None), tail, in_sem.at[0])
    wqkvb_copy = pltpu.make_async_copy(wqkvb_hbm, wqkvb_ref, in_sem.at[1])
    wphi_copy = pltpu.make_async_copy(wphi_hbm, wphi_ref, in_sem.at[5])
    mem0_copy = pltpu.make_async_copy(mem0_hbm, mem0_ref, in_sem.at[6])
    wob_copy = pltpu.make_async_copy(wob_hbm, wob_ref, in_sem.at[2])

    wphi_copy.start()
    xt_copy.start()
    start_w(0, 1, 2)
    wphi_copy.wait()
    _expand_phi(wphi_ref, phi_ref)
    xt_copy.wait()

    xp_ref[...] = _layernorm(y_ref[:, tail, :].astype(F32).reshape(n_seg * PRE, d)).astype(BF16)

    mem0_copy.start()
    start_w(0, 0)
    start_w(1, 1, 2, 0)

    def pre_project(p, carry):
        @pl.when(p + 2 < n_pairs)
        def _():
            start_w(jnp.minimum(p + 2, n_pairs - 1), 0, 1, 2)

        part = pl.ds(p * (n_seg // n_pairs), n_seg // n_pairs)
        x_copy(part, head, in_sem.at[3]).start()
        for i in range(2):
            pltpu.make_async_copy(
                wo_hbm.at[p, i], wo_ref.at[pl.ds(3 * p, 3), i], in_sem.at[4]).start()
        before = jnp.maximum(p - 1, 0)

        @pl.when(p > 0)
        def _():
            wait_w(before, 0)

        wait_w(p, 1, 2)
        pre_ref[p] = lax.dot_general(xp_ref[...], staged(p, slice(3, 9)), NT,
                                     preferred_element_type=F32)
        w_ref[before, :, 0:pw] = _pack(staged(before, pl.ds(jnp.where(p > 0, 0, 3), 3)).T)
        for j in (1, 2):
            w_ref[p, :, j * pw:(j + 1) * pw] = _pack(staged(p, slice(3 * j, 3 * j + 3)).T)
        return carry

    lax.fori_loop(0, n_pairs, pre_project, 0)

    wait_w(n_pairs - 1, 0)
    w_ref[n_pairs - 1, :, 0:pw] = _pack(staged(n_pairs - 1, slice(0, 3)).T)
    x_copy(slice(None), head, in_sem.at[3]).wait()
    pltpu.make_async_copy(wo_ref, wo_ref, in_sem.at[4]).wait()

    wqkvb_copy.start()
    wob_copy.start()
    mem0_copy.wait()
    x_ref[0] = y_ref[0].astype(F32)

    def layer_a(layer, x_in, pre):
        unroll = A_UNROLL[layer]
        step = functools.partial(_a_step, layer=layer, dh=dh, x_in=x_in, x_ref=x_ref, xb_ref=xb_ref,
                                 w_ref=w_ref, wo_ref=wo_ref, pre_ref=pre, o_ref=o_ref,
                                 near_ref=near_ref)

        def steps(it, carry):
            for i in range(unroll):
                carry = step(it * unroll + i, carry, i == 0, i == unroll - 1)
            return carry

        lax.fori_loop(0, n_seg // unroll, steps,
                      (mem0_ref[...].astype(F32), _layernorm(x_ref[0])))

    b_keys = functools.partial(_b_keys, x_ref=x_ref, xb_ref=xb_ref, bkv_ref=bkv_ref,
                               kv_ref=kv_ref, z_ref=z_ref)
    b_queries = functools.partial(_b_queries, x_ref=x_ref, xb_ref=xb_ref, y_ref=y_ref,
                                  bq_ref=bq_ref, bo_ref=bo_ref, kv_ref=kv_ref, z_ref=z_ref,
                                  ot_ref=ot_ref, on_ref=on_ref)

    def layer_pair(layer, carry):
        @pl.when(layer == 0)
        def _():
            layer_a(0, y_ref, pre_ref)

        @pl.when(layer == 0)
        def _():
            wqkvb_copy.wait()
            wob_copy.wait()
            _b_weights(wqkvb_ref, phi_ref, wob_ref, bq_ref, bkv_ref, bo_ref)

        @pl.when(layer == 1)
        def _():
            layer_a(1, x_ref, None)

        lax.fori_loop(0, n_iter, b_keys, 0)

        def queries(it, carry):
            def send(i):
                @pl.when(layer == 1)
                def _():
                    out_copy(it, i).start()

            b_queries(it, send)
            return carry

        lax.fori_loop(0, n_iter, queries, 0)

        return carry

    lax.fori_loop(0, 2, layer_pair, 0)
    pltpu.make_async_copy(y_ref, out_hbm, out_sem.at[0]).wait()


@functools.partial(jax.jit, static_argnames=("A_seg_len",))
def pallas_interleave_layers__memory_aug_recurrent_mem_tr__linear_kernel_hedgehog__prompt_kernel(
    A_x, A_mem0, A_Wq, A_Wk, A_Wv, A_Wo, A_seg_len, B_x, B_wqkv, B_w_phi, B_wo,
):
    del B_x
    batch, s_len, d = A_x.shape
    _, heads, dh = A_Wq.shape
    n_mem = A_mem0.shape[1]
    seg = int(A_seg_len)
    b_heads, b_dh, _ = B_w_phi.shape
    rows = n_mem + seg
    n_pairs = heads // 2
    gr = 2 * b_dh
    half = K_PAIRS * gr
    n_seg = s_len // seg
    assert batch == 1 and dh == 192 and heads == 2 * O_SPLITS[0][-1]
    assert n_mem % 8 == 0 and seg % 16 == 0 and 128 % seg == 0 and 2 * rows <= 128
    assert s_len % TB == 0 and s_len > TB == sum(O_ROWS) and n_seg % n_pairs == 0
    assert b_heads * b_dh == d and b_dh % 8 == 4 and d % half == 0

    def head_major(w):
        return w.transpose(1, 2, 0)

    hbm = pl.BlockSpec(memory_space=pltpu.HBM)
    out = pl.pallas_call(
        functools.partial(_kernel, dh=dh),
        out_shape=jax.ShapeDtypeStruct((n_seg, seg, d), A_x.dtype),
        in_specs=[hbm] * 9,
        out_specs=hbm,
        scratch_shapes=[
            pltpu.VMEM((n_seg, seg, d), F32),
            pltpu.VMEM((n_seg, seg, d), BF16),
            pltpu.VMEM((n_seg, seg, d), BF16),
            pltpu.VMEM((n_seg * PRE, d), BF16),
            pltpu.VMEM((n_pairs, 9, 2, 64, d), BF16),
            pltpu.VMEM((n_pairs, n_seg * PRE, 4 * dh), F32),
            pltpu.VMEM((n_pairs, d // 2, 6 * dh), jnp.uint32),
            pltpu.VMEM((3 * n_pairs, 2, 64, d), BF16),
            pltpu.VMEM((rows, heads * dh), F32),
            pltpu.VMEM((n_pairs, n_mem + 16, 4 * dh), F32),
            pltpu.VMEM((n_mem, d), BF16),
            pltpu.VMEM((b_dh, b_dh, b_heads), BF16),
            pltpu.VMEM((d // (F_PAIRS * gr), F_PAIRS * gr // 2, 256), jnp.uint32),
            pltpu.VMEM(B_wqkv.shape, BF16),
            pltpu.VMEM(B_wo.shape, BF16),
            pltpu.VMEM((d // 2, d), jnp.uint32),
            pltpu.VMEM((d // 2, d), jnp.uint32),
            pltpu.VMEM((d // half, half, d), jnp.uint32),
            pltpu.VMEM((b_heads // 2, gr, 2 * gr), F32),
            pltpu.VMEM((b_heads // 2, 2 * gr, 128), F32),
            pltpu.VMEM((d // 2, TB), jnp.uint32),
            pltpu.VMEM((TB // 2, d), jnp.uint32),
            pltpu.SemaphoreType.DMA((n_pairs, 4)),
            pltpu.SemaphoreType.DMA((7,)),
            pltpu.SemaphoreType.DMA((1,)),
        ],
        compiler_params=pltpu.CompilerParams(vmem_limit_bytes=120 * 1024 * 1024),
    )(
        A_x.reshape(n_seg, seg, d), A_mem0.reshape(n_mem, d),
        head_major(A_Wq).reshape(n_pairs, 3, 2, 64, d),
        head_major(A_Wk).reshape(n_pairs, 3, 2, 64, d),
        head_major(A_Wv).reshape(n_pairs, 2, 3, 64, d), A_Wo.reshape(n_pairs, 2, 3, 64, d),
        B_wqkv, B_w_phi.transpose(1, 2, 0), B_wo,
    )
    return out.reshape(batch, s_len, d)
```

```python
import functools
import math

import jax
import jax.numpy as jnp
from jax import lax
import jax.experimental.pallas as pl
import jax.experimental.pallas.tpu as pltpu

F32 = jnp.float32
BF16 = jnp.bfloat16
NT = (((1,), (1,)), ((), ()))
LOG2E = math.log2(math.e)
MASKED = -1e9

LAG_S = (2, 2)
LAG_PV = (2, 2)
O_SPLITS = ((0, 1, 2, 4, 6, 13, 16), (0, 2, 4, 6, 8, 12, 16))
VPU_ROWS = ((range(16), (2, 5, 8)), (range(16), (0, 1, 2, 4, 5, 6, 8, 9)))
VPU_DUE = (2, 2)
EXP_AHEAD = (1, 1)
A_UNROLL = (2, 2)
K_SPLIT = 512
NORM_AT = ((1, 2), (1, 3))
PRE = 8
WO_LAG = 3
ORD = (0, 0)
LNC = (2, 2)
VPU_LAG = (0, 1)
KEY_AHEAD = (10, 12)
XW = (3, 1)
GM = (2, 2)
TB = 512
K_PAIRS = 8
Q_PAIRS = 8
F_PAIRS = 2
O_ROWS = (128, 128, 128, 128)


def _iota(shape, axis):
    return lax.broadcasted_iota(jnp.int32, shape, axis)


def _div(v, d):
    return (v * ((1 << 18) // d + 1)) >> 18


def _pack(x):
    return pltpu.bitcast(x.astype(BF16), jnp.uint32)


def _unpack(x):
    return pltpu.bitcast(x, BF16)


def _recip(x):
    r = pl.reciprocal(x, approx=True)
    return r * (2.0 - x * r)


def _layernorm(x):
    m = jnp.mean(x, axis=-1, keepdims=True)
    c = x - m
    v = jnp.mean(c * c, axis=-1, keepdims=True)
    return c * lax.rsqrt(v + 1e-5)


def _a_step(s, carry, opens, closes, *, layer, dh, x_in, x_ref, xb_ref, w_ref, wo_ref, pre_ref,
            o_ref, near_ref):
    mem, xn = carry
    n_mem, seg = mem.shape[0], xn.shape[0]
    rows = n_mem + seg
    pw = 2 * dh
    n_pairs = w_ref.shape[0]
    scale = dh ** -0.5

    nxt = jnp.minimum(s + 1, x_ref.shape[0] - 1)
    prv = jnp.maximum(s - 1, 0)
    def slow_norm(x, last=None):
        if not LNC[layer]:
            return _layernorm(x)
        outs = []
        for i in range(0, seg, 8):
            t = x[i:i + 8]
            if len(outs) >= LNC[layer]:
                t = jnp.where(s < 0, outs[-LNC[layer]], t)
            outs.append(_layernorm(t))
        return jnp.concatenate(outs, axis=0)

    xn_next = slow_norm(x_in[nxt].astype(F32))
    xb_prev = slow_norm(x_ref[prv])
    xb_ref[prv] = xb_prev.astype(BF16)

    def after(early, value):
        return value if early is None else jnp.where(s < 0, early[:, :value.shape[1]], value)

    def after_all(early, value):
        t = functools.reduce(jnp.maximum, [early[i:i + 8, j:j + 128]
                                           for i in range(0, early.shape[0], 8)
                                           for j in range(0, early.shape[1], 128)])
        return jnp.concatenate([after(t, value[0:8]), value[8:]], axis=0)

    h = jnp.concatenate([mem, xn], axis=0)
    h_short = h[:rows - PRE].astype(BF16)

    first = _iota((rows, 128), 1) < 64
    zero = jnp.zeros((rows, 128), F32)

    def key_blocks(t):
        t0, t1, t2 = t[:, 0:128], t[:, 128:256], t[:, 256:384]
        top = jnp.concatenate([t0, jnp.where(first, t1, 0.0), zero], axis=1)
        bot = jnp.concatenate([zero, jnp.where(first, 0.0, t1), t2], axis=1)
        return jnp.concatenate([top, bot], axis=0).astype(BF16)

    def value_blocks(t):
        mine = jnp.concatenate([first] * 3, axis=1)
        return jnp.concatenate(
            [jnp.where(mine, t, 0.0), jnp.where(mine, 0.0, t)], axis=0).astype(BF16)

    def vpu_rows(p):
        return [n_mem + 8 * i for i, pairs in enumerate(VPU_ROWS[layer]) if p in pairs]

    def mxu_rows(p):
        return [r for r in range(0, rows, 8) if r not in vpu_rows(p)]

    def pick(t, starts):
        return jnp.concatenate([t[r:r + 8] for r in starts], axis=0)

    q, k, v, probs, near_done = {}, {}, {}, {}, {}

    def times_w(lhs, p, lo, hi):
        def part(k0, k1):
            w = _unpack(w_ref[p, k0 // 2:k1 // 2, lo:hi])
            return jnp.dot(lhs[:, k0:k1], w, preferred_element_type=F32)

        if p == 0 and lo == 0 and not opens:
            return part(K_SPLIT, lhs.shape[1]) + part(0, K_SPLIT)
        return part(0, lhs.shape[1])

    def project_short(p, j):
        done = pre_ref[p, pl.ds(pl.multiple_of(s * PRE, PRE), PRE), (j - 1) * pw:j * pw]
        return jnp.concatenate([times_w(h_short, p, j * pw, (j + 1) * pw), done], axis=0)

    def scores(p):
        col = pick(_iota((rows, 2 * rows), 1), mxu_rows(p))
        row = pick(_iota((rows, 2 * rows), 0), mxu_rows(p))
        is_a = col < rows
        visible = (row < n_mem) | (row >= jnp.where(is_a, col, col - rows))
        sc = lax.dot_general(pick(q[p], mxu_rows(p)), key_blocks(k[p]), NT,
                             preferred_element_type=F32)
        sc = jnp.where(visible, sc * scale, MASKED)
        max_a = jnp.max(jnp.where(is_a, sc, -jnp.inf), axis=1, keepdims=True)
        max_b = jnp.max(jnp.where(is_a, -jnp.inf, sc), axis=1, keepdims=True)
        e = jnp.exp(sc - jnp.where(is_a, max_a, max_b))
        sum_a = jnp.sum(jnp.where(is_a, e, 0.0), axis=1, keepdims=True)
        sum_b = jnp.sum(jnp.where(is_a, 0.0, e), axis=1, keepdims=True)
        probs[p] = e * _recip(jnp.where(is_a, sum_a, sum_b))
        if p == NORM_AT[layer][0]:
            probs[p] = after_all(xn_next, probs[p])
        if p == NORM_AT[layer][1]:
            probs[p] = after_all(xb_prev, probs[p])
        if VPU_DUE[layer] and p - VPU_DUE[layer] in near_done:
            probs[p] = after_all(near_done[p - VPU_DUE[layer]], probs[p])

    def values(p):
        o = jnp.dot(probs[p], value_blocks(v[p]), preferred_element_type=F32)
        for i, r in enumerate(mxu_rows(p)):
            o_ref[r:r + 8, p * pw:(p + 1) * pw] = o[8 * i:8 * i + 8]

    chain = [None, None]
    scored, summed = [], []

    def attend_on_vpu(p, r):
        def key_row(j, i):
            return jnp.broadcast_to(near_ref[p, j:j + 1, 128 * i:128 * (i + 1)], (8, 128))

        half, sub = first[0:8], _iota((8, 128), 0)
        t = q[p][r:r + 8] * (scale * LOG2E)
        q0, q2 = t[:, 0:128], t[:, 256:384]
        q1a, q1b = jnp.where(half, t[:, 128:256], 0.0), jnp.where(half, 0.0, t[:, 128:256])
        sc = []
        if not XW[layer] & 1:
            scored.clear()
        if not XW[layer] & 2:
            summed.clear()
        for j in range(r + 8):
            if KEY_AHEAD[layer] and len(scored) >= KEY_AHEAD[layer]:
                chain[0] = after(scored[-KEY_AHEAD[layer]], chain[0])
            k1 = after(chain[0], key_row(j, 1))
            m0 = q0 * after(chain[0] if GM[layer] else None, key_row(j, 0))
            dot_a = m0 + q1a * k1
            chain[0] = q2 * after((None, chain[0], dot_a, m0)[GM[layer]], key_row(j, 2)) + q1b * k1
            t = jnp.where(half, jnp.sum(dot_a, axis=1, keepdims=True),
                          jnp.sum(chain[0], axis=1, keepdims=True))
            sc.append(t if j <= r else jnp.where(sub >= j - r, t, MASKED * LOG2E))
            scored.append(sc[-1])
        top = functools.reduce(jnp.maximum, sc)
        for j in range(r + 8):
            e = jnp.exp2(sc[j] - after(summed[-EXP_AHEAD[layer]] if len(summed) >= EXP_AHEAD[layer] else None, top))
            total = e if j == 0 else total + e
            weight = after(chain[1], e)
            terms = [weight * key_row(j, 3 + i) for i in range(3)]
            acc = terms if j == 0 else [a + b for a, b in zip(acc, terms)]
            chain[1] = acc[2]
            summed.append(acc[2])
        inv = _recip(total)
        o_ref[r:r + 8, p * pw:(p + 1) * pw] = jnp.concatenate([a * inv for a in acc], axis=1)
        near_done[p] = acc[2]

    def attend_early_rows(p):
        if vpu_rows(p):
            n = vpu_rows(p)[-1] + 8
            near_ref[p, 0:n, 0:pw] = k[p][0:n]
            near_ref[p, 0:n, pw:2 * pw] = v[p][0:n]
        for r in vpu_rows(p):
            attend_on_vpu(p, r)

    def project_out(p0, p1, acc):
        lo, hi = 3 * p0, 3 * p1

        def part(k0, k1, c0, c1):
            w = _unpack(wo_ref[k0:k1, :, c0:c1].reshape((k1 - k0) * 64, c1 - c0))
            return jnp.dot(o_ref[:, k0 * 128:k1 * 128], w, preferred_element_type=F32)

        d = wo_ref.shape[-1]
        if p1 < n_pairs:
            r = part(lo, hi, 0, d)
        elif closes:
            return part(hi - 1, hi, 0, d) + (part(lo, hi - 1, 0, d) + acc)
        else:
            r = jnp.concatenate([part(lo, hi, 0, K_SPLIT), part(lo, hi, K_SPLIT, d)], axis=1)
        return r if acc is None else r + acc

    out = None
    lag_s, lag_v = LAG_S[layer], LAG_S[layer] + LAG_PV[layer]
    todo = list(zip(O_SPLITS[layer][:-1], O_SPLITS[layer][1:]))
    for t in range(n_pairs + lag_v):
        if t >= n_pairs:
            out = project_out(*todo.pop(0), out)
        elif pre_ref is None:
            r = times_w(h, t, 0, 3 * pw)
            q[t], k[t], v[t] = r[:, 0:pw], r[:, pw:2 * pw], r[:, 2 * pw:3 * pw]
        else:
            q[t] = times_w(h, t, 0, pw)
            if ORD[layer] == 2 and 0 <= t - lag_s < n_pairs:
                scores(t - lag_s)
            k[t] = project_short(t, 1)
        if (ORD[layer] == 0 or (ORD[layer] == 2 and (t >= n_pairs or pre_ref is None))) and 0 <= t - lag_s < n_pairs:
            scores(t - lag_s)
        if 0 <= t - lag_v < n_pairs:
            values(t - lag_v)
        if t < n_pairs and pre_ref is not None:
            v[t] = project_short(t, 2)
        if ORD[layer] == 1 and 0 <= t - lag_s < n_pairs:
            scores(t - lag_s)
        if 0 <= t - VPU_LAG[layer] < n_pairs:
            attend_early_rows(t - VPU_LAG[layer])
    for part in todo:
        out = project_out(*part, out)

    x_ref[s] = x_in[s].astype(F32) + out[n_mem:, :]
    return out[:n_mem, :], xn_next


def _pair_reduce(t, op):
    r = t[0:8]
    for i in range(8, t.shape[0], 8):
        r = op(r, t[i:i + 8])
    r = op(r, pltpu.roll(r, 4, 0))
    return op(r, pltpu.roll(r, 2, 0))


def _tile_rows(r, n):
    return jnp.concatenate([r] * (n // 8), axis=0)


def _feature_map(p):
    n = p.shape[0]
    e_pos = jnp.exp2(p - _tile_rows(_pair_reduce(p, jnp.maximum), n))
    e_neg = jnp.exp2(_tile_rows(_pair_reduce(p, jnp.minimum), n) - p)
    inv_pos = _recip(_pair_reduce(e_pos, jnp.add))
    inv_neg = _recip(_pair_reduce(e_neg, jnp.add))
    return jnp.concatenate(
        [e_pos * _tile_rows(inv_pos, n), e_neg * _tile_rows(inv_neg, n)], axis=0)


def _fold_span(b, blk):
    return b * blk // 128 * 128, -(-(b + 1) * blk // 128) * 128


def _expand_phi(wphi_ref, phi_ref):
    dh, _, heads = wphi_ref.shape
    d = dh * heads
    gr = 2 * dh
    c = _iota((dh, d), 1)
    c_feat = c - _div(c, dh) * dh
    spread = (_div(_iota((heads, d), 1), dh) == _iota((heads, d), 0)).astype(BF16)
    by_feat = jnp.zeros((dh, d), F32)
    for e in range(dh):
        t = jnp.dot(wphi_ref[e], spread, preferred_element_type=F32)
        by_feat = jnp.where(c_feat == e, t, by_feat)
    by_feat = by_feat.astype(BF16)
    blk = F_PAIRS * gr
    r = _iota((blk, dh), 0)
    sel = (((r - _div(r, gr) * gr) >> 1) == _iota((blk, dh), 1)).astype(BF16)
    for b in range(d // blk):
        lo, hi = _fold_span(b, blk)
        r = _iota((blk, hi - lo), 0)
        head = 2 * (_div(r, gr) + b * F_PAIRS) + (r & 1)
        phi = jnp.dot(sel, by_feat[:, lo:hi], preferred_element_type=F32)
        phi_ref[b, :, 0:hi - lo] = _pack(
            jnp.where(_div(_iota((1, hi - lo), 1) + lo, dh) == head, phi, 0.0))


def _b_weights(wqkv_ref, phi_ref, wob_ref, bq_ref, bkv_ref, bo_ref):
    d = wqkv_ref.shape[0]
    blk = 2 * phi_ref.shape[1]
    half = bkv_ref.shape[1]
    bo_ref[...] = _pack(wob_ref[...])
    wv = wqkv_ref[:, 2 * d:3 * d].T
    for b in range(d // half):
        bkv_ref[b, half // 2:half, :] = _pack(wv[b * half:(b + 1) * half])
    for b in range(d // blk):
        lo, hi = _fold_span(b, blk)
        phi = _unpack(phi_ref[b, :, 0:hi - lo])
        wq = lax.dot_general(phi, wqkv_ref[:, lo:hi], NT, preferred_element_type=F32)
        wk = lax.dot_general(phi, wqkv_ref[:, d + lo:d + hi], NT, preferred_element_type=F32)
        bq_ref[b * blk // 2:(b + 1) * blk // 2, :] = _pack(wq * LOG2E)
        at = b * blk % half // 2
        bkv_ref[b * blk // half, at:at + blk // 2, :] = _pack(wk * LOG2E)


def _chunk_rows(ref, it, r0, n):
    seg = ref.shape[1]
    return pl.ds(it * (TB // seg) + r0 // seg, n // seg)


def _b_keys(it, carry, *, x_ref, xb_ref, bkv_ref, kv_ref, z_ref):
    n_blk, half, _ = bkv_ref.shape
    gr = half // K_PAIRS
    xb = xb_ref[_chunk_rows(xb_ref, it, 0, TB)].reshape(TB, -1)
    last = x_ref.shape[0] - 1
    xb_ref[last] = _layernorm(x_ref[last]).astype(BF16)
    same_head = (_iota((gr, 2 * gr), 0) >= gr // 2) == ((_iota((gr, 2 * gr), 1) & 1) == 1)

    def accumulate(b, t):
        for i in range(K_PAIRS):
            g = b * K_PAIRS + i
            phi = _feature_map(t[i * gr:(i + 1) * gr])
            z_ref[g] = jnp.where(it > 0, z_ref[g], 0.0) + jnp.sum(phi, axis=1, keepdims=True)
            kv = lax.dot_general(t[half + i * gr:half + (i + 1) * gr], phi.astype(BF16), NT,
                                 preferred_element_type=F32)
            kv_ref[g] = jnp.where(it > 0, kv_ref[g], 0.0) + jnp.where(same_head, kv, 0.0)

    pending = None
    for b in range(n_blk):
        t = lax.dot_general(_unpack(bkv_ref[b]), xb, NT, preferred_element_type=F32)
        if pending is not None:
            accumulate(*pending)
        pending = (b, t)
    accumulate(*pending)
    return carry


def _b_queries(it, send, *, x_ref, xb_ref, y_ref, bq_ref, bo_ref, kv_ref, z_ref, ot_ref, on_ref):
    n_groups, gr, _ = kv_ref.shape
    blk = Q_PAIRS * gr
    sub = _iota((8, TB), 0)
    xb = xb_ref[_chunk_rows(xb_ref, it, 0, TB)].reshape(TB, -1)

    def attend(b, t):
        outs = []
        for i in range(Q_PAIRS):
            g = b * Q_PAIRS + i
            phi = _feature_map(t[i * gr:(i + 1) * gr])
            num = jnp.dot(kv_ref[g], phi.astype(BF16), preferred_element_type=F32)
            z = jnp.concatenate([z_ref[g]] * (TB // 128), axis=1)
            inv = _recip(_pair_reduce(phi * z, jnp.add) + 1e-6)
            other = pltpu.roll(inv, 1, 0)
            inv_a = jnp.where((sub & 1) == 0, inv, other)
            inv_b = jnp.where((sub & 1) == 0, other, inv)
            n = (gr - 8) // 16
            inv = jnp.concatenate(
                [inv_a] * n + [jnp.where(sub < 4, inv_a, inv_b)] + [inv_b] * n, axis=0)
            outs.append(num * inv)
        ot_ref[b * blk // 2:(b + 1) * blk // 2, :] = _pack(jnp.concatenate(outs, axis=0))

    n_blk = n_groups // Q_PAIRS
    proj = {}
    for b in range(n_blk + 1):
        if b < n_blk:
            proj[b] = lax.dot_general(_unpack(bq_ref[b * blk // 2:(b + 1) * blk // 2, :]), xb,
                                      NT, preferred_element_type=F32)
        if b > 0:
            attend(b - 1, proj[b - 1])
    on_ref[...] = _pack(_unpack(ot_ref[...]).T)
    r0 = 0
    for i, n in enumerate(O_ROWS):
        at = _chunk_rows(x_ref, it, r0, n)
        y = jnp.dot(_unpack(on_ref[r0 // 2:(r0 + n) // 2, :]), _unpack(bo_ref[...]),
                    preferred_element_type=F32)
        x = x_ref[at] + y.reshape((-1,) + x_ref.shape[1:])
        x_ref[at] = x
        y_ref[at] = x.astype(BF16)
        send(i)
        r0 += n


def _kernel(x_hbm, mem0_hbm, wq_hbm, wk_hbm, wv_hbm, wo_hbm, wqkvb_hbm, wphi_hbm, wob_hbm,
            out_hbm,
            x_ref, xb_ref, y_ref, xp_ref, stage_ref, pre_ref, w_ref, wo_ref, o_ref, near_ref,
            mem0_ref, wphi_ref, phi_ref, wqkvb_ref, wob_ref, bo_ref, bq_ref, bkv_ref,
            kv_ref, z_ref, ot_ref, on_ref,
            w_sem, in_sem, out_sem, *, dh):
    n_seg, seg, d = x_ref.shape
    n_pairs = w_ref.shape[0]
    pw = 2 * dh
    n_iter = n_seg * seg // TB

    def w_copies(p, j):
        src = (wq_hbm, wk_hbm, wv_hbm, wo_hbm)[j]
        if j < 2:
            return [pltpu.make_async_copy(src.at[p], stage_ref.at[p, 3 * j:3 * j + 3],
                                          w_sem.at[p, j])]
        return [pltpu.make_async_copy(src.at[p, i], stage_ref.at[p, 3 * j:3 * j + 3, i],
                                      w_sem.at[p, 2 * j - 2 + i]) for i in range(2)]

    def start_w(p, *slots):
        for j in slots:
            for copy in w_copies(p, j):
                copy.start()

    def wait_w(p, *slots):
        for j in slots:
            for copy in w_copies(p, j):
                copy.wait()

    def staged(p, tiles):
        return stage_ref[p, tiles].reshape(-1, d)

    def out_copy(it, i):
        part = _chunk_rows(y_ref, it, sum(O_ROWS[:i]), O_ROWS[i])
        return pltpu.make_async_copy(y_ref.at[part], out_hbm.at[part], out_sem.at[0])

    def x_copy(part, rows, sem):
        return pltpu.make_async_copy(x_hbm.at[part, rows, :], y_ref.at[part, rows, :], sem)

    head, tail = slice(0, seg - PRE), slice(seg - PRE, seg)
    xt_copy = x_copy(slice(None), tail, in_sem.at[0])
    wqkvb_copy = pltpu.make_async_copy(wqkvb_hbm, wqkvb_ref, in_sem.at[1])
    wphi_copy = pltpu.make_async_copy(wphi_hbm, wphi_ref, in_sem.at[5])
    mem0_copy = pltpu.make_async_copy(mem0_hbm, mem0_ref, in_sem.at[4])
    wob_copy = pltpu.make_async_copy(wob_hbm, wob_ref, in_sem.at[2])

    wphi_copy.start()
    xt_copy.start()
    start_w(0, 1, 2)
    wphi_copy.wait()
    _expand_phi(wphi_ref, phi_ref)
    xt_copy.wait()

    xp_ref[...] = _layernorm(y_ref[:, tail, :].astype(F32).reshape(n_seg * PRE, d)).astype(BF16)

    mem0_copy.start()
    start_w(1, 1, 2)
    start_w(0, 0)
    start_w(1, 0)

    def pre_project(p, carry):
        @pl.when(p + 2 < n_pairs)
        def _():
            start_w(jnp.minimum(p + 2, n_pairs - 1), 0, 1, 2)

        part = pl.ds(p * (n_seg // n_pairs), n_seg // n_pairs)
        x_copy(part, head, in_sem.at[3]).start()
        start_w(p, 3)
        p_q, p_o = jnp.maximum(p - 1, 0), jnp.maximum(p - WO_LAG, 0)

        @pl.when(p >= 1)
        def _():
            wait_w(p_q, 0)

        @pl.when(p >= WO_LAG)
        def _():
            wait_w(p_o, 3)

        wait_w(p, 1, 2)
        pre_ref[p] = lax.dot_general(xp_ref[...], staged(p, slice(3, 9)), NT,
                                     preferred_element_type=F32)
        w_ref[p_q, :, 0:pw] = _pack(staged(p_q, pl.ds(jnp.where(p >= 1, 0, 3), 3)).T)
        wo_ref[pl.ds(3 * p_o, 3)] = _pack(
            staged(p_o, pl.ds(jnp.where(p >= WO_LAG, 9, 3), 3))).reshape(3, 64, d)
        for j in (1, 2):
            w_ref[p, :, j * pw:(j + 1) * pw] = _pack(staged(p, slice(3 * j, 3 * j + 3)).T)
        return carry

    lax.fori_loop(0, n_pairs, pre_project, 0)

    wait_w(n_pairs - 1, 0)
    w_ref[n_pairs - 1, :, 0:pw] = _pack(staged(n_pairs - 1, slice(0, 3)).T)
    for p in range(n_pairs - WO_LAG, n_pairs):
        wait_w(p, 3)
        wo_ref[3 * p:3 * p + 3] = _pack(staged(p, slice(9, 12))).reshape(3, 64, d)
    x_copy(slice(None), head, in_sem.at[3]).wait()

    wqkvb_copy.start()
    wob_copy.start()
    mem0_copy.wait()
    x_ref[0] = y_ref[0].astype(F32)

    def layer_a(layer, x_in, pre):
        unroll = A_UNROLL[layer]
        step = functools.partial(_a_step, layer=layer, dh=dh, x_in=x_in, x_ref=x_ref, xb_ref=xb_ref,
                                 w_ref=w_ref, wo_ref=wo_ref, pre_ref=pre, o_ref=o_ref,
                                 near_ref=near_ref)

        def steps(it, carry):
            for i in range(unroll):
                carry = step(it * unroll + i, carry, i == 0, i == unroll - 1)
            return carry

        lax.fori_loop(0, n_seg // unroll, steps,
                      (mem0_ref[...].astype(F32), _layernorm(x_ref[0])))

    b_keys = functools.partial(_b_keys, x_ref=x_ref, xb_ref=xb_ref, bkv_ref=bkv_ref,
                               kv_ref=kv_ref, z_ref=z_ref)
    b_queries = functools.partial(_b_queries, x_ref=x_ref, xb_ref=xb_ref, y_ref=y_ref,
                                  bq_ref=bq_ref, bo_ref=bo_ref, kv_ref=kv_ref, z_ref=z_ref,
                                  ot_ref=ot_ref, on_ref=on_ref)

    def layer_pair(layer, carry):
        @pl.when(layer == 0)
        def _():
            layer_a(0, y_ref, pre_ref)

        @pl.when(layer == 0)
        def _():
            wqkvb_copy.wait()
            wob_copy.wait()
            _b_weights(wqkvb_ref, phi_ref, wob_ref, bq_ref, bkv_ref, bo_ref)

        @pl.when(layer == 1)
        def _():
            layer_a(1, x_ref, None)

        lax.fori_loop(0, n_iter, b_keys, 0)

        def queries(it, carry):
            def send(i):
                @pl.when(layer == 1)
                def _():
                    out_copy(it, i).start()

            b_queries(it, send)
            return carry

        lax.fori_loop(0, n_iter, queries, 0)

        return carry

    lax.fori_loop(0, 2, layer_pair, 0)
    pltpu.make_async_copy(y_ref, out_hbm, out_sem.at[0]).wait()


@functools.partial(jax.jit, static_argnames=("A_seg_len",))
def pallas_interleave_layers__memory_aug_recurrent_mem_tr__linear_kernel_hedgehog__prompt_kernel(
    A_x, A_mem0, A_Wq, A_Wk, A_Wv, A_Wo, A_seg_len, B_x, B_wqkv, B_w_phi, B_wo,
):
    del B_x
    batch, s_len, d = A_x.shape
    _, heads, dh = A_Wq.shape
    n_mem = A_mem0.shape[1]
    seg = int(A_seg_len)
    b_heads, b_dh, _ = B_w_phi.shape
    rows = n_mem + seg
    n_pairs = heads // 2
    gr = 2 * b_dh
    half = K_PAIRS * gr
    n_seg = s_len // seg
    assert batch == 1 and dh == 192 and heads == 2 * O_SPLITS[0][-1]
    assert n_mem % 8 == 0 and seg % 16 == 0 and 128 % seg == 0 and 2 * rows <= 128
    assert s_len % TB == 0 and s_len > TB == sum(O_ROWS) and n_seg % n_pairs == 0
    assert b_heads * b_dh == d and b_dh % 8 == 4 and d % half == 0

    def head_major(w):
        return w.transpose(1, 2, 0)

    hbm = pl.BlockSpec(memory_space=pltpu.HBM)
    out = pl.pallas_call(
        functools.partial(_kernel, dh=dh),
        out_shape=jax.ShapeDtypeStruct((n_seg, seg, d), A_x.dtype),
        in_specs=[hbm] * 9,
        out_specs=hbm,
        scratch_shapes=[
            pltpu.VMEM((n_seg, seg, d), F32),
            pltpu.VMEM((n_seg, seg, d), BF16),
            pltpu.VMEM((n_seg, seg, d), BF16),
            pltpu.VMEM((n_seg * PRE, d), BF16),
            pltpu.VMEM((n_pairs, 12, 2, 64, d), BF16),
            pltpu.VMEM((n_pairs, n_seg * PRE, 4 * dh), F32),
            pltpu.VMEM((n_pairs, d // 2, 6 * dh), jnp.uint32),
            pltpu.VMEM((3 * n_pairs, 64, d), jnp.uint32),
            pltpu.VMEM((rows, heads * dh), F32),
            pltpu.VMEM((n_pairs, n_mem + 16, 4 * dh), F32),
            pltpu.VMEM((n_mem, d), BF16),
            pltpu.VMEM((b_dh, b_dh, b_heads), BF16),
            pltpu.VMEM((d // (F_PAIRS * gr), F_PAIRS * gr // 2, 256), jnp.uint32),
            pltpu.VMEM(B_wqkv.shape, BF16),
            pltpu.VMEM(B_wo.shape, BF16),
            pltpu.VMEM((d // 2, d), jnp.uint32),
            pltpu.VMEM((d // 2, d), jnp.uint32),
            pltpu.VMEM((d // half, half, d), jnp.uint32),
            pltpu.VMEM((b_heads // 2, gr, 2 * gr), F32),
            pltpu.VMEM((b_heads // 2, 2 * gr, 128), F32),
            pltpu.VMEM((d // 2, TB), jnp.uint32),
            pltpu.VMEM((TB // 2, d), jnp.uint32),
            pltpu.SemaphoreType.DMA((n_pairs, 6)),
            pltpu.SemaphoreType.DMA((6,)),
            pltpu.SemaphoreType.DMA((1,)),
        ],
        compiler_params=pltpu.CompilerParams(vmem_limit_bytes=120 * 1024 * 1024),
    )(
        A_x.reshape(n_seg, seg, d), A_mem0.reshape(n_mem, d),
        head_major(A_Wq).reshape(n_pairs, 3, 2, 64, d),
        head_major(A_Wk).reshape(n_pairs, 3, 2, 64, d),
        head_major(A_Wv).reshape(n_pairs, 2, 3, 64, d), A_Wo.reshape(n_pairs, 2, 3, 64, d),
        B_wqkv, B_w_phi.transpose(1, 2, 0), B_wo,
    )
    return out.reshape(batch, s_len, d)
```

```python
import functools
import math

import jax
import jax.numpy as jnp
from jax import lax
import jax.experimental.pallas as pl
import jax.experimental.pallas.tpu as pltpu

F32 = jnp.float32
BF16 = jnp.bfloat16
NT = (((1,), (1,)), ((), ()))
LOG2E = math.log2(math.e)
MASKED = -1e9

LAG_S = (2, 1)
LAG_PV = (2, 3)
O_SPLITS = ((0, 2, 4, 6, 8, 13, 16), (0, 2, 4, 6, 8, 11, 14, 16))
O_EARLY = ((), ())
VPU_ROWS = ((range(16), (2, 7)), (range(16), range(10)))
VPU_DUE = (2, 2)
EXP_AHEAD = (1, 1)
A_UNROLL = (2, 2)
K_SPLIT = 512
NORM_AT = ((1, 2), (1, 3))
PRE = 8
WO_LAG = 3
ORD = (0, 0)
LNC = (2, 2)
VPU_LAG = (0, 1)
KEY_AHEAD = (10, 11)
XW = (3, 3)
GM = (2, 3)
TB = 512
K_PAIRS = 8
Q_PAIRS = 8
F_PAIRS = 2
O_ROWS = (128, 128, 128, 128)


def _iota(shape, axis):
    return lax.broadcasted_iota(jnp.int32, shape, axis)


def _div(v, d):
    return (v * ((1 << 18) // d + 1)) >> 18


def _pack(x):
    return pltpu.bitcast(x.astype(BF16), jnp.uint32)


def _unpack(x):
    return pltpu.bitcast(x, BF16)


def _recip(x):
    r = pl.reciprocal(x, approx=True)
    return r * (2.0 - x * r)


def _layernorm(x):
    m = jnp.mean(x, axis=-1, keepdims=True)
    c = x - m
    v = jnp.mean(c * c, axis=-1, keepdims=True)
    return c * lax.rsqrt(v + 1e-5)


def _a_step(s, carry, opens, closes, *, layer, dh, x_in, x_ref, xb_ref, w_ref, wo_ref, pre_ref,
            o_ref, near_ref):
    mem, xn = carry
    n_mem, seg = mem.shape[0], xn.shape[0]
    rows = n_mem + seg
    pw = 2 * dh
    n_pairs = w_ref.shape[0]
    scale = dh ** -0.5

    nxt = jnp.minimum(s + 1, x_ref.shape[0] - 1)
    prv = jnp.maximum(s - 1, 0)
    def slow_norm(x, last=None):
        if not LNC[layer]:
            return _layernorm(x)
        outs = []
        for i in range(0, seg, 8):
            t = x[i:i + 8]
            if len(outs) >= LNC[layer]:
                t = jnp.where(s < 0, outs[-LNC[layer]], t)
            outs.append(_layernorm(t))
        return jnp.concatenate(outs, axis=0)

    xn_next = slow_norm(x_in[nxt].astype(F32))
    xb_prev = slow_norm(x_ref[prv])
    xb_ref[prv] = xb_prev.astype(BF16)

    def after(early, value):
        return value if early is None else jnp.where(s < 0, early[:, :value.shape[1]], value)

    def after_all(early, value):
        t = functools.reduce(jnp.maximum, [early[i:i + 8, j:j + 128]
                                           for i in range(0, early.shape[0], 8)
                                           for j in range(0, early.shape[1], 128)])
        return jnp.concatenate([after(t, value[0:8]), value[8:]], axis=0)

    h = jnp.concatenate([mem, xn], axis=0)
    h_short = h[:rows - PRE].astype(BF16)

    first = _iota((rows, 128), 1) < 64
    zero = jnp.zeros((rows, 128), F32)

    def key_blocks(t):
        t0, t1, t2 = t[:, 0:128], t[:, 128:256], t[:, 256:384]
        top = jnp.concatenate([t0, jnp.where(first, t1, 0.0), zero], axis=1)
        bot = jnp.concatenate([zero, jnp.where(first, 0.0, t1), t2], axis=1)
        return jnp.concatenate([top, bot], axis=0).astype(BF16)

    def value_blocks(t):
        mine = jnp.concatenate([first] * 3, axis=1)
        return jnp.concatenate(
            [jnp.where(mine, t, 0.0), jnp.where(mine, 0.0, t)], axis=0).astype(BF16)

    def vpu_rows(p):
        return [n_mem + 8 * i for i, pairs in enumerate(VPU_ROWS[layer]) if p in pairs]

    def mxu_rows(p):
        return [r for r in range(0, rows, 8) if r not in vpu_rows(p)]

    def pick(t, starts):
        return jnp.concatenate([t[r:r + 8] for r in starts], axis=0)

    q, k, v, probs, near_done = {}, {}, {}, {}, {}

    def times_w(lhs, p, lo, hi):
        def part(k0, k1):
            w = _unpack(w_ref[p, k0 // 2:k1 // 2, lo:hi])
            return jnp.dot(lhs[:, k0:k1], w, preferred_element_type=F32)

        if p == 0 and lo == 0 and not opens:
            return part(K_SPLIT, lhs.shape[1]) + part(0, K_SPLIT)
        return part(0, lhs.shape[1])

    def project_short(p, j):
        done = pre_ref[p, pl.ds(pl.multiple_of(s * PRE, PRE), PRE), (j - 1) * pw:j * pw]
        return jnp.concatenate([times_w(h_short, p, j * pw, (j + 1) * pw), done], axis=0)

    def scores(p):
        col = pick(_iota((rows, 2 * rows), 1), mxu_rows(p))
        row = pick(_iota((rows, 2 * rows), 0), mxu_rows(p))
        is_a = col < rows
        visible = (row < n_mem) | (row >= jnp.where(is_a, col, col - rows))
        sc = lax.dot_general(pick(q[p], mxu_rows(p)), key_blocks(k[p]), NT,
                             preferred_element_type=F32)
        sc = jnp.where(visible, sc * scale, MASKED)
        max_a = jnp.max(jnp.where(is_a, sc, -jnp.inf), axis=1, keepdims=True)
        max_b = jnp.max(jnp.where(is_a, -jnp.inf, sc), axis=1, keepdims=True)
        e = jnp.exp(sc - jnp.where(is_a, max_a, max_b))
        sum_a = jnp.sum(jnp.where(is_a, e, 0.0), axis=1, keepdims=True)
        sum_b = jnp.sum(jnp.where(is_a, 0.0, e), axis=1, keepdims=True)
        probs[p] = e * _recip(jnp.where(is_a, sum_a, sum_b))
        if p == NORM_AT[layer][0]:
            probs[p] = after_all(xn_next, probs[p])
        if p == NORM_AT[layer][1]:
            probs[p] = after_all(xb_prev, probs[p])
        if VPU_DUE[layer] and p - VPU_DUE[layer] in near_done:
            probs[p] = after_all(near_done[p - VPU_DUE[layer]], probs[p])

    def values(p):
        o = jnp.dot(probs[p], value_blocks(v[p]), preferred_element_type=F32)
        for i, r in enumerate(mxu_rows(p)):
            o_ref[r:r + 8, p * pw:(p + 1) * pw] = o[8 * i:8 * i + 8]

    chain = [None, None]
    scored, summed = [], []

    def attend_on_vpu(p, r):
        def key_row(j, i):
            return jnp.broadcast_to(near_ref[p, j:j + 1, 128 * i:128 * (i + 1)], (8, 128))

        half, sub = first[0:8], _iota((8, 128), 0)
        t = q[p][r:r + 8] * (scale * LOG2E)
        q0, q2 = t[:, 0:128], t[:, 256:384]
        q1a, q1b = jnp.where(half, t[:, 128:256], 0.0), jnp.where(half, 0.0, t[:, 128:256])
        sc = []
        if not XW[layer] & 1:
            scored.clear()
        if not XW[layer] & 2:
            summed.clear()
        for j in range(r + 8):
            if KEY_AHEAD[layer] and len(scored) >= KEY_AHEAD[layer]:
                chain[0] = after(scored[-KEY_AHEAD[layer]], chain[0])
            k1 = after(chain[0], key_row(j, 1))
            m0 = q0 * after(chain[0] if GM[layer] else None, key_row(j, 0))
            dot_a = m0 + q1a * k1
            chain[0] = q2 * after((None, chain[0], dot_a, m0)[GM[layer]], key_row(j, 2)) + q1b * k1
            t = jnp.where(half, jnp.sum(dot_a, axis=1, keepdims=True),
                          jnp.sum(chain[0], axis=1, keepdims=True))
            sc.append(t if j <= r else jnp.where(sub >= j - r, t, MASKED * LOG2E))
            scored.append(sc[-1])
        top = functools.reduce(jnp.maximum, sc)
        for j in range(r + 8):
            e = jnp.exp2(sc[j] - after(summed[-EXP_AHEAD[layer]] if len(summed) >= EXP_AHEAD[layer] else None, top))
            total = e if j == 0 else total + e
            weight = after(chain[1], e)
            terms = [weight * key_row(j, 3 + i) for i in range(3)]
            acc = terms if j == 0 else [a + b for a, b in zip(acc, terms)]
            chain[1] = acc[2]
            summed.append(acc[2])
        inv = _recip(total)
        o_ref[r:r + 8, p * pw:(p + 1) * pw] = jnp.concatenate([a * inv for a in acc], axis=1)
        near_done[p] = acc[2]

    def attend_early_rows(p):
        if vpu_rows(p):
            n = vpu_rows(p)[-1] + 8
            near_ref[p, 0:n, 0:pw] = k[p][0:n]
            near_ref[p, 0:n, pw:2 * pw] = v[p][0:n]
        for r in vpu_rows(p):
            attend_on_vpu(p, r)

    def project_out(p0, p1, acc):
        lo, hi = 3 * p0, 3 * p1

        def part(k0, k1, c0, c1):
            w = _unpack(wo_ref[k0:k1, :, c0:c1].reshape((k1 - k0) * 64, c1 - c0))
            return jnp.dot(o_ref[:, k0 * 128:k1 * 128], w, preferred_element_type=F32)

        d = wo_ref.shape[-1]
        if p1 < n_pairs:
            r = part(lo, hi, 0, d)
        elif closes:
            return part(hi - 1, hi, 0, d) + (part(lo, hi - 1, 0, d) + acc)
        else:
            r = jnp.concatenate([part(lo, hi, 0, K_SPLIT), part(lo, hi, K_SPLIT, d)], axis=1)
        return r if acc is None else r + acc

    out = None
    lag_s, lag_v = LAG_S[layer], LAG_S[layer] + LAG_PV[layer]
    todo = list(zip(O_SPLITS[layer][:-1], O_SPLITS[layer][1:]))
    for t in range(n_pairs + lag_v):
        if t >= n_pairs:
            out = project_out(*todo.pop(0), out)
        elif pre_ref is None:
            r = times_w(h, t, 0, 3 * pw)
            q[t], k[t], v[t] = r[:, 0:pw], r[:, pw:2 * pw], r[:, 2 * pw:3 * pw]
        else:
            q[t] = times_w(h, t, 0, pw)
            if ORD[layer] == 2 and 0 <= t - lag_s < n_pairs:
                scores(t - lag_s)
            k[t] = project_short(t, 1)
        if (ORD[layer] == 0 or (ORD[layer] == 2 and (t >= n_pairs or pre_ref is None))) and 0 <= t - lag_s < n_pairs:
            scores(t - lag_s)
        if 0 <= t - lag_v < n_pairs:
            values(t - lag_v)
        if t < n_pairs and pre_ref is not None:
            v[t] = project_short(t, 2)
        if ORD[layer] == 1 and 0 <= t - lag_s < n_pairs:
            scores(t - lag_s)
        if t in O_EARLY[layer]:
            out = project_out(*todo.pop(0), out)
        if 0 <= t - VPU_LAG[layer] < n_pairs:
            attend_early_rows(t - VPU_LAG[layer])
    for part in todo:
        out = project_out(*part, out)

    x_ref[s] = x_in[s].astype(F32) + out[n_mem:, :]
    return out[:n_mem, :], xn_next


def _pair_reduce(t, op):
    r = t[0:8]
    for i in range(8, t.shape[0], 8):
        r = op(r, t[i:i + 8])
    r = op(r, pltpu.roll(r, 4, 0))
    return op(r, pltpu.roll(r, 2, 0))


def _tile_rows(r, n):
    return jnp.concatenate([r] * (n // 8), axis=0)


def _feature_map(p):
    n = p.shape[0]
    e_pos = jnp.exp2(p - _tile_rows(_pair_reduce(p, jnp.maximum), n))
    e_neg = jnp.exp2(_tile_rows(_pair_reduce(p, jnp.minimum), n) - p)
    inv_pos = _recip(_pair_reduce(e_pos, jnp.add))
    inv_neg = _recip(_pair_reduce(e_neg, jnp.add))
    return jnp.concatenate(
        [e_pos * _tile_rows(inv_pos, n), e_neg * _tile_rows(inv_neg, n)], axis=0)


def _fold_span(b, blk):
    return b * blk // 128 * 128, -(-(b + 1) * blk // 128) * 128


def _expand_phi(wphi_ref, phi_ref):
    dh, _, heads = wphi_ref.shape
    d = dh * heads
    gr = 2 * dh
    c = _iota((dh, d), 1)
    c_feat = c - _div(c, dh) * dh
    spread = (_div(_iota((heads, d), 1), dh) == _iota((heads, d), 0)).astype(BF16)
    by_feat = jnp.zeros((dh, d), F32)
    for e in range(dh):
        t = jnp.dot(wphi_ref[e], spread, preferred_element_type=F32)
        by_feat = jnp.where(c_feat == e, t, by_feat)
    by_feat = by_feat.astype(BF16)
    blk = F_PAIRS * gr
    r = _iota((blk, dh), 0)
    sel = (((r - _div(r, gr) * gr) >> 1) == _iota((blk, dh), 1)).astype(BF16)
    for b in range(d // blk):
        lo, hi = _fold_span(b, blk)
        r = _iota((blk, hi - lo), 0)
        head = 2 * (_div(r, gr) + b * F_PAIRS) + (r & 1)
        phi = jnp.dot(sel, by_feat[:, lo:hi], preferred_element_type=F32)
        phi_ref[b, :, 0:hi - lo] = _pack(
            jnp.where(_div(_iota((1, hi - lo), 1) + lo, dh) == head, phi, 0.0))


def _b_weights(wqkv_ref, phi_ref, wob_ref, bq_ref, bkv_ref, bo_ref):
    d = wqkv_ref.shape[0]
    blk = 2 * phi_ref.shape[1]
    half = bkv_ref.shape[1]
    bo_ref[...] = _pack(wob_ref[...])
    wv = wqkv_ref[:, 2 * d:3 * d].T
    for b in range(d // half):
        bkv_ref[b, half // 2:half, :] = _pack(wv[b * half:(b + 1) * half])
    for b in range(d // blk):
        lo, hi = _fold_span(b, blk)
        phi = _unpack(phi_ref[b, :, 0:hi - lo])
        wq = lax.dot_general(phi, wqkv_ref[:, lo:hi], NT, preferred_element_type=F32)
        wk = lax.dot_general(phi, wqkv_ref[:, d + lo:d + hi], NT, preferred_element_type=F32)
        bq_ref[b * blk // 2:(b + 1) * blk // 2, :] = _pack(wq * LOG2E)
        at = b * blk % half // 2
        bkv_ref[b * blk // half, at:at + blk // 2, :] = _pack(wk * LOG2E)


def _chunk_rows(ref, it, r0, n):
    seg = ref.shape[1]
    return pl.ds(it * (TB // seg) + r0 // seg, n // seg)


def _b_keys(it, carry, *, x_ref, xb_ref, bkv_ref, kv_ref, z_ref):
    n_blk, half, _ = bkv_ref.shape
    gr = half // K_PAIRS
    xb = xb_ref[_chunk_rows(xb_ref, it, 0, TB)].reshape(TB, -1)
    last = x_ref.shape[0] - 1
    xb_ref[last] = _layernorm(x_ref[last]).astype(BF16)
    same_head = (_iota((gr, 2 * gr), 0) >= gr // 2) == ((_iota((gr, 2 * gr), 1) & 1) == 1)

    def accumulate(b, t):
        for i in range(K_PAIRS):
            g = b * K_PAIRS + i
            phi = _feature_map(t[i * gr:(i + 1) * gr])
            z_ref[g] = jnp.where(it > 0, z_ref[g], 0.0) + jnp.sum(phi, axis=1, keepdims=True)
            kv = lax.dot_general(t[half + i * gr:half + (i + 1) * gr], phi.astype(BF16), NT,
                                 preferred_element_type=F32)
            kv_ref[g] = jnp.where(it > 0, kv_ref[g], 0.0) + jnp.where(same_head, kv, 0.0)

    pending = None
    for b in range(n_blk):
        t = lax.dot_general(_unpack(bkv_ref[b]), xb, NT, preferred_element_type=F32)
        if pending is not None:
            accumulate(*pending)
        pending = (b, t)
    accumulate(*pending)
    return carry


def _b_queries(it, send, *, x_ref, xb_ref, y_ref, bq_ref, bo_ref, kv_ref, z_ref, ot_ref, on_ref):
    n_groups, gr, _ = kv_ref.shape
    blk = Q_PAIRS * gr
    sub = _iota((8, TB), 0)
    xb = xb_ref[_chunk_rows(xb_ref, it, 0, TB)].reshape(TB, -1)

    def attend(b, t):
        outs = []
        for i in range(Q_PAIRS):
            g = b * Q_PAIRS + i
            phi = _feature_map(t[i * gr:(i + 1) * gr])
            num = jnp.dot(kv_ref[g], phi.astype(BF16), preferred_element_type=F32)
            z = jnp.concatenate([z_ref[g]] * (TB // 128), axis=1)
            inv = _recip(_pair_reduce(phi * z, jnp.add) + 1e-6)
            other = pltpu.roll(inv, 1, 0)
            inv_a = jnp.where((sub & 1) == 0, inv, other)
            inv_b = jnp.where((sub & 1) == 0, other, inv)
            n = (gr - 8) // 16
            inv = jnp.concatenate(
                [inv_a] * n + [jnp.where(sub < 4, inv_a, inv_b)] + [inv_b] * n, axis=0)
            outs.append(num * inv)
        ot_ref[b * blk // 2:(b + 1) * blk // 2, :] = _pack(jnp.concatenate(outs, axis=0))

    n_blk = n_groups // Q_PAIRS
    proj = {}
    for b in range(n_blk + 1):
        if b < n_blk:
            proj[b] = lax.dot_general(_unpack(bq_ref[b * blk // 2:(b + 1) * blk // 2, :]), xb,
                                      NT, preferred_element_type=F32)
        if b > 0:
            attend(b - 1, proj[b - 1])
    on_ref[...] = _pack(_unpack(ot_ref[...]).T)
    r0 = 0
    for i, n in enumerate(O_ROWS):
        at = _chunk_rows(x_ref, it, r0, n)
        y = jnp.dot(_unpack(on_ref[r0 // 2:(r0 + n) // 2, :]), _unpack(bo_ref[...]),
                    preferred_element_type=F32)
        x = x_ref[at] + y.reshape((-1,) + x_ref.shape[1:])
        x_ref[at] = x
        y_ref[at] = x.astype(BF16)
        send(i)
        r0 += n


def _kernel(x_hbm, mem0_hbm, wq_hbm, wk_hbm, wv_hbm, wo_hbm, wqkvb_hbm, wphi_hbm, wob_hbm,
            out_hbm,
            x_ref, xb_ref, y_ref, xp_ref, stage_ref, pre_ref, w_ref, wo_ref, o_ref, near_ref,
            mem0_ref, wphi_ref, phi_ref, wqkvb_ref, wob_ref, bo_ref, bq_ref, bkv_ref,
            kv_ref, z_ref, ot_ref, on_ref,
            w_sem, in_sem, out_sem, *, dh):
    n_seg, seg, d = x_ref.shape
    n_pairs = w_ref.shape[0]
    pw = 2 * dh
    n_iter = n_seg * seg // TB

    def w_copies(p, j):
        src = (wq_hbm, wk_hbm, wv_hbm, wo_hbm)[j]
        if j < 2:
            return [pltpu.make_async_copy(src.at[p], stage_ref.at[p, 3 * j:3 * j + 3],
                                          w_sem.at[p, j])]
        return [pltpu.make_async_copy(src.at[p, i], stage_ref.at[p, 3 * j:3 * j + 3, i],
                                      w_sem.at[p, 2 * j - 2 + i]) for i in range(2)]

    def start_w(p, *slots):
        for j in slots:
            for copy in w_copies(p, j):
                copy.start()

    def wait_w(p, *slots):
        for j in slots:
            for copy in w_copies(p, j):
                copy.wait()

    def staged(p, tiles):
        return stage_ref[p, tiles].reshape(-1, d)

    def out_copy(it, i):
        part = _chunk_rows(y_ref, it, sum(O_ROWS[:i]), O_ROWS[i])
        return pltpu.make_async_copy(y_ref.at[part], out_hbm.at[part], out_sem.at[0])

    def x_copy(part, rows, sem):
        return pltpu.make_async_copy(x_hbm.at[part, rows, :], y_ref.at[part, rows, :], sem)

    head, tail = slice(0, seg - PRE), slice(seg - PRE, seg)
    xt_copy = x_copy(slice(None), tail, in_sem.at[0])
    wqkvb_copy = pltpu.make_async_copy(wqkvb_hbm, wqkvb_ref, in_sem.at[1])
    wphi_copy = pltpu.make_async_copy(wphi_hbm, wphi_ref, in_sem.at[5])
    mem0_copy = pltpu.make_async_copy(mem0_hbm, mem0_ref, in_sem.at[4])
    wob_copy = pltpu.make_async_copy(wob_hbm, wob_ref, in_sem.at[2])

    wphi_copy.start()
    xt_copy.start()
    start_w(0, 1, 2)
    wphi_copy.wait()
    _expand_phi(wphi_ref, phi_ref)
    xt_copy.wait()

    xp_ref[...] = _layernorm(y_ref[:, tail, :].astype(F32).reshape(n_seg * PRE, d)).astype(BF16)

    mem0_copy.start()
    start_w(1, 1, 2)
    start_w(0, 0)
    start_w(1, 0)

    def pre_project(p, carry):
        @pl.when(p + 2 < n_pairs)
        def _():
            start_w(jnp.minimum(p + 2, n_pairs - 1), 0, 1, 2)

        part = pl.ds(p * (n_seg // n_pairs), n_seg // n_pairs)
        x_copy(part, head, in_sem.at[3]).start()
        start_w(p, 3)
        p_q, p_o = jnp.maximum(p - 1, 0), jnp.maximum(p - WO_LAG, 0)

        @pl.when(p >= 1)
        def _():
            wait_w(p_q, 0)

        @pl.when(p >= WO_LAG)
        def _():
            wait_w(p_o, 3)

        wait_w(p, 1, 2)
        pre_ref[p] = lax.dot_general(xp_ref[...], staged(p, slice(3, 9)), NT,
                                     preferred_element_type=F32)
        w_ref[p_q, :, 0:pw] = _pack(staged(p_q, pl.ds(jnp.where(p >= 1, 0, 3), 3)).T)
        wo_ref[pl.ds(3 * p_o, 3)] = _pack(
            staged(p_o, pl.ds(jnp.where(p >= WO_LAG, 9, 3), 3))).reshape(3, 64, d)
        for j in (1, 2):
            w_ref[p, :, j * pw:(j + 1) * pw] = _pack(staged(p, slice(3 * j, 3 * j + 3)).T)
        return carry

    lax.fori_loop(0, n_pairs, pre_project, 0)

    wait_w(n_pairs - 1, 0)
    w_ref[n_pairs - 1, :, 0:pw] = _pack(staged(n_pairs - 1, slice(0, 3)).T)
    for p in range(n_pairs - WO_LAG, n_pairs):
        wait_w(p, 3)
        wo_ref[3 * p:3 * p + 3] = _pack(staged(p, slice(9, 12))).reshape(3, 64, d)
    x_copy(slice(None), head, in_sem.at[3]).wait()

    wqkvb_copy.start()
    wob_copy.start()
    mem0_copy.wait()
    x_ref[0] = y_ref[0].astype(F32)

    def layer_a(layer, x_in, pre):
        unroll = A_UNROLL[layer]
        step = functools.partial(_a_step, layer=layer, dh=dh, x_in=x_in, x_ref=x_ref, xb_ref=xb_ref,
                                 w_ref=w_ref, wo_ref=wo_ref, pre_ref=pre, o_ref=o_ref,
                                 near_ref=near_ref)

        def steps(it, carry):
            for i in range(unroll):
                carry = step(it * unroll + i, carry, i == 0, i == unroll - 1)
            return carry

        lax.fori_loop(0, n_seg // unroll, steps,
                      (mem0_ref[...].astype(F32), _layernorm(x_ref[0])))

    b_keys = functools.partial(_b_keys, x_ref=x_ref, xb_ref=xb_ref, bkv_ref=bkv_ref,
                               kv_ref=kv_ref, z_ref=z_ref)
    b_queries = functools.partial(_b_queries, x_ref=x_ref, xb_ref=xb_ref, y_ref=y_ref,
                                  bq_ref=bq_ref, bo_ref=bo_ref, kv_ref=kv_ref, z_ref=z_ref,
                                  ot_ref=ot_ref, on_ref=on_ref)

    def layer_pair(layer, carry):
        @pl.when(layer == 0)
        def _():
            layer_a(0, y_ref, pre_ref)

        @pl.when(layer == 0)
        def _():
            wqkvb_copy.wait()
            wob_copy.wait()
            _b_weights(wqkvb_ref, phi_ref, wob_ref, bq_ref, bkv_ref, bo_ref)

        @pl.when(layer == 1)
        def _():
            layer_a(1, x_ref, None)

        lax.fori_loop(0, n_iter, b_keys, 0)

        def queries(it, carry):
            def send(i):
                @pl.when(layer == 1)
                def _():
                    out_copy(it, i).start()

            b_queries(it, send)
            return carry

        lax.fori_loop(0, n_iter, queries, 0)

        return carry

    lax.fori_loop(0, 2, layer_pair, 0)
    pltpu.make_async_copy(y_ref, out_hbm, out_sem.at[0]).wait()


@functools.partial(jax.jit, static_argnames=("A_seg_len",))
def pallas_interleave_layers__memory_aug_recurrent_mem_tr__linear_kernel_hedgehog__prompt_kernel(
    A_x, A_mem0, A_Wq, A_Wk, A_Wv, A_Wo, A_seg_len, B_x, B_wqkv, B_w_phi, B_wo,
):
    del B_x
    batch, s_len, d = A_x.shape
    _, heads, dh = A_Wq.shape
    n_mem = A_mem0.shape[1]
    seg = int(A_seg_len)
    b_heads, b_dh, _ = B_w_phi.shape
    rows = n_mem + seg
    n_pairs = heads // 2
    gr = 2 * b_dh
    half = K_PAIRS * gr
    n_seg = s_len // seg
    assert batch == 1 and dh == 192 and heads == 2 * O_SPLITS[0][-1]
    assert n_mem % 8 == 0 and seg % 16 == 0 and 128 % seg == 0 and 2 * rows <= 128
    assert s_len % TB == 0 and s_len > TB == sum(O_ROWS) and n_seg % n_pairs == 0
    assert b_heads * b_dh == d and b_dh % 8 == 4 and d % half == 0

    def head_major(w):
        return w.transpose(1, 2, 0)

    hbm = pl.BlockSpec(memory_space=pltpu.HBM)
    out = pl.pallas_call(
        functools.partial(_kernel, dh=dh),
        out_shape=jax.ShapeDtypeStruct((n_seg, seg, d), A_x.dtype),
        in_specs=[hbm] * 9,
        out_specs=hbm,
        scratch_shapes=[
            pltpu.VMEM((n_seg, seg, d), F32),
            pltpu.VMEM((n_seg, seg, d), BF16),
            pltpu.VMEM((n_seg, seg, d), BF16),
            pltpu.VMEM((n_seg * PRE, d), BF16),
            pltpu.VMEM((n_pairs, 12, 2, 64, d), BF16),
            pltpu.VMEM((n_pairs, n_seg * PRE, 4 * dh), F32),
            pltpu.VMEM((n_pairs, d // 2, 6 * dh), jnp.uint32),
            pltpu.VMEM((3 * n_pairs, 64, d), jnp.uint32),
            pltpu.VMEM((rows, heads * dh), F32),
            pltpu.VMEM((n_pairs, n_mem + 16, 4 * dh), F32),
            pltpu.VMEM((n_mem, d), BF16),
            pltpu.VMEM((b_dh, b_dh, b_heads), BF16),
            pltpu.VMEM((d // (F_PAIRS * gr), F_PAIRS * gr // 2, 256), jnp.uint32),
            pltpu.VMEM(B_wqkv.shape, BF16),
            pltpu.VMEM(B_wo.shape, BF16),
            pltpu.VMEM((d // 2, d), jnp.uint32),
            pltpu.VMEM((d // 2, d), jnp.uint32),
            pltpu.VMEM((d // half, half, d), jnp.uint32),
            pltpu.VMEM((b_heads // 2, gr, 2 * gr), F32),
            pltpu.VMEM((b_heads // 2, 2 * gr, 128), F32),
            pltpu.VMEM((d // 2, TB), jnp.uint32),
            pltpu.VMEM((TB // 2, d), jnp.uint32),
            pltpu.SemaphoreType.DMA((n_pairs, 6)),
            pltpu.SemaphoreType.DMA((6,)),
            pltpu.SemaphoreType.DMA((1,)),
        ],
        compiler_params=pltpu.CompilerParams(vmem_limit_bytes=120 * 1024 * 1024),
    )(
        A_x.reshape(n_seg, seg, d), A_mem0.reshape(n_mem, d),
        head_major(A_Wq).reshape(n_pairs, 3, 2, 64, d),
        head_major(A_Wk).reshape(n_pairs, 3, 2, 64, d),
        head_major(A_Wv).reshape(n_pairs, 2, 3, 64, d), A_Wo.reshape(n_pairs, 2, 3, 64, d),
        B_wqkv, B_w_phi.transpose(1, 2, 0), B_wo,
    )
    return out.reshape(batch, s_len, d)
```

```python
import functools
import math

import jax
import jax.numpy as jnp
from jax import lax
import jax.experimental.pallas as pl
import jax.experimental.pallas.tpu as pltpu

F32 = jnp.float32
BF16 = jnp.bfloat16
NT = (((1,), (1,)), ((), ()))
LOG2E = math.log2(math.e)
MASKED = -1e9

LAG_S = (2, 1)
LAG_PV = (2, 3)
O_SPLITS = ((0, 2, 4, 6, 8, 13, 16), (0, 2, 4, 6, 8, 12, 16))
O_EARLY = ((), ())
ISSUE = ("qkSVv", "aSV")
VPU_ROWS = ((range(16), (2, 7)), (range(16), range(12)))
VPU_DUE = (2, 3)
EXP_AHEAD = (1, 1)
A_UNROLL = (2, 2)
K_SPLIT = 512
NORM_AT = ((1, 2), (1, 2))
PRE = 8
WO_LAG = 3
LNC = (2, 2)
VPU_LAG = (0, 0)
KEY_AHEAD = (10, 10)
XW = (3, 1)
GM = (2, 2)
TB = 512
K_PAIRS = 8
Q_PAIRS = 8
F_PAIRS = 2
O_ROWS = (128, 128, 128, 128)


def _iota(shape, axis):
    return lax.broadcasted_iota(jnp.int32, shape, axis)


def _div(v, d):
    return (v * ((1 << 18) // d + 1)) >> 18


def _pack(x):
    return pltpu.bitcast(x.astype(BF16), jnp.uint32)


def _unpack(x):
    return pltpu.bitcast(x, BF16)


def _recip(x):
    r = pl.reciprocal(x, approx=True)
    return r * (2.0 - x * r)


def _layernorm(x):
    m = jnp.mean(x, axis=-1, keepdims=True)
    c = x - m
    v = jnp.mean(c * c, axis=-1, keepdims=True)
    return c * lax.rsqrt(v + 1e-5)


def _a_step(s, carry, opens, closes, *, layer, dh, x_in, x_ref, xb_ref, w_ref, wo_ref, pre_ref,
            o_ref, near_ref):
    mem, xn = carry
    n_mem, seg = mem.shape[0], xn.shape[0]
    rows = n_mem + seg
    pw = 2 * dh
    n_pairs = w_ref.shape[0]
    scale = dh ** -0.5

    nxt = jnp.minimum(s + 1, x_ref.shape[0] - 1)
    prv = jnp.maximum(s - 1, 0)
    def slow_norm(x, last=None):
        if not LNC[layer]:
            return _layernorm(x)
        outs = []
        for i in range(0, seg, 8):
            t = x[i:i + 8]
            if len(outs) >= LNC[layer]:
                t = jnp.where(s < 0, outs[-LNC[layer]], t)
            outs.append(_layernorm(t))
        return jnp.concatenate(outs, axis=0)

    xn_next = slow_norm(x_in[nxt].astype(F32))
    xb_prev = slow_norm(x_ref[prv])
    xb_ref[prv] = xb_prev.astype(BF16)

    def after(early, value):
        return value if early is None else jnp.where(s < 0, early[:, :value.shape[1]], value)

    def after_all(early, value):
        t = functools.reduce(jnp.maximum, [early[i:i + 8, j:j + 128]
                                           for i in range(0, early.shape[0], 8)
                                           for j in range(0, early.shape[1], 128)])
        return jnp.concatenate([after(t, value[0:8]), value[8:]], axis=0)

    h = jnp.concatenate([mem, xn], axis=0)
    h_short = h[:rows - PRE].astype(BF16)

    first = _iota((rows, 128), 1) < 64
    zero = jnp.zeros((rows, 128), F32)

    def key_blocks(t):
        t0, t1, t2 = t[:, 0:128], t[:, 128:256], t[:, 256:384]
        top = jnp.concatenate([t0, jnp.where(first, t1, 0.0), zero], axis=1)
        bot = jnp.concatenate([zero, jnp.where(first, 0.0, t1), t2], axis=1)
        return jnp.concatenate([top, bot], axis=0).astype(BF16)

    def value_blocks(t):
        mine = jnp.concatenate([first] * 3, axis=1)
        return jnp.concatenate(
            [jnp.where(mine, t, 0.0), jnp.where(mine, 0.0, t)], axis=0).astype(BF16)

    def vpu_rows(p):
        return [n_mem + 8 * i for i, pairs in enumerate(VPU_ROWS[layer]) if p in pairs]

    def mxu_rows(p):
        return [r for r in range(0, rows, 8) if r not in vpu_rows(p)]

    def pick(t, starts):
        return jnp.concatenate([t[r:r + 8] for r in starts], axis=0)

    q, k, v, probs, near_done = {}, {}, {}, {}, {}

    def times_w(lhs, p, lo, hi):
        def part(k0, k1):
            w = _unpack(w_ref[p, k0 // 2:k1 // 2, lo:hi])
            return jnp.dot(lhs[:, k0:k1], w, preferred_element_type=F32)

        if p == 0 and lo == 0 and not opens:
            return part(K_SPLIT, lhs.shape[1]) + part(0, K_SPLIT)
        return part(0, lhs.shape[1])

    def project_short(p, j):
        done = pre_ref[p, pl.ds(pl.multiple_of(s * PRE, PRE), PRE), (j - 1) * pw:j * pw]
        return jnp.concatenate([times_w(h_short, p, j * pw, (j + 1) * pw), done], axis=0)

    def scores(p):
        col = pick(_iota((rows, 2 * rows), 1), mxu_rows(p))
        row = pick(_iota((rows, 2 * rows), 0), mxu_rows(p))
        is_a = col < rows
        visible = (row < n_mem) | (row >= jnp.where(is_a, col, col - rows))
        sc = lax.dot_general(pick(q[p], mxu_rows(p)), key_blocks(k[p]), NT,
                             preferred_element_type=F32)
        sc = jnp.where(visible, sc * scale, MASKED)
        max_a = jnp.max(jnp.where(is_a, sc, -jnp.inf), axis=1, keepdims=True)
        max_b = jnp.max(jnp.where(is_a, -jnp.inf, sc), axis=1, keepdims=True)
        e = jnp.exp(sc - jnp.where(is_a, max_a, max_b))
        sum_a = jnp.sum(jnp.where(is_a, e, 0.0), axis=1, keepdims=True)
        sum_b = jnp.sum(jnp.where(is_a, 0.0, e), axis=1, keepdims=True)
        probs[p] = e * _recip(jnp.where(is_a, sum_a, sum_b))
        if p == NORM_AT[layer][0]:
            probs[p] = after_all(xn_next, probs[p])
        if p == NORM_AT[layer][1]:
            probs[p] = after_all(xb_prev, probs[p])
        if VPU_DUE[layer] and p - VPU_DUE[layer] in near_done:
            probs[p] = after_all(near_done[p - VPU_DUE[layer]], probs[p])

    def values(p):
        o = jnp.dot(probs[p], value_blocks(v[p]), preferred_element_type=F32)
        for i, r in enumerate(mxu_rows(p)):
            o_ref[r:r + 8, p * pw:(p + 1) * pw] = o[8 * i:8 * i + 8]

    chain = [None, None]
    scored, summed = [], []

    def attend_on_vpu(p, r):
        def key_row(j, i):
            return jnp.broadcast_to(near_ref[p, j:j + 1, 128 * i:128 * (i + 1)], (8, 128))

        half, sub = first[0:8], _iota((8, 128), 0)
        t = q[p][r:r + 8] * (scale * LOG2E)
        q0, q2 = t[:, 0:128], t[:, 256:384]
        q1a, q1b = jnp.where(half, t[:, 128:256], 0.0), jnp.where(half, 0.0, t[:, 128:256])
        sc = []
        if not XW[layer] & 1:
            scored.clear()
        if not XW[layer] & 2:
            summed.clear()
        for j in range(r + 8):
            if KEY_AHEAD[layer] and len(scored) >= KEY_AHEAD[layer]:
                chain[0] = after(scored[-KEY_AHEAD[layer]], chain[0])
            k1 = after(chain[0], key_row(j, 1))
            m0 = q0 * after(chain[0] if GM[layer] else None, key_row(j, 0))
            dot_a = m0 + q1a * k1
            chain[0] = q2 * after((None, chain[0], dot_a, m0)[GM[layer]], key_row(j, 2)) + q1b * k1
            t = jnp.where(half, jnp.sum(dot_a, axis=1, keepdims=True),
                          jnp.sum(chain[0], axis=1, keepdims=True))
            sc.append(t if j <= r else jnp.where(sub >= j - r, t, MASKED * LOG2E))
            scored.append(sc[-1])
        top = functools.reduce(jnp.maximum, sc)
        for j in range(r + 8):
            e = jnp.exp2(sc[j] - after(summed[-EXP_AHEAD[layer]] if len(summed) >= EXP_AHEAD[layer] else None, top))
            total = e if j == 0 else total + e
            weight = after(chain[1], e)
            terms = [weight * key_row(j, 3 + i) for i in range(3)]
            acc = terms if j == 0 else [a + b for a, b in zip(acc, terms)]
            chain[1] = acc[2]
            summed.append(acc[2])
        inv = _recip(total)
        o_ref[r:r + 8, p * pw:(p + 1) * pw] = jnp.concatenate([a * inv for a in acc], axis=1)
        near_done[p] = acc[2]

    def attend_early_rows(p):
        if vpu_rows(p):
            n = vpu_rows(p)[-1] + 8
            near_ref[p, 0:n, 0:pw] = k[p][0:n]
            near_ref[p, 0:n, pw:2 * pw] = v[p][0:n]
        for r in vpu_rows(p):
            attend_on_vpu(p, r)

    def project_out(p0, p1, acc):
        lo, hi = 3 * p0, 3 * p1

        def part(k0, k1, c0, c1):
            w = _unpack(wo_ref[k0:k1, :, c0:c1].reshape((k1 - k0) * 64, c1 - c0))
            return jnp.dot(o_ref[:, k0 * 128:k1 * 128], w, preferred_element_type=F32)

        d = wo_ref.shape[-1]
        if p1 < n_pairs:
            r = part(lo, hi, 0, d)
        elif closes:
            return part(hi - 1, hi, 0, d) + (part(lo, hi - 1, 0, d) + acc)
        else:
            r = jnp.concatenate([part(lo, hi, 0, K_SPLIT), part(lo, hi, K_SPLIT, d)], axis=1)
        return r if acc is None else r + acc

    out = None
    lag_s, lag_v = LAG_S[layer], LAG_S[layer] + LAG_PV[layer]
    todo = list(zip(O_SPLITS[layer][:-1], O_SPLITS[layer][1:]))
    for t in range(n_pairs + lag_v):
        if t >= n_pairs:
            out = project_out(*todo.pop(0), out)
        for c in ISSUE[layer]:
            if c == "S" and 0 <= t - lag_s < n_pairs:
                scores(t - lag_s)
            elif c == "V" and 0 <= t - lag_v < n_pairs:
                values(t - lag_v)
            elif c == "a" and t < n_pairs:
                r = times_w(h, t, 0, 3 * pw)
                q[t], k[t], v[t] = r[:, 0:pw], r[:, pw:2 * pw], r[:, 2 * pw:3 * pw]
            elif c in "qkv" and t < n_pairs:
                j = "qkv".index(c)
                (q, k, v)[j][t] = (project_short(t, j) if j and pre_ref is not None
                                   else times_w(h, t, j * pw, (j + 1) * pw))
        if t in O_EARLY[layer]:
            out = project_out(*todo.pop(0), out)
        if 0 <= t - VPU_LAG[layer] < n_pairs:
            attend_early_rows(t - VPU_LAG[layer])
    for part in todo:
        out = project_out(*part, out)

    x_ref[s] = x_in[s].astype(F32) + out[n_mem:, :]
    return out[:n_mem, :], xn_next


def _pair_reduce(t, op):
    r = t[0:8]
    for i in range(8, t.shape[0], 8):
        r = op(r, t[i:i + 8])
    r = op(r, pltpu.roll(r, 4, 0))
    return op(r, pltpu.roll(r, 2, 0))


def _tile_rows(r, n):
    return jnp.concatenate([r] * (n // 8), axis=0)


def _feature_map(p):
    n = p.shape[0]
    e_pos = jnp.exp2(p - _tile_rows(_pair_reduce(p, jnp.maximum), n))
    e_neg = jnp.exp2(_tile_rows(_pair_reduce(p, jnp.minimum), n) - p)
    inv_pos = _recip(_pair_reduce(e_pos, jnp.add))
    inv_neg = _recip(_pair_reduce(e_neg, jnp.add))
    return jnp.concatenate(
        [e_pos * _tile_rows(inv_pos, n), e_neg * _tile_rows(inv_neg, n)], axis=0)


def _fold_span(b, blk):
    return b * blk // 128 * 128, -(-(b + 1) * blk // 128) * 128


def _expand_phi(wphi_ref, phi_ref):
    dh, _, heads = wphi_ref.shape
    d = dh * heads
    gr = 2 * dh
    c = _iota((dh, d), 1)
    c_feat = c - _div(c, dh) * dh
    spread = (_div(_iota((heads, d), 1), dh) == _iota((heads, d), 0)).astype(BF16)
    by_feat = jnp.zeros((dh, d), F32)
    for e in range(dh):
        t = jnp.dot(wphi_ref[e], spread, preferred_element_type=F32)
        by_feat = jnp.where(c_feat == e, t, by_feat)
    by_feat = by_feat.astype(BF16)
    blk = F_PAIRS * gr
    r = _iota((blk, dh), 0)
    sel = (((r - _div(r, gr) * gr) >> 1) == _iota((blk, dh), 1)).astype(BF16)
    for b in range(d // blk):
        lo, hi = _fold_span(b, blk)
        r = _iota((blk, hi - lo), 0)
        head = 2 * (_div(r, gr) + b * F_PAIRS) + (r & 1)
        phi = jnp.dot(sel, by_feat[:, lo:hi], preferred_element_type=F32)
        phi_ref[b, :, 0:hi - lo] = _pack(
            jnp.where(_div(_iota((1, hi - lo), 1) + lo, dh) == head, phi, 0.0))


def _b_weights(wqkv_ref, phi_ref, wob_ref, bq_ref, bkv_ref, bo_ref):
    d = wqkv_ref.shape[0]
    blk = 2 * phi_ref.shape[1]
    half = bkv_ref.shape[1]
    bo_ref[...] = _pack(wob_ref[...])
    wv = wqkv_ref[:, 2 * d:3 * d].T
    for b in range(d // half):
        bkv_ref[b, half // 2:half, :] = _pack(wv[b * half:(b + 1) * half])
    for b in range(d // blk):
        lo, hi = _fold_span(b, blk)
        phi = _unpack(phi_ref[b, :, 0:hi - lo])
        wq = lax.dot_general(phi, wqkv_ref[:, lo:hi], NT, preferred_element_type=F32)
        wk = lax.dot_general(phi, wqkv_ref[:, d + lo:d + hi], NT, preferred_element_type=F32)
        bq_ref[b * blk // 2:(b + 1) * blk // 2, :] = _pack(wq * LOG2E)
        at = b * blk % half // 2
        bkv_ref[b * blk // half, at:at + blk // 2, :] = _pack(wk * LOG2E)


def _chunk_rows(ref, it, r0, n):
    seg = ref.shape[1]
    return pl.ds(it * (TB // seg) + r0 // seg, n // seg)


def _b_keys(it, carry, *, x_ref, xb_ref, bkv_ref, kv_ref, z_ref):
    n_blk, half, _ = bkv_ref.shape
    gr = half // K_PAIRS
    xb = xb_ref[_chunk_rows(xb_ref, it, 0, TB)].reshape(TB, -1)
    last = x_ref.shape[0] - 1
    xb_ref[last] = _layernorm(x_ref[last]).astype(BF16)
    same_head = (_iota((gr, 2 * gr), 0) >= gr // 2) == ((_iota((gr, 2 * gr), 1) & 1) == 1)

    def accumulate(b, t):
        for i in range(K_PAIRS):
            g = b * K_PAIRS + i
            phi = _feature_map(t[i * gr:(i + 1) * gr])
            z_ref[g] = jnp.where(it > 0, z_ref[g], 0.0) + jnp.sum(phi, axis=1, keepdims=True)
            kv = lax.dot_general(t[half + i * gr:half + (i + 1) * gr], phi.astype(BF16), NT,
                                 preferred_element_type=F32)
            kv_ref[g] = jnp.where(it > 0, kv_ref[g], 0.0) + jnp.where(same_head, kv, 0.0)

    pending = None
    for b in range(n_blk):
        t = lax.dot_general(_unpack(bkv_ref[b]), xb, NT, preferred_element_type=F32)
        if pending is not None:
            accumulate(*pending)
        pending = (b, t)
    accumulate(*pending)
    return carry


def _b_queries(it, send, *, x_ref, xb_ref, y_ref, bq_ref, bo_ref, kv_ref, z_ref, ot_ref, on_ref):
    n_groups, gr, _ = kv_ref.shape
    blk = Q_PAIRS * gr
    sub = _iota((8, TB), 0)
    xb = xb_ref[_chunk_rows(xb_ref, it, 0, TB)].reshape(TB, -1)

    def attend(b, t):
        outs = []
        for i in range(Q_PAIRS):
            g = b * Q_PAIRS + i
            phi = _feature_map(t[i * gr:(i + 1) * gr])
            num = jnp.dot(kv_ref[g], phi.astype(BF16), preferred_element_type=F32)
            z = jnp.concatenate([z_ref[g]] * (TB // 128), axis=1)
            inv = _recip(_pair_reduce(phi * z, jnp.add) + 1e-6)
            other = pltpu.roll(inv, 1, 0)
            inv_a = jnp.where((sub & 1) == 0, inv, other)
            inv_b = jnp.where((sub & 1) == 0, other, inv)
            n = (gr - 8) // 16
            inv = jnp.concatenate(
                [inv_a] * n + [jnp.where(sub < 4, inv_a, inv_b)] + [inv_b] * n, axis=0)
            outs.append(num * inv)
        ot_ref[b * blk // 2:(b + 1) * blk // 2, :] = _pack(jnp.concatenate(outs, axis=0))

    n_blk = n_groups // Q_PAIRS
    proj = {}
    for b in range(n_blk + 1):
        if b < n_blk:
            proj[b] = lax.dot_general(_unpack(bq_ref[b * blk // 2:(b + 1) * blk // 2, :]), xb,
                                      NT, preferred_element_type=F32)
        if b > 0:
            attend(b - 1, proj[b - 1])
    on_ref[...] = _pack(_unpack(ot_ref[...]).T)
    r0 = 0
    for i, n in enumerate(O_ROWS):
        at = _chunk_rows(x_ref, it, r0, n)
        y = jnp.dot(_unpack(on_ref[r0 // 2:(r0 + n) // 2, :]), _unpack(bo_ref[...]),
                    preferred_element_type=F32)
        x = x_ref[at] + y.reshape((-1,) + x_ref.shape[1:])
        x_ref[at] = x
        y_ref[at] = x.astype(BF16)
        send(i)
        r0 += n


def _kernel(x_hbm, mem0_hbm, wq_hbm, wk_hbm, wv_hbm, wo_hbm, wqkvb_hbm, wphi_hbm, wob_hbm,
            out_hbm,
            x_ref, xb_ref, y_ref, xp_ref, stage_ref, pre_ref, w_ref, wo_ref, o_ref, near_ref,
            mem0_ref, wphi_ref, phi_ref, wqkvb_ref, wob_ref, bo_ref, bq_ref, bkv_ref,
            kv_ref, z_ref, ot_ref, on_ref,
            w_sem, in_sem, out_sem, *, dh):
    n_seg, seg, d = x_ref.shape
    n_pairs = w_ref.shape[0]
    pw = 2 * dh
    n_iter = n_seg * seg // TB

    def w_copies(p, j):
        src = (wq_hbm, wk_hbm, wv_hbm, wo_hbm)[j]
        if j < 2:
            return [pltpu.make_async_copy(src.at[p], stage_ref.at[p, 3 * j:3 * j + 3],
                                          w_sem.at[p, j])]
        return [pltpu.make_async_copy(src.at[p, i], stage_ref.at[p, 3 * j:3 * j + 3, i],
                                      w_sem.at[p, 2 * j - 2 + i]) for i in range(2)]

    def start_w(p, *slots):
        for j in slots:
            for copy in w_copies(p, j):
                copy.start()

    def wait_w(p, *slots):
        for j in slots:
            for copy in w_copies(p, j):
                copy.wait()

    def staged(p, tiles):
        return stage_ref[p, tiles].reshape(-1, d)

    def out_copy(it, i):
        part = _chunk_rows(y_ref, it, sum(O_ROWS[:i]), O_ROWS[i])
        return pltpu.make_async_copy(y_ref.at[part], out_hbm.at[part], out_sem.at[0])

    def x_copy(part, rows, sem):
        return pltpu.make_async_copy(x_hbm.at[part, rows, :], y_ref.at[part, rows, :], sem)

    head, tail = slice(0, seg - PRE), slice(seg - PRE, seg)
    xt_copy = x_copy(slice(None), tail, in_sem.at[0])
    wqkvb_copy = pltpu.make_async_copy(wqkvb_hbm, wqkvb_ref, in_sem.at[1])
    wphi_copy = pltpu.make_async_copy(wphi_hbm, wphi_ref, in_sem.at[5])
    mem0_copy = pltpu.make_async_copy(mem0_hbm, mem0_ref, in_sem.at[4])
    wob_copy = pltpu.make_async_copy(wob_hbm, wob_ref, in_sem.at[2])

    wphi_copy.start()
    xt_copy.start()
    start_w(0, 1, 2)
    wphi_copy.wait()
    _expand_phi(wphi_ref, phi_ref)
    xt_copy.wait()

    xp_ref[...] = _layernorm(y_ref[:, tail, :].astype(F32).reshape(n_seg * PRE, d)).astype(BF16)

    mem0_copy.start()
    start_w(1, 1, 2)
    start_w(0, 0)
    start_w(1, 0)

    def pre_project(p, carry):
        @pl.when(p + 2 < n_pairs)
        def _():
            start_w(jnp.minimum(p + 2, n_pairs - 1), 0, 1, 2)

        part = pl.ds(p * (n_seg // n_pairs), n_seg // n_pairs)
        x_copy(part, head, in_sem.at[3]).start()
        start_w(p, 3)
        p_q, p_o = jnp.maximum(p - 1, 0), jnp.maximum(p - WO_LAG, 0)

        @pl.when(p >= 1)
        def _():
            wait_w(p_q, 0)

        @pl.when(p >= WO_LAG)
        def _():
            wait_w(p_o, 3)

        wait_w(p, 1, 2)
        pre_ref[p] = lax.dot_general(xp_ref[...], staged(p, slice(3, 9)), NT,
                                     preferred_element_type=F32)
        w_ref[p_q, :, 0:pw] = _pack(staged(p_q, pl.ds(jnp.where(p >= 1, 0, 3), 3)).T)
        wo_ref[pl.ds(3 * p_o, 3)] = _pack(
            staged(p_o, pl.ds(jnp.where(p >= WO_LAG, 9, 3), 3))).reshape(3, 64, d)
        for j in (1, 2):
            w_ref[p, :, j * pw:(j + 1) * pw] = _pack(staged(p, slice(3 * j, 3 * j + 3)).T)
        return carry

    lax.fori_loop(0, n_pairs, pre_project, 0)

    wait_w(n_pairs - 1, 0)
    w_ref[n_pairs - 1, :, 0:pw] = _pack(staged(n_pairs - 1, slice(0, 3)).T)
    for p in range(n_pairs - WO_LAG, n_pairs):
        wait_w(p, 3)
        wo_ref[3 * p:3 * p + 3] = _pack(staged(p, slice(9, 12))).reshape(3, 64, d)
    x_copy(slice(None), head, in_sem.at[3]).wait()

    wqkvb_copy.start()
    wob_copy.start()
    mem0_copy.wait()
    x_ref[0] = y_ref[0].astype(F32)

    def layer_a(layer, x_in, pre):
        unroll = A_UNROLL[layer]
        step = functools.partial(_a_step, layer=layer, dh=dh, x_in=x_in, x_ref=x_ref, xb_ref=xb_ref,
                                 w_ref=w_ref, wo_ref=wo_ref, pre_ref=pre, o_ref=o_ref,
                                 near_ref=near_ref)

        def steps(it, carry):
            for i in range(unroll):
                carry = step(it * unroll + i, carry, i == 0, i == unroll - 1)
            return carry

        lax.fori_loop(0, n_seg // unroll, steps,
                      (mem0_ref[...].astype(F32), _layernorm(x_ref[0])))

    b_keys = functools.partial(_b_keys, x_ref=x_ref, xb_ref=xb_ref, bkv_ref=bkv_ref,
                               kv_ref=kv_ref, z_ref=z_ref)
    b_queries = functools.partial(_b_queries, x_ref=x_ref, xb_ref=xb_ref, y_ref=y_ref,
                                  bq_ref=bq_ref, bo_ref=bo_ref, kv_ref=kv_ref, z_ref=z_ref,
                                  ot_ref=ot_ref, on_ref=on_ref)

    def layer_pair(layer, carry):
        @pl.when(layer == 0)
        def _():
            layer_a(0, y_ref, pre_ref)

        @pl.when(layer == 0)
        def _():
            wqkvb_copy.wait()
            wob_copy.wait()
            _b_weights(wqkvb_ref, phi_ref, wob_ref, bq_ref, bkv_ref, bo_ref)

        @pl.when(layer == 1)
        def _():
            layer_a(1, x_ref, None)

        lax.fori_loop(0, n_iter, b_keys, 0)

        def queries(it, carry):
            def send(i):
                @pl.when(layer == 1)
                def _():
                    out_copy(it, i).start()

            b_queries(it, send)
            return carry

        lax.fori_loop(0, n_iter, queries, 0)

        return carry

    lax.fori_loop(0, 2, layer_pair, 0)
    pltpu.make_async_copy(y_ref, out_hbm, out_sem.at[0]).wait()


@functools.partial(jax.jit, static_argnames=("A_seg_len",))
def pallas_interleave_layers__memory_aug_recurrent_mem_tr__linear_kernel_hedgehog__prompt_kernel(
    A_x, A_mem0, A_Wq, A_Wk, A_Wv, A_Wo, A_seg_len, B_x, B_wqkv, B_w_phi, B_wo,
):
    del B_x
    batch, s_len, d = A_x.shape
    _, heads, dh = A_Wq.shape
    n_mem = A_mem0.shape[1]
    seg = int(A_seg_len)
    b_heads, b_dh, _ = B_w_phi.shape
    rows = n_mem + seg
    n_pairs = heads // 2
    gr = 2 * b_dh
    half = K_PAIRS * gr
    n_seg = s_len // seg
    assert batch == 1 and dh == 192 and heads == 2 * O_SPLITS[0][-1]
    assert n_mem % 8 == 0 and seg % 16 == 0 and 128 % seg == 0 and 2 * rows <= 128
    assert s_len % TB == 0 and s_len > TB == sum(O_ROWS) and n_seg % n_pairs == 0
    assert b_heads * b_dh == d and b_dh % 8 == 4 and d % half == 0

    def head_major(w):
        return w.transpose(1, 2, 0)

    hbm = pl.BlockSpec(memory_space=pltpu.HBM)
    out = pl.pallas_call(
        functools.partial(_kernel, dh=dh),
        out_shape=jax.ShapeDtypeStruct((n_seg, seg, d), A_x.dtype),
        in_specs=[hbm] * 9,
        out_specs=hbm,
        scratch_shapes=[
            pltpu.VMEM((n_seg, seg, d), F32),
            pltpu.VMEM((n_seg, seg, d), BF16),
            pltpu.VMEM((n_seg, seg, d), BF16),
            pltpu.VMEM((n_seg * PRE, d), BF16),
            pltpu.VMEM((n_pairs, 12, 2, 64, d), BF16),
            pltpu.VMEM((n_pairs, n_seg * PRE, 4 * dh), F32),
            pltpu.VMEM((n_pairs, d // 2, 6 * dh), jnp.uint32),
            pltpu.VMEM((3 * n_pairs, 64, d), jnp.uint32),
            pltpu.VMEM((rows, heads * dh), F32),
            pltpu.VMEM((n_pairs, n_mem + 16, 4 * dh), F32),
            pltpu.VMEM((n_mem, d), BF16),
            pltpu.VMEM((b_dh, b_dh, b_heads), BF16),
            pltpu.VMEM((d // (F_PAIRS * gr), F_PAIRS * gr // 2, 256), jnp.uint32),
            pltpu.VMEM(B_wqkv.shape, BF16),
            pltpu.VMEM(B_wo.shape, BF16),
            pltpu.VMEM((d // 2, d), jnp.uint32),
            pltpu.VMEM((d // 2, d), jnp.uint32),
            pltpu.VMEM((d // half, half, d), jnp.uint32),
            pltpu.VMEM((b_heads // 2, gr, 2 * gr), F32),
            pltpu.VMEM((b_heads // 2, 2 * gr, 128), F32),
            pltpu.VMEM((d // 2, TB), jnp.uint32),
            pltpu.VMEM((TB // 2, d), jnp.uint32),
            pltpu.SemaphoreType.DMA((n_pairs, 6)),
            pltpu.SemaphoreType.DMA((6,)),
            pltpu.SemaphoreType.DMA((1,)),
        ],
        compiler_params=pltpu.CompilerParams(vmem_limit_bytes=120 * 1024 * 1024),
    )(
        A_x.reshape(n_seg, seg, d), A_mem0.reshape(n_mem, d),
        head_major(A_Wq).reshape(n_pairs, 3, 2, 64, d),
        head_major(A_Wk).reshape(n_pairs, 3, 2, 64, d),
        head_major(A_Wv).reshape(n_pairs, 2, 3, 64, d), A_Wo.reshape(n_pairs, 2, 3, 64, d),
        B_wqkv, B_w_phi.transpose(1, 2, 0), B_wo,
    )
    return out.reshape(batch, s_len, d)
```

```python
import functools
import math

import jax
import jax.numpy as jnp
from jax import lax
import jax.experimental.pallas as pl
import jax.experimental.pallas.tpu as pltpu

F32 = jnp.float32
BF16 = jnp.bfloat16
NT = (((1,), (1,)), ((), ()))
LOG2E = math.log2(math.e)
MASKED = -1e9

ISSUE = ("qkSVv", "aSV")
LAG_S = (2, 1)
LAG_PV = (2, 3)
O_SPLITS = ((0, 2, 4, 6, 8, 13, 16), (0, 2, 4, 6, 8, 10, 13, 16))
VPU_ROWS = ((range(16), (2, 7)), (range(16), range(14)))
VPU_DUE = (2, 3)
KEYS_AHEAD = (10, 11)
LOAD_ON_SUM = (True, False)
NORM_DUE = ((1, 2), (1, 3))
A_UNROLL = 2
K_SPLIT = 512
PRE = 8
WO_LAG = 3
TB = 512
K_PAIRS = 8
Q_PAIRS = 8
F_PAIRS = 2
O_ROWS = (128, 128, 128, 128)


def _iota(shape, axis):
    return lax.broadcasted_iota(jnp.int32, shape, axis)


def _div(v, d):
    return (v * ((1 << 18) // d + 1)) >> 18


def _pack(x):
    return pltpu.bitcast(x.astype(BF16), jnp.uint32)


def _unpack(x):
    return pltpu.bitcast(x, BF16)


def _recip(x):
    r = pl.reciprocal(x, approx=True)
    return r * (2.0 - x * r)


def _layernorm(x):
    m = jnp.mean(x, axis=-1, keepdims=True)
    c = x - m
    v = jnp.mean(c * c, axis=-1, keepdims=True)
    return c * lax.rsqrt(v + 1e-5)


def _a_step(s, carry, opens, closes, *, layer, dh, x_in, x_ref, xb_ref, w_ref, wo_ref, pre_ref,
            o_ref, near_ref):
    mem, xn = carry
    n_mem, seg = mem.shape[0], xn.shape[0]
    rows = n_mem + seg
    pw = 2 * dh
    n_pairs = w_ref.shape[0]
    scale = dh ** -0.5

    def after(early, value):
        return value if early is None else jnp.where(s < 0, early[:, :value.shape[1]], value)

    def after_all(early, value):
        t = functools.reduce(jnp.maximum, [early[i:i + 8, j:j + 128]
                                           for i in range(0, early.shape[0], 8)
                                           for j in range(0, early.shape[1], 128)])
        return jnp.concatenate([after(t, value[0:8]), value[8:]], axis=0)

    def slow_norm(x):
        outs = [None, None]
        for i in range(0, seg, 8):
            outs.append(_layernorm(after(outs[-2], x[i:i + 8])))
        return jnp.concatenate(outs[2:], axis=0)

    nxt = jnp.minimum(s + 1, x_ref.shape[0] - 1)
    prv = jnp.maximum(s - 1, 0)
    xn_next = slow_norm(x_in[nxt].astype(F32))
    xb_prev = slow_norm(x_ref[prv])
    xb_ref[prv] = xb_prev.astype(BF16)

    h = jnp.concatenate([mem, xn], axis=0)
    h_short = h[:rows - PRE].astype(BF16)

    first = _iota((rows, 128), 1) < 64
    zero = jnp.zeros((rows, 128), F32)

    def key_blocks(t):
        t0, t1, t2 = t[:, 0:128], t[:, 128:256], t[:, 256:384]
        top = jnp.concatenate([t0, jnp.where(first, t1, 0.0), zero], axis=1)
        bot = jnp.concatenate([zero, jnp.where(first, 0.0, t1), t2], axis=1)
        return jnp.concatenate([top, bot], axis=0).astype(BF16)

    def value_blocks(t):
        mine = jnp.concatenate([first] * 3, axis=1)
        return jnp.concatenate(
            [jnp.where(mine, t, 0.0), jnp.where(mine, 0.0, t)], axis=0).astype(BF16)

    def vpu_rows(p):
        return [n_mem + 8 * i for i, pairs in enumerate(VPU_ROWS[layer]) if p in pairs]

    def mxu_rows(p):
        return [r for r in range(0, rows, 8) if r not in vpu_rows(p)]

    def pick(t, starts):
        return jnp.concatenate([t[r:r + 8] for r in starts], axis=0)

    q, k, v, probs, near_done = {}, {}, {}, {}, {}

    def times_w(lhs, p, lo, hi):
        def part(k0, k1):
            w = _unpack(w_ref[p, k0 // 2:k1 // 2, lo:hi])
            return jnp.dot(lhs[:, k0:k1], w, preferred_element_type=F32)

        if p == 0 and lo == 0 and not opens:
            return part(K_SPLIT, lhs.shape[1]) + part(0, K_SPLIT)
        return part(0, lhs.shape[1])

    def project_short(p, j):
        done = pre_ref[p, pl.ds(pl.multiple_of(s * PRE, PRE), PRE), (j - 1) * pw:j * pw]
        return jnp.concatenate([times_w(h_short, p, j * pw, (j + 1) * pw), done], axis=0)

    def scores(p):
        col = pick(_iota((rows, 2 * rows), 1), mxu_rows(p))
        row = pick(_iota((rows, 2 * rows), 0), mxu_rows(p))
        is_a = col < rows
        visible = (row < n_mem) | (row >= jnp.where(is_a, col, col - rows))
        sc = lax.dot_general(pick(q[p], mxu_rows(p)), key_blocks(k[p]), NT,
                             preferred_element_type=F32)
        sc = jnp.where(visible, sc * scale, MASKED)
        max_a = jnp.max(jnp.where(is_a, sc, -jnp.inf), axis=1, keepdims=True)
        max_b = jnp.max(jnp.where(is_a, -jnp.inf, sc), axis=1, keepdims=True)
        e = jnp.exp(sc - jnp.where(is_a, max_a, max_b))
        sum_a = jnp.sum(jnp.where(is_a, e, 0.0), axis=1, keepdims=True)
        sum_b = jnp.sum(jnp.where(is_a, 0.0, e), axis=1, keepdims=True)
        probs[p] = e * _recip(jnp.where(is_a, sum_a, sum_b))
        if p == NORM_DUE[layer][0]:
            probs[p] = after_all(xn_next, probs[p])
        if p == NORM_DUE[layer][1]:
            probs[p] = after_all(xb_prev, probs[p])
        if p - VPU_DUE[layer] in near_done:
            probs[p] = after_all(near_done[p - VPU_DUE[layer]], probs[p])

    def values(p):
        o = jnp.dot(probs[p], value_blocks(v[p]), preferred_element_type=F32)
        for i, r in enumerate(mxu_rows(p)):
            o_ref[r:r + 8, p * pw:(p + 1) * pw] = o[8 * i:8 * i + 8]

    chain = [None, None]
    scored = [None] * KEYS_AHEAD[layer]

    def attend_on_vpu(p, r):
        def key_row(j, i):
            return jnp.broadcast_to(near_ref[p, j:j + 1, 128 * i:128 * (i + 1)], (8, 128))

        half, sub = first[0:8], _iota((8, 128), 0)
        t = q[p][r:r + 8] * (scale * LOG2E)
        q0, q2 = t[:, 0:128], t[:, 256:384]
        q1a, q1b = jnp.where(half, t[:, 128:256], 0.0), jnp.where(half, 0.0, t[:, 128:256])
        for j in range(r + 8):
            ready = after(scored[-KEYS_AHEAD[layer]], chain[0])
            k1 = after(ready, key_row(j, 1))
            m0 = q0 * after(ready, key_row(j, 0))
            dot_a = m0 + q1a * k1
            dot_b = q2 * after(dot_a if LOAD_ON_SUM[layer] else m0, key_row(j, 2)) + q1b * k1
            t = jnp.where(half, jnp.sum(dot_a, axis=1, keepdims=True),
                          jnp.sum(dot_b, axis=1, keepdims=True))
            scored.append(t if j <= r else jnp.where(sub >= j - r, t, MASKED * LOG2E))
            chain[0] = dot_b
        sc = scored[-(r + 8):]
        top = functools.reduce(jnp.maximum, sc)
        for j in range(r + 8):
            e = jnp.exp2(sc[j] - after(chain[1], top))
            weight = after(chain[1], e)
            terms = [weight * key_row(j, 3 + i) for i in range(3)]
            total = e if j == 0 else total + e
            acc = terms if j == 0 else [a + b for a, b in zip(acc, terms)]
            chain[1] = acc[2]
        inv = _recip(total)
        o_ref[r:r + 8, p * pw:(p + 1) * pw] = jnp.concatenate([a * inv for a in acc], axis=1)
        near_done[p] = acc[2]

    def attend_early_rows(p):
        if vpu_rows(p):
            n = vpu_rows(p)[-1] + 8
            near_ref[p, 0:n, 0:pw] = k[p][0:n]
            near_ref[p, 0:n, pw:2 * pw] = v[p][0:n]
        for r in vpu_rows(p):
            attend_on_vpu(p, r)

    def project_out(p0, p1, acc):
        lo, hi = 3 * p0, 3 * p1

        def part(k0, k1, c0, c1):
            w = _unpack(wo_ref[k0:k1, :, c0:c1].reshape((k1 - k0) * 64, c1 - c0))
            return jnp.dot(o_ref[:, k0 * 128:k1 * 128], w, preferred_element_type=F32)

        d = wo_ref.shape[-1]
        if p1 < n_pairs:
            r = part(lo, hi, 0, d)
        elif closes:
            return part(hi - 1, hi, 0, d) + (part(lo, hi - 1, 0, d) + acc)
        else:
            r = jnp.concatenate([part(lo, hi, 0, K_SPLIT), part(lo, hi, K_SPLIT, d)], axis=1)
        return r if acc is None else r + acc

    out = None
    lag_s, lag_v = LAG_S[layer], LAG_S[layer] + LAG_PV[layer]
    todo = list(zip(O_SPLITS[layer][:-1], O_SPLITS[layer][1:]))
    for t in range(n_pairs + lag_v):
        if t >= n_pairs:
            out = project_out(*todo.pop(0), out)
        for c in ISSUE[layer]:
            if c == "S" and 0 <= t - lag_s < n_pairs:
                scores(t - lag_s)
            elif c == "V" and 0 <= t - lag_v < n_pairs:
                values(t - lag_v)
            elif c == "a" and t < n_pairs:
                r = times_w(h, t, 0, 3 * pw)
                q[t], k[t], v[t] = r[:, 0:pw], r[:, pw:2 * pw], r[:, 2 * pw:3 * pw]
            elif c in "qkv" and t < n_pairs:
                j = "qkv".index(c)
                (q, k, v)[j][t] = (project_short(t, j) if j and pre_ref is not None
                                   else times_w(h, t, j * pw, (j + 1) * pw))
        if t < n_pairs:
            attend_early_rows(t)
    for part in todo:
        out = project_out(*part, out)

    x_ref[s] = x_in[s].astype(F32) + out[n_mem:, :]
    return out[:n_mem, :], xn_next


def _pair_reduce(t, op):
    r = t[0:8]
    for i in range(8, t.shape[0], 8):
        r = op(r, t[i:i + 8])
    r = op(r, pltpu.roll(r, 4, 0))
    return op(r, pltpu.roll(r, 2, 0))


def _tile_rows(r, n):
    return jnp.concatenate([r] * (n // 8), axis=0)


def _feature_map(p):
    n = p.shape[0]
    e_pos = jnp.exp2(p - _tile_rows(_pair_reduce(p, jnp.maximum), n))
    e_neg = jnp.exp2(_tile_rows(_pair_reduce(p, jnp.minimum), n) - p)
    inv_pos = _recip(_pair_reduce(e_pos, jnp.add))
    inv_neg = _recip(_pair_reduce(e_neg, jnp.add))
    return jnp.concatenate(
        [e_pos * _tile_rows(inv_pos, n), e_neg * _tile_rows(inv_neg, n)], axis=0)


def _fold_span(b, blk):
    return b * blk // 128 * 128, -(-(b + 1) * blk // 128) * 128


def _expand_phi(wphi_ref, phi_ref):
    dh, _, heads = wphi_ref.shape
    d = dh * heads
    gr = 2 * dh
    c = _iota((dh, d), 1)
    c_feat = c - _div(c, dh) * dh
    spread = (_div(_iota((heads, d), 1), dh) == _iota((heads, d), 0)).astype(BF16)
    by_feat = jnp.zeros((dh, d), F32)
    for e in range(dh):
        t = jnp.dot(wphi_ref[e], spread, preferred_element_type=F32)
        by_feat = jnp.where(c_feat == e, t, by_feat)
    by_feat = by_feat.astype(BF16)
    blk = F_PAIRS * gr
    r = _iota((blk, dh), 0)
    sel = (((r - _div(r, gr) * gr) >> 1) == _iota((blk, dh), 1)).astype(BF16)
    for b in range(d // blk):
        lo, hi = _fold_span(b, blk)
        r = _iota((blk, hi - lo), 0)
        head = 2 * (_div(r, gr) + b * F_PAIRS) + (r & 1)
        phi = jnp.dot(sel, by_feat[:, lo:hi], preferred_element_type=F32)
        phi_ref[b, :, 0:hi - lo] = _pack(
            jnp.where(_div(_iota((1, hi - lo), 1) + lo, dh) == head, phi, 0.0))


def _b_weights(wqkv_ref, phi_ref, wob_ref, bq_ref, bkv_ref, bo_ref):
    d = wqkv_ref.shape[0]
    blk = 2 * phi_ref.shape[1]
    half = bkv_ref.shape[1]
    bo_ref[...] = _pack(wob_ref[...])
    wv = wqkv_ref[:, 2 * d:3 * d].T
    for b in range(d // half):
        bkv_ref[b, half // 2:half, :] = _pack(wv[b * half:(b + 1) * half])
    for b in range(d // blk):
        lo, hi = _fold_span(b, blk)
        phi = _unpack(phi_ref[b, :, 0:hi - lo])
        wq = lax.dot_general(phi, wqkv_ref[:, lo:hi], NT, preferred_element_type=F32)
        wk = lax.dot_general(phi, wqkv_ref[:, d + lo:d + hi], NT, preferred_element_type=F32)
        bq_ref[b * blk // 2:(b + 1) * blk // 2, :] = _pack(wq * LOG2E)
        at = b * blk % half // 2
        bkv_ref[b * blk // half, at:at + blk // 2, :] = _pack(wk * LOG2E)


def _chunk_rows(ref, it, r0, n):
    seg = ref.shape[1]
    return pl.ds(it * (TB // seg) + r0 // seg, n // seg)


def _b_keys(it, carry, *, x_ref, xb_ref, bkv_ref, kv_ref, z_ref):
    n_blk, half, _ = bkv_ref.shape
    gr = half // K_PAIRS
    xb = xb_ref[_chunk_rows(xb_ref, it, 0, TB)].reshape(TB, -1)
    last = x_ref.shape[0] - 1
    xb_ref[last] = _layernorm(x_ref[last]).astype(BF16)
    same_head = (_iota((gr, 2 * gr), 0) >= gr // 2) == ((_iota((gr, 2 * gr), 1) & 1) == 1)

    def accumulate(b, t):
        for i in range(K_PAIRS):
            g = b * K_PAIRS + i
            phi = _feature_map(t[i * gr:(i + 1) * gr])
            z_ref[g] = jnp.where(it > 0, z_ref[g], 0.0) + jnp.sum(phi, axis=1, keepdims=True)
            kv = lax.dot_general(t[half + i * gr:half + (i + 1) * gr], phi.astype(BF16), NT,
                                 preferred_element_type=F32)
            kv_ref[g] = jnp.where(it > 0, kv_ref[g], 0.0) + jnp.where(same_head, kv, 0.0)

    pending = None
    for b in range(n_blk):
        t = lax.dot_general(_unpack(bkv_ref[b]), xb, NT, preferred_element_type=F32)
        if pending is not None:
            accumulate(*pending)
        pending = (b, t)
    accumulate(*pending)
    return carry


def _b_queries(it, send, *, x_ref, xb_ref, y_ref, bq_ref, bo_ref, kv_ref, z_ref, ot_ref, on_ref):
    n_groups, gr, _ = kv_ref.shape
    blk = Q_PAIRS * gr
    sub = _iota((8, TB), 0)
    xb = xb_ref[_chunk_rows(xb_ref, it, 0, TB)].reshape(TB, -1)

    def attend(b, t):
        outs = []
        for i in range(Q_PAIRS):
            g = b * Q_PAIRS + i
            phi = _feature_map(t[i * gr:(i + 1) * gr])
            num = jnp.dot(kv_ref[g], phi.astype(BF16), preferred_element_type=F32)
            z = jnp.concatenate([z_ref[g]] * (TB // 128), axis=1)
            inv = _recip(_pair_reduce(phi * z, jnp.add) + 1e-6)
            other = pltpu.roll(inv, 1, 0)
            inv_a = jnp.where((sub & 1) == 0, inv, other)
            inv_b = jnp.where((sub & 1) == 0, other, inv)
            n = (gr - 8) // 16
            inv = jnp.concatenate(
                [inv_a] * n + [jnp.where(sub < 4, inv_a, inv_b)] + [inv_b] * n, axis=0)
            outs.append(num * inv)
        ot_ref[b * blk // 2:(b + 1) * blk // 2, :] = _pack(jnp.concatenate(outs, axis=0))

    n_blk = n_groups // Q_PAIRS
    proj = {}
    for b in range(n_blk + 1):
        if b < n_blk:
            proj[b] = lax.dot_general(_unpack(bq_ref[b * blk // 2:(b + 1) * blk // 2, :]), xb,
                                      NT, preferred_element_type=F32)
        if b > 0:
            attend(b - 1, proj[b - 1])
    on_ref[...] = _pack(_unpack(ot_ref[...]).T)
    r0 = 0
    for i, n in enumerate(O_ROWS):
        at = _chunk_rows(x_ref, it, r0, n)
        y = jnp.dot(_unpack(on_ref[r0 // 2:(r0 + n) // 2, :]), _unpack(bo_ref[...]),
                    preferred_element_type=F32)
        x = x_ref[at] + y.reshape((-1,) + x_ref.shape[1:])
        x_ref[at] = x
        y_ref[at] = x.astype(BF16)
        send(i)
        r0 += n


def _kernel(x_hbm, mem0_hbm, wq_hbm, wk_hbm, wv_hbm, wo_hbm, wqkvb_hbm, wphi_hbm, wob_hbm,
            out_hbm,
            x_ref, xb_ref, y_ref, xp_ref, stage_ref, pre_ref, w_ref, wo_ref, o_ref, near_ref,
            mem0_ref, wphi_ref, phi_ref, wqkvb_ref, wob_ref, bo_ref, bq_ref, bkv_ref,
            kv_ref, z_ref, ot_ref, on_ref,
            w_sem, in_sem, out_sem, *, dh):
    n_seg, seg, d = x_ref.shape
    n_pairs = w_ref.shape[0]
    pw = 2 * dh
    n_iter = n_seg * seg // TB

    def w_copies(p, j):
        src = (wq_hbm, wk_hbm, wv_hbm, wo_hbm)[j]
        if j < 2:
            return [pltpu.make_async_copy(src.at[p], stage_ref.at[p, 3 * j:3 * j + 3],
                                          w_sem.at[p, j])]
        return [pltpu.make_async_copy(src.at[p, i], stage_ref.at[p, 3 * j:3 * j + 3, i],
                                      w_sem.at[p, 2 * j - 2 + i]) for i in range(2)]

    def start_w(p, *slots):
        for j in slots:
            for copy in w_copies(p, j):
                copy.start()

    def wait_w(p, *slots):
        for j in slots:
            for copy in w_copies(p, j):
                copy.wait()

    def staged(p, tiles):
        return stage_ref[p, tiles].reshape(-1, d)

    def out_copy(it, i):
        part = _chunk_rows(y_ref, it, sum(O_ROWS[:i]), O_ROWS[i])
        return pltpu.make_async_copy(y_ref.at[part], out_hbm.at[part], out_sem.at[0])

    def x_copy(part, rows, sem):
        return pltpu.make_async_copy(x_hbm.at[part, rows, :], y_ref.at[part, rows, :], sem)

    head, tail = slice(0, seg - PRE), slice(seg - PRE, seg)
    xt_copy = x_copy(slice(None), tail, in_sem.at[0])
    wqkvb_copy = pltpu.make_async_copy(wqkvb_hbm, wqkvb_ref, in_sem.at[1])
    wphi_copy = pltpu.make_async_copy(wphi_hbm, wphi_ref, in_sem.at[5])
    mem0_copy = pltpu.make_async_copy(mem0_hbm, mem0_ref, in_sem.at[4])
    wob_copy = pltpu.make_async_copy(wob_hbm, wob_ref, in_sem.at[2])

    wphi_copy.start()
    xt_copy.start()
    start_w(0, 1, 2)
    wphi_copy.wait()
    _expand_phi(wphi_ref, phi_ref)
    xt_copy.wait()

    xp_ref[...] = _layernorm(y_ref[:, tail, :].astype(F32).reshape(n_seg * PRE, d)).astype(BF16)

    mem0_copy.start()
    start_w(1, 1, 2)
    start_w(0, 0)
    start_w(1, 0)

    def pre_project(p, carry):
        @pl.when(p + 2 < n_pairs)
        def _():
            start_w(jnp.minimum(p + 2, n_pairs - 1), 0, 1, 2)

        part = pl.ds(p * (n_seg // n_pairs), n_seg // n_pairs)
        x_copy(part, head, in_sem.at[3]).start()
        start_w(p, 3)
        p_q, p_o = jnp.maximum(p - 1, 0), jnp.maximum(p - WO_LAG, 0)

        @pl.when(p >= 1)
        def _():
            wait_w(p_q, 0)

        @pl.when(p >= WO_LAG)
        def _():
            wait_w(p_o, 3)

        wait_w(p, 1, 2)
        pre_ref[p] = lax.dot_general(xp_ref[...], staged(p, slice(3, 9)), NT,
                                     preferred_element_type=F32)
        w_ref[p_q, :, 0:pw] = _pack(staged(p_q, pl.ds(jnp.where(p >= 1, 0, 3), 3)).T)
        wo_ref[pl.ds(3 * p_o, 3)] = _pack(
            staged(p_o, pl.ds(jnp.where(p >= WO_LAG, 9, 3), 3))).reshape(3, 64, d)
        for j in (1, 2):
            w_ref[p, :, j * pw:(j + 1) * pw] = _pack(staged(p, slice(3 * j, 3 * j + 3)).T)
        return carry

    lax.fori_loop(0, n_pairs, pre_project, 0)

    wait_w(n_pairs - 1, 0)
    w_ref[n_pairs - 1, :, 0:pw] = _pack(staged(n_pairs - 1, slice(0, 3)).T)
    for p in range(n_pairs - WO_LAG, n_pairs):
        wait_w(p, 3)
        wo_ref[3 * p:3 * p + 3] = _pack(staged(p, slice(9, 12))).reshape(3, 64, d)
    x_copy(slice(None), head, in_sem.at[3]).wait()

    wqkvb_copy.start()
    wob_copy.start()
    mem0_copy.wait()
    x_ref[0] = y_ref[0].astype(F32)

    def layer_a(layer, x_in, pre):
        unroll = A_UNROLL
        step = functools.partial(_a_step, layer=layer, dh=dh, x_in=x_in, x_ref=x_ref, xb_ref=xb_ref,
                                 w_ref=w_ref, wo_ref=wo_ref, pre_ref=pre, o_ref=o_ref,
                                 near_ref=near_ref)

        def steps(it, carry):
            for i in range(unroll):
                carry = step(it * unroll + i, carry, i == 0, i == unroll - 1)
            return carry

        lax.fori_loop(0, n_seg // unroll, steps,
                      (mem0_ref[...].astype(F32), _layernorm(x_ref[0])))

    b_keys = functools.partial(_b_keys, x_ref=x_ref, xb_ref=xb_ref, bkv_ref=bkv_ref,
                               kv_ref=kv_ref, z_ref=z_ref)
    b_queries = functools.partial(_b_queries, x_ref=x_ref, xb_ref=xb_ref, y_ref=y_ref,
                                  bq_ref=bq_ref, bo_ref=bo_ref, kv_ref=kv_ref, z_ref=z_ref,
                                  ot_ref=ot_ref, on_ref=on_ref)

    def layer_pair(layer, carry):
        @pl.when(layer == 0)
        def _():
            layer_a(0, y_ref, pre_ref)

        @pl.when(layer == 0)
        def _():
            wqkvb_copy.wait()
            wob_copy.wait()
            _b_weights(wqkvb_ref, phi_ref, wob_ref, bq_ref, bkv_ref, bo_ref)

        @pl.when(layer == 1)
        def _():
            layer_a(1, x_ref, None)

        lax.fori_loop(0, n_iter, b_keys, 0)

        def queries(it, carry):
            def send(i):
                @pl.when(layer == 1)
                def _():
                    out_copy(it, i).start()

            b_queries(it, send)
            return carry

        lax.fori_loop(0, n_iter, queries, 0)

        return carry

    lax.fori_loop(0, 2, layer_pair, 0)
    pltpu.make_async_copy(y_ref, out_hbm, out_sem.at[0]).wait()


@functools.partial(jax.jit, static_argnames=("A_seg_len",))
def pallas_interleave_layers__memory_aug_recurrent_mem_tr__linear_kernel_hedgehog__prompt_kernel(
    A_x, A_mem0, A_Wq, A_Wk, A_Wv, A_Wo, A_seg_len, B_x, B_wqkv, B_w_phi, B_wo,
):
    del B_x
    batch, s_len, d = A_x.shape
    _, heads, dh = A_Wq.shape
    n_mem = A_mem0.shape[1]
    seg = int(A_seg_len)
    b_heads, b_dh, _ = B_w_phi.shape
    rows = n_mem + seg
    n_pairs = heads // 2
    gr = 2 * b_dh
    half = K_PAIRS * gr
    n_seg = s_len // seg
    assert batch == 1 and dh == 192 and heads == 2 * O_SPLITS[0][-1]
    assert n_mem % 8 == 0 and seg % 16 == 0 and 128 % seg == 0 and 2 * rows <= 128
    assert s_len % TB == 0 and s_len > TB == sum(O_ROWS) and n_seg % n_pairs == 0
    assert b_heads * b_dh == d and b_dh % 8 == 4 and d % half == 0

    def head_major(w):
        return w.transpose(1, 2, 0)

    hbm = pl.BlockSpec(memory_space=pltpu.HBM)
    out = pl.pallas_call(
        functools.partial(_kernel, dh=dh),
        out_shape=jax.ShapeDtypeStruct((n_seg, seg, d), A_x.dtype),
        in_specs=[hbm] * 9,
        out_specs=hbm,
        scratch_shapes=[
            pltpu.VMEM((n_seg, seg, d), F32),
            pltpu.VMEM((n_seg, seg, d), BF16),
            pltpu.VMEM((n_seg, seg, d), BF16),
            pltpu.VMEM((n_seg * PRE, d), BF16),
            pltpu.VMEM((n_pairs, 12, 2, 64, d), BF16),
            pltpu.VMEM((n_pairs, n_seg * PRE, 4 * dh), F32),
            pltpu.VMEM((n_pairs, d // 2, 6 * dh), jnp.uint32),
            pltpu.VMEM((3 * n_pairs, 64, d), jnp.uint32),
            pltpu.VMEM((rows, heads * dh), F32),
            pltpu.VMEM((n_pairs, n_mem + 16, 4 * dh), F32),
            pltpu.VMEM((n_mem, d), BF16),
            pltpu.VMEM((b_dh, b_dh, b_heads), BF16),
            pltpu.VMEM((d // (F_PAIRS * gr), F_PAIRS * gr // 2, 256), jnp.uint32),
            pltpu.VMEM(B_wqkv.shape, BF16),
            pltpu.VMEM(B_wo.shape, BF16),
            pltpu.VMEM((d // 2, d), jnp.uint32),
            pltpu.VMEM((d // 2, d), jnp.uint32),
            pltpu.VMEM((d // half, half, d), jnp.uint32),
            pltpu.VMEM((b_heads // 2, gr, 2 * gr), F32),
            pltpu.VMEM((b_heads // 2, 2 * gr, 128), F32),
            pltpu.VMEM((d // 2, TB), jnp.uint32),
            pltpu.VMEM((TB // 2, d), jnp.uint32),
            pltpu.SemaphoreType.DMA((n_pairs, 6)),
            pltpu.SemaphoreType.DMA((6,)),
            pltpu.SemaphoreType.DMA((1,)),
        ],
        compiler_params=pltpu.CompilerParams(vmem_limit_bytes=120 * 1024 * 1024),
    )(
        A_x.reshape(n_seg, seg, d), A_mem0.reshape(n_mem, d),
        head_major(A_Wq).reshape(n_pairs, 3, 2, 64, d),
        head_major(A_Wk).reshape(n_pairs, 3, 2, 64, d),
        head_major(A_Wv).reshape(n_pairs, 2, 3, 64, d), A_Wo.reshape(n_pairs, 2, 3, 64, d),
        B_wqkv, B_w_phi.transpose(1, 2, 0), B_wo,
    )
    return out.reshape(batch, s_len, d)
```

```python
import functools
import math

import jax
import jax.numpy as jnp
from jax import lax
import jax.experimental.pallas as pl
import jax.experimental.pallas.tpu as pltpu

F32 = jnp.float32
BF16 = jnp.bfloat16
NT = (((1,), (1,)), ((), ()))
LOG2E = math.log2(math.e)
MASKED = -1e9

ISSUE = ("qkSVv", "aSV")
LAG_S = (2, 1)
LAG_PV = (2, 3)
O_SPLITS = ((0, 2, 4, 6, 8, 13, 16), (0, 2, 4, 6, 8, 10, 13, 16))
VPU_ROWS = ((range(16), (2, 7, 8, 11)), (range(16), range(14)))
VPU_DUE = (2, 3)
KEYS_AHEAD = (10, 11)
NORM_DUE = ((0, 1), (1, 3))
A_UNROLL = 2
K_SPLIT = 512
PRE = 8
WO_LAG = 3
TB = 512
K_PAIRS = 8
Q_PAIRS = 8
F_PAIRS = 2
O_ROWS = (128, 128, 128, 128)


def _iota(shape, axis):
    return lax.broadcasted_iota(jnp.int32, shape, axis)


def _div(v, d):
    return (v * ((1 << 18) // d + 1)) >> 18


def _pack(x):
    return pltpu.bitcast(x.astype(BF16), jnp.uint32)


def _unpack(x):
    return pltpu.bitcast(x, BF16)


def _recip(x):
    r = pl.reciprocal(x, approx=True)
    return r * (2.0 - x * r)


def _layernorm(x):
    m = jnp.mean(x, axis=-1, keepdims=True)
    c = x - m
    v = jnp.mean(c * c, axis=-1, keepdims=True)
    return c * lax.rsqrt(v + 1e-5)


def _a_step(s, carry, opens, closes, *, layer, dh, x_in, x_ref, xb_ref, w_ref, wo_ref, pre_ref,
            o_ref, near_ref):
    mem, xn = carry
    n_mem, seg = mem.shape[0], xn.shape[0]
    rows = n_mem + seg
    pw = 2 * dh
    n_pairs = w_ref.shape[0]
    scale = dh ** -0.5

    def after(early, value):
        return value if early is None else jnp.where(s < 0, early[:, :value.shape[1]], value)

    def after_all(early, value):
        t = functools.reduce(jnp.maximum, [early[i:i + 8, j:j + 128]
                                           for i in range(0, early.shape[0], 8)
                                           for j in range(0, early.shape[1], 128)])
        return jnp.concatenate([after(t, value[0:8]), value[8:]], axis=0)

    def slow_norm(x):
        outs = [None, None]
        for i in range(0, seg, 8):
            outs.append(_layernorm(after(outs[-2], x[i:i + 8])))
        return jnp.concatenate(outs[2:], axis=0)

    nxt = jnp.minimum(s + 1, x_ref.shape[0] - 1)
    prv = jnp.maximum(s - 1, 0)
    xn_next = slow_norm(x_in[nxt].astype(F32))
    xb_prev = slow_norm(x_ref[prv])
    xb_ref[prv] = xb_prev.astype(BF16)

    h = jnp.concatenate([mem, xn], axis=0)
    h_short = h[:rows - PRE].astype(BF16)

    first = _iota((rows, 128), 1) < 64
    zero = jnp.zeros((rows, 128), F32)

    def key_blocks(t):
        t0, t1, t2 = t[:, 0:128], t[:, 128:256], t[:, 256:384]
        top = jnp.concatenate([t0, jnp.where(first, t1, 0.0), zero], axis=1)
        bot = jnp.concatenate([zero, jnp.where(first, 0.0, t1), t2], axis=1)
        return jnp.concatenate([top, bot], axis=0).astype(BF16)

    def value_blocks(t):
        mine = jnp.concatenate([first] * 3, axis=1)
        return jnp.concatenate(
            [jnp.where(mine, t, 0.0), jnp.where(mine, 0.0, t)], axis=0).astype(BF16)

    def vpu_rows(p):
        return [n_mem + 8 * i for i, pairs in enumerate(VPU_ROWS[layer]) if p in pairs]

    def mxu_rows(p):
        return [r for r in range(0, rows, 8) if r not in vpu_rows(p)]

    def pick(t, starts):
        return jnp.concatenate([t[r:r + 8] for r in starts], axis=0)

    q, k, v, probs, near_done = {}, {}, {}, {}, {}

    def times_w(lhs, p, lo, hi):
        def part(k0, k1):
            w = _unpack(w_ref[p, k0 // 2:k1 // 2, lo:hi])
            return jnp.dot(lhs[:, k0:k1], w, preferred_element_type=F32)

        if p == 0 and lo == 0 and not opens:
            return part(K_SPLIT, lhs.shape[1]) + part(0, K_SPLIT)
        return part(0, lhs.shape[1])

    def project_short(p, j):
        done = pre_ref[p, pl.ds(pl.multiple_of(s * PRE, PRE), PRE), (j - 1) * pw:j * pw]
        return jnp.concatenate([times_w(h_short, p, j * pw, (j + 1) * pw), done], axis=0)

    def scores(p):
        col = pick(_iota((rows, 2 * rows), 1), mxu_rows(p))
        row = pick(_iota((rows, 2 * rows), 0), mxu_rows(p))
        is_a = col < rows
        visible = (row < n_mem) | (row >= jnp.where(is_a, col, col - rows))
        sc = lax.dot_general(pick(q[p], mxu_rows(p)), key_blocks(k[p]), NT,
                             preferred_element_type=F32)
        sc = jnp.where(visible, sc * scale, MASKED)
        max_a = jnp.max(jnp.where(is_a, sc, -jnp.inf), axis=1, keepdims=True)
        max_b = jnp.max(jnp.where(is_a, -jnp.inf, sc), axis=1, keepdims=True)
        e = jnp.exp(sc - jnp.where(is_a, max_a, max_b))
        sum_a = jnp.sum(jnp.where(is_a, e, 0.0), axis=1, keepdims=True)
        sum_b = jnp.sum(jnp.where(is_a, 0.0, e), axis=1, keepdims=True)
        probs[p] = e * _recip(jnp.where(is_a, sum_a, sum_b))
        if p == NORM_DUE[layer][0]:
            probs[p] = after_all(xn_next, probs[p])
        if p == NORM_DUE[layer][1]:
            probs[p] = after_all(xb_prev, probs[p])
        if p - VPU_DUE[layer] in near_done:
            probs[p] = after_all(near_done[p - VPU_DUE[layer]], probs[p])

    def values(p):
        o = jnp.dot(probs[p], value_blocks(v[p]), preferred_element_type=F32)
        for i, r in enumerate(mxu_rows(p)):
            o_ref[r:r + 8, p * pw:(p + 1) * pw] = o[8 * i:8 * i + 8]

    chain = [None, None]
    scored = [None] * KEYS_AHEAD[layer]

    def attend_on_vpu(p, r):
        def key_row(j, i):
            return jnp.broadcast_to(near_ref[p, j:j + 1, 128 * i:128 * (i + 1)], (8, 128))

        half, sub = first[0:8], _iota((8, 128), 0)
        t = q[p][r:r + 8] * (scale * LOG2E)
        q0, q2 = t[:, 0:128], t[:, 256:384]
        q1a, q1b = jnp.where(half, t[:, 128:256], 0.0), jnp.where(half, 0.0, t[:, 128:256])
        for j in range(r + 8):
            ready = after(scored[-KEYS_AHEAD[layer]], chain[0])
            k1 = after(ready, key_row(j, 1))
            dot_a = q0 * after(ready, key_row(j, 0)) + q1a * k1
            dot_b = q2 * after(dot_a, key_row(j, 2)) + q1b * k1
            t = jnp.where(half, jnp.sum(dot_a, axis=1, keepdims=True),
                          jnp.sum(dot_b, axis=1, keepdims=True))
            scored.append(t if j <= r else jnp.where(sub >= j - r, t, MASKED * LOG2E))
            chain[0] = dot_b
        sc = scored[-(r + 8):]
        top = functools.reduce(jnp.maximum, sc)
        for j in range(r + 8):
            e = jnp.exp2(sc[j] - after(chain[1], top))
            weight = after(chain[1], e)
            terms = [weight * key_row(j, 3 + i) for i in range(3)]
            total = e if j == 0 else total + e
            acc = terms if j == 0 else [a + b for a, b in zip(acc, terms)]
            chain[1] = acc[2]
        inv = _recip(total)
        o_ref[r:r + 8, p * pw:(p + 1) * pw] = jnp.concatenate([a * inv for a in acc], axis=1)
        near_done[p] = acc[2]

    def attend_early_rows(p):
        if vpu_rows(p):
            n = vpu_rows(p)[-1] + 8
            near_ref[p, 0:n, 0:pw] = k[p][0:n]
            near_ref[p, 0:n, pw:2 * pw] = v[p][0:n]
        for r in reversed(vpu_rows(p)):
            attend_on_vpu(p, r)

    def project_out(p0, p1, acc):
        lo, hi = 3 * p0, 3 * p1

        def part(k0, k1, c0, c1):
            w = _unpack(wo_ref[k0:k1, :, c0:c1].reshape((k1 - k0) * 64, c1 - c0))
            return jnp.dot(o_ref[:, k0 * 128:k1 * 128], w, preferred_element_type=F32)

        d = wo_ref.shape[-1]
        if p1 < n_pairs:
            r = part(lo, hi, 0, d)
        elif closes:
            return part(hi - 1, hi, 0, d) + (part(lo, hi - 1, 0, d) + acc)
        else:
            r = jnp.concatenate([part(lo, hi, 0, K_SPLIT), part(lo, hi, K_SPLIT, d)], axis=1)
        return r if acc is None else r + acc

    out = None
    lag_s, lag_v = LAG_S[layer], LAG_S[layer] + LAG_PV[layer]
    todo = list(zip(O_SPLITS[layer][:-1], O_SPLITS[layer][1:]))
    for t in range(n_pairs + lag_v):
        if t >= n_pairs:
            out = project_out(*todo.pop(0), out)
        for c in ISSUE[layer]:
            if c == "S" and 0 <= t - lag_s < n_pairs:
                scores(t - lag_s)
            elif c == "V" and 0 <= t - lag_v < n_pairs:
                values(t - lag_v)
            elif c == "a" and t < n_pairs:
                r = times_w(h, t, 0, 3 * pw)
                q[t], k[t], v[t] = r[:, 0:pw], r[:, pw:2 * pw], r[:, 2 * pw:3 * pw]
            elif c in "qkv" and t < n_pairs:
                j = "qkv".index(c)
                (q, k, v)[j][t] = (project_short(t, j) if j and pre_ref is not None
                                   else times_w(h, t, j * pw, (j + 1) * pw))
        if t < n_pairs:
            attend_early_rows(t)
    for part in todo:
        out = project_out(*part, out)

    x_ref[s] = x_in[s].astype(F32) + out[n_mem:, :]
    return out[:n_mem, :], xn_next


def _pair_reduce(t, op):
    r = t[0:8]
    for i in range(8, t.shape[0], 8):
        r = op(r, t[i:i + 8])
    r = op(r, pltpu.roll(r, 4, 0))
    return op(r, pltpu.roll(r, 2, 0))


def _tile_rows(r, n):
    return jnp.concatenate([r] * (n // 8), axis=0)


def _feature_map(p):
    n = p.shape[0]
    e_pos = jnp.exp2(p - _tile_rows(_pair_reduce(p, jnp.maximum), n))
    e_neg = jnp.exp2(_tile_rows(_pair_reduce(p, jnp.minimum), n) - p)
    inv_pos = _recip(_pair_reduce(e_pos, jnp.add))
    inv_neg = _recip(_pair_reduce(e_neg, jnp.add))
    return jnp.concatenate(
        [e_pos * _tile_rows(inv_pos, n), e_neg * _tile_rows(inv_neg, n)], axis=0)


def _fold_span(b, blk):
    return b * blk // 128 * 128, -(-(b + 1) * blk // 128) * 128


def _expand_phi(wphi_ref, phi_ref):
    dh, _, heads = wphi_ref.shape
    d = dh * heads
    gr = 2 * dh
    c = _iota((dh, d), 1)
    c_feat = c - _div(c, dh) * dh
    spread = (_div(_iota((heads, d), 1), dh) == _iota((heads, d), 0)).astype(BF16)
    by_feat = jnp.zeros((dh, d), F32)
    for e in range(dh):
        t = jnp.dot(wphi_ref[e], spread, preferred_element_type=F32)
        by_feat = jnp.where(c_feat == e, t, by_feat)
    by_feat = by_feat.astype(BF16)
    blk = F_PAIRS * gr
    r = _iota((blk, dh), 0)
    sel = (((r - _div(r, gr) * gr) >> 1) == _iota((blk, dh), 1)).astype(BF16)
    for b in range(d // blk):
        lo, hi = _fold_span(b, blk)
        r = _iota((blk, hi - lo), 0)
        head = 2 * (_div(r, gr) + b * F_PAIRS) + (r & 1)
        phi = jnp.dot(sel, by_feat[:, lo:hi], preferred_element_type=F32)
        phi_ref[b, :, 0:hi - lo] = _pack(
            jnp.where(_div(_iota((1, hi - lo), 1) + lo, dh) == head, phi, 0.0))


def _b_weights(wqkv_ref, phi_ref, wob_ref, bq_ref, bkv_ref, bo_ref):
    d = wqkv_ref.shape[0]
    blk = 2 * phi_ref.shape[1]
    half = bkv_ref.shape[1]
    bo_ref[...] = _pack(wob_ref[...])
    wv = wqkv_ref[:, 2 * d:3 * d].T
    for b in range(d // half):
        bkv_ref[b, half // 2:half, :] = _pack(wv[b * half:(b + 1) * half])
    for b in range(d // blk):
        lo, hi = _fold_span(b, blk)
        phi = _unpack(phi_ref[b, :, 0:hi - lo])
        wq = lax.dot_general(phi, wqkv_ref[:, lo:hi], NT, preferred_element_type=F32)
        wk = lax.dot_general(phi, wqkv_ref[:, d + lo:d + hi], NT, preferred_element_type=F32)
        bq_ref[b * blk // 2:(b + 1) * blk // 2, :] = _pack(wq * LOG2E)
        at = b * blk % half // 2
        bkv_ref[b * blk // half, at:at + blk // 2, :] = _pack(wk * LOG2E)


def _chunk_rows(ref, it, r0, n):
    seg = ref.shape[1]
    return pl.ds(it * (TB // seg) + r0 // seg, n // seg)


def _b_keys(it, carry, *, x_ref, xb_ref, bkv_ref, kv_ref, z_ref):
    n_blk, half, _ = bkv_ref.shape
    gr = half // K_PAIRS
    xb = xb_ref[_chunk_rows(xb_ref, it, 0, TB)].reshape(TB, -1)
    last = x_ref.shape[0] - 1
    xb_ref[last] = _layernorm(x_ref[last]).astype(BF16)
    same_head = (_iota((gr, 2 * gr), 0) >= gr // 2) == ((_iota((gr, 2 * gr), 1) & 1) == 1)

    def accumulate(b, t):
        for i in range(K_PAIRS):
            g = b * K_PAIRS + i
            phi = _feature_map(t[i * gr:(i + 1) * gr])
            z_ref[g] = jnp.where(it > 0, z_ref[g], 0.0) + jnp.sum(phi, axis=1, keepdims=True)
            kv = lax.dot_general(t[half + i * gr:half + (i + 1) * gr], phi.astype(BF16), NT,
                                 preferred_element_type=F32)
            kv_ref[g] = jnp.where(it > 0, kv_ref[g], 0.0) + jnp.where(same_head, kv, 0.0)

    pending = None
    for b in range(n_blk):
        t = lax.dot_general(_unpack(bkv_ref[b]), xb, NT, preferred_element_type=F32)
        if pending is not None:
            accumulate(*pending)
        pending = (b, t)
    accumulate(*pending)
    return carry


def _b_queries(it, send, *, x_ref, xb_ref, y_ref, bq_ref, bo_ref, kv_ref, z_ref, ot_ref, on_ref):
    n_groups, gr, _ = kv_ref.shape
    blk = Q_PAIRS * gr
    sub = _iota((8, TB), 0)
    xb = xb_ref[_chunk_rows(xb_ref, it, 0, TB)].reshape(TB, -1)

    def attend(b, t):
        outs = []
        for i in range(Q_PAIRS):
            g = b * Q_PAIRS + i
            phi = _feature_map(t[i * gr:(i + 1) * gr])
            num = jnp.dot(kv_ref[g], phi.astype(BF16), preferred_element_type=F32)
            z = jnp.concatenate([z_ref[g]] * (TB // 128), axis=1)
            inv = _recip(_pair_reduce(phi * z, jnp.add) + 1e-6)
            other = pltpu.roll(inv, 1, 0)
            inv_a = jnp.where((sub & 1) == 0, inv, other)
            inv_b = jnp.where((sub & 1) == 0, other, inv)
            n = (gr - 8) // 16
            inv = jnp.concatenate(
                [inv_a] * n + [jnp.where(sub < 4, inv_a, inv_b)] + [inv_b] * n, axis=0)
            outs.append(num * inv)
        ot_ref[b * blk // 2:(b + 1) * blk // 2, :] = _pack(jnp.concatenate(outs, axis=0))

    n_blk = n_groups // Q_PAIRS
    proj = {}
    for b in range(n_blk + 1):
        if b < n_blk:
            proj[b] = lax.dot_general(_unpack(bq_ref[b * blk // 2:(b + 1) * blk // 2, :]), xb,
                                      NT, preferred_element_type=F32)
        if b > 0:
            attend(b - 1, proj[b - 1])
    on_ref[...] = _pack(_unpack(ot_ref[...]).T)
    r0 = 0
    for i, n in enumerate(O_ROWS):
        at = _chunk_rows(x_ref, it, r0, n)
        y = jnp.dot(_unpack(on_ref[r0 // 2:(r0 + n) // 2, :]), _unpack(bo_ref[...]),
                    preferred_element_type=F32)
        x = x_ref[at] + y.reshape((-1,) + x_ref.shape[1:])
        x_ref[at] = x
        y_ref[at] = x.astype(BF16)
        send(i)
        r0 += n


def _kernel(x_hbm, mem0_hbm, wq_hbm, wk_hbm, wv_hbm, wo_hbm, wqkvb_hbm, wphi_hbm, wob_hbm,
            out_hbm,
            x_ref, xb_ref, y_ref, xp_ref, stage_ref, pre_ref, w_ref, wo_ref, o_ref, near_ref,
            mem0_ref, wphi_ref, phi_ref, wqkvb_ref, wob_ref, bo_ref, bq_ref, bkv_ref,
            kv_ref, z_ref, ot_ref, on_ref,
            w_sem, in_sem, out_sem, *, dh):
    n_seg, seg, d = x_ref.shape
    n_pairs = w_ref.shape[0]
    pw = 2 * dh
    n_iter = n_seg * seg // TB

    def w_copies(p, j):
        src = (wq_hbm, wk_hbm, wv_hbm, wo_hbm)[j]
        if j < 2:
            return [pltpu.make_async_copy(src.at[p], stage_ref.at[p, 3 * j:3 * j + 3],
                                          w_sem.at[p, j])]
        return [pltpu.make_async_copy(src.at[p, i], stage_ref.at[p, 3 * j:3 * j + 3, i],
                                      w_sem.at[p, 2 * j - 2 + i]) for i in range(2)]

    def start_w(p, *slots):
        for j in slots:
            for copy in w_copies(p, j):
                copy.start()

    def wait_w(p, *slots):
        for j in slots:
            for copy in w_copies(p, j):
                copy.wait()

    def staged(p, tiles):
        return stage_ref[p, tiles].reshape(-1, d)

    def out_copy(it, i):
        part = _chunk_rows(y_ref, it, sum(O_ROWS[:i]), O_ROWS[i])
        return pltpu.make_async_copy(y_ref.at[part], out_hbm.at[part], out_sem.at[0])

    def x_copy(part, rows, sem):
        return pltpu.make_async_copy(x_hbm.at[part, rows, :], y_ref.at[part, rows, :], sem)

    head, tail = slice(0, seg - PRE), slice(seg - PRE, seg)
    xt_copy = x_copy(slice(None), tail, in_sem.at[0])
    wqkvb_copy = pltpu.make_async_copy(wqkvb_hbm, wqkvb_ref, in_sem.at[1])
    wphi_copy = pltpu.make_async_copy(wphi_hbm, wphi_ref, in_sem.at[5])
    mem0_copy = pltpu.make_async_copy(mem0_hbm, mem0_ref, in_sem.at[4])
    wob_copy = pltpu.make_async_copy(wob_hbm, wob_ref, in_sem.at[2])

    wphi_copy.start()
    xt_copy.start()
    start_w(0, 1, 2)
    wphi_copy.wait()
    _expand_phi(wphi_ref, phi_ref)
    xt_copy.wait()

    xp_ref[...] = _layernorm(y_ref[:, tail, :].astype(F32).reshape(n_seg * PRE, d)).astype(BF16)

    mem0_copy.start()
    start_w(1, 1, 2)
    start_w(0, 0)
    start_w(1, 0)

    def pre_project(p, carry):
        @pl.when(p + 2 < n_pairs)
        def _():
            start_w(jnp.minimum(p + 2, n_pairs - 1), 0, 1, 2)

        part = pl.ds(p * (n_seg // n_pairs), n_seg // n_pairs)
        x_copy(part, head, in_sem.at[3]).start()
        start_w(p, 3)
        p_q, p_o = jnp.maximum(p - 1, 0), jnp.maximum(p - WO_LAG, 0)

        @pl.when(p >= 1)
        def _():
            wait_w(p_q, 0)

        @pl.when(p >= WO_LAG)
        def _():
            wait_w(p_o, 3)

        wait_w(p, 1, 2)
        pre_ref[p] = lax.dot_general(xp_ref[...], staged(p, slice(3, 9)), NT,
                                     preferred_element_type=F32)
        w_ref[p_q, :, 0:pw] = _pack(staged(p_q, pl.ds(jnp.where(p >= 1, 0, 3), 3)).T)
        wo_ref[pl.ds(3 * p_o, 3)] = _pack(
            staged(p_o, pl.ds(jnp.where(p >= WO_LAG, 9, 3), 3))).reshape(3, 64, d)
        for j in (1, 2):
            w_ref[p, :, j * pw:(j + 1) * pw] = _pack(staged(p, slice(3 * j, 3 * j + 3)).T)
        return carry

    lax.fori_loop(0, n_pairs, pre_project, 0)

    wait_w(n_pairs - 1, 0)
    w_ref[n_pairs - 1, :, 0:pw] = _pack(staged(n_pairs - 1, slice(0, 3)).T)
    for p in range(n_pairs - WO_LAG, n_pairs):
        wait_w(p, 3)
        wo_ref[3 * p:3 * p + 3] = _pack(staged(p, slice(9, 12))).reshape(3, 64, d)
    x_copy(slice(None), head, in_sem.at[3]).wait()

    wqkvb_copy.start()
    wob_copy.start()
    mem0_copy.wait()
    x_ref[0] = y_ref[0].astype(F32)

    def layer_a(layer, x_in, pre):
        unroll = A_UNROLL
        step = functools.partial(_a_step, layer=layer, dh=dh, x_in=x_in, x_ref=x_ref, xb_ref=xb_ref,
                                 w_ref=w_ref, wo_ref=wo_ref, pre_ref=pre, o_ref=o_ref,
                                 near_ref=near_ref)

        def steps(it, carry):
            for i in range(unroll):
                carry = step(it * unroll + i, carry, i == 0, i == unroll - 1)
            return carry

        lax.fori_loop(0, n_seg // unroll, steps,
                      (mem0_ref[...].astype(F32), _layernorm(x_ref[0])))

    b_keys = functools.partial(_b_keys, x_ref=x_ref, xb_ref=xb_ref, bkv_ref=bkv_ref,
                               kv_ref=kv_ref, z_ref=z_ref)
    b_queries = functools.partial(_b_queries, x_ref=x_ref, xb_ref=xb_ref, y_ref=y_ref,
                                  bq_ref=bq_ref, bo_ref=bo_ref, kv_ref=kv_ref, z_ref=z_ref,
                                  ot_ref=ot_ref, on_ref=on_ref)

    def layer_pair(layer, carry):
        @pl.when(layer == 0)
        def _():
            layer_a(0, y_ref, pre_ref)

        @pl.when(layer == 0)
        def _():
            wqkvb_copy.wait()
            wob_copy.wait()
            _b_weights(wqkvb_ref, phi_ref, wob_ref, bq_ref, bkv_ref, bo_ref)

        @pl.when(layer == 1)
        def _():
            layer_a(1, x_ref, None)

        lax.fori_loop(0, n_iter, b_keys, 0)

        def queries(it, carry):
            def send(i):
                @pl.when(layer == 1)
                def _():
                    out_copy(it, i).start()

            b_queries(it, send)
            return carry

        lax.fori_loop(0, n_iter, queries, 0)

        return carry

    lax.fori_loop(0, 2, layer_pair, 0)
    pltpu.make_async_copy(y_ref, out_hbm, out_sem.at[0]).wait()


@functools.partial(jax.jit, static_argnames=("A_seg_len",))
def pallas_interleave_layers__memory_aug_recurrent_mem_tr__linear_kernel_hedgehog__prompt_kernel(
    A_x, A_mem0, A_Wq, A_Wk, A_Wv, A_Wo, A_seg_len, B_x, B_wqkv, B_w_phi, B_wo,
):
    del B_x
    batch, s_len, d = A_x.shape
    _, heads, dh = A_Wq.shape
    n_mem = A_mem0.shape[1]
    seg = int(A_seg_len)
    b_heads, b_dh, _ = B_w_phi.shape
    rows = n_mem + seg
    n_pairs = heads // 2
    gr = 2 * b_dh
    half = K_PAIRS * gr
    n_seg = s_len // seg
    assert batch == 1 and dh == 192 and heads == 2 * O_SPLITS[0][-1]
    assert n_mem % 8 == 0 and seg % 16 == 0 and 128 % seg == 0 and 2 * rows <= 128
    assert s_len % TB == 0 and s_len > TB == sum(O_ROWS) and n_seg % n_pairs == 0
    assert b_heads * b_dh == d and b_dh % 8 == 4 and d % half == 0

    def head_major(w):
        return w.transpose(1, 2, 0)

    hbm = pl.BlockSpec(memory_space=pltpu.HBM)
    out = pl.pallas_call(
        functools.partial(_kernel, dh=dh),
        out_shape=jax.ShapeDtypeStruct((n_seg, seg, d), A_x.dtype),
        in_specs=[hbm] * 9,
        out_specs=hbm,
        scratch_shapes=[
            pltpu.VMEM((n_seg, seg, d), F32),
            pltpu.VMEM((n_seg, seg, d), BF16),
            pltpu.VMEM((n_seg, seg, d), BF16),
            pltpu.VMEM((n_seg * PRE, d), BF16),
            pltpu.VMEM((n_pairs, 12, 2, 64, d), BF16),
            pltpu.VMEM((n_pairs, n_seg * PRE, 4 * dh), F32),
            pltpu.VMEM((n_pairs, d // 2, 6 * dh), jnp.uint32),
            pltpu.VMEM((3 * n_pairs, 64, d), jnp.uint32),
            pltpu.VMEM((rows, heads * dh), F32),
            pltpu.VMEM((n_pairs, n_mem + 16, 4 * dh), F32),
            pltpu.VMEM((n_mem, d), BF16),
            pltpu.VMEM((b_dh, b_dh, b_heads), BF16),
            pltpu.VMEM((d // (F_PAIRS * gr), F_PAIRS * gr // 2, 256), jnp.uint32),
            pltpu.VMEM(B_wqkv.shape, BF16),
            pltpu.VMEM(B_wo.shape, BF16),
            pltpu.VMEM((d // 2, d), jnp.uint32),
            pltpu.VMEM((d // 2, d), jnp.uint32),
            pltpu.VMEM((d // half, half, d), jnp.uint32),
            pltpu.VMEM((b_heads // 2, gr, 2 * gr), F32),
            pltpu.VMEM((b_heads // 2, 2 * gr, 128), F32),
            pltpu.VMEM((d // 2, TB), jnp.uint32),
            pltpu.VMEM((TB // 2, d), jnp.uint32),
            pltpu.SemaphoreType.DMA((n_pairs, 6)),
            pltpu.SemaphoreType.DMA((6,)),
            pltpu.SemaphoreType.DMA((1,)),
        ],
        compiler_params=pltpu.CompilerParams(vmem_limit_bytes=120 * 1024 * 1024),
    )(
        A_x.reshape(n_seg, seg, d), A_mem0.reshape(n_mem, d),
        head_major(A_Wq).reshape(n_pairs, 3, 2, 64, d),
        head_major(A_Wk).reshape(n_pairs, 3, 2, 64, d),
        head_major(A_Wv).reshape(n_pairs, 2, 3, 64, d), A_Wo.reshape(n_pairs, 2, 3, 64, d),
        B_wqkv, B_w_phi.transpose(1, 2, 0), B_wo,
    )
    return out.reshape(batch, s_len, d)
```

```python
import functools
import math

import jax
import jax.numpy as jnp
from jax import lax
import jax.experimental.pallas as pl
import jax.experimental.pallas.tpu as pltpu

F32 = jnp.float32
BF16 = jnp.bfloat16
NT = (((1,), (1,)), ((), ()))
LOG2E = math.log2(math.e)
MASKED = -1e9

ISSUE = ("qkSVv", "aSV")
LAG_S = (2, 1)
LAG_PV = (2, 3)
O_SPLITS = ((0, 1, 2, 3, 4, 6, 8), (0, 1, 2, 3, 4, 6, 8))
VPU_ROWS = ((range(16), ()), (range(16), ()))
VPU_DUE = (2, 3)
KEYS_AHEAD = (10, 11)
NORM_DUE = ((0, 1), (1, 3))
HALF = 256
PACE = 256
RING = 8
PRE = 8
WO_LAG = 3
TB = 512
K_PAIRS = 8
Q_PAIRS = 8
F_PAIRS = 2
O_ROWS = (128, 128, 128, 128)


def _iota(shape, axis):
    return lax.broadcasted_iota(jnp.int32, shape, axis)


def _div(v, d):
    return (v * ((1 << 18) // d + 1)) >> 18


def _pack(x):
    return pltpu.bitcast(x.astype(BF16), jnp.uint32)


def _unpack(x):
    return pltpu.bitcast(x, BF16)


def _recip(x):
    r = pl.reciprocal(x, approx=True)
    return r * (2.0 - x * r)


def _layernorm(x):
    m = jnp.mean(x, axis=-1, keepdims=True)
    c = x - m
    v = jnp.mean(c * c, axis=-1, keepdims=True)
    return c * lax.rsqrt(v + 1e-5)


def _rows(*parts):
    return jnp.concatenate(parts, axis=0)


def _cols(*parts):
    return jnp.concatenate(parts, axis=1)


def _strassen_weights(b11, b12, b21, b22):
    f11, f12, f21, f22 = (b.astype(F32) for b in (b11, b12, b21, b22))
    return [r.astype(BF16)
            for r in (f11 + f22, b11, f12 - f22, f21 - f11, b22, f11 + f12, f21 + f22)]


def _left_product(a1, a2, times):
    return times(a2, 3) + times(a1 + a2, 1)


def _right_product(a1, a2, times):
    return times(a1 + a2, 4) + times(a1, 2)


def _token_operands(a1, a2, b1, b2):
    low = b1 + b2
    n = low.shape[0] // 2
    return ({1: low[:n], 3: b2, 2: a1, 4: a1 + a2},
            {1: low[n:], 0: a1 + b2, 6: a2 - b2, 5: b1 - a1})


def _memory_operands(m1, m2):
    both = m1 + m2
    return {0: m2, 1: both, 2: m1, 3: m2, 4: both, 5: m1, 6: m2}


def _first_results(p, n):
    m1 = _rows(p[1][n:], jnp.zeros_like(p[1][n:]))
    return ((p[1][:n] + p[3][:n], p[2][:n] + p[4][:n]),
            (p[2][n:] + p[4][n:], p[3][n:] - p[4][n:], p[3][n:] + m1, p[2][n:] - m1))


def _second_left(p, n, c11, c21):
    m1 = _rows(jnp.zeros_like(p[1][n:]), p[1][n:])
    return p[1][:n] + p[6][:n] - p[0][:n], c11 + p[0][n:] + p[6][n:], c21 + m1


def _second_right(p, n, c22):
    m1 = _rows(jnp.zeros_like(p[1][n:]), p[1][n:])
    return p[5][:n] + p[0][:n] - p[1][:n], c22 + p[0][n:] + p[5][n:] - m1


def _a_step(s, mem, xn, shared, *, layer, dh, x_in, x_ref, xb_ref, ws_ref, wp_ref, wos_ref,
            wop_ref, pre_ref, ahead_ref, o_refs, near_ref):
    odd = bool(shared)
    n_mem, seg = mem.shape[0], xn[0].shape[0]
    n_seg = xb_ref.shape[0]
    rows = n_mem + seg
    pw = 2 * dh
    n_pairs = wp_ref.shape[0]
    o_ref = o_refs[odd]
    scale = dh ** -0.5

    def after(early, value):
        return value if early is None else jnp.where(s < 0, early[:, :value.shape[1]], value)

    def after_all(early, value):
        t = functools.reduce(jnp.maximum, [early[i:i + 8, j:j + 128]
                                           for i in range(0, early.shape[0], 8)
                                           for j in range(0, early.shape[1], 128)])
        return jnp.concatenate([after(t, value[0:8]), value[8:]], axis=0)

    def slow_norm(x):
        outs = [None, None]
        for i in range(0, seg, 8):
            outs.append(_layernorm(after(outs[-2], x[i:i + 8])))
        return jnp.concatenate(outs[2:], axis=0)

    xn_next = slow_norm(x_in[jnp.minimum(s + len(xn), n_seg - 1)].astype(F32))
    done = jnp.maximum(s - 3, 0)
    xb_done = slow_norm(x_ref[done])
    xb_ref[done] = xb_done.astype(BF16)

    h = _rows(mem, xn[0])

    first = _iota((rows, 128), 1) < 64
    zero = jnp.zeros((rows, 128), F32)

    def key_blocks(t):
        t0, t1, t2 = t[:, 0:128], t[:, 128:256], t[:, 256:384]
        top = jnp.concatenate([t0, jnp.where(first, t1, 0.0), zero], axis=1)
        bot = jnp.concatenate([zero, jnp.where(first, 0.0, t1), t2], axis=1)
        return jnp.concatenate([top, bot], axis=0).astype(BF16)

    def value_blocks(t):
        mine = jnp.concatenate([first] * 3, axis=1)
        return jnp.concatenate(
            [jnp.where(mine, t, 0.0), jnp.where(mine, 0.0, t)], axis=0).astype(BF16)

    def vpu_rows(p):
        return [n_mem + 8 * i for i, pairs in enumerate(VPU_ROWS[layer]) if p in pairs]

    def mxu_rows(p):
        return [r for r in range(0, rows, 8) if r not in vpu_rows(p)]

    def pick(t, starts):
        return jnp.concatenate([t[r:r + 8] for r in starts], axis=0)

    q, k, v, probs, near_done = {}, {}, {}, {}, {}

    def project(p, lo, hi, n):
        def dot(a, w):
            return jnp.dot(a if n % 16 else a.astype(BF16), _unpack(w),
                           preferred_element_type=F32)

        most = (_left_product, _right_product)[p % 2](
            h[:n, :HALF], h[:n, HALF:2 * HALF], lambda a, i: dot(a, ws_ref[p // 2, i, :, lo:hi]))
        return dot(h[:n, 2 * HALF:], wp_ref[p, :, lo:hi]) + most

    def project_short(p, j):
        return _rows(project(p, j * pw, (j + 1) * pw, rows - PRE),
                     pre_ref[p, pl.ds(pl.multiple_of(s * PRE, PRE), PRE), (j - 1) * pw:j * pw])

    if pre_ref is None:
        if not odd:
            shared["in"] = _token_operands(*(t[:, c:c + HALF] for t in xn[1:3] for c in (0, HALF)))
        m_in = _memory_operands(mem[:, :HALF], mem[:, HALF:2 * HALF])
        lhs_in = {i: _rows(m_in[i], t) for i, t in shared["in"][odd].items()}
    products = {}

    def project_shared(p):
        g, right = divmod(p, 2)
        for i in (((1, 3), (2, 4)), ((1, 0, 6), (5,)))[odd][right]:
            products[i] = jnp.dot(lhs_in[i], _unpack(ws_ref[g, i]), preferred_element_type=F32)
        if not odd:
            tokens = ahead_ref[p]
            if right:
                (_, m), shared[g] = _first_results(products, n_mem)
            else:
                m = products[1][:n_mem] + products[3][:n_mem]
        elif right:
            tokens = shared[g][0]
            m, ahead_ref[p] = _second_right(products, n_mem, shared[g][3])
        else:
            m, tokens, ahead_ref[p] = _second_left(products, n_mem, *shared[g][1:3])
        return jnp.dot(h[:, 2 * HALF:], _unpack(wp_ref[p]),
                       preferred_element_type=F32) + _rows(m, tokens)

    def scores(p):
        col = pick(_iota((rows, 2 * rows), 1), mxu_rows(p))
        row = pick(_iota((rows, 2 * rows), 0), mxu_rows(p))
        is_a = col < rows
        visible = (row < n_mem) | (row >= jnp.where(is_a, col, col - rows))
        sc = lax.dot_general(pick(q[p], mxu_rows(p)), key_blocks(k[p]), NT,
                             preferred_element_type=F32)
        sc = jnp.where(visible, sc * scale, MASKED)
        max_a = jnp.max(jnp.where(is_a, sc, -jnp.inf), axis=1, keepdims=True)
        max_b = jnp.max(jnp.where(is_a, -jnp.inf, sc), axis=1, keepdims=True)
        e = jnp.exp(sc - jnp.where(is_a, max_a, max_b))
        sum_a = jnp.sum(jnp.where(is_a, e, 0.0), axis=1, keepdims=True)
        sum_b = jnp.sum(jnp.where(is_a, 0.0, e), axis=1, keepdims=True)
        probs[p] = e * _recip(jnp.where(is_a, sum_a, sum_b))
        if p == NORM_DUE[layer][0]:
            probs[p] = after_all(xn_next, probs[p])
        if p == NORM_DUE[layer][1]:
            probs[p] = after_all(xb_done, probs[p])
        if p - VPU_DUE[layer] in near_done:
            probs[p] = after_all(near_done[p - VPU_DUE[layer]], probs[p])

    def values(p):
        o = jnp.dot(probs[p], value_blocks(v[p]), preferred_element_type=F32)
        for i, r in enumerate(mxu_rows(p)):
            o_ref[r:r + 8, p * pw:(p + 1) * pw] = o[8 * i:8 * i + 8]

    chain = [None, None]
    scored = [None] * KEYS_AHEAD[layer]

    def attend_on_vpu(p, r):
        def key_row(j, i):
            return jnp.broadcast_to(near_ref[p, j:j + 1, 128 * i:128 * (i + 1)], (8, 128))

        half, sub = first[0:8], _iota((8, 128), 0)
        t = q[p][r:r + 8] * (scale * LOG2E)
        q0, q2 = t[:, 0:128], t[:, 256:384]
        q1a, q1b = jnp.where(half, t[:, 128:256], 0.0), jnp.where(half, 0.0, t[:, 128:256])
        for j in range(r + 8):
            ready = after(scored[-KEYS_AHEAD[layer]], chain[0])
            k1 = after(ready, key_row(j, 1))
            dot_a = q0 * after(ready, key_row(j, 0)) + q1a * k1
            dot_b = q2 * after(dot_a, key_row(j, 2)) + q1b * k1
            t = jnp.where(half, jnp.sum(dot_a, axis=1, keepdims=True),
                          jnp.sum(dot_b, axis=1, keepdims=True))
            scored.append(t if j <= r else jnp.where(sub >= j - r, t, MASKED * LOG2E))
            chain[0] = dot_b
        sc = scored[-(r + 8):]
        top = functools.reduce(jnp.maximum, sc)
        for j in range(r + 8):
            e = jnp.exp2(sc[j] - after(chain[1], top))
            weight = after(chain[1], e)
            terms = [weight * key_row(j, 3 + i) for i in range(3)]
            total = e if j == 0 else total + e
            acc = terms if j == 0 else [a + b for a, b in zip(acc, terms)]
            chain[1] = acc[2]
        inv = _recip(total)
        o_ref[r:r + 8, p * pw:(p + 1) * pw] = jnp.concatenate([a * inv for a in acc], axis=1)
        near_done[p] = acc[2]

    def attend_early_rows(p):
        if vpu_rows(p):
            n = vpu_rows(p)[-1] + 8
            near_ref[p, 0:n, 0:pw] = k[p][0:n]
            near_ref[p, 0:n, pw:2 * pw] = v[p][0:n]
        for r in reversed(vpu_rows(p)):
            attend_on_vpu(p, r)

    out = {}

    def project_out(g0, g1):
        def halves(ref, lo, hi):
            return [_cols(*(ref[lo:hi, (2 * g + i) * pw:(2 * g + i + 1) * pw]
                            for g in range(g0, g1))) for i in range(2)]

        if not odd:
            shared["out", g0] = _token_operands(*halves(o_refs[0], n_mem, rows),
                                                *halves(o_refs[1], n_mem, rows))
        m = _memory_operands(*halves(o_ref, 0, n_mem))
        for i, t in shared["out", g0][odd].items():
            r = jnp.dot(_rows(m[i], t), _unpack(wos_ref[g0:g1, i].reshape(-1, HALF)),
                        preferred_element_type=F32)
            out[i] = r + out[i] if i in out else r

    lag_s, lag_v = LAG_S[layer], LAG_S[layer] + LAG_PV[layer]
    todo = list(zip(O_SPLITS[layer][:-1], O_SPLITS[layer][1:]))
    for t in range(n_pairs + lag_v):
        if t >= n_pairs:
            project_out(*todo.pop(0))
        for c in ISSUE[layer]:
            if c == "S" and 0 <= t - lag_s < n_pairs:
                scores(t - lag_s)
            elif c == "V" and 0 <= t - lag_v < n_pairs:
                values(t - lag_v)
            elif c == "a" and t < n_pairs:
                r = project_shared(t)
                q[t], k[t], v[t] = r[:, 0:pw], r[:, pw:2 * pw], r[:, 2 * pw:3 * pw]
            elif c in "qkv" and t < n_pairs:
                j = "qkv".index(c)
                (q, k, v)[j][t] = project_short(t, j) if j else project(t, 0, pw, rows)
        if t < n_pairs:
            attend_early_rows(t)
    for part in todo:
        project_out(*part)
    rest = jnp.dot(o_ref[...], _unpack(wop_ref[...].reshape(-1, wop_ref.shape[-1])),
                   preferred_element_type=F32)

    most, tail = slice(0, 2 * HALF), slice(2 * HALF, None)
    x_ref[s, :, tail] = x_in[s, :, tail].astype(F32) + rest[n_mem:]
    if odd:
        c12, c11, c21, c22 = shared["out"]
        m1, c11, c21 = _second_left(out, n_mem, c11, c21)
        m2, c22 = _second_right(out, n_mem, c22)
        x_ref[s - 1, :, most] = x_in[s - 1, :, most].astype(F32) + _cols(c11, c12)
        back = jnp.maximum(s - 2, 1)
        x_ref[back, :, most] = (x_in[back, :, most].astype(F32)
                                + jnp.where(s > 1, _cols(c21, c22), 0.0))
    else:
        (m1, m2), shared["out"] = _first_results(out, n_mem)
    return _cols(m1, m2, rest[:n_mem]), xn_next


def _pair_reduce(t, op):
    r = t[0:8]
    for i in range(8, t.shape[0], 8):
        r = op(r, t[i:i + 8])
    r = op(r, pltpu.roll(r, 4, 0))
    return op(r, pltpu.roll(r, 2, 0))


def _tile_rows(r, n):
    return jnp.concatenate([r] * (n // 8), axis=0)


def _feature_map(p):
    n = p.shape[0]
    e_pos = jnp.exp2(p - _tile_rows(_pair_reduce(p, jnp.maximum), n))
    e_neg = jnp.exp2(_tile_rows(_pair_reduce(p, jnp.minimum), n) - p)
    inv_pos = _recip(_pair_reduce(e_pos, jnp.add))
    inv_neg = _recip(_pair_reduce(e_neg, jnp.add))
    return jnp.concatenate(
        [e_pos * _tile_rows(inv_pos, n), e_neg * _tile_rows(inv_neg, n)], axis=0)


def _fold_span(b, blk):
    return b * blk // 128 * 128, -(-(b + 1) * blk // 128) * 128


def _expand_phi(wphi_ref, phi_ref):
    dh, _, heads = wphi_ref.shape
    d = dh * heads
    gr = 2 * dh
    c = _iota((dh, d), 1)
    c_feat = c - _div(c, dh) * dh
    spread = (_div(_iota((heads, d), 1), dh) == _iota((heads, d), 0)).astype(BF16)

    def gather(j, by_feat):
        for e in (j * (dh // 4) + i for i in range(dh // 4)):
            t = jnp.dot(wphi_ref[e], spread, preferred_element_type=F32)
            by_feat = jnp.where(c_feat == e, t, by_feat)
        return by_feat

    by_feat = lax.fori_loop(0, 4, gather, jnp.zeros((dh, d), F32)).astype(BF16)
    blk = F_PAIRS * gr
    r = _iota((blk, dh), 0)
    sel = (((r - _div(r, gr) * gr) >> 1) == _iota((blk, dh), 1)).astype(BF16)
    for b in range(d // blk):
        lo, hi = _fold_span(b, blk)
        r = _iota((blk, hi - lo), 0)
        head = 2 * (_div(r, gr) + b * F_PAIRS) + (r & 1)
        phi = jnp.dot(sel, by_feat[:, lo:hi], preferred_element_type=F32)
        phi_ref[b, :, 0:hi - lo] = _pack(
            jnp.where(_div(_iota((1, hi - lo), 1) + lo, dh) == head, phi, 0.0))


def _b_weights(wqkv_ref, phi_ref, wob_ref, bq_ref, bkv_ref, bo_ref):
    d = wqkv_ref.shape[0]
    blk = 2 * phi_ref.shape[1]
    half = bkv_ref.shape[1]
    bo_ref[...] = _pack(wob_ref[...])
    wv = wqkv_ref[:, 2 * d:3 * d].T
    for b in range(d // half):
        bkv_ref[b, half // 2:half, :] = _pack(wv[b * half:(b + 1) * half])
    for b in range(d // blk):
        lo, hi = _fold_span(b, blk)
        phi = _unpack(phi_ref[b, :, 0:hi - lo])
        wq = lax.dot_general(phi, wqkv_ref[:, lo:hi], NT, preferred_element_type=F32)
        wk = lax.dot_general(phi, wqkv_ref[:, d + lo:d + hi], NT, preferred_element_type=F32)
        bq_ref[b * blk // 2:(b + 1) * blk // 2, :] = _pack(wq * LOG2E)
        at = b * blk % half // 2
        bkv_ref[b * blk // half, at:at + blk // 2, :] = _pack(wk * LOG2E)


def _chunk_rows(ref, it, r0, n):
    seg = ref.shape[1]
    return pl.ds(it * (TB // seg) + r0 // seg, n // seg)


def _b_keys(it, carry, *, x_ref, xb_ref, bkv_ref, kv_ref, z_ref):
    n_blk, half, _ = bkv_ref.shape
    gr = half // K_PAIRS
    xb = xb_ref[_chunk_rows(xb_ref, it, 0, TB)].reshape(TB, -1)
    last = x_ref.shape[0] - 1 - jnp.minimum(it, 2)
    xb_ref[last] = _layernorm(x_ref[last]).astype(BF16)
    same_head = (_iota((gr, 2 * gr), 0) >= gr // 2) == ((_iota((gr, 2 * gr), 1) & 1) == 1)

    def accumulate(b, t):
        for i in range(K_PAIRS):
            g = b * K_PAIRS + i
            phi = _feature_map(t[i * gr:(i + 1) * gr])
            z_ref[g] = jnp.where(it > 0, z_ref[g], 0.0) + jnp.sum(phi, axis=1, keepdims=True)
            kv = lax.dot_general(t[half + i * gr:half + (i + 1) * gr], phi.astype(BF16), NT,
                                 preferred_element_type=F32)
            kv_ref[g] = jnp.where(it > 0, kv_ref[g], 0.0) + jnp.where(same_head, kv, 0.0)

    pending = None
    for b in range(n_blk):
        t = lax.dot_general(_unpack(bkv_ref[b]), xb, NT, preferred_element_type=F32)
        if pending is not None:
            accumulate(*pending)
        pending = (b, t)
    accumulate(*pending)
    return carry


def _b_queries(it, send, *, x_ref, xb_ref, y_ref, bq_ref, bo_ref, kv_ref, z_ref, ot_ref, on_ref):
    n_groups, gr, _ = kv_ref.shape
    blk = Q_PAIRS * gr
    sub = _iota((8, TB), 0)
    xb = xb_ref[_chunk_rows(xb_ref, it, 0, TB)].reshape(TB, -1)

    def attend(b, t):
        outs = []
        for i in range(Q_PAIRS):
            g = b * Q_PAIRS + i
            phi = _feature_map(t[i * gr:(i + 1) * gr])
            num = jnp.dot(kv_ref[g], phi.astype(BF16), preferred_element_type=F32)
            z = jnp.concatenate([z_ref[g]] * (TB // 128), axis=1)
            inv = _recip(_pair_reduce(phi * z, jnp.add) + 1e-6)
            other = pltpu.roll(inv, 1, 0)
            inv_a = jnp.where((sub & 1) == 0, inv, other)
            inv_b = jnp.where((sub & 1) == 0, other, inv)
            n = (gr - 8) // 16
            inv = jnp.concatenate(
                [inv_a] * n + [jnp.where(sub < 4, inv_a, inv_b)] + [inv_b] * n, axis=0)
            outs.append(num * inv)
        ot_ref[b * blk // 2:(b + 1) * blk // 2, :] = _pack(jnp.concatenate(outs, axis=0))

    n_blk = n_groups // Q_PAIRS
    proj = {}
    for b in range(n_blk + 1):
        if b < n_blk:
            proj[b] = lax.dot_general(_unpack(bq_ref[b * blk // 2:(b + 1) * blk // 2, :]), xb,
                                      NT, preferred_element_type=F32)
        if b > 0:
            attend(b - 1, proj[b - 1])
    on_ref[...] = _pack(_unpack(ot_ref[...]).T)
    r0 = 0
    for i, n in enumerate(O_ROWS):
        at = _chunk_rows(x_ref, it, r0, n)
        y = jnp.dot(_unpack(on_ref[r0 // 2:(r0 + n) // 2, :]), _unpack(bo_ref[...]),
                    preferred_element_type=F32)
        x = x_ref[at] + y.reshape((-1,) + x_ref.shape[1:])
        x_ref[at] = x
        y_ref[at] = x.astype(BF16)
        send(i)
        r0 += n


def _kernel(x_hbm, mem0_hbm, wq_hbm, wk_hbm, wv_hbm, wo_hbm, wqkvb_hbm, wphi_hbm, wob_hbm,
            out_hbm,
            x_ref, xb_ref, y_ref, xp_ref, stage_ref, pre_ref, ahead_ref,
            ws_ref, wp_ref, wos_ref, wop_ref, o_even_ref, o_odd_ref, near_ref,
            mem0_ref, wphi_ref, phi_ref, wqkvb_ref, wob_ref, bo_ref, bq_ref, bkv_ref,
            kv_ref, z_ref, ot_ref, on_ref,
            w_sem, in_sem, out_sem, *, dh):
    n_seg, seg, d = x_ref.shape
    n_pairs = wp_ref.shape[0]
    n_mem = mem0_ref.shape[0]
    pw = 2 * dh
    n_iter = n_seg * seg // TB

    def w_copies(p, j):
        src = (wq_hbm, wk_hbm, wv_hbm, wo_hbm)[j]
        if j < 2:
            return [pltpu.make_async_copy(src.at[p], stage_ref.at[p % RING, 3 * j:3 * j + 3],
                                          w_sem.at[p, j])]
        return [pltpu.make_async_copy(src.at[p, i], stage_ref.at[p % RING, 3 * j:3 * j + 3, i],
                                      w_sem.at[p, 2 * j - 2 + i]) for i in range(2)]

    def start_w(p, *slots):
        for j in slots:
            for copy in w_copies(p, j):
                copy.start()

    def wait_w(p, *slots):
        for j in slots:
            for copy in w_copies(p, j):
                copy.wait()

    def prepare_in(u, tiles, live=True, pace=lambda t, b: b):
        g, i = u // 2, u % 2
        for t in tiles:
            cols = pl.ds(pl.multiple_of(128 * t, 128), 128)
            blocks = [stage_ref[p % RING, t, :, :, pl.ds(pl.multiple_of(c + i * 128, 128), 128)]
                      .reshape(128, 128)
                      for c in (0, HALF) for p in (2 * g, jnp.where(live, 2 * g + 1, 0))]
            for n, r in enumerate(_strassen_weights(*(pace(t, b) for b in blocks))):
                ws_ref[g, n, pl.ds(pl.multiple_of(i * 64, 64), 64), cols] = _pack(r.T)
            wp_ref[u, :, cols] = _pack(stage_ref[u % RING, t, :, :, 2 * HALF:].reshape(128, -1).T)

    def wait_out(u):
        for i in range(2):
            pltpu.make_async_copy(stage_ref.at[0, 9:12, 0], stage_ref.at[0, 9:12, 0],
                                  w_sem.at[u // 2 * 2 + i, 4 + u % 2]).wait()

    def prepare_out(u, live=True, pace=lambda t, b: b):
        g, i = u // 2, u % 2
        for t in range(3):
            parts = [pace(3 * t + 1, stage_ref[p % RING, jnp.where(live, 9, 3) + t, i])
                     for p in (2 * g, jnp.where(live, 2 * g + 1, 0))]
            blocks = [part[:, c:c + HALF] for part in parts for c in (0, HALF)]
            for n, r in enumerate(_strassen_weights(*blocks)):
                wos_ref[g, n, t, i] = _pack(r)
            for n, part in enumerate(parts):
                wop_ref[2 * g + n, t, i] = _pack(part[:, 2 * HALF:])

    def out_copy(it, i):
        part = _chunk_rows(y_ref, it, sum(O_ROWS[:i]), O_ROWS[i])
        return pltpu.make_async_copy(y_ref.at[part], out_hbm.at[part], out_sem.at[0])

    def x_copy(part, rows, sem):
        return pltpu.make_async_copy(x_hbm.at[part, rows, :], y_ref.at[part, rows, :], sem)

    head, tail = slice(0, seg - PRE), slice(seg - PRE, seg)
    xt_copy = x_copy(slice(None), tail, in_sem.at[0])
    wqkvb_copy = pltpu.make_async_copy(wqkvb_hbm, wqkvb_ref, in_sem.at[1])
    wphi_copy = pltpu.make_async_copy(wphi_hbm, wphi_ref, in_sem.at[5])
    mem0_copy = pltpu.make_async_copy(mem0_hbm, mem0_ref, in_sem.at[4])
    wob_copy = pltpu.make_async_copy(wob_hbm, wob_ref, in_sem.at[2])

    wphi_copy.start()
    xt_copy.start()
    start_w(0, 0, 1, 2)
    wphi_copy.wait()
    _expand_phi(wphi_ref, phi_ref)
    xt_copy.wait()

    xp_ref[...] = _layernorm(y_ref[:, tail, :].astype(F32).reshape(n_seg * PRE, d)).astype(BF16)

    mem0_copy.start()
    start_w(1, 0, 1, 2)

    def pre_project(p, carry):
        @pl.when(p + 2 < n_pairs)
        def _():
            start_w(jnp.minimum(p + 2, n_pairs - 1), 0, 1, 2)

        part = pl.ds(p * (n_seg // n_pairs), n_seg // n_pairs)
        x_copy(part, head, in_sem.at[3]).start()
        start_w(p, 3)

        @pl.when(p >= WO_LAG)
        def _():
            wait_out(jnp.maximum(p - WO_LAG, 0))

        wait_w(p, 0, 1, 2)
        kv = lax.dot_general(xp_ref[...], stage_ref[p % RING, 3:9].reshape(-1, d), NT,
                             preferred_element_type=F32)
        pre_ref[p] = kv

        def pace(t, block):
            c, r = divmod(t * PACE, xp_ref.shape[0])
            early = kv[r:r + block.shape[0], 128 * c:128 * (c + 1)].astype(BF16)
            return jnp.where(p < 0, _cols(*[early] * (block.shape[1] // 128)), block)

        prepare_in(jnp.maximum(p - 1, 0), range(9), p >= 1, pace)
        prepare_out(jnp.maximum(p - WO_LAG, 0), p >= WO_LAG, pace)
        return carry

    lax.fori_loop(0, n_pairs, pre_project, 0)

    @pl.loop(0, 3)
    def _(j):
        prepare_in(n_pairs - 1, [3 * j + i for i in range(3)])

    @pl.loop(n_pairs - WO_LAG, n_pairs)
    def _(u):
        wait_out(u)
        prepare_out(u)

    x_copy(slice(None), head, in_sem.at[3]).wait()

    wqkvb_copy.start()
    wob_copy.start()
    mem0_copy.wait()
    x_ref[0] = y_ref[0].astype(F32)

    def layer_a(layer, x_in, pre):
        step = functools.partial(
            _a_step, layer=layer, dh=dh, x_in=x_in, x_ref=x_ref, xb_ref=xb_ref, ws_ref=ws_ref,
            wp_ref=wp_ref, wos_ref=wos_ref, wop_ref=wop_ref, pre_ref=pre, ahead_ref=ahead_ref,
            o_refs=(o_even_ref, o_odd_ref), near_ref=near_ref)
        xn = [_layernorm(x_in[i].astype(F32)) for i in range(1 if pre is not None else 3)]
        o_odd_ref[...] = jnp.zeros(o_odd_ref.shape, F32)
        if pre is None:
            @pl.loop(0, n_pairs // 2)
            def _(g):
                for i, product in enumerate((_left_product, _right_product)):
                    ahead_ref[2 * g + i] = product(
                        xn[0][:, :HALF], xn[0][:, HALF:2 * HALF],
                        lambda a, n: jnp.dot(a.astype(BF16), _unpack(ws_ref[g, n]),
                                             preferred_element_type=F32))

        def two_steps(it, carry):
            mem, *xn = carry
            shared = {}
            for i in range(2):
                mem, xn_next = step(2 * it + i, mem, xn, shared)
                xn = xn[1:] + [xn_next]
            return (mem, *xn)

        lax.fori_loop(0, n_seg // 2, two_steps, (mem0_ref[...].astype(F32), *xn))

    def finish_a(layer):
        a = [_cols(*(o_odd_ref[n_mem:, (2 * g + i) * pw:(2 * g + i + 1) * pw]
                     for g in range(n_pairs // 2))) for i in range(2)]
        y = _cols(*(product(*a, lambda t, n: jnp.dot(
            t.astype(BF16), _unpack(wos_ref[:, n].reshape(-1, HALF)), preferred_element_type=F32))
            for product in (_left_product, _right_product)))
        at = (n_seg - 1, slice(None), slice(0, 2 * HALF))
        x_ref[at] = jnp.where(layer == 0, y_ref[at].astype(F32), x_ref[at]) + y

    b_keys = functools.partial(_b_keys, x_ref=x_ref, xb_ref=xb_ref, bkv_ref=bkv_ref,
                               kv_ref=kv_ref, z_ref=z_ref)
    b_queries = functools.partial(_b_queries, x_ref=x_ref, xb_ref=xb_ref, y_ref=y_ref,
                                  bq_ref=bq_ref, bo_ref=bo_ref, kv_ref=kv_ref, z_ref=z_ref,
                                  ot_ref=ot_ref, on_ref=on_ref)

    def layer_pair(layer, carry):
        @pl.when(layer == 0)
        def _():
            layer_a(0, y_ref, pre_ref)

        @pl.when(layer == 0)
        def _():
            wqkvb_copy.wait()
            wob_copy.wait()
            _b_weights(wqkvb_ref, phi_ref, wob_ref, bq_ref, bkv_ref, bo_ref)

        @pl.when(layer == 1)
        def _():
            layer_a(1, x_ref, None)

        finish_a(layer)

        lax.fori_loop(0, n_iter, b_keys, 0)

        def queries(it, carry):
            def send(i):
                @pl.when(layer == 1)
                def _():
                    out_copy(it, i).start()

            b_queries(it, send)
            return carry

        lax.fori_loop(0, n_iter, queries, 0)

        return carry

    lax.fori_loop(0, 2, layer_pair, 0)
    pltpu.make_async_copy(y_ref, out_hbm, out_sem.at[0]).wait()


@functools.partial(jax.jit, static_argnames=("A_seg_len",))
def pallas_interleave_layers__memory_aug_recurrent_mem_tr__linear_kernel_hedgehog__prompt_kernel(
    A_x, A_mem0, A_Wq, A_Wk, A_Wv, A_Wo, A_seg_len, B_x, B_wqkv, B_w_phi, B_wo,
):
    del B_x
    batch, s_len, d = A_x.shape
    _, heads, dh = A_Wq.shape
    n_mem = A_mem0.shape[1]
    seg = int(A_seg_len)
    b_heads, b_dh, _ = B_w_phi.shape
    rows = n_mem + seg
    n_pairs = heads // 2
    gr = 2 * b_dh
    half = K_PAIRS * gr
    n_seg = s_len // seg
    assert batch == 1 and dh == 192 and heads == 4 * O_SPLITS[0][-1] and d == 2 * HALF + 128
    assert n_mem % 8 == 0 and seg % 16 == 0 and 128 % seg == 0 and 2 * rows <= 128
    assert s_len % TB == 0 and s_len > 3 * TB == 3 * sum(O_ROWS) and n_seg % n_pairs == 0
    assert b_heads * b_dh == d and b_dh % 8 == 4 and d % half == 0

    def head_major(w):
        return w.transpose(1, 2, 0)

    hbm = pl.BlockSpec(memory_space=pltpu.HBM)
    out = pl.pallas_call(
        functools.partial(_kernel, dh=dh),
        out_shape=jax.ShapeDtypeStruct((n_seg, seg, d), A_x.dtype),
        in_specs=[hbm] * 9,
        out_specs=hbm,
        scratch_shapes=[
            pltpu.VMEM((n_seg, seg, d), F32),
            pltpu.VMEM((n_seg, seg, d), BF16),
            pltpu.VMEM((n_seg, seg, d), BF16),
            pltpu.VMEM((n_seg * PRE, d), BF16),
            pltpu.VMEM((RING, 12, 2, 64, d), BF16),
            pltpu.VMEM((n_pairs, n_seg * PRE, 4 * dh), F32),
            pltpu.VMEM((n_pairs, seg, 6 * dh), F32),
            pltpu.VMEM((n_pairs // 2, 7, HALF // 2, 6 * dh), jnp.uint32),
            pltpu.VMEM((n_pairs, d // 2 - HALF, 6 * dh), jnp.uint32),
            pltpu.VMEM((n_pairs // 2, 7, 3, 2, 32, HALF), jnp.uint32),
            pltpu.VMEM((n_pairs, 3, 2, 32, d - 2 * HALF), jnp.uint32),
            pltpu.VMEM((rows, heads * dh), F32),
            pltpu.VMEM((rows, heads * dh), F32),
            pltpu.VMEM((n_pairs, n_mem + 16, 4 * dh), F32),
            pltpu.VMEM((n_mem, d), BF16),
            pltpu.VMEM((b_dh, b_dh, b_heads), BF16),
            pltpu.VMEM((d // (F_PAIRS * gr), F_PAIRS * gr // 2, 256), jnp.uint32),
            pltpu.VMEM(B_wqkv.shape, BF16),
            pltpu.VMEM(B_wo.shape, BF16),
            pltpu.VMEM((d // 2, d), jnp.uint32),
            pltpu.VMEM((d // 2, d), jnp.uint32),
            pltpu.VMEM((d // half, half, d), jnp.uint32),
            pltpu.VMEM((b_heads // 2, gr, 2 * gr), F32),
            pltpu.VMEM((b_heads // 2, 2 * gr, 128), F32),
            pltpu.VMEM((d // 2, TB), jnp.uint32),
            pltpu.VMEM((TB // 2, d), jnp.uint32),
            pltpu.SemaphoreType.DMA((n_pairs, 6)),
            pltpu.SemaphoreType.DMA((6,)),
            pltpu.SemaphoreType.DMA((1,)),
        ],
        compiler_params=pltpu.CompilerParams(vmem_limit_bytes=124 * 1024 * 1024),
    )(
        A_x.reshape(n_seg, seg, d), A_mem0.reshape(n_mem, d),
        head_major(A_Wq).reshape(n_pairs, 3, 2, 64, d),
        head_major(A_Wk).reshape(n_pairs, 3, 2, 64, d),
        head_major(A_Wv).reshape(n_pairs, 2, 3, 64, d), A_Wo.reshape(n_pairs, 2, 3, 64, d),
        B_wqkv, B_w_phi.transpose(1, 2, 0), B_wo,
    )
    return out.reshape(batch, s_len, d)
```

```python
import functools
import math

import jax
import jax.numpy as jnp
from jax import lax
import jax.experimental.pallas as pl
import jax.experimental.pallas.tpu as pltpu

F32 = jnp.float32
BF16 = jnp.bfloat16
NT = (((1,), (1,)), ((), ()))
LOG2E = math.log2(math.e)
MASKED = -1e9

ISSUE = ("qkSVv", "aSV")
LAG_S = (2, 1)
LAG_PV = (2, 3)
O_SPLITS = ((0, 1, 2, 3, 4, 6, 8), (0, 1, 2, 3, 4, 6, 8))
VPU_ROWS = ((range(16), ()), (range(16), ()))
VPU_DUE = (2, 3)
KEYS_AHEAD = (10, 11)
NORM_DUE = ((0, 1), (1, 3))
HALF = 256
PACE = 256
RING = 8
PRE = 8
WO_LAG = 3
TB = 512
K_PAIRS = 8
Q_PAIRS = 8
F_PAIRS = 2
O_ROWS = (128, 128, 128, 128)


def _iota(shape, axis):
    return lax.broadcasted_iota(jnp.int32, shape, axis)


def _div(v, d):
    return (v * ((1 << 18) // d + 1)) >> 18


def _pack(x):
    return pltpu.bitcast(x.astype(BF16), jnp.uint32)


def _unpack(x):
    return pltpu.bitcast(x, BF16)


def _recip(x):
    r = pl.reciprocal(x, approx=True)
    return r * (2.0 - x * r)


def _layernorm(x):
    m = jnp.mean(x, axis=-1, keepdims=True)
    c = x - m
    v = jnp.mean(c * c, axis=-1, keepdims=True)
    return c * lax.rsqrt(v + 1e-5)


def _rows(*parts):
    return jnp.concatenate(parts, axis=0)


def _cols(*parts):
    return jnp.concatenate(parts, axis=1)


def _strassen_weights(b11, b12, b21, b22):
    f11, f12, f21, f22 = (b.astype(F32) for b in (b11, b12, b21, b22))
    return [r.astype(BF16)
            for r in (f11 + f22, b11, f12 - f22, f21 - f11, b22, f11 + f12, f21 + f22)]


def _left_product(a1, a2, times):
    return times(a2, 3) + times(a1 + a2, 1)


def _right_product(a1, a2, times):
    return times(a1 + a2, 4) + times(a1, 2)


def _token_operands(a1, a2, b1, b2):
    low = b1 + b2
    n = low.shape[0] // 2
    return ({1: low[:n], 3: b2, 2: a1, 4: a1 + a2},
            {1: low[n:], 0: a1 + b2, 6: a2 - b2, 5: b1 - a1})


def _memory_operands(m1, m2):
    both = m1 + m2
    return {0: m2, 1: both, 2: m1, 3: m2, 4: both, 5: m1, 6: m2}


def _first_results(p, n):
    m1 = _rows(p[1][n:], jnp.zeros_like(p[1][n:]))
    return ((p[1][:n] + p[3][:n], p[2][:n] + p[4][:n]),
            (p[2][n:] + p[4][n:], p[3][n:] - p[4][n:], p[3][n:] + m1, p[2][n:] - m1))


def _second_left(p, n, c11, c21):
    m1 = _rows(jnp.zeros_like(p[1][n:]), p[1][n:])
    return p[1][:n] + p[6][:n] - p[0][:n], c11 + p[0][n:] + p[6][n:], c21 + m1


def _second_right(p, n, c22):
    m1 = _rows(jnp.zeros_like(p[1][n:]), p[1][n:])
    return p[5][:n] + p[0][:n] - p[1][:n], c22 + p[0][n:] + p[5][n:] - m1


def _a_step(s, mem, xn, shared, *, layer, dh, x_in, x_ref, xb_ref, ws_ref, wp_ref, wos_ref,
            wop_ref, pre_ref, ahead_ref, o_refs, near_ref):
    odd = bool(shared)
    n_mem, seg = mem.shape[0], xn[0].shape[0]
    n_seg = xb_ref.shape[0]
    rows = n_mem + seg
    pw = 2 * dh
    n_pairs = wp_ref.shape[0]
    o_ref = o_refs[odd]
    scale = dh ** -0.5

    def after(early, value):
        return value if early is None else jnp.where(s < 0, early[:, :value.shape[1]], value)

    def after_all(early, value):
        t = functools.reduce(jnp.maximum, [early[i:i + 8, j:j + 128]
                                           for i in range(0, early.shape[0], 8)
                                           for j in range(0, early.shape[1], 128)])
        return jnp.concatenate([after(t, value[0:8]), value[8:]], axis=0)

    def slow_norm(x):
        outs = [None, None]
        for i in range(0, seg, 8):
            outs.append(_layernorm(after(outs[-2], x[i:i + 8])))
        return jnp.concatenate(outs[2:], axis=0)

    xn_next = slow_norm(x_in[jnp.minimum(s + len(xn), n_seg - 1)].astype(F32))
    done = jnp.maximum(s - 3, 0)
    xb_done = slow_norm(x_ref[done])
    xb_ref[done] = xb_done.astype(BF16)

    h = _rows(mem, xn[0])

    first = _iota((rows, 128), 1) < 64
    zero = jnp.zeros((rows, 128), F32)

    def key_blocks(t):
        t0, t1, t2 = t[:, 0:128], t[:, 128:256], t[:, 256:384]
        top = jnp.concatenate([t0, jnp.where(first, t1, 0.0), zero], axis=1)
        bot = jnp.concatenate([zero, jnp.where(first, 0.0, t1), t2], axis=1)
        return jnp.concatenate([top, bot], axis=0).astype(BF16)

    def value_blocks(t):
        mine = jnp.concatenate([first] * 3, axis=1)
        return jnp.concatenate(
            [jnp.where(mine, t, 0.0), jnp.where(mine, 0.0, t)], axis=0).astype(BF16)

    def vpu_rows(p):
        return [n_mem + 8 * i for i, pairs in enumerate(VPU_ROWS[layer]) if p in pairs]

    def mxu_rows(p):
        return [r for r in range(0, rows, 8) if r not in vpu_rows(p)]

    def pick(t, starts):
        return jnp.concatenate([t[r:r + 8] for r in starts], axis=0)

    q, k, v, probs, near_done = {}, {}, {}, {}, {}

    def project_short(p, j):
        def dot(a, w):
            return jnp.dot(a.astype(BF16), _unpack(w), preferred_element_type=F32)

        cols, top = slice(j * pw, (j + 1) * pw), h[:rows - PRE]
        most = (_left_product, _right_product)[p % 2](
            top[:, :HALF], top[:, HALF:2 * HALF], lambda a, i: dot(a, ws_ref[p // 2, i, :, cols]))
        return _rows(dot(top[:, 2 * HALF:], wp_ref[p, :, cols]) + most,
                     pre_ref[p, pl.ds(pl.multiple_of(s * PRE, PRE), PRE), (j - 1) * pw:j * pw])

    if not odd:
        shared["in"] = _token_operands(*(t[:, c:c + HALF] for t in xn[1:3] for c in (0, HALF)))
    m_in = _memory_operands(mem[:, :HALF], mem[:, HALF:2 * HALF])
    lhs_in = {i: _rows(m_in[i], t) for i, t in shared["in"][odd].items()}
    products = {}

    def project_shared(p, cols):
        g, right = divmod(p, 2)
        for i in (((1, 3), (2, 4)), ((1, 0, 6), (5,)))[odd][right]:
            products[i] = jnp.dot(lhs_in[i], _unpack(ws_ref[g, i, :, cols]),
                                  preferred_element_type=F32)
        if not odd:
            tokens = ahead_ref[p, :, cols]
            if right:
                (_, m), shared[g] = _first_results(products, n_mem)
            else:
                m = products[1][:n_mem] + products[3][:n_mem]
        elif right:
            tokens = shared[g][0]
            m, ahead_ref[p, :, cols] = _second_right(products, n_mem, shared[g][3])
        else:
            m, tokens, ahead_ref[p, :, cols] = _second_left(products, n_mem, *shared[g][1:3])
        return jnp.dot(h[:, 2 * HALF:], _unpack(wp_ref[p, :, cols]),
                       preferred_element_type=F32) + _rows(m, tokens)

    def scores(p):
        col = pick(_iota((rows, 2 * rows), 1), mxu_rows(p))
        row = pick(_iota((rows, 2 * rows), 0), mxu_rows(p))
        is_a = col < rows
        visible = (row < n_mem) | (row >= jnp.where(is_a, col, col - rows))
        sc = lax.dot_general(pick(q[p], mxu_rows(p)), key_blocks(k[p]), NT,
                             preferred_element_type=F32)
        sc = jnp.where(visible, sc * scale, MASKED)
        max_a = jnp.max(jnp.where(is_a, sc, -jnp.inf), axis=1, keepdims=True)
        max_b = jnp.max(jnp.where(is_a, -jnp.inf, sc), axis=1, keepdims=True)
        e = jnp.exp(sc - jnp.where(is_a, max_a, max_b))
        sum_a = jnp.sum(jnp.where(is_a, e, 0.0), axis=1, keepdims=True)
        sum_b = jnp.sum(jnp.where(is_a, 0.0, e), axis=1, keepdims=True)
        probs[p] = e * _recip(jnp.where(is_a, sum_a, sum_b))
        if p == NORM_DUE[layer][0]:
            probs[p] = after_all(xn_next, probs[p])
        if p == NORM_DUE[layer][1]:
            probs[p] = after_all(xb_done, probs[p])
        if p - VPU_DUE[layer] in near_done:
            probs[p] = after_all(near_done[p - VPU_DUE[layer]], probs[p])

    def values(p):
        o = jnp.dot(probs[p], value_blocks(v[p]), preferred_element_type=F32)
        for i, r in enumerate(mxu_rows(p)):
            o_ref[r:r + 8, p * pw:(p + 1) * pw] = o[8 * i:8 * i + 8]

    chain = [None, None]
    scored = [None] * KEYS_AHEAD[layer]

    def attend_on_vpu(p, r):
        def key_row(j, i):
            return jnp.broadcast_to(near_ref[p, j:j + 1, 128 * i:128 * (i + 1)], (8, 128))

        half, sub = first[0:8], _iota((8, 128), 0)
        t = q[p][r:r + 8] * (scale * LOG2E)
        q0, q2 = t[:, 0:128], t[:, 256:384]
        q1a, q1b = jnp.where(half, t[:, 128:256], 0.0), jnp.where(half, 0.0, t[:, 128:256])
        for j in range(r + 8):
            ready = after(scored[-KEYS_AHEAD[layer]], chain[0])
            k1 = after(ready, key_row(j, 1))
            dot_a = q0 * after(ready, key_row(j, 0)) + q1a * k1
            dot_b = q2 * after(dot_a, key_row(j, 2)) + q1b * k1
            t = jnp.where(half, jnp.sum(dot_a, axis=1, keepdims=True),
                          jnp.sum(dot_b, axis=1, keepdims=True))
            scored.append(t if j <= r else jnp.where(sub >= j - r, t, MASKED * LOG2E))
            chain[0] = dot_b
        sc = scored[-(r + 8):]
        top = functools.reduce(jnp.maximum, sc)
        for j in range(r + 8):
            e = jnp.exp2(sc[j] - after(chain[1], top))
            weight = after(chain[1], e)
            terms = [weight * key_row(j, 3 + i) for i in range(3)]
            total = e if j == 0 else total + e
            acc = terms if j == 0 else [a + b for a, b in zip(acc, terms)]
            chain[1] = acc[2]
        inv = _recip(total)
        o_ref[r:r + 8, p * pw:(p + 1) * pw] = jnp.concatenate([a * inv for a in acc], axis=1)
        near_done[p] = acc[2]

    def attend_early_rows(p):
        if vpu_rows(p):
            n = vpu_rows(p)[-1] + 8
            near_ref[p, 0:n, 0:pw] = k[p][0:n]
            near_ref[p, 0:n, pw:2 * pw] = v[p][0:n]
        for r in reversed(vpu_rows(p)):
            attend_on_vpu(p, r)

    out = {}

    def project_out(g0, g1):
        def halves(ref, lo, hi):
            return [_cols(*(ref[lo:hi, (2 * g + i) * pw:(2 * g + i + 1) * pw]
                            for g in range(g0, g1))) for i in range(2)]

        if not odd:
            shared["out", g0] = _token_operands(*halves(o_refs[0], n_mem, rows),
                                                *halves(o_refs[1], n_mem, rows))
        m = _memory_operands(*halves(o_ref, 0, n_mem))
        for i, t in shared["out", g0][odd].items():
            r = jnp.dot(_rows(m[i], t), _unpack(wos_ref[g0:g1, i].reshape(-1, HALF)),
                        preferred_element_type=F32)
            out[i] = r + out[i] if i in out else r

    lag_s, lag_v = LAG_S[layer], LAG_S[layer] + LAG_PV[layer]
    todo = list(zip(O_SPLITS[layer][:-1], O_SPLITS[layer][1:]))
    for t in range(n_pairs + lag_v):
        if t >= n_pairs:
            project_out(*todo.pop(0))
        for c in ISSUE[layer]:
            if c == "S" and 0 <= t - lag_s < n_pairs:
                scores(t - lag_s)
            elif c == "V" and 0 <= t - lag_v < n_pairs:
                values(t - lag_v)
            elif c == "a" and t < n_pairs:
                r = project_shared(t, slice(0, 3 * pw))
                q[t], k[t], v[t] = r[:, 0:pw], r[:, pw:2 * pw], r[:, 2 * pw:3 * pw]
            elif c in "qkv" and t < n_pairs:
                j = "qkv".index(c)
                (q, k, v)[j][t] = project_short(t, j) if j else project_shared(t, slice(0, pw))
        if t < n_pairs:
            attend_early_rows(t)
    for part in todo:
        project_out(*part)
    rest = jnp.dot(o_ref[...], _unpack(wop_ref[...].reshape(-1, wop_ref.shape[-1])),
                   preferred_element_type=F32)

    most, tail = slice(0, 2 * HALF), slice(2 * HALF, None)
    x_ref[s, :, tail] = x_in[s, :, tail].astype(F32) + rest[n_mem:]
    if odd:
        c12, c11, c21, c22 = shared["out"]
        m1, c11, c21 = _second_left(out, n_mem, c11, c21)
        m2, c22 = _second_right(out, n_mem, c22)
        x_ref[s - 1, :, most] = x_in[s - 1, :, most].astype(F32) + _cols(c11, c12)
        back = jnp.maximum(s - 2, 1)
        x_ref[back, :, most] = (x_in[back, :, most].astype(F32)
                                + jnp.where(s > 1, _cols(c21, c22), 0.0))
    else:
        (m1, m2), shared["out"] = _first_results(out, n_mem)
    return _cols(m1, m2, rest[:n_mem]), xn_next


def _pair_reduce(t, op):
    r = t[0:8]
    for i in range(8, t.shape[0], 8):
        r = op(r, t[i:i + 8])
    r = op(r, pltpu.roll(r, 4, 0))
    return op(r, pltpu.roll(r, 2, 0))


def _tile_rows(r, n):
    return jnp.concatenate([r] * (n // 8), axis=0)


def _feature_map(p):
    n = p.shape[0]
    e_pos = jnp.exp2(p - _tile_rows(_pair_reduce(p, jnp.maximum), n))
    e_neg = jnp.exp2(_tile_rows(_pair_reduce(p, jnp.minimum), n) - p)
    inv_pos = _recip(_pair_reduce(e_pos, jnp.add))
    inv_neg = _recip(_pair_reduce(e_neg, jnp.add))
    return jnp.concatenate(
        [e_pos * _tile_rows(inv_pos, n), e_neg * _tile_rows(inv_neg, n)], axis=0)


def _fold_span(b, blk):
    return b * blk // 128 * 128, -(-(b + 1) * blk // 128) * 128


def _expand_phi(wphi_ref, phi_ref):
    dh, _, heads = wphi_ref.shape
    d = dh * heads
    gr = 2 * dh
    c = _iota((dh, d), 1)
    c_feat = c - _div(c, dh) * dh
    spread = (_div(_iota((heads, d), 1), dh) == _iota((heads, d), 0)).astype(BF16)

    def gather(j, by_feat):
        for e in (j * (dh // 4) + i for i in range(dh // 4)):
            t = jnp.dot(wphi_ref[e], spread, preferred_element_type=F32)
            by_feat = jnp.where(c_feat == e, t, by_feat)
        return by_feat

    by_feat = lax.fori_loop(0, 4, gather, jnp.zeros((dh, d), F32)).astype(BF16)
    blk = F_PAIRS * gr
    r = _iota((blk, dh), 0)
    sel = (((r - _div(r, gr) * gr) >> 1) == _iota((blk, dh), 1)).astype(BF16)
    for b in range(d // blk):
        lo, hi = _fold_span(b, blk)
        r = _iota((blk, hi - lo), 0)
        head = 2 * (_div(r, gr) + b * F_PAIRS) + (r & 1)
        phi = jnp.dot(sel, by_feat[:, lo:hi], preferred_element_type=F32)
        phi_ref[b, :, 0:hi - lo] = _pack(
            jnp.where(_div(_iota((1, hi - lo), 1) + lo, dh) == head, phi, 0.0))


def _b_weights(wqkv_ref, phi_ref, wob_ref, bq_ref, bkv_ref, bo_ref):
    d = wqkv_ref.shape[0]
    blk = 2 * phi_ref.shape[1]
    half = bkv_ref.shape[1]
    bo_ref[...] = _pack(wob_ref[...])
    wv = wqkv_ref[:, 2 * d:3 * d].T
    for b in range(d // half):
        bkv_ref[b, half // 2:half, :] = _pack(wv[b * half:(b + 1) * half])
    for b in range(d // blk):
        lo, hi = _fold_span(b, blk)
        phi = _unpack(phi_ref[b, :, 0:hi - lo])
        wq = lax.dot_general(phi, wqkv_ref[:, lo:hi], NT, preferred_element_type=F32)
        wk = lax.dot_general(phi, wqkv_ref[:, d + lo:d + hi], NT, preferred_element_type=F32)
        bq_ref[b * blk // 2:(b + 1) * blk // 2, :] = _pack(wq * LOG2E)
        at = b * blk % half // 2
        bkv_ref[b * blk // half, at:at + blk // 2, :] = _pack(wk * LOG2E)


def _chunk_rows(ref, it, r0, n):
    seg = ref.shape[1]
    return pl.ds(it * (TB // seg) + r0 // seg, n // seg)


def _b_keys(it, carry, *, x_ref, xb_ref, bkv_ref, kv_ref, z_ref):
    n_blk, half, _ = bkv_ref.shape
    gr = half // K_PAIRS
    xb = xb_ref[_chunk_rows(xb_ref, it, 0, TB)].reshape(TB, -1)
    last = x_ref.shape[0] - 1 - jnp.minimum(it, 2)
    xb_ref[last] = _layernorm(x_ref[last]).astype(BF16)
    same_head = (_iota((gr, 2 * gr), 0) >= gr // 2) == ((_iota((gr, 2 * gr), 1) & 1) == 1)

    def accumulate(b, t):
        for i in range(K_PAIRS):
            g = b * K_PAIRS + i
            phi = _feature_map(t[i * gr:(i + 1) * gr])
            z_ref[g] = jnp.where(it > 0, z_ref[g], 0.0) + jnp.sum(phi, axis=1, keepdims=True)
            kv = lax.dot_general(t[half + i * gr:half + (i + 1) * gr], phi.astype(BF16), NT,
                                 preferred_element_type=F32)
            kv_ref[g] = jnp.where(it > 0, kv_ref[g], 0.0) + jnp.where(same_head, kv, 0.0)

    pending = None
    for b in range(n_blk):
        t = lax.dot_general(_unpack(bkv_ref[b]), xb, NT, preferred_element_type=F32)
        if pending is not None:
            accumulate(*pending)
        pending = (b, t)
    accumulate(*pending)
    return carry


def _b_queries(it, send, *, x_ref, xb_ref, y_ref, bq_ref, bo_ref, kv_ref, z_ref, ot_ref, on_ref):
    n_groups, gr, _ = kv_ref.shape
    blk = Q_PAIRS * gr
    sub = _iota((8, TB), 0)
    xb = xb_ref[_chunk_rows(xb_ref, it, 0, TB)].reshape(TB, -1)

    def attend(b, t):
        outs = []
        for i in range(Q_PAIRS):
            g = b * Q_PAIRS + i
            phi = _feature_map(t[i * gr:(i + 1) * gr])
            num = jnp.dot(kv_ref[g], phi.astype(BF16), preferred_element_type=F32)
            z = jnp.concatenate([z_ref[g]] * (TB // 128), axis=1)
            inv = _recip(_pair_reduce(phi * z, jnp.add) + 1e-6)
            other = pltpu.roll(inv, 1, 0)
            inv_a = jnp.where((sub & 1) == 0, inv, other)
            inv_b = jnp.where((sub & 1) == 0, other, inv)
            n = (gr - 8) // 16
            inv = jnp.concatenate(
                [inv_a] * n + [jnp.where(sub < 4, inv_a, inv_b)] + [inv_b] * n, axis=0)
            outs.append(num * inv)
        ot_ref[b * blk // 2:(b + 1) * blk // 2, :] = _pack(jnp.concatenate(outs, axis=0))

    n_blk = n_groups // Q_PAIRS
    proj = {}
    for b in range(n_blk + 1):
        if b < n_blk:
            proj[b] = lax.dot_general(_unpack(bq_ref[b * blk // 2:(b + 1) * blk // 2, :]), xb,
                                      NT, preferred_element_type=F32)
        if b > 0:
            attend(b - 1, proj[b - 1])
    on_ref[...] = _pack(_unpack(ot_ref[...]).T)
    r0 = 0
    for i, n in enumerate(O_ROWS):
        at = _chunk_rows(x_ref, it, r0, n)
        y = jnp.dot(_unpack(on_ref[r0 // 2:(r0 + n) // 2, :]), _unpack(bo_ref[...]),
                    preferred_element_type=F32)
        x = x_ref[at] + y.reshape((-1,) + x_ref.shape[1:])
        x_ref[at] = x
        y_ref[at] = x.astype(BF16)
        send(i)
        r0 += n


def _kernel(x_hbm, mem0_hbm, wq_hbm, wk_hbm, wv_hbm, wo_hbm, wqkvb_hbm, wphi_hbm, wob_hbm,
            out_hbm,
            x_ref, xb_ref, y_ref, xp_ref, stage_ref, pre_ref, ahead_ref,
            ws_ref, wp_ref, wos_ref, wop_ref, o_even_ref, o_odd_ref, near_ref,
            mem0_ref, wphi_ref, phi_ref, wqkvb_ref, wob_ref, bo_ref, bq_ref, bkv_ref,
            kv_ref, z_ref, ot_ref, on_ref,
            w_sem, in_sem, out_sem, *, dh):
    n_seg, seg, d = x_ref.shape
    n_pairs = wp_ref.shape[0]
    n_mem = mem0_ref.shape[0]
    pw = 2 * dh
    n_iter = n_seg * seg // TB

    def w_copies(p, j):
        src = (wq_hbm, wk_hbm, wv_hbm, wo_hbm)[j]
        if j < 2:
            return [pltpu.make_async_copy(src.at[p], stage_ref.at[p % RING, 3 * j:3 * j + 3],
                                          w_sem.at[p, j])]
        return [pltpu.make_async_copy(src.at[p, i], stage_ref.at[p % RING, 3 * j:3 * j + 3, i],
                                      w_sem.at[p, 2 * j - 2 + i]) for i in range(2)]

    def start_w(p, *slots):
        for j in slots:
            for copy in w_copies(p, j):
                copy.start()

    def wait_w(p, *slots):
        for j in slots:
            for copy in w_copies(p, j):
                copy.wait()

    def prepare_in(u, tiles, live=True, pace=lambda t, b: b):
        g, i = u // 2, u % 2
        for t in tiles:
            cols = pl.ds(pl.multiple_of(128 * t, 128), 128)
            blocks = [stage_ref[p % RING, t, :, :, pl.ds(pl.multiple_of(c + i * 128, 128), 128)]
                      .reshape(128, 128)
                      for c in (0, HALF) for p in (2 * g, jnp.where(live, 2 * g + 1, 0))]
            for n, r in enumerate(_strassen_weights(*(pace(t, b) for b in blocks))):
                ws_ref[g, n, pl.ds(pl.multiple_of(i * 64, 64), 64), cols] = _pack(r.T)
            wp_ref[u, :, cols] = _pack(stage_ref[u % RING, t, :, :, 2 * HALF:].reshape(128, -1).T)

    def wait_out(u):
        for i in range(2):
            pltpu.make_async_copy(stage_ref.at[0, 9:12, 0], stage_ref.at[0, 9:12, 0],
                                  w_sem.at[u // 2 * 2 + i, 4 + u % 2]).wait()

    def prepare_out(u, live=True, pace=lambda t, b: b):
        g, i = u // 2, u % 2
        for t in range(3):
            parts = [pace(3 * t + 1, stage_ref[p % RING, jnp.where(live, 9, 3) + t, i])
                     for p in (2 * g, jnp.where(live, 2 * g + 1, 0))]
            blocks = [part[:, c:c + HALF] for part in parts for c in (0, HALF)]
            for n, r in enumerate(_strassen_weights(*blocks)):
                wos_ref[g, n, t, i] = _pack(r)
            for n, part in enumerate(parts):
                wop_ref[2 * g + n, t, i] = _pack(part[:, 2 * HALF:])

    def out_copy(it, i):
        part = _chunk_rows(y_ref, it, sum(O_ROWS[:i]), O_ROWS[i])
        return pltpu.make_async_copy(y_ref.at[part], out_hbm.at[part], out_sem.at[0])

    def x_copy(part, rows, sem):
        return pltpu.make_async_copy(x_hbm.at[part, rows, :], y_ref.at[part, rows, :], sem)

    head, tail = slice(0, seg - PRE), slice(seg - PRE, seg)
    xt_copy = x_copy(slice(None), tail, in_sem.at[0])
    wqkvb_copy = pltpu.make_async_copy(wqkvb_hbm, wqkvb_ref, in_sem.at[1])
    wphi_copy = pltpu.make_async_copy(wphi_hbm, wphi_ref, in_sem.at[5])
    mem0_copy = pltpu.make_async_copy(mem0_hbm, mem0_ref, in_sem.at[4])
    wob_copy = pltpu.make_async_copy(wob_hbm, wob_ref, in_sem.at[2])

    wphi_copy.start()
    xt_copy.start()
    start_w(0, 0, 1, 2)
    wphi_copy.wait()
    _expand_phi(wphi_ref, phi_ref)
    xt_copy.wait()

    xp_ref[...] = _layernorm(y_ref[:, tail, :].astype(F32).reshape(n_seg * PRE, d)).astype(BF16)

    mem0_copy.start()
    start_w(1, 0, 1, 2)

    def pre_project(p, carry):
        @pl.when(p + 2 < n_pairs)
        def _():
            start_w(jnp.minimum(p + 2, n_pairs - 1), 0, 1, 2)

        part = pl.ds(p * (n_seg // n_pairs), n_seg // n_pairs)
        x_copy(part, head, in_sem.at[3]).start()
        start_w(p, 3)

        @pl.when(p >= WO_LAG)
        def _():
            wait_out(jnp.maximum(p - WO_LAG, 0))

        wait_w(p, 0, 1, 2)
        kv = lax.dot_general(xp_ref[...], stage_ref[p % RING, 3:9].reshape(-1, d), NT,
                             preferred_element_type=F32)
        pre_ref[p] = kv

        def pace(t, block):
            c, r = divmod(t * PACE, xp_ref.shape[0])
            early = kv[r:r + block.shape[0], 128 * c:128 * (c + 1)].astype(BF16)
            return jnp.where(p < 0, _cols(*[early] * (block.shape[1] // 128)), block)

        prepare_in(jnp.maximum(p - 1, 0), range(9), p >= 1, pace)
        prepare_out(jnp.maximum(p - WO_LAG, 0), p >= WO_LAG, pace)
        return carry

    lax.fori_loop(0, n_pairs, pre_project, 0)

    @pl.loop(0, 3)
    def _(j):
        prepare_in(n_pairs - 1, [3 * j + i for i in range(3)])

    @pl.loop(n_pairs - WO_LAG, n_pairs)
    def _(u):
        wait_out(u)
        prepare_out(u)

    x_copy(slice(None), head, in_sem.at[3]).wait()

    wqkvb_copy.start()
    wob_copy.start()
    mem0_copy.wait()
    x_ref[0] = y_ref[0].astype(F32)

    def layer_a(layer, x_in, pre):
        step = functools.partial(
            _a_step, layer=layer, dh=dh, x_in=x_in, x_ref=x_ref, xb_ref=xb_ref, ws_ref=ws_ref,
            wp_ref=wp_ref, wos_ref=wos_ref, wop_ref=wop_ref, pre_ref=pre, ahead_ref=ahead_ref,
            o_refs=(o_even_ref, o_odd_ref), near_ref=near_ref)
        xn = [_layernorm(x_in[i].astype(F32)) for i in range(3)]
        o_odd_ref[...] = jnp.zeros(o_odd_ref.shape, F32)
        cols, per = (slice(0, 3 * pw), 1) if pre is None else (slice(0, pw), 2)

        @pl.loop(0, n_pairs // 2 // per)
        def _(j):
            for g in (j * per + i for i in range(per)):
                for i, product in enumerate((_left_product, _right_product)):
                    ahead_ref[2 * g + i, :, cols] = product(
                        xn[0][:, :HALF], xn[0][:, HALF:2 * HALF],
                        lambda a, n: jnp.dot(a.astype(BF16), _unpack(ws_ref[g, n, :, cols]),
                                             preferred_element_type=F32))

        def two_steps(it, carry):
            mem, *xn = carry
            shared = {}
            for i in range(2):
                mem, xn_next = step(2 * it + i, mem, xn, shared)
                xn = xn[1:] + [xn_next]
            return (mem, *xn)

        lax.fori_loop(0, n_seg // 2, two_steps, (mem0_ref[...].astype(F32), *xn))

    def finish_a(layer):
        a = [_cols(*(o_odd_ref[n_mem:, (2 * g + i) * pw:(2 * g + i + 1) * pw]
                     for g in range(n_pairs // 2))) for i in range(2)]
        y = _cols(*(product(*a, lambda t, n: jnp.dot(
            t.astype(BF16), _unpack(wos_ref[:, n].reshape(-1, HALF)), preferred_element_type=F32))
            for product in (_left_product, _right_product)))
        at = (n_seg - 1, slice(None), slice(0, 2 * HALF))
        x_ref[at] = jnp.where(layer == 0, y_ref[at].astype(F32), x_ref[at]) + y

    b_keys = functools.partial(_b_keys, x_ref=x_ref, xb_ref=xb_ref, bkv_ref=bkv_ref,
                               kv_ref=kv_ref, z_ref=z_ref)
    b_queries = functools.partial(_b_queries, x_ref=x_ref, xb_ref=xb_ref, y_ref=y_ref,
                                  bq_ref=bq_ref, bo_ref=bo_ref, kv_ref=kv_ref, z_ref=z_ref,
                                  ot_ref=ot_ref, on_ref=on_ref)

    def layer_pair(layer, carry):
        @pl.when(layer == 0)
        def _():
            layer_a(0, y_ref, pre_ref)

        @pl.when(layer == 0)
        def _():
            wqkvb_copy.wait()
            wob_copy.wait()
            _b_weights(wqkvb_ref, phi_ref, wob_ref, bq_ref, bkv_ref, bo_ref)

        @pl.when(layer == 1)
        def _():
            layer_a(1, x_ref, None)

        finish_a(layer)

        lax.fori_loop(0, n_iter, b_keys, 0)

        def queries(it, carry):
            def send(i):
                @pl.when(layer == 1)
                def _():
                    out_copy(it, i).start()

            b_queries(it, send)
            return carry

        lax.fori_loop(0, n_iter, queries, 0)

        return carry

    lax.fori_loop(0, 2, layer_pair, 0)
    pltpu.make_async_copy(y_ref, out_hbm, out_sem.at[0]).wait()


@functools.partial(jax.jit, static_argnames=("A_seg_len",))
def pallas_interleave_layers__memory_aug_recurrent_mem_tr__linear_kernel_hedgehog__prompt_kernel(
    A_x, A_mem0, A_Wq, A_Wk, A_Wv, A_Wo, A_seg_len, B_x, B_wqkv, B_w_phi, B_wo,
):
    del B_x
    batch, s_len, d = A_x.shape
    _, heads, dh = A_Wq.shape
    n_mem = A_mem0.shape[1]
    seg = int(A_seg_len)
    b_heads, b_dh, _ = B_w_phi.shape
    rows = n_mem + seg
    n_pairs = heads // 2
    gr = 2 * b_dh
    half = K_PAIRS * gr
    n_seg = s_len // seg
    assert batch == 1 and dh == 192 and heads == 4 * O_SPLITS[0][-1] and d == 2 * HALF + 128
    assert n_mem % 8 == 0 and seg % 16 == 0 and 128 % seg == 0 and 2 * rows <= 128
    assert s_len % TB == 0 and s_len > 3 * TB == 3 * sum(O_ROWS) and n_seg % n_pairs == 0
    assert b_heads * b_dh == d and b_dh % 8 == 4 and d % half == 0

    def head_major(w):
        return w.transpose(1, 2, 0)

    hbm = pl.BlockSpec(memory_space=pltpu.HBM)
    out = pl.pallas_call(
        functools.partial(_kernel, dh=dh),
        out_shape=jax.ShapeDtypeStruct((n_seg, seg, d), A_x.dtype),
        in_specs=[hbm] * 9,
        out_specs=hbm,
        scratch_shapes=[
            pltpu.VMEM((n_seg, seg, d), F32),
            pltpu.VMEM((n_seg, seg, d), BF16),
            pltpu.VMEM((n_seg, seg, d), BF16),
            pltpu.VMEM((n_seg * PRE, d), BF16),
            pltpu.VMEM((RING, 12, 2, 64, d), BF16),
            pltpu.VMEM((n_pairs, n_seg * PRE, 4 * dh), F32),
            pltpu.VMEM((n_pairs, seg, 6 * dh), F32),
            pltpu.VMEM((n_pairs // 2, 7, HALF // 2, 6 * dh), jnp.uint32),
            pltpu.VMEM((n_pairs, d // 2 - HALF, 6 * dh), jnp.uint32),
            pltpu.VMEM((n_pairs // 2, 7, 3, 2, 32, HALF), jnp.uint32),
            pltpu.VMEM((n_pairs, 3, 2, 32, d - 2 * HALF), jnp.uint32),
            pltpu.VMEM((rows, heads * dh), F32),
            pltpu.VMEM((rows, heads * dh), F32),
            pltpu.VMEM((n_pairs, n_mem + 16, 4 * dh), F32),
            pltpu.VMEM((n_mem, d), BF16),
            pltpu.VMEM((b_dh, b_dh, b_heads), BF16),
            pltpu.VMEM((d // (F_PAIRS * gr), F_PAIRS * gr // 2, 256), jnp.uint32),
            pltpu.VMEM(B_wqkv.shape, BF16),
            pltpu.VMEM(B_wo.shape, BF16),
            pltpu.VMEM((d // 2, d), jnp.uint32),
            pltpu.VMEM((d // 2, d), jnp.uint32),
            pltpu.VMEM((d // half, half, d), jnp.uint32),
            pltpu.VMEM((b_heads // 2, gr, 2 * gr), F32),
            pltpu.VMEM((b_heads // 2, 2 * gr, 128), F32),
            pltpu.VMEM((d // 2, TB), jnp.uint32),
            pltpu.VMEM((TB // 2, d), jnp.uint32),
            pltpu.SemaphoreType.DMA((n_pairs, 6)),
            pltpu.SemaphoreType.DMA((6,)),
            pltpu.SemaphoreType.DMA((1,)),
        ],
        compiler_params=pltpu.CompilerParams(vmem_limit_bytes=124 * 1024 * 1024),
    )(
        A_x.reshape(n_seg, seg, d), A_mem0.reshape(n_mem, d),
        head_major(A_Wq).reshape(n_pairs, 3, 2, 64, d),
        head_major(A_Wk).reshape(n_pairs, 3, 2, 64, d),
        head_major(A_Wv).reshape(n_pairs, 2, 3, 64, d), A_Wo.reshape(n_pairs, 2, 3, 64, d),
        B_wqkv, B_w_phi.transpose(1, 2, 0), B_wo,
    )
    return out.reshape(batch, s_len, d)
```

```python
import functools
import math

import jax
import jax.numpy as jnp
from jax import lax
import jax.experimental.pallas as pl
import jax.experimental.pallas.tpu as pltpu

F32 = jnp.float32
BF16 = jnp.bfloat16
NT = (((1,), (1,)), ((), ()))
LOG2E = math.log2(math.e)
MASKED = -1e9

ISSUE = ("kqSVv", "aSV")
LAG_S = (2, 1)
LAG_PV = (2, 3)
O_SPLITS = ((0, 1, 2, 3, 4, 5, 6, 8), (0, 1, 2, 3, 4, 6, 8))
VPU_ROWS = ((range(16), ()), (range(16), ()))
VPU_DUE = (3, 3)
KEYS_AHEAD = (13, 9)
NORM_DUE = ((0, 2), (2, 3))
HALF = 256
PACE = 256
RING = 8
PRE = 8
WO_LAG = 3
TB = 512
K_PAIRS = 8
Q_PAIRS = 8
F_PAIRS = 2
O_ROWS = (128, 128, 128, 128)


def _iota(shape, axis):
    return lax.broadcasted_iota(jnp.int32, shape, axis)


def _div(v, d):
    return (v * ((1 << 18) // d + 1)) >> 18


def _pack(x):
    return pltpu.bitcast(x.astype(BF16), jnp.uint32)


def _unpack(x):
    return pltpu.bitcast(x, BF16)


def _recip(x):
    r = pl.reciprocal(x, approx=True)
    return r * (2.0 - x * r)


def _layernorm(x):
    m = jnp.mean(x, axis=-1, keepdims=True)
    c = x - m
    v = jnp.mean(c * c, axis=-1, keepdims=True)
    return c * lax.rsqrt(v + 1e-5)


def _rows(*parts):
    return jnp.concatenate(parts, axis=0)


def _cols(*parts):
    return jnp.concatenate(parts, axis=1)


def _strassen_weights(b11, b12, b21, b22):
    f11, f12, f21, f22 = (b.astype(F32) for b in (b11, b12, b21, b22))
    return [r.astype(BF16)
            for r in (f11 + f22, b11, f12 - f22, f21 - f11, b22, f11 + f12, f21 + f22)]


def _left_product(a1, a2, times):
    return times(a2, 3) + times(a1 + a2, 1)


def _right_product(a1, a2, times):
    return times(a1 + a2, 4) + times(a1, 2)


def _token_operands(a1, a2, b1, b2):
    low = b1 + b2
    n = low.shape[0] // 2
    return ({1: low[:n], 3: b2, 2: a1, 4: a1 + a2},
            {1: low[n:], 0: a1 + b2, 6: a2 - b2, 5: b1 - a1})


def _memory_operands(m1, m2):
    both = m1 + m2
    return {0: m2, 1: both, 2: m1, 3: m2, 4: both, 5: m1, 6: m2}


def _first_results(p, n):
    m1 = _rows(p[1][n:], jnp.zeros_like(p[1][n:]))
    return ((p[1][:n] + p[3][:n], p[2][:n] + p[4][:n]),
            (p[2][n:] + p[4][n:], p[3][n:] - p[4][n:], p[3][n:] + m1, p[2][n:] - m1))


def _second_left(p, n, c11, c21):
    m1 = _rows(jnp.zeros_like(p[1][n:]), p[1][n:])
    return p[1][:n] + p[6][:n] - p[0][:n], c11 + p[0][n:] + p[6][n:], c21 + m1


def _second_right(p, n, c22):
    m1 = _rows(jnp.zeros_like(p[1][n:]), p[1][n:])
    return p[5][:n] + p[0][:n] - p[1][:n], c22 + p[0][n:] + p[5][n:] - m1


def _a_step(s, mem, xn, shared, *, layer, dh, x_in, x_ref, xb_ref, ws_ref, wp_ref, wos_ref,
            wop_ref, pre_ref, ahead_ref, o_refs, near_ref):
    odd = bool(shared)
    n_mem, seg = mem.shape[0], xn[0].shape[0]
    n_seg = xb_ref.shape[0]
    rows = n_mem + seg
    pw = 2 * dh
    n_pairs = wp_ref.shape[0]
    o_ref = o_refs[odd]
    scale = dh ** -0.5

    def after(early, value):
        return value if early is None else jnp.where(s < 0, early[:, :value.shape[1]], value)

    def after_all(early, value):
        t = functools.reduce(jnp.maximum, [early[i:i + 8, j:j + 128]
                                           for i in range(0, early.shape[0], 8)
                                           for j in range(0, early.shape[1], 128)])
        return jnp.concatenate([after(t, value[0:8]), value[8:]], axis=0)

    def slow_norm(x):
        outs = [None, None]
        for i in range(0, seg, 8):
            outs.append(_layernorm(after(outs[-2], x[i:i + 8])))
        return jnp.concatenate(outs[2:], axis=0)

    xn_next = slow_norm(x_in[jnp.minimum(s + len(xn), n_seg - 1)].astype(F32))
    done = jnp.maximum(s - 3, 0)
    xb_done = slow_norm(x_ref[done])
    xb_ref[done] = xb_done.astype(BF16)

    h = _rows(mem, xn[0])

    first = _iota((rows, 128), 1) < 64
    zero = jnp.zeros((rows, 128), F32)

    def key_blocks(t):
        t0, t1, t2 = t[:, 0:128], t[:, 128:256], t[:, 256:384]
        top = jnp.concatenate([t0, jnp.where(first, t1, 0.0), zero], axis=1)
        bot = jnp.concatenate([zero, jnp.where(first, 0.0, t1), t2], axis=1)
        return jnp.concatenate([top, bot], axis=0).astype(BF16)

    def value_blocks(t):
        mine = jnp.concatenate([first] * 3, axis=1)
        return jnp.concatenate(
            [jnp.where(mine, t, 0.0), jnp.where(mine, 0.0, t)], axis=0).astype(BF16)

    def vpu_rows(p):
        return [n_mem + 8 * i for i, pairs in enumerate(VPU_ROWS[layer]) if p in pairs]

    def mxu_rows(p):
        return [r for r in range(0, rows, 8) if r not in vpu_rows(p)]

    def pick(t, starts):
        return jnp.concatenate([t[r:r + 8] for r in starts], axis=0)

    q, k, v, probs, near_done = {}, {}, {}, {}, {}

    def project_short(p, j):
        def dot(a, w):
            return jnp.dot(a.astype(BF16), _unpack(w), preferred_element_type=F32)

        cols, top = slice(j * pw, (j + 1) * pw), h[:rows - PRE]
        most = (_left_product, _right_product)[p % 2](
            top[:, :HALF], top[:, HALF:2 * HALF], lambda a, i: dot(a, ws_ref[p // 2, i, :, cols]))
        return _rows(dot(top[:, 2 * HALF:], wp_ref[p, :, cols]) + most,
                     pre_ref[p, pl.ds(pl.multiple_of(s * PRE, PRE), PRE), (j - 1) * pw:j * pw])

    if not odd:
        shared["in"] = _token_operands(*(t[:, c:c + HALF] for t in xn[1:3] for c in (0, HALF)))
    m_in = _memory_operands(mem[:, :HALF], mem[:, HALF:2 * HALF])
    lhs_in = {i: _rows(m_in[i], t) for i, t in shared["in"][odd].items()}
    products = {}

    def project_shared(p, cols):
        g, right = divmod(p, 2)
        for i in (((1, 3), (2, 4)), ((1, 0, 6), (5,)))[odd][right]:
            products[i] = jnp.dot(lhs_in[i], _unpack(ws_ref[g, i, :, cols]),
                                  preferred_element_type=F32)
        if not odd:
            tokens = ahead_ref[p, :, cols]
            if right:
                (_, m), shared[g] = _first_results(products, n_mem)
            else:
                m = products[1][:n_mem] + products[3][:n_mem]
        elif right:
            tokens = shared[g][0]
            m, ahead_ref[p, :, cols] = _second_right(products, n_mem, shared[g][3])
        else:
            m, tokens, ahead_ref[p, :, cols] = _second_left(products, n_mem, *shared[g][1:3])
        return jnp.dot(h[:, 2 * HALF:], _unpack(wp_ref[p, :, cols]),
                       preferred_element_type=F32) + _rows(m, tokens)

    def scores(p):
        col = pick(_iota((rows, 2 * rows), 1), mxu_rows(p))
        row = pick(_iota((rows, 2 * rows), 0), mxu_rows(p))
        is_a = col < rows
        visible = (row < n_mem) | (row >= jnp.where(is_a, col, col - rows))
        sc = lax.dot_general(pick(q[p], mxu_rows(p)), key_blocks(k[p]), NT,
                             preferred_element_type=F32)
        sc = jnp.where(visible, sc * scale, MASKED)
        max_a = jnp.max(jnp.where(is_a, sc, -jnp.inf), axis=1, keepdims=True)
        max_b = jnp.max(jnp.where(is_a, -jnp.inf, sc), axis=1, keepdims=True)
        e = jnp.exp(sc - jnp.where(is_a, max_a, max_b))
        sum_a = jnp.sum(jnp.where(is_a, e, 0.0), axis=1, keepdims=True)
        sum_b = jnp.sum(jnp.where(is_a, 0.0, e), axis=1, keepdims=True)
        probs[p] = e * _recip(jnp.where(is_a, sum_a, sum_b))
        if p == NORM_DUE[layer][0]:
            probs[p] = after_all(xn_next, probs[p])
        if p == NORM_DUE[layer][1]:
            probs[p] = after_all(xb_done, probs[p])
        if p - VPU_DUE[layer] in near_done:
            probs[p] = after_all(near_done[p - VPU_DUE[layer]], probs[p])

    def values(p):
        o = jnp.dot(probs[p], value_blocks(v[p]), preferred_element_type=F32)
        for i, r in enumerate(mxu_rows(p)):
            o_ref[r:r + 8, p * pw:(p + 1) * pw] = o[8 * i:8 * i + 8]

    chain = [None, None]
    scored = [None] * KEYS_AHEAD[layer]

    def attend_on_vpu(p, r):
        def key_row(j, i):
            return jnp.broadcast_to(near_ref[p, j:j + 1, 128 * i:128 * (i + 1)], (8, 128))

        half, sub = first[0:8], _iota((8, 128), 0)
        t = q[p][r:r + 8] * (scale * LOG2E)
        q0, q2 = t[:, 0:128], t[:, 256:384]
        q1a, q1b = jnp.where(half, t[:, 128:256], 0.0), jnp.where(half, 0.0, t[:, 128:256])
        for j in range(r + 8):
            ready = after(scored[-KEYS_AHEAD[layer]], chain[0])
            k1 = after(ready, key_row(j, 1))
            dot_a = q0 * after(ready, key_row(j, 0)) + q1a * k1
            dot_b = q2 * after(dot_a, key_row(j, 2)) + q1b * k1
            t = jnp.where(half, jnp.sum(dot_a, axis=1, keepdims=True),
                          jnp.sum(dot_b, axis=1, keepdims=True))
            scored.append(t if j <= r else jnp.where(sub >= j - r, t, MASKED * LOG2E))
            chain[0] = dot_b
        sc = scored[-(r + 8):]
        top = functools.reduce(jnp.maximum, sc)
        for j in range(r + 8):
            e = jnp.exp2(sc[j] - after(chain[1], top))
            weight = after(chain[1], e)
            terms = [weight * key_row(j, 3 + i) for i in range(3)]
            total = e if j == 0 else total + e
            acc = terms if j == 0 else [a + b for a, b in zip(acc, terms)]
            chain[1] = acc[2]
        inv = _recip(total)
        o_ref[r:r + 8, p * pw:(p + 1) * pw] = jnp.concatenate([a * inv for a in acc], axis=1)
        near_done[p] = acc[2]

    def attend_early_rows(p):
        if vpu_rows(p):
            n = vpu_rows(p)[-1] + 8
            near_ref[p, 0:n, 0:pw] = k[p][0:n]
            near_ref[p, 0:n, pw:2 * pw] = v[p][0:n]
        for r in reversed(vpu_rows(p)):
            attend_on_vpu(p, r)

    out = {}

    def project_out(g0, g1):
        def halves(ref, lo, hi):
            return [_cols(*(ref[lo:hi, (2 * g + i) * pw:(2 * g + i + 1) * pw]
                            for g in range(g0, g1))) for i in range(2)]

        if not odd:
            shared["out", g0] = _token_operands(*halves(o_refs[0], n_mem, rows),
                                                *halves(o_refs[1], n_mem, rows))
        m = _memory_operands(*halves(o_ref, 0, n_mem))
        for i, t in shared["out", g0][odd].items():
            r = jnp.dot(_rows(m[i], t), _unpack(wos_ref[g0:g1, i].reshape(-1, HALF)),
                        preferred_element_type=F32)
            out[i] = r + out[i] if i in out else r

    lag_s, lag_v = LAG_S[layer], LAG_S[layer] + LAG_PV[layer]
    todo = list(zip(O_SPLITS[layer][:-1], O_SPLITS[layer][1:]))
    for t in range(n_pairs + lag_v):
        if t >= n_pairs:
            project_out(*todo.pop(0))
        for c in ISSUE[layer]:
            if c == "S" and 0 <= t - lag_s < n_pairs:
                scores(t - lag_s)
            elif c == "V" and 0 <= t - lag_v < n_pairs:
                values(t - lag_v)
            elif c == "a" and t < n_pairs:
                r = project_shared(t, slice(0, 3 * pw))
                q[t], k[t], v[t] = r[:, 0:pw], r[:, pw:2 * pw], r[:, 2 * pw:3 * pw]
            elif c in "qkv" and t < n_pairs:
                j = "qkv".index(c)
                (q, k, v)[j][t] = project_short(t, j) if j else project_shared(t, slice(0, pw))
        if t < n_pairs:
            attend_early_rows(t)
    for part in todo:
        project_out(*part)
    rest = jnp.dot(o_ref[...], _unpack(wop_ref[...].reshape(-1, wop_ref.shape[-1])),
                   preferred_element_type=F32)

    most, tail = slice(0, 2 * HALF), slice(2 * HALF, None)
    x_ref[s, :, tail] = x_in[s, :, tail].astype(F32) + rest[n_mem:]
    if odd:
        c12, c11, c21, c22 = shared["out"]
        m1, c11, c21 = _second_left(out, n_mem, c11, c21)
        m2, c22 = _second_right(out, n_mem, c22)
        x_ref[s - 1, :, most] = x_in[s - 1, :, most].astype(F32) + _cols(c11, c12)
        back = jnp.maximum(s - 2, 1)
        x_ref[back, :, most] = (x_in[back, :, most].astype(F32)
                                + jnp.where(s > 1, _cols(c21, c22), 0.0))
    else:
        (m1, m2), shared["out"] = _first_results(out, n_mem)
    return _cols(m1, m2, rest[:n_mem]), xn_next


def _pair_reduce(t, op):
    r = t[0:8]
    for i in range(8, t.shape[0], 8):
        r = op(r, t[i:i + 8])
    r = op(r, pltpu.roll(r, 4, 0))
    return op(r, pltpu.roll(r, 2, 0))


def _tile_rows(r, n):
    return jnp.concatenate([r] * (n // 8), axis=0)


def _feature_map(p):
    n = p.shape[0]
    e_pos = jnp.exp2(p - _tile_rows(_pair_reduce(p, jnp.maximum), n))
    e_neg = jnp.exp2(_tile_rows(_pair_reduce(p, jnp.minimum), n) - p)
    inv_pos = _recip(_pair_reduce(e_pos, jnp.add))
    inv_neg = _recip(_pair_reduce(e_neg, jnp.add))
    return jnp.concatenate(
        [e_pos * _tile_rows(inv_pos, n), e_neg * _tile_rows(inv_neg, n)], axis=0)


def _fold_span(b, blk):
    return b * blk // 128 * 128, -(-(b + 1) * blk // 128) * 128


def _expand_phi(wphi_ref, phi_ref):
    dh, _, heads = wphi_ref.shape
    d = dh * heads
    gr = 2 * dh
    c = _iota((dh, d), 1)
    c_feat = c - _div(c, dh) * dh
    spread = (_div(_iota((heads, d), 1), dh) == _iota((heads, d), 0)).astype(BF16)

    def gather(j, by_feat):
        for e in (j * (dh // 4) + i for i in range(dh // 4)):
            t = jnp.dot(wphi_ref[e], spread, preferred_element_type=F32)
            by_feat = jnp.where(c_feat == e, t, by_feat)
        return by_feat

    by_feat = lax.fori_loop(0, 4, gather, jnp.zeros((dh, d), F32)).astype(BF16)
    blk = F_PAIRS * gr
    r = _iota((blk, dh), 0)
    sel = (((r - _div(r, gr) * gr) >> 1) == _iota((blk, dh), 1)).astype(BF16)
    for b in range(d // blk):
        lo, hi = _fold_span(b, blk)
        r = _iota((blk, hi - lo), 0)
        head = 2 * (_div(r, gr) + b * F_PAIRS) + (r & 1)
        phi = jnp.dot(sel, by_feat[:, lo:hi], preferred_element_type=F32)
        phi_ref[b, :, 0:hi - lo] = _pack(
            jnp.where(_div(_iota((1, hi - lo), 1) + lo, dh) == head, phi, 0.0))


def _b_weights(wqkv_ref, phi_ref, wob_ref, bq_ref, bkv_ref, bo_ref):
    d = wqkv_ref.shape[0]
    blk = 2 * phi_ref.shape[1]
    half = bkv_ref.shape[1]
    bo_ref[...] = _pack(wob_ref[...])
    wv = wqkv_ref[:, 2 * d:3 * d].T
    for b in range(d // half):
        bkv_ref[b, half // 2:half, :] = _pack(wv[b * half:(b + 1) * half])
    for b in range(d // blk):
        lo, hi = _fold_span(b, blk)
        phi = _unpack(phi_ref[b, :, 0:hi - lo])
        wq = lax.dot_general(phi, wqkv_ref[:, lo:hi], NT, preferred_element_type=F32)
        wk = lax.dot_general(phi, wqkv_ref[:, d + lo:d + hi], NT, preferred_element_type=F32)
        bq_ref[b * blk // 2:(b + 1) * blk // 2, :] = _pack(wq * LOG2E)
        at = b * blk % half // 2
        bkv_ref[b * blk // half, at:at + blk // 2, :] = _pack(wk * LOG2E)


def _chunk_rows(ref, it, r0, n):
    seg = ref.shape[1]
    return pl.ds(it * (TB // seg) + r0 // seg, n // seg)


def _b_keys(it, carry, *, x_ref, xb_ref, bkv_ref, kv_ref, z_ref):
    n_blk, half, _ = bkv_ref.shape
    gr = half // K_PAIRS
    xb = xb_ref[_chunk_rows(xb_ref, it, 0, TB)].reshape(TB, -1)
    last = x_ref.shape[0] - 1 - jnp.minimum(it, 2)
    xb_ref[last] = _layernorm(x_ref[last]).astype(BF16)
    same_head = (_iota((gr, 2 * gr), 0) >= gr // 2) == ((_iota((gr, 2 * gr), 1) & 1) == 1)

    def accumulate(b, t):
        for i in range(K_PAIRS):
            g = b * K_PAIRS + i
            phi = _feature_map(t[i * gr:(i + 1) * gr])
            z_ref[g] = jnp.where(it > 0, z_ref[g], 0.0) + jnp.sum(phi, axis=1, keepdims=True)
            kv = lax.dot_general(t[half + i * gr:half + (i + 1) * gr], phi.astype(BF16), NT,
                                 preferred_element_type=F32)
            kv_ref[g] = jnp.where(it > 0, kv_ref[g], 0.0) + jnp.where(same_head, kv, 0.0)

    pending = None
    for b in range(n_blk):
        t = lax.dot_general(_unpack(bkv_ref[b]), xb, NT, preferred_element_type=F32)
        if pending is not None:
            accumulate(*pending)
        pending = (b, t)
    accumulate(*pending)
    return carry


def _b_queries(it, send, *, x_ref, xb_ref, y_ref, bq_ref, bo_ref, kv_ref, z_ref, ot_ref, on_ref):
    n_groups, gr, _ = kv_ref.shape
    blk = Q_PAIRS * gr
    sub = _iota((8, TB), 0)
    xb = xb_ref[_chunk_rows(xb_ref, it, 0, TB)].reshape(TB, -1)

    def attend(b, t):
        outs = []
        for i in range(Q_PAIRS):
            g = b * Q_PAIRS + i
            phi = _feature_map(t[i * gr:(i + 1) * gr])
            num = jnp.dot(kv_ref[g], phi.astype(BF16), preferred_element_type=F32)
            z = jnp.concatenate([z_ref[g]] * (TB // 128), axis=1)
            inv = _recip(_pair_reduce(phi * z, jnp.add) + 1e-6)
            other = pltpu.roll(inv, 1, 0)
            inv_a = jnp.where((sub & 1) == 0, inv, other)
            inv_b = jnp.where((sub & 1) == 0, other, inv)
            n = (gr - 8) // 16
            inv = jnp.concatenate(
                [inv_a] * n + [jnp.where(sub < 4, inv_a, inv_b)] + [inv_b] * n, axis=0)
            outs.append(num * inv)
        ot_ref[b * blk // 2:(b + 1) * blk // 2, :] = _pack(jnp.concatenate(outs, axis=0))

    n_blk = n_groups // Q_PAIRS
    proj = {}
    for b in range(n_blk + 1):
        if b < n_blk:
            proj[b] = lax.dot_general(_unpack(bq_ref[b * blk // 2:(b + 1) * blk // 2, :]), xb,
                                      NT, preferred_element_type=F32)
        if b > 0:
            attend(b - 1, proj[b - 1])
    on_ref[...] = _pack(_unpack(ot_ref[...]).T)
    r0 = 0
    for i, n in enumerate(O_ROWS):
        at = _chunk_rows(x_ref, it, r0, n)
        y = jnp.dot(_unpack(on_ref[r0 // 2:(r0 + n) // 2, :]), _unpack(bo_ref[...]),
                    preferred_element_type=F32)
        x = x_ref[at] + y.reshape((-1,) + x_ref.shape[1:])
        x_ref[at] = x
        y_ref[at] = x.astype(BF16)
        send(i)
        r0 += n


def _kernel(x_hbm, mem0_hbm, wq_hbm, wk_hbm, wv_hbm, wo_hbm, wqkvb_hbm, wphi_hbm, wob_hbm,
            out_hbm,
            x_ref, xb_ref, y_ref, xp_ref, stage_ref, pre_ref, ahead_ref,
            ws_ref, wp_ref, wos_ref, wop_ref, o_even_ref, o_odd_ref, near_ref,
            mem0_ref, wphi_ref, phi_ref, wqkvb_ref, wob_ref, bo_ref, bq_ref, bkv_ref,
            kv_ref, z_ref, ot_ref, on_ref,
            w_sem, in_sem, out_sem, *, dh):
    n_seg, seg, d = x_ref.shape
    n_pairs = wp_ref.shape[0]
    n_mem = mem0_ref.shape[0]
    pw = 2 * dh
    n_iter = n_seg * seg // TB

    def w_copies(p, j):
        src = (wq_hbm, wk_hbm, wv_hbm, wo_hbm)[j]
        if j < 2:
            return [pltpu.make_async_copy(src.at[p], stage_ref.at[p % RING, 3 * j:3 * j + 3],
                                          w_sem.at[p, j])]
        return [pltpu.make_async_copy(src.at[p, i], stage_ref.at[p % RING, 3 * j:3 * j + 3, i],
                                      w_sem.at[p, 2 * j - 2 + i]) for i in range(2)]

    def start_w(p, *slots):
        for j in slots:
            for copy in w_copies(p, j):
                copy.start()

    def wait_w(p, *slots):
        for j in slots:
            for copy in w_copies(p, j):
                copy.wait()

    def prepare_in(u, tiles, live=True, pace=lambda t, b: b):
        g, i = u // 2, u % 2
        for t in tiles:
            cols = pl.ds(pl.multiple_of(128 * t, 128), 128)
            blocks = [stage_ref[p % RING, t, :, :, pl.ds(pl.multiple_of(c + i * 128, 128), 128)]
                      .reshape(128, 128)
                      for c in (0, HALF) for p in (2 * g, jnp.where(live, 2 * g + 1, 0))]
            for n, r in enumerate(_strassen_weights(*(pace(t, b) for b in blocks))):
                ws_ref[g, n, pl.ds(pl.multiple_of(i * 64, 64), 64), cols] = _pack(r.T)
            wp_ref[u, :, cols] = _pack(stage_ref[u % RING, t, :, :, 2 * HALF:].reshape(128, -1).T)

    def wait_out(u):
        for i in range(2):
            pltpu.make_async_copy(stage_ref.at[0, 9:12, 0], stage_ref.at[0, 9:12, 0],
                                  w_sem.at[u // 2 * 2 + i, 4 + u % 2]).wait()

    def prepare_out(u, live=True, pace=lambda t, b: b):
        g, i = u // 2, u % 2
        for t in range(3):
            parts = [pace(3 * t + 1, stage_ref[p % RING, jnp.where(live, 9, 3) + t, i])
                     for p in (2 * g, jnp.where(live, 2 * g + 1, 0))]
            blocks = [part[:, c:c + HALF] for part in parts for c in (0, HALF)]
            for n, r in enumerate(_strassen_weights(*blocks)):
                wos_ref[g, n, t, i] = _pack(r)
            for n, part in enumerate(parts):
                wop_ref[2 * g + n, t, i] = _pack(part[:, 2 * HALF:])

    def out_copy(it, i):
        part = _chunk_rows(y_ref, it, sum(O_ROWS[:i]), O_ROWS[i])
        return pltpu.make_async_copy(y_ref.at[part], out_hbm.at[part], out_sem.at[0])

    def x_copy(part, rows, sem):
        return pltpu.make_async_copy(x_hbm.at[part, rows, :], y_ref.at[part, rows, :], sem)

    head, tail = slice(0, seg - PRE), slice(seg - PRE, seg)
    xt_copy = x_copy(slice(None), tail, in_sem.at[0])
    wqkvb_copy = pltpu.make_async_copy(wqkvb_hbm, wqkvb_ref, in_sem.at[1])
    wphi_copy = pltpu.make_async_copy(wphi_hbm, wphi_ref, in_sem.at[5])
    mem0_copy = pltpu.make_async_copy(mem0_hbm, mem0_ref, in_sem.at[4])
    wob_copy = pltpu.make_async_copy(wob_hbm, wob_ref, in_sem.at[2])

    wphi_copy.start()
    xt_copy.start()
    start_w(0, 0, 1, 2)
    wphi_copy.wait()
    _expand_phi(wphi_ref, phi_ref)
    xt_copy.wait()

    xp_ref[...] = _layernorm(y_ref[:, tail, :].astype(F32).reshape(n_seg * PRE, d)).astype(BF16)

    mem0_copy.start()
    start_w(1, 0, 1, 2)

    def pre_project(p, carry):
        @pl.when(p + 2 < n_pairs)
        def _():
            start_w(jnp.minimum(p + 2, n_pairs - 1), 0, 1, 2)

        part = pl.ds(p * (n_seg // n_pairs), n_seg // n_pairs)
        x_copy(part, head, in_sem.at[3]).start()
        start_w(p, 3)

        @pl.when(p >= WO_LAG)
        def _():
            wait_out(jnp.maximum(p - WO_LAG, 0))

        wait_w(p, 0, 1, 2)
        kv = lax.dot_general(xp_ref[...], stage_ref[p % RING, 3:9].reshape(-1, d), NT,
                             preferred_element_type=F32)
        pre_ref[p] = kv

        def pace(t, block):
            c, r = divmod(t * PACE, xp_ref.shape[0])
            early = kv[r:r + block.shape[0], 128 * c:128 * (c + 1)].astype(BF16)
            return jnp.where(p < 0, _cols(*[early] * (block.shape[1] // 128)), block)

        prepare_in(jnp.maximum(p - 1, 0), range(9), p >= 1, pace)
        prepare_out(jnp.maximum(p - WO_LAG, 0), p >= WO_LAG, pace)
        return carry

    lax.fori_loop(0, n_pairs, pre_project, 0)

    @pl.loop(0, 3)
    def _(j):
        prepare_in(n_pairs - 1, [3 * j + i for i in range(3)])

    @pl.loop(n_pairs - WO_LAG, n_pairs)
    def _(u):
        wait_out(u)
        prepare_out(u)

    x_copy(slice(None), head, in_sem.at[3]).wait()

    wqkvb_copy.start()
    wob_copy.start()
    mem0_copy.wait()
    x_ref[0] = y_ref[0].astype(F32)

    def layer_a(layer, x_in, pre):
        step = functools.partial(
            _a_step, layer=layer, dh=dh, x_in=x_in, x_ref=x_ref, xb_ref=xb_ref, ws_ref=ws_ref,
            wp_ref=wp_ref, wos_ref=wos_ref, wop_ref=wop_ref, pre_ref=pre, ahead_ref=ahead_ref,
            o_refs=(o_even_ref, o_odd_ref), near_ref=near_ref)
        xn = [_layernorm(x_in[i].astype(F32)) for i in range(3)]
        o_odd_ref[...] = jnp.zeros(o_odd_ref.shape, F32)
        cols, per = (slice(0, 3 * pw), 1) if pre is None else (slice(0, pw), 2)

        @pl.loop(0, n_pairs // 2 // per)
        def _(j):
            for g in (j * per + i for i in range(per)):
                for i, product in enumerate((_left_product, _right_product)):
                    ahead_ref[2 * g + i, :, cols] = product(
                        xn[0][:, :HALF], xn[0][:, HALF:2 * HALF],
                        lambda a, n: jnp.dot(a.astype(BF16), _unpack(ws_ref[g, n, :, cols]),
                                             preferred_element_type=F32))

        def two_steps(it, carry):
            mem, *xn = carry
            shared = {}
            for i in range(2):
                mem, xn_next = step(2 * it + i, mem, xn, shared)
                xn = xn[1:] + [xn_next]
            return (mem, *xn)

        lax.fori_loop(0, n_seg // 2, two_steps, (mem0_ref[...].astype(F32), *xn))

    def finish_a(layer):
        a = [_cols(*(o_odd_ref[n_mem:, (2 * g + i) * pw:(2 * g + i + 1) * pw]
                     for g in range(n_pairs // 2))) for i in range(2)]
        y = _cols(*(product(*a, lambda t, n: jnp.dot(
            t.astype(BF16), _unpack(wos_ref[:, n].reshape(-1, HALF)), preferred_element_type=F32))
            for product in (_left_product, _right_product)))
        at = (n_seg - 1, slice(None), slice(0, 2 * HALF))
        x_ref[at] = jnp.where(layer == 0, y_ref[at].astype(F32), x_ref[at]) + y

    b_keys = functools.partial(_b_keys, x_ref=x_ref, xb_ref=xb_ref, bkv_ref=bkv_ref,
                               kv_ref=kv_ref, z_ref=z_ref)
    b_queries = functools.partial(_b_queries, x_ref=x_ref, xb_ref=xb_ref, y_ref=y_ref,
                                  bq_ref=bq_ref, bo_ref=bo_ref, kv_ref=kv_ref, z_ref=z_ref,
                                  ot_ref=ot_ref, on_ref=on_ref)

    def layer_pair(layer, carry):
        @pl.when(layer == 0)
        def _():
            layer_a(0, y_ref, pre_ref)

        @pl.when(layer == 0)
        def _():
            wqkvb_copy.wait()
            wob_copy.wait()
            _b_weights(wqkvb_ref, phi_ref, wob_ref, bq_ref, bkv_ref, bo_ref)

        @pl.when(layer == 1)
        def _():
            layer_a(1, x_ref, None)

        finish_a(layer)

        lax.fori_loop(0, n_iter, b_keys, 0)

        def queries(it, carry):
            def send(i):
                @pl.when(layer == 1)
                def _():
                    out_copy(it, i).start()

            b_queries(it, send)
            return carry

        lax.fori_loop(0, n_iter, queries, 0)

        return carry

    lax.fori_loop(0, 2, layer_pair, 0)
    pltpu.make_async_copy(y_ref, out_hbm, out_sem.at[0]).wait()


@functools.partial(jax.jit, static_argnames=("A_seg_len",))
def pallas_interleave_layers__memory_aug_recurrent_mem_tr__linear_kernel_hedgehog__prompt_kernel(
    A_x, A_mem0, A_Wq, A_Wk, A_Wv, A_Wo, A_seg_len, B_x, B_wqkv, B_w_phi, B_wo,
):
    del B_x
    batch, s_len, d = A_x.shape
    _, heads, dh = A_Wq.shape
    n_mem = A_mem0.shape[1]
    seg = int(A_seg_len)
    b_heads, b_dh, _ = B_w_phi.shape
    rows = n_mem + seg
    n_pairs = heads // 2
    gr = 2 * b_dh
    half = K_PAIRS * gr
    n_seg = s_len // seg
    assert batch == 1 and dh == 192 and heads == 4 * O_SPLITS[0][-1] and d == 2 * HALF + 128
    assert n_mem % 8 == 0 and seg % 16 == 0 and 128 % seg == 0 and 2 * rows <= 128
    assert s_len % TB == 0 and s_len > 3 * TB == 3 * sum(O_ROWS) and n_seg % n_pairs == 0
    assert b_heads * b_dh == d and b_dh % 8 == 4 and d % half == 0

    def head_major(w):
        return w.transpose(1, 2, 0)

    hbm = pl.BlockSpec(memory_space=pltpu.HBM)
    out = pl.pallas_call(
        functools.partial(_kernel, dh=dh),
        out_shape=jax.ShapeDtypeStruct((n_seg, seg, d), A_x.dtype),
        in_specs=[hbm] * 9,
        out_specs=hbm,
        scratch_shapes=[
            pltpu.VMEM((n_seg, seg, d), F32),
            pltpu.VMEM((n_seg, seg, d), BF16),
            pltpu.VMEM((n_seg, seg, d), BF16),
            pltpu.VMEM((n_seg * PRE, d), BF16),
            pltpu.VMEM((RING, 12, 2, 64, d), BF16),
            pltpu.VMEM((n_pairs, n_seg * PRE, 4 * dh), F32),
            pltpu.VMEM((n_pairs, seg, 6 * dh), F32),
            pltpu.VMEM((n_pairs // 2, 7, HALF // 2, 6 * dh), jnp.uint32),
            pltpu.VMEM((n_pairs, d // 2 - HALF, 6 * dh), jnp.uint32),
            pltpu.VMEM((n_pairs // 2, 7, 3, 2, 32, HALF), jnp.uint32),
            pltpu.VMEM((n_pairs, 3, 2, 32, d - 2 * HALF), jnp.uint32),
            pltpu.VMEM((rows, heads * dh), F32),
            pltpu.VMEM((rows, heads * dh), F32),
            pltpu.VMEM((n_pairs, n_mem + 16, 4 * dh), F32),
            pltpu.VMEM((n_mem, d), BF16),
            pltpu.VMEM((b_dh, b_dh, b_heads), BF16),
            pltpu.VMEM((d // (F_PAIRS * gr), F_PAIRS * gr // 2, 256), jnp.uint32),
            pltpu.VMEM(B_wqkv.shape, BF16),
            pltpu.VMEM(B_wo.shape, BF16),
            pltpu.VMEM((d // 2, d), jnp.uint32),
            pltpu.VMEM((d // 2, d), jnp.uint32),
            pltpu.VMEM((d // half, half, d), jnp.uint32),
            pltpu.VMEM((b_heads // 2, gr, 2 * gr), F32),
            pltpu.VMEM((b_heads // 2, 2 * gr, 128), F32),
            pltpu.VMEM((d // 2, TB), jnp.uint32),
            pltpu.VMEM((TB // 2, d), jnp.uint32),
            pltpu.SemaphoreType.DMA((n_pairs, 6)),
            pltpu.SemaphoreType.DMA((6,)),
            pltpu.SemaphoreType.DMA((1,)),
        ],
        compiler_params=pltpu.CompilerParams(vmem_limit_bytes=124 * 1024 * 1024),
    )(
        A_x.reshape(n_seg, seg, d), A_mem0.reshape(n_mem, d),
        head_major(A_Wq).reshape(n_pairs, 3, 2, 64, d),
        head_major(A_Wk).reshape(n_pairs, 3, 2, 64, d),
        head_major(A_Wv).reshape(n_pairs, 2, 3, 64, d), A_Wo.reshape(n_pairs, 2, 3, 64, d),
        B_wqkv, B_w_phi.transpose(1, 2, 0), B_wo,
    )
    return out.reshape(batch, s_len, d)
```

```python
import functools
import math

import jax
import jax.numpy as jnp
from jax import lax
import jax.experimental.pallas as pl
import jax.experimental.pallas.tpu as pltpu

F32 = jnp.float32
BF16 = jnp.bfloat16
NT = (((1,), (1,)), ((), ()))
LOG2E = math.log2(math.e)
MASKED = -1e9

ISSUE = ("kqSVv", "kqSVv")
LAG_S = (2, 1)
LAG_PV = (2, 3)
O_SPLITS = ((0, 1, 2, 3, 4, 5, 6, 8), (0, 1, 2, 3, 4, 6, 8))
VPU_ROWS = ((range(16), ()), (range(16), ()))
VPU_DUE = (3, 3)
KEYS_AHEAD = (13, 9)
NORM_DUE = ((0, 2), (2, 3))
HALF = 256
PACE = 256
P_ORDER = ((((1, 3), (2, 4)), ((1, 0, 6), (5,))),) * 2
O_ORDER = (((1, 3, 2, 4), (1, 0, 6, 5)), ((3, 2, 1, 4), (0, 6, 1, 5)))
A_SPLITS = (0, 1152)
RING = 8
PRE = 8
WO_LAG = 3
TB = 512
K_PAIRS = 8
Q_PAIRS = 8
F_PAIRS = 2
O_ROWS = (128, 128, 128, 128)


def _iota(shape, axis):
    return lax.broadcasted_iota(jnp.int32, shape, axis)


def _div(v, d):
    return (v * ((1 << 18) // d + 1)) >> 18


def _pack(x):
    return pltpu.bitcast(x.astype(BF16), jnp.uint32)


def _unpack(x):
    return pltpu.bitcast(x, BF16)


def _recip(x):
    r = pl.reciprocal(x, approx=True)
    return r * (2.0 - x * r)


def _layernorm(x):
    m = jnp.mean(x, axis=-1, keepdims=True)
    c = x - m
    v = jnp.mean(c * c, axis=-1, keepdims=True)
    return c * lax.rsqrt(v + 1e-5)


def _rows(*parts):
    return jnp.concatenate(parts, axis=0)


def _cols(*parts):
    return jnp.concatenate(parts, axis=1)


def _strassen_weights(b11, b12, b21, b22):
    f11, f12, f21, f22 = (b.astype(F32) for b in (b11, b12, b21, b22))
    return [r.astype(BF16)
            for r in (f11 + f22, b11, f12 - f22, f21 - f11, b22, f11 + f12, f21 + f22)]


def _left_product(a1, a2, times):
    return times(a2, 3) + times(a1 + a2, 1)


def _right_product(a1, a2, times):
    return times(a1 + a2, 4) + times(a1, 2)


def _token_operands(a1, a2, b1, b2):
    low = b1 + b2
    n = low.shape[0] // 2
    return ({3: b2, 2: a1, 1: low[:n], 4: a1 + a2},
            {0: a1 + b2, 6: a2 - b2, 1: low[n:], 5: b1 - a1})


def _memory_operands(m1, m2):
    both = m1 + m2
    return {0: m2, 1: both, 2: m1, 3: m2, 4: both, 5: m1, 6: m2}


def _first_results(p, n):
    m1 = _rows(p[1][n:], jnp.zeros_like(p[1][n:]))
    return ((p[1][:n] + p[3][:n], p[2][:n] + p[4][:n]),
            (p[2][n:] + p[4][n:], p[3][n:] - p[4][n:], p[3][n:] + m1, p[2][n:] - m1))


def _second_left(p, n, c11, c21):
    m1 = _rows(jnp.zeros_like(p[1][n:]), p[1][n:])
    return p[1][:n] + p[6][:n] - p[0][:n], c11 + p[0][n:] + p[6][n:], c21 + m1


def _second_right(p, n, c22):
    m1 = _rows(jnp.zeros_like(p[1][n:]), p[1][n:])
    return p[5][:n] + p[0][:n] - p[1][:n], c22 + p[0][n:] + p[5][n:] - m1


def _a_step(s, mem, xn, shared, *, layer, dh, x_in, x_ref, xb_ref, ws_ref, wp_ref, wos_ref,
            wop_ref, pre_ref, ahead_ref, o_refs, near_ref):
    odd = bool(shared)
    n_mem, seg = mem.shape[0], xn[0].shape[0]
    n_seg = xb_ref.shape[0]
    rows = n_mem + seg
    pw = 2 * dh
    n_pairs = wp_ref.shape[0]
    o_ref = o_refs[odd]
    scale = dh ** -0.5

    def after(early, value):
        return value if early is None else jnp.where(s < 0, early[:, :value.shape[1]], value)

    def after_all(early, value):
        t = functools.reduce(jnp.maximum, [early[i:i + 8, j:j + 128]
                                           for i in range(0, early.shape[0], 8)
                                           for j in range(0, early.shape[1], 128)])
        return jnp.concatenate([after(t, value[0:8]), value[8:]], axis=0)

    def slow_norm(x):
        outs = [None, None]
        for i in range(0, seg, 8):
            outs.append(_layernorm(after(outs[-2], x[i:i + 8])))
        return jnp.concatenate(outs[2:], axis=0)

    xn_next = slow_norm(x_in[jnp.minimum(s + len(xn), n_seg - 1)].astype(F32))
    done = jnp.maximum(s - 3, 0)
    xb_done = slow_norm(x_ref[done])
    xb_ref[done] = xb_done.astype(BF16)

    h = _rows(mem, xn[0])

    first = _iota((rows, 128), 1) < 64
    zero = jnp.zeros((rows, 128), F32)

    def key_blocks(t):
        t0, t1, t2 = t[:, 0:128], t[:, 128:256], t[:, 256:384]
        top = jnp.concatenate([t0, jnp.where(first, t1, 0.0), zero], axis=1)
        bot = jnp.concatenate([zero, jnp.where(first, 0.0, t1), t2], axis=1)
        return jnp.concatenate([top, bot], axis=0).astype(BF16)

    def value_blocks(t):
        mine = jnp.concatenate([first] * 3, axis=1)
        return jnp.concatenate(
            [jnp.where(mine, t, 0.0), jnp.where(mine, 0.0, t)], axis=0).astype(BF16)

    def vpu_rows(p):
        return [n_mem + 8 * i for i, pairs in enumerate(VPU_ROWS[layer]) if p in pairs]

    def mxu_rows(p):
        return [r for r in range(0, rows, 8) if r not in vpu_rows(p)]

    def pick(t, starts):
        return jnp.concatenate([t[r:r + 8] for r in starts], axis=0)

    q, k, v, probs, near_done = {}, {}, {}, {}, {}

    def project_short(p, j):
        def dot(a, w):
            return jnp.dot(a.astype(BF16), _unpack(w), preferred_element_type=F32)

        cols, top = slice(j * pw, (j + 1) * pw), h[:rows - PRE]
        most = (_left_product, _right_product)[p % 2](
            top[:, :HALF], top[:, HALF:2 * HALF], lambda a, i: dot(a, ws_ref[p // 2, i, :, cols]))
        return _rows(dot(top[:, 2 * HALF:], wp_ref[p, :, cols]) + most,
                     pre_ref[p, pl.ds(pl.multiple_of(s * PRE, PRE), PRE), (j - 1) * pw:j * pw])

    if not odd:
        shared["in"] = _token_operands(*(t[:, c:c + HALF] for t in xn[1:3] for c in (0, HALF)))
    m_in = _memory_operands(mem[:, :HALF], mem[:, HALF:2 * HALF])
    lhs_in = {i: _rows(m_in[i], t) for i, t in shared["in"][odd].items()}
    products = {}

    def project_shared(p, lo, hi):
        g, right = divmod(p, 2)
        cols, prod = slice(lo, hi), products.setdefault(lo, {})
        for i in P_ORDER[layer][odd][right]:
            prod[i] = jnp.dot(lhs_in[i], _unpack(ws_ref[g, i, :, cols]),
                              preferred_element_type=F32)
        if not odd:
            tokens = ahead_ref[p, :, cols]
            if right:
                (_, m), shared[g, lo] = _first_results(prod, n_mem)
            else:
                m = prod[1][:n_mem] + prod[3][:n_mem]
        elif right:
            tokens = shared[g, lo][0]
            m, ahead_ref[p, :, cols] = _second_right(prod, n_mem, shared[g, lo][3])
        else:
            m, tokens, ahead_ref[p, :, cols] = _second_left(prod, n_mem, *shared[g, lo][1:3])
        return jnp.dot(h[:, 2 * HALF:], _unpack(wp_ref[p, :, cols]),
                       preferred_element_type=F32) + _rows(m, tokens)

    def scores(p):
        col = pick(_iota((rows, 2 * rows), 1), mxu_rows(p))
        row = pick(_iota((rows, 2 * rows), 0), mxu_rows(p))
        is_a = col < rows
        visible = (row < n_mem) | (row >= jnp.where(is_a, col, col - rows))
        sc = lax.dot_general(pick(q[p], mxu_rows(p)), key_blocks(k[p]), NT,
                             preferred_element_type=F32)
        sc = jnp.where(visible, sc * scale, MASKED)
        max_a = jnp.max(jnp.where(is_a, sc, -jnp.inf), axis=1, keepdims=True)
        max_b = jnp.max(jnp.where(is_a, -jnp.inf, sc), axis=1, keepdims=True)
        e = jnp.exp(sc - jnp.where(is_a, max_a, max_b))
        sum_a = jnp.sum(jnp.where(is_a, e, 0.0), axis=1, keepdims=True)
        sum_b = jnp.sum(jnp.where(is_a, 0.0, e), axis=1, keepdims=True)
        probs[p] = e * _recip(jnp.where(is_a, sum_a, sum_b))
        if p == NORM_DUE[layer][0]:
            probs[p] = after_all(xn_next, probs[p])
        if p == NORM_DUE[layer][1]:
            probs[p] = after_all(xb_done, probs[p])
        if p - VPU_DUE[layer] in near_done:
            probs[p] = after_all(near_done[p - VPU_DUE[layer]], probs[p])

    def values(p):
        o = jnp.dot(probs[p], value_blocks(v[p]), preferred_element_type=F32)
        for i, r in enumerate(mxu_rows(p)):
            o_ref[r:r + 8, p * pw:(p + 1) * pw] = o[8 * i:8 * i + 8]

    chain = [None, None]
    scored = [None] * KEYS_AHEAD[layer]

    def attend_on_vpu(p, r):
        def key_row(j, i):
            return jnp.broadcast_to(near_ref[p, j:j + 1, 128 * i:128 * (i + 1)], (8, 128))

        half, sub = first[0:8], _iota((8, 128), 0)
        t = q[p][r:r + 8] * (scale * LOG2E)
        q0, q2 = t[:, 0:128], t[:, 256:384]
        q1a, q1b = jnp.where(half, t[:, 128:256], 0.0), jnp.where(half, 0.0, t[:, 128:256])
        for j in range(r + 8):
            ready = after(scored[-KEYS_AHEAD[layer]], chain[0])
            k1 = after(ready, key_row(j, 1))
            dot_a = q0 * after(ready, key_row(j, 0)) + q1a * k1
            dot_b = q2 * after(dot_a, key_row(j, 2)) + q1b * k1
            t = jnp.where(half, jnp.sum(dot_a, axis=1, keepdims=True),
                          jnp.sum(dot_b, axis=1, keepdims=True))
            scored.append(t if j <= r else jnp.where(sub >= j - r, t, MASKED * LOG2E))
            chain[0] = dot_b
        sc = scored[-(r + 8):]
        top = functools.reduce(jnp.maximum, sc)
        for j in range(r + 8):
            e = jnp.exp2(sc[j] - after(chain[1], top))
            weight = after(chain[1], e)
            terms = [weight * key_row(j, 3 + i) for i in range(3)]
            total = e if j == 0 else total + e
            acc = terms if j == 0 else [a + b for a, b in zip(acc, terms)]
            chain[1] = acc[2]
        inv = _recip(total)
        o_ref[r:r + 8, p * pw:(p + 1) * pw] = jnp.concatenate([a * inv for a in acc], axis=1)
        near_done[p] = acc[2]

    def attend_early_rows(p):
        if vpu_rows(p):
            n = vpu_rows(p)[-1] + 8
            near_ref[p, 0:n, 0:pw] = k[p][0:n]
            near_ref[p, 0:n, pw:2 * pw] = v[p][0:n]
        for r in reversed(vpu_rows(p)):
            attend_on_vpu(p, r)

    out = {}

    def project_out(g0, g1):
        def halves(ref, lo, hi):
            return [_cols(*(ref[lo:hi, (2 * g + i) * pw:(2 * g + i + 1) * pw]
                            for g in range(g0, g1))) for i in range(2)]

        if not odd:
            shared["out", g0] = _token_operands(*halves(o_refs[0], n_mem, rows),
                                                *halves(o_refs[1], n_mem, rows))
        m = _memory_operands(*halves(o_ref, 0, n_mem))
        for i in O_ORDER[layer][odd]:
            r = jnp.dot(_rows(m[i], shared["out", g0][odd][i]), _unpack(wos_ref[g0:g1, i].reshape(-1, HALF)),
                        preferred_element_type=F32)
            out[i] = r + out[i] if i in out else r

    lag_s, lag_v = LAG_S[layer], LAG_S[layer] + LAG_PV[layer]
    todo = list(zip(O_SPLITS[layer][:-1], O_SPLITS[layer][1:]))
    for t in range(n_pairs + lag_v):
        if t >= n_pairs:
            project_out(*todo.pop(0))
        for c in ISSUE[layer]:
            if c == "S" and 0 <= t - lag_s < n_pairs:
                scores(t - lag_s)
            elif c == "V" and 0 <= t - lag_v < n_pairs:
                values(t - lag_v)
            elif c == "a" and t < n_pairs:
                r = _cols(*(project_shared(t, lo, hi) for lo, hi in zip(A_SPLITS, A_SPLITS[1:])))
                q[t], k[t], v[t] = r[:, 0:pw], r[:, pw:2 * pw], r[:, 2 * pw:3 * pw]
            elif c in "qkv" and t < n_pairs:
                j = "qkv".index(c)
                (q, k, v)[j][t] = (project_short(t, j) if j and pre_ref is not None
                                   else project_shared(t, j * pw, (j + 1) * pw))
        if t < n_pairs:
            attend_early_rows(t)
    for part in todo:
        project_out(*part)
    rest = jnp.dot(o_ref[...], _unpack(wop_ref[...].reshape(-1, wop_ref.shape[-1])),
                   preferred_element_type=F32)

    most, tail = slice(0, 2 * HALF), slice(2 * HALF, None)
    x_ref[s, :, tail] = x_in[s, :, tail].astype(F32) + rest[n_mem:]
    if odd:
        c12, c11, c21, c22 = shared["out"]
        m1, c11, c21 = _second_left(out, n_mem, c11, c21)
        m2, c22 = _second_right(out, n_mem, c22)
        x_ref[s - 1, :, most] = x_in[s - 1, :, most].astype(F32) + _cols(c11, c12)
        back = jnp.maximum(s - 2, 1)
        x_ref[back, :, most] = (x_in[back, :, most].astype(F32)
                                + jnp.where(s > 1, _cols(c21, c22), 0.0))
    else:
        (m1, m2), shared["out"] = _first_results(out, n_mem)
    return _cols(m1, m2, rest[:n_mem]), xn_next


def _pair_reduce(t, op):
    r = t[0:8]
    for i in range(8, t.shape[0], 8):
        r = op(r, t[i:i + 8])
    r = op(r, pltpu.roll(r, 4, 0))
    return op(r, pltpu.roll(r, 2, 0))


def _tile_rows(r, n):
    return jnp.concatenate([r] * (n // 8), axis=0)


def _feature_map(p):
    n = p.shape[0]
    e_pos = jnp.exp2(p - _tile_rows(_pair_reduce(p, jnp.maximum), n))
    e_neg = jnp.exp2(_tile_rows(_pair_reduce(p, jnp.minimum), n) - p)
    inv_pos = _recip(_pair_reduce(e_pos, jnp.add))
    inv_neg = _recip(_pair_reduce(e_neg, jnp.add))
    return jnp.concatenate(
        [e_pos * _tile_rows(inv_pos, n), e_neg * _tile_rows(inv_neg, n)], axis=0)


def _fold_span(b, blk):
    return b * blk // 128 * 128, -(-(b + 1) * blk // 128) * 128


def _expand_phi(wphi_ref, phi_ref):
    dh, _, heads = wphi_ref.shape
    d = dh * heads
    gr = 2 * dh
    c = _iota((dh, d), 1)
    c_feat = c - _div(c, dh) * dh
    spread = (_div(_iota((heads, d), 1), dh) == _iota((heads, d), 0)).astype(BF16)

    def gather(j, by_feat):
        for e in (j * (dh // 4) + i for i in range(dh // 4)):
            t = jnp.dot(wphi_ref[e], spread, preferred_element_type=F32)
            by_feat = jnp.where(c_feat == e, t, by_feat)
        return by_feat

    by_feat = lax.fori_loop(0, 4, gather, jnp.zeros((dh, d), F32)).astype(BF16)
    blk = F_PAIRS * gr
    r = _iota((blk, dh), 0)
    sel = (((r - _div(r, gr) * gr) >> 1) == _iota((blk, dh), 1)).astype(BF16)
    for b in range(d // blk):
        lo, hi = _fold_span(b, blk)
        r = _iota((blk, hi - lo), 0)
        head = 2 * (_div(r, gr) + b * F_PAIRS) + (r & 1)
        phi = jnp.dot(sel, by_feat[:, lo:hi], preferred_element_type=F32)
        phi_ref[b, :, 0:hi - lo] = _pack(
            jnp.where(_div(_iota((1, hi - lo), 1) + lo, dh) == head, phi, 0.0))


def _b_weights(wqkv_ref, phi_ref, wob_ref, bq_ref, bkv_ref, bo_ref):
    d = wqkv_ref.shape[0]
    blk = 2 * phi_ref.shape[1]
    half = bkv_ref.shape[1]
    bo_ref[...] = _pack(wob_ref[...])
    wv = wqkv_ref[:, 2 * d:3 * d].T
    for b in range(d // half):
        bkv_ref[b, half // 2:half, :] = _pack(wv[b * half:(b + 1) * half])
    for b in range(d // blk):
        lo, hi = _fold_span(b, blk)
        phi = _unpack(phi_ref[b, :, 0:hi - lo])
        wq = lax.dot_general(phi, wqkv_ref[:, lo:hi], NT, preferred_element_type=F32)
        wk = lax.dot_general(phi, wqkv_ref[:, d + lo:d + hi], NT, preferred_element_type=F32)
        bq_ref[b * blk // 2:(b + 1) * blk // 2, :] = _pack(wq * LOG2E)
        at = b * blk % half // 2
        bkv_ref[b * blk // half, at:at + blk // 2, :] = _pack(wk * LOG2E)


def _chunk_rows(ref, it, r0, n):
    seg = ref.shape[1]
    return pl.ds(it * (TB // seg) + r0 // seg, n // seg)


def _b_keys(it, carry, *, x_ref, xb_ref, bkv_ref, kv_ref, z_ref):
    n_blk, half, _ = bkv_ref.shape
    gr = half // K_PAIRS
    xb = xb_ref[_chunk_rows(xb_ref, it, 0, TB)].reshape(TB, -1)
    last = x_ref.shape[0] - 1 - jnp.minimum(it, 2)
    xb_ref[last] = _layernorm(x_ref[last]).astype(BF16)
    same_head = (_iota((gr, 2 * gr), 0) >= gr // 2) == ((_iota((gr, 2 * gr), 1) & 1) == 1)

    def accumulate(b, t):
        for i in range(K_PAIRS):
            g = b * K_PAIRS + i
            phi = _feature_map(t[i * gr:(i + 1) * gr])
            z_ref[g] = jnp.where(it > 0, z_ref[g], 0.0) + jnp.sum(phi, axis=1, keepdims=True)
            kv = lax.dot_general(t[half + i * gr:half + (i + 1) * gr], phi.astype(BF16), NT,
                                 preferred_element_type=F32)
            kv_ref[g] = jnp.where(it > 0, kv_ref[g], 0.0) + jnp.where(same_head, kv, 0.0)

    pending = None
    for b in range(n_blk):
        t = lax.dot_general(_unpack(bkv_ref[b]), xb, NT, preferred_element_type=F32)
        if pending is not None:
            accumulate(*pending)
        pending = (b, t)
    accumulate(*pending)
    return carry


def _b_queries(it, send, *, x_ref, xb_ref, y_ref, bq_ref, bo_ref, kv_ref, z_ref, ot_ref, on_ref):
    n_groups, gr, _ = kv_ref.shape
    blk = Q_PAIRS * gr
    sub = _iota((8, TB), 0)
    xb = xb_ref[_chunk_rows(xb_ref, it, 0, TB)].reshape(TB, -1)

    def attend(b, t):
        outs = []
        for i in range(Q_PAIRS):
            g = b * Q_PAIRS + i
            phi = _feature_map(t[i * gr:(i + 1) * gr])
            num = jnp.dot(kv_ref[g], phi.astype(BF16), preferred_element_type=F32)
            z = jnp.concatenate([z_ref[g]] * (TB // 128), axis=1)
            inv = _recip(_pair_reduce(phi * z, jnp.add) + 1e-6)
            other = pltpu.roll(inv, 1, 0)
            inv_a = jnp.where((sub & 1) == 0, inv, other)
            inv_b = jnp.where((sub & 1) == 0, other, inv)
            n = (gr - 8) // 16
            inv = jnp.concatenate(
                [inv_a] * n + [jnp.where(sub < 4, inv_a, inv_b)] + [inv_b] * n, axis=0)
            outs.append(num * inv)
        ot_ref[b * blk // 2:(b + 1) * blk // 2, :] = _pack(jnp.concatenate(outs, axis=0))

    n_blk = n_groups // Q_PAIRS
    proj = {}
    for b in range(n_blk + 1):
        if b < n_blk:
            proj[b] = lax.dot_general(_unpack(bq_ref[b * blk // 2:(b + 1) * blk // 2, :]), xb,
                                      NT, preferred_element_type=F32)
        if b > 0:
            attend(b - 1, proj[b - 1])
    on_ref[...] = _pack(_unpack(ot_ref[...]).T)
    r0 = 0
    for i, n in enumerate(O_ROWS):
        at = _chunk_rows(x_ref, it, r0, n)
        y = jnp.dot(_unpack(on_ref[r0 // 2:(r0 + n) // 2, :]), _unpack(bo_ref[...]),
                    preferred_element_type=F32)
        x = x_ref[at] + y.reshape((-1,) + x_ref.shape[1:])
        x_ref[at] = x
        y_ref[at] = x.astype(BF16)
        send(i)
        r0 += n


def _kernel(x_hbm, mem0_hbm, wq_hbm, wk_hbm, wv_hbm, wo_hbm, wqkvb_hbm, wphi_hbm, wob_hbm,
            out_hbm,
            x_ref, xb_ref, y_ref, xp_ref, stage_ref, pre_ref, ahead_ref,
            ws_ref, wp_ref, wos_ref, wop_ref, o_even_ref, o_odd_ref, near_ref,
            mem0_ref, wphi_ref, phi_ref, wqkvb_ref, wob_ref, bo_ref, bq_ref, bkv_ref,
            kv_ref, z_ref, ot_ref, on_ref,
            w_sem, in_sem, out_sem, *, dh):
    n_seg, seg, d = x_ref.shape
    n_pairs = wp_ref.shape[0]
    n_mem = mem0_ref.shape[0]
    pw = 2 * dh
    n_iter = n_seg * seg // TB

    def w_copies(p, j):
        src = (wq_hbm, wk_hbm, wv_hbm, wo_hbm)[j]
        if j < 2:
            return [pltpu.make_async_copy(src.at[p], stage_ref.at[p % RING, 3 * j:3 * j + 3],
                                          w_sem.at[p, j])]
        return [pltpu.make_async_copy(src.at[p, i], stage_ref.at[p % RING, 3 * j:3 * j + 3, i],
                                      w_sem.at[p, 2 * j - 2 + i]) for i in range(2)]

    def start_w(p, *slots):
        for j in slots:
            for copy in w_copies(p, j):
                copy.start()

    def wait_w(p, *slots):
        for j in slots:
            for copy in w_copies(p, j):
                copy.wait()

    def prepare_in(u, tiles, live=True, pace=lambda t, b: b):
        g, i = u // 2, u % 2
        for t in tiles:
            cols = pl.ds(pl.multiple_of(128 * t, 128), 128)
            blocks = [stage_ref[p % RING, t, :, :, pl.ds(pl.multiple_of(c + i * 128, 128), 128)]
                      .reshape(128, 128)
                      for c in (0, HALF) for p in (2 * g, jnp.where(live, 2 * g + 1, 0))]
            for n, r in enumerate(_strassen_weights(*(pace(t, b) for b in blocks))):
                ws_ref[g, n, pl.ds(pl.multiple_of(i * 64, 64), 64), cols] = _pack(r.T)
            wp_ref[u, :, cols] = _pack(stage_ref[u % RING, t, :, :, 2 * HALF:].reshape(128, -1).T)

    def wait_out(u):
        for i in range(2):
            pltpu.make_async_copy(stage_ref.at[0, 9:12, 0], stage_ref.at[0, 9:12, 0],
                                  w_sem.at[u // 2 * 2 + i, 4 + u % 2]).wait()

    def prepare_out(u, live=True, pace=lambda t, b: b):
        g, i = u // 2, u % 2
        for t in range(3):
            parts = [pace(3 * t + 1, stage_ref[p % RING, jnp.where(live, 9, 3) + t, i])
                     for p in (2 * g, jnp.where(live, 2 * g + 1, 0))]
            blocks = [part[:, c:c + HALF] for part in parts for c in (0, HALF)]
            for n, r in enumerate(_strassen_weights(*blocks)):
                wos_ref[g, n, t, i] = _pack(r)
            for n, part in enumerate(parts):
                wop_ref[2 * g + n, t, i] = _pack(part[:, 2 * HALF:])

    def out_copy(it, i):
        part = _chunk_rows(y_ref, it, sum(O_ROWS[:i]), O_ROWS[i])
        return pltpu.make_async_copy(y_ref.at[part], out_hbm.at[part], out_sem.at[0])

    def x_copy(part, rows, sem):
        return pltpu.make_async_copy(x_hbm.at[part, rows, :], y_ref.at[part, rows, :], sem)

    head, tail = slice(0, seg - PRE), slice(seg - PRE, seg)
    xt_copy = x_copy(slice(None), tail, in_sem.at[0])
    wqkvb_copy = pltpu.make_async_copy(wqkvb_hbm, wqkvb_ref, in_sem.at[1])
    wphi_copy = pltpu.make_async_copy(wphi_hbm, wphi_ref, in_sem.at[5])
    mem0_copy = pltpu.make_async_copy(mem0_hbm, mem0_ref, in_sem.at[4])
    wob_copy = pltpu.make_async_copy(wob_hbm, wob_ref, in_sem.at[2])

    wphi_copy.start()
    xt_copy.start()
    start_w(0, 0, 1, 2)
    wphi_copy.wait()
    _expand_phi(wphi_ref, phi_ref)
    xt_copy.wait()

    xp_ref[...] = _layernorm(y_ref[:, tail, :].astype(F32).reshape(n_seg * PRE, d)).astype(BF16)

    mem0_copy.start()
    start_w(1, 0, 1, 2)

    def pre_project(p, carry):
        @pl.when(p + 2 < n_pairs)
        def _():
            start_w(jnp.minimum(p + 2, n_pairs - 1), 0, 1, 2)

        part = pl.ds(p * (n_seg // n_pairs), n_seg // n_pairs)
        x_copy(part, head, in_sem.at[3]).start()
        start_w(p, 3)

        @pl.when(p >= WO_LAG)
        def _():
            wait_out(jnp.maximum(p - WO_LAG, 0))

        wait_w(p, 0, 1, 2)
        kv = lax.dot_general(xp_ref[...], stage_ref[p % RING, 3:9].reshape(-1, d), NT,
                             preferred_element_type=F32)
        pre_ref[p] = kv

        def pace(t, block):
            c, r = divmod(t * PACE, xp_ref.shape[0])
            early = kv[r:r + block.shape[0], 128 * c:128 * (c + 1)].astype(BF16)
            return jnp.where(p < 0, _cols(*[early] * (block.shape[1] // 128)), block)

        prepare_in(jnp.maximum(p - 1, 0), range(9), p >= 1, pace)
        prepare_out(jnp.maximum(p - WO_LAG, 0), p >= WO_LAG, pace)
        return carry

    lax.fori_loop(0, n_pairs, pre_project, 0)

    @pl.loop(0, 3)
    def _(j):
        prepare_in(n_pairs - 1, [3 * j + i for i in range(3)])

    @pl.loop(n_pairs - WO_LAG, n_pairs)
    def _(u):
        wait_out(u)
        prepare_out(u)

    x_copy(slice(None), head, in_sem.at[3]).wait()

    wqkvb_copy.start()
    wob_copy.start()
    mem0_copy.wait()
    x_ref[0] = y_ref[0].astype(F32)

    def layer_a(layer, x_in, pre):
        step = functools.partial(
            _a_step, layer=layer, dh=dh, x_in=x_in, x_ref=x_ref, xb_ref=xb_ref, ws_ref=ws_ref,
            wp_ref=wp_ref, wos_ref=wos_ref, wop_ref=wop_ref, pre_ref=pre, ahead_ref=ahead_ref,
            o_refs=(o_even_ref, o_odd_ref), near_ref=near_ref)
        xn = [_layernorm(x_in[i].astype(F32)) for i in range(3)]
        o_odd_ref[...] = jnp.zeros(o_odd_ref.shape, F32)
        cols, per = (slice(0, 3 * pw), 1) if pre is None else (slice(0, pw), 2)

        @pl.loop(0, n_pairs // 2 // per)
        def _(j):
            for g in (j * per + i for i in range(per)):
                for i, product in enumerate((_left_product, _right_product)):
                    ahead_ref[2 * g + i, :, cols] = product(
                        xn[0][:, :HALF], xn[0][:, HALF:2 * HALF],
                        lambda a, n: jnp.dot(a.astype(BF16), _unpack(ws_ref[g, n, :, cols]),
                                             preferred_element_type=F32))

        def two_steps(it, carry):
            mem, *xn = carry
            shared = {}
            for i in range(2):
                mem, xn_next = step(2 * it + i, mem, xn, shared)
                xn = xn[1:] + [xn_next]
            return (mem, *xn)

        lax.fori_loop(0, n_seg // 2, two_steps, (mem0_ref[...].astype(F32), *xn))

    def finish_a(layer):
        a = [_cols(*(o_odd_ref[n_mem:, (2 * g + i) * pw:(2 * g + i + 1) * pw]
                     for g in range(n_pairs // 2))) for i in range(2)]
        y = _cols(*(product(*a, lambda t, n: jnp.dot(
            t.astype(BF16), _unpack(wos_ref[:, n].reshape(-1, HALF)), preferred_element_type=F32))
            for product in (_left_product, _right_product)))
        at = (n_seg - 1, slice(None), slice(0, 2 * HALF))
        x_ref[at] = jnp.where(layer == 0, y_ref[at].astype(F32), x_ref[at]) + y

    b_keys = functools.partial(_b_keys, x_ref=x_ref, xb_ref=xb_ref, bkv_ref=bkv_ref,
                               kv_ref=kv_ref, z_ref=z_ref)
    b_queries = functools.partial(_b_queries, x_ref=x_ref, xb_ref=xb_ref, y_ref=y_ref,
                                  bq_ref=bq_ref, bo_ref=bo_ref, kv_ref=kv_ref, z_ref=z_ref,
                                  ot_ref=ot_ref, on_ref=on_ref)

    def layer_pair(layer, carry):
        @pl.when(layer == 0)
        def _():
            layer_a(0, y_ref, pre_ref)

        @pl.when(layer == 0)
        def _():
            wqkvb_copy.wait()
            wob_copy.wait()
            _b_weights(wqkvb_ref, phi_ref, wob_ref, bq_ref, bkv_ref, bo_ref)

        @pl.when(layer == 1)
        def _():
            layer_a(1, x_ref, None)

        finish_a(layer)

        lax.fori_loop(0, n_iter, b_keys, 0)

        def queries(it, carry):
            def send(i):
                @pl.when(layer == 1)
                def _():
                    out_copy(it, i).start()

            b_queries(it, send)
            return carry

        lax.fori_loop(0, n_iter, queries, 0)

        return carry

    lax.fori_loop(0, 2, layer_pair, 0)
    pltpu.make_async_copy(y_ref, out_hbm, out_sem.at[0]).wait()


@functools.partial(jax.jit, static_argnames=("A_seg_len",))
def pallas_interleave_layers__memory_aug_recurrent_mem_tr__linear_kernel_hedgehog__prompt_kernel(
    A_x, A_mem0, A_Wq, A_Wk, A_Wv, A_Wo, A_seg_len, B_x, B_wqkv, B_w_phi, B_wo,
):
    del B_x
    batch, s_len, d = A_x.shape
    _, heads, dh = A_Wq.shape
    n_mem = A_mem0.shape[1]
    seg = int(A_seg_len)
    b_heads, b_dh, _ = B_w_phi.shape
    rows = n_mem + seg
    n_pairs = heads // 2
    gr = 2 * b_dh
    half = K_PAIRS * gr
    n_seg = s_len // seg
    assert batch == 1 and dh == 192 and heads == 4 * O_SPLITS[0][-1] and d == 2 * HALF + 128
    assert n_mem % 8 == 0 and seg % 16 == 0 and 128 % seg == 0 and 2 * rows <= 128
    assert s_len % TB == 0 and s_len > 3 * TB == 3 * sum(O_ROWS) and n_seg % n_pairs == 0
    assert b_heads * b_dh == d and b_dh % 8 == 4 and d % half == 0

    def head_major(w):
        return w.transpose(1, 2, 0)

    hbm = pl.BlockSpec(memory_space=pltpu.HBM)
    out = pl.pallas_call(
        functools.partial(_kernel, dh=dh),
        out_shape=jax.ShapeDtypeStruct((n_seg, seg, d), A_x.dtype),
        in_specs=[hbm] * 9,
        out_specs=hbm,
        scratch_shapes=[
            pltpu.VMEM((n_seg, seg, d), F32),
            pltpu.VMEM((n_seg, seg, d), BF16),
            pltpu.VMEM((n_seg, seg, d), BF16),
            pltpu.VMEM((n_seg * PRE, d), BF16),
            pltpu.VMEM((RING, 12, 2, 64, d), BF16),
            pltpu.VMEM((n_pairs, n_seg * PRE, 4 * dh), F32),
            pltpu.VMEM((n_pairs, seg, 6 * dh), F32),
            pltpu.VMEM((n_pairs // 2, 7, HALF // 2, 6 * dh), jnp.uint32),
            pltpu.VMEM((n_pairs, d // 2 - HALF, 6 * dh), jnp.uint32),
            pltpu.VMEM((n_pairs // 2, 7, 3, 2, 32, HALF), jnp.uint32),
            pltpu.VMEM((n_pairs, 3, 2, 32, d - 2 * HALF), jnp.uint32),
            pltpu.VMEM((rows, heads * dh), F32),
            pltpu.VMEM((rows, heads * dh), F32),
            pltpu.VMEM((n_pairs, n_mem + 16, 4 * dh), F32),
            pltpu.VMEM((n_mem, d), BF16),
            pltpu.VMEM((b_dh, b_dh, b_heads), BF16),
            pltpu.VMEM((d // (F_PAIRS * gr), F_PAIRS * gr // 2, 256), jnp.uint32),
            pltpu.VMEM(B_wqkv.shape, BF16),
            pltpu.VMEM(B_wo.shape, BF16),
            pltpu.VMEM((d // 2, d), jnp.uint32),
            pltpu.VMEM((d // 2, d), jnp.uint32),
            pltpu.VMEM((d // half, half, d), jnp.uint32),
            pltpu.VMEM((b_heads // 2, gr, 2 * gr), F32),
            pltpu.VMEM((b_heads // 2, 2 * gr, 128), F32),
            pltpu.VMEM((d // 2, TB), jnp.uint32),
            pltpu.VMEM((TB // 2, d), jnp.uint32),
            pltpu.SemaphoreType.DMA((n_pairs, 6)),
            pltpu.SemaphoreType.DMA((6,)),
            pltpu.SemaphoreType.DMA((1,)),
        ],
        compiler_params=pltpu.CompilerParams(vmem_limit_bytes=124 * 1024 * 1024),
    )(
        A_x.reshape(n_seg, seg, d), A_mem0.reshape(n_mem, d),
        head_major(A_Wq).reshape(n_pairs, 3, 2, 64, d),
        head_major(A_Wk).reshape(n_pairs, 3, 2, 64, d),
        head_major(A_Wv).reshape(n_pairs, 2, 3, 64, d), A_Wo.reshape(n_pairs, 2, 3, 64, d),
        B_wqkv, B_w_phi.transpose(1, 2, 0), B_wo,
    )
    return out.reshape(batch, s_len, d)
```

```python
import functools
import math

import jax
import jax.numpy as jnp
from jax import lax
import jax.experimental.pallas as pl
import jax.experimental.pallas.tpu as pltpu

F32 = jnp.float32
BF16 = jnp.bfloat16
NT = (((1,), (1,)), ((), ()))
LOG2E = math.log2(math.e)
MASKED = -1e9

ISSUE = ("kqSVv", "qkVSv")
LAG_S = (2, 1)
LAG_PV = (2, 3)
O_SPLITS = ((0, 1, 2, 3, 4, 5, 6, 8), (0, 1, 2, 3, 4, 6, 8))
P_ORDER = ((((1, 3), (2, 4)), ((1, 0, 6), (5,))), (((1, 3), (4, 2)), ((1, 0, 6), (5,))))
O_ORDER = (((1, 3, 2, 4), (0, 6, 5, 1)), ((3, 2, 1, 4), (5, 6, 1, 0)))
VPU_DUE = 3
KEYS_AHEAD = (14, 9)
NORM_DUE = ((0, 2), (0, 1))
HALF = 256
PRE = 8
RING = 8
WO_LAG = 3
PACE = 256
TB = 512
K_PAIRS = 8
Q_PAIRS = 8
F_PAIRS = 2
O_ROWS = (128, 128, 128, 128)


def _iota(shape, axis):
    return lax.broadcasted_iota(jnp.int32, shape, axis)


def _div(v, d):
    return (v * ((1 << 18) // d + 1)) >> 18


def _pack(x):
    return pltpu.bitcast(x.astype(BF16), jnp.uint32)


def _unpack(x):
    return pltpu.bitcast(x, BF16)


def _recip(x):
    r = pl.reciprocal(x, approx=True)
    return r * (2.0 - x * r)


def _layernorm(x):
    m = jnp.mean(x, axis=-1, keepdims=True)
    c = x - m
    v = jnp.mean(c * c, axis=-1, keepdims=True)
    return c * lax.rsqrt(v + 1e-5)


def _rows(*parts):
    return jnp.concatenate(parts, axis=0)


def _cols(*parts):
    return jnp.concatenate(parts, axis=1)


def _strassen_weights(b11, b12, b21, b22):
    f11, f12, f21, f22 = (b.astype(F32) for b in (b11, b12, b21, b22))
    return [r.astype(BF16)
            for r in (f11 + f22, b11, f12 - f22, f21 - f11, b22, f11 + f12, f21 + f22)]


def _left_product(a1, a2, times):
    return times(a2, 3) + times(a1 + a2, 1)


def _right_product(a1, a2, times):
    return times(a1 + a2, 4) + times(a1, 2)


def _token_operands(a1, a2, b1, b2):
    low = b1 + b2
    n = low.shape[0] // 2
    return ({3: b2, 2: a1, 1: low[:n], 4: a1 + a2},
            {0: a1 + b2, 6: a2 - b2, 1: low[n:], 5: b1 - a1})


def _memory_operands(m1, m2):
    both = m1 + m2
    return {0: m2, 1: both, 2: m1, 3: m2, 4: both, 5: m1, 6: m2}


def _first_results(p, n):
    m1 = _rows(p[1][n:], jnp.zeros_like(p[1][n:]))
    return ((p[1][:n] + p[3][:n], p[2][:n] + p[4][:n]),
            (p[2][n:] + p[4][n:], p[3][n:] - p[4][n:], p[3][n:] + m1, p[2][n:] - m1))


def _second_left(p, n, c11, c21):
    m1 = _rows(jnp.zeros_like(p[1][n:]), p[1][n:])
    return p[1][:n] + p[6][:n] - p[0][:n], c11 + p[0][n:] + p[6][n:], c21 + m1


def _second_right(p, n, c22):
    m1 = _rows(jnp.zeros_like(p[1][n:]), p[1][n:])
    return p[5][:n] + p[0][:n] - p[1][:n], c22 + p[0][n:] + p[5][n:] - m1


def _a_step(s, mem, xn, shared, *, layer, dh, x_in, x_ref, xb_ref, ws_ref, wp_ref, wos_ref,
            wop_ref, pre_ref, ahead_ref, o_refs, near_ref):
    odd = bool(shared)
    n_mem, seg = mem.shape[0], xn[0].shape[0]
    n_seg = xb_ref.shape[0]
    rows = n_mem + seg
    pw = 2 * dh
    n_pairs = wp_ref.shape[0]
    o_ref = o_refs[odd]
    scale = dh ** -0.5

    def after(early, value):
        return value if early is None else jnp.where(s < 0, early[:, :value.shape[1]], value)

    def after_all(early, value):
        t = functools.reduce(jnp.maximum, [early[i:i + 8, j:j + 128]
                                           for i in range(0, early.shape[0], 8)
                                           for j in range(0, early.shape[1], 128)])
        return jnp.concatenate([after(t, value[0:8]), value[8:]], axis=0)

    def slow_norm(x):
        outs = [None, None]
        for i in range(0, seg, 8):
            outs.append(_layernorm(after(outs[-2], x[i:i + 8])))
        return jnp.concatenate(outs[2:], axis=0)

    xn_next = slow_norm(x_in[jnp.minimum(s + len(xn), n_seg - 1)].astype(F32))
    done = jnp.maximum(s - 3, 0)
    xb_done = slow_norm(x_ref[done])
    xb_ref[done] = xb_done.astype(BF16)

    h = _rows(mem, xn[0])

    first = _iota((rows, 128), 1) < 64
    zero = jnp.zeros((rows, 128), F32)

    def key_blocks(t):
        t0, t1, t2 = t[:, 0:128], t[:, 128:256], t[:, 256:384]
        top = jnp.concatenate([t0, jnp.where(first, t1, 0.0), zero], axis=1)
        bot = jnp.concatenate([zero, jnp.where(first, 0.0, t1), t2], axis=1)
        return jnp.concatenate([top, bot], axis=0).astype(BF16)

    def value_blocks(t):
        mine = jnp.concatenate([first] * 3, axis=1)
        return jnp.concatenate(
            [jnp.where(mine, t, 0.0), jnp.where(mine, 0.0, t)], axis=0).astype(BF16)

    near = n_mem + 8

    def far_rows(t):
        return _rows(t[:n_mem], t[near:])

    q, k, v, probs, near_done = {}, {}, {}, {}, {}

    def project_short(p, j):
        def dot(a, w):
            return jnp.dot(a.astype(BF16), _unpack(w), preferred_element_type=F32)

        cols, top = slice(j * pw, (j + 1) * pw), h[:rows - PRE]
        most = (_left_product, _right_product)[p % 2](
            top[:, :HALF], top[:, HALF:2 * HALF], lambda a, i: dot(a, ws_ref[p // 2, i, :, cols]))
        return _rows(dot(top[:, 2 * HALF:], wp_ref[p, :, cols]) + most,
                     pre_ref[p, pl.ds(pl.multiple_of(s * PRE, PRE), PRE), (j - 1) * pw:j * pw])

    if not odd:
        shared["in"] = _token_operands(*(t[:, c:c + HALF] for t in xn[1:3] for c in (0, HALF)))
    m_in = _memory_operands(mem[:, :HALF], mem[:, HALF:2 * HALF])
    lhs_in = {i: _rows(m_in[i], t) for i, t in shared["in"][odd].items()}
    products = {}

    def project_shared(p, j):
        g, right = divmod(p, 2)
        cols, prod = slice(j * pw, (j + 1) * pw), products.setdefault(j, {})
        for i in P_ORDER[layer][odd][right]:
            prod[i] = jnp.dot(lhs_in[i], _unpack(ws_ref[g, i, :, cols]),
                              preferred_element_type=F32)
        if not odd:
            tokens = ahead_ref[p, :, cols]
            if right:
                (_, m), shared[g, j] = _first_results(prod, n_mem)
            else:
                m = prod[1][:n_mem] + prod[3][:n_mem]
        elif right:
            tokens = shared[g, j][0]
            m, ahead_ref[p, :, cols] = _second_right(prod, n_mem, shared[g, j][3])
        else:
            m, tokens, ahead_ref[p, :, cols] = _second_left(prod, n_mem, *shared[g, j][1:3])
        return jnp.dot(h[:, 2 * HALF:], _unpack(wp_ref[p, :, cols]),
                       preferred_element_type=F32) + _rows(m, tokens)

    def scores(p):
        col = far_rows(_iota((rows, 2 * rows), 1))
        row = far_rows(_iota((rows, 2 * rows), 0))
        is_a = col < rows
        visible = (row < n_mem) | (row >= jnp.where(is_a, col, col - rows))
        sc = lax.dot_general(far_rows(q[p]), key_blocks(k[p]), NT, preferred_element_type=F32)
        sc = jnp.where(visible, sc * scale, MASKED)
        max_a = jnp.max(jnp.where(is_a, sc, -jnp.inf), axis=1, keepdims=True)
        max_b = jnp.max(jnp.where(is_a, -jnp.inf, sc), axis=1, keepdims=True)
        e = jnp.exp(sc - jnp.where(is_a, max_a, max_b))
        sum_a = jnp.sum(jnp.where(is_a, e, 0.0), axis=1, keepdims=True)
        sum_b = jnp.sum(jnp.where(is_a, 0.0, e), axis=1, keepdims=True)
        probs[p] = e * _recip(jnp.where(is_a, sum_a, sum_b))
        if p == NORM_DUE[layer][0]:
            probs[p] = after_all(xn_next, probs[p])
        if p == NORM_DUE[layer][1]:
            probs[p] = after_all(xb_done, probs[p])
        if p - VPU_DUE in near_done:
            probs[p] = after_all(near_done[p - VPU_DUE], probs[p])

    def values(p):
        o = jnp.dot(probs[p], value_blocks(v[p]), preferred_element_type=F32)
        o_ref[:n_mem, p * pw:(p + 1) * pw] = o[:n_mem]
        o_ref[near:, p * pw:(p + 1) * pw] = o[n_mem:]

    chain = [None, None]
    scored = [None] * KEYS_AHEAD[layer]

    def attend_near(p):
        def key_row(j, i):
            return jnp.broadcast_to(near_ref[p, j:j + 1, 128 * i:128 * (i + 1)], (8, 128))

        near_ref[p, :, 0:pw] = k[p][:near]
        near_ref[p, :, pw:2 * pw] = v[p][:near]
        half, sub = first[0:8], _iota((8, 128), 0)
        t = q[p][n_mem:near] * (scale * LOG2E)
        q0, q2 = t[:, 0:128], t[:, 256:384]
        q1a, q1b = jnp.where(half, t[:, 128:256], 0.0), jnp.where(half, 0.0, t[:, 128:256])
        for j in range(near):
            ready = after(scored[-KEYS_AHEAD[layer]], chain[0])
            k1 = after(ready, key_row(j, 1))
            dot_a = q0 * after(ready, key_row(j, 0)) + q1a * k1
            dot_b = q2 * after(dot_a, key_row(j, 2)) + q1b * k1
            t = jnp.where(half, jnp.sum(dot_a, axis=1, keepdims=True),
                          jnp.sum(dot_b, axis=1, keepdims=True))
            scored.append(t if j <= n_mem else jnp.where(sub >= j - n_mem, t, MASKED * LOG2E))
            chain[0] = dot_b
        sc = scored[-near:]
        top = functools.reduce(jnp.maximum, sc)
        for j in range(near):
            e = jnp.exp2(sc[j] - after(chain[1], top))
            weight = after(chain[1], e)
            terms = [weight * key_row(j, 3 + i) for i in range(3)]
            total = e if j == 0 else total + e
            acc = terms if j == 0 else [a + b for a, b in zip(acc, terms)]
            chain[1] = acc[2]
        inv = _recip(total)
        o_ref[n_mem:near, p * pw:(p + 1) * pw] = _cols(*(a * inv for a in acc))
        near_done[p] = acc[2]

    out = {}

    def project_out(g0, g1):
        def halves(ref, lo, hi):
            return [_cols(*(ref[lo:hi, (2 * g + i) * pw:(2 * g + i + 1) * pw]
                            for g in range(g0, g1))) for i in range(2)]

        if not odd:
            shared["out", g0] = _token_operands(*halves(o_refs[0], n_mem, rows),
                                                *halves(o_refs[1], n_mem, rows))
        m = _memory_operands(*halves(o_ref, 0, n_mem))
        for i in O_ORDER[layer][odd]:
            r = jnp.dot(_rows(m[i], shared["out", g0][odd][i]), _unpack(wos_ref[g0:g1, i].reshape(-1, HALF)),
                        preferred_element_type=F32)
            out[i] = r + out[i] if i in out else r

    lag_s, lag_v = LAG_S[layer], LAG_S[layer] + LAG_PV[layer]
    todo = list(zip(O_SPLITS[layer][:-1], O_SPLITS[layer][1:]))
    for t in range(n_pairs + lag_v):
        if t >= n_pairs:
            project_out(*todo.pop(0))
        for c in ISSUE[layer]:
            if c == "S" and 0 <= t - lag_s < n_pairs:
                scores(t - lag_s)
            elif c == "V" and 0 <= t - lag_v < n_pairs:
                values(t - lag_v)
            elif c in "qkv" and t < n_pairs:
                j = "qkv".index(c)
                (q, k, v)[j][t] = (project_short(t, j) if j and pre_ref is not None
                                   else project_shared(t, j))
        if t < n_pairs:
            attend_near(t)
    for part in todo:
        project_out(*part)
    rest = jnp.dot(o_ref[...], _unpack(wop_ref[...].reshape(-1, wop_ref.shape[-1])),
                   preferred_element_type=F32)

    most, tail = slice(0, 2 * HALF), slice(2 * HALF, None)
    x_ref[s, :, tail] = x_in[s, :, tail].astype(F32) + rest[n_mem:]
    if odd:
        c12, c11, c21, c22 = shared["out"]
        m1, c11, c21 = _second_left(out, n_mem, c11, c21)
        m2, c22 = _second_right(out, n_mem, c22)
        x_ref[s - 1, :, most] = x_in[s - 1, :, most].astype(F32) + _cols(c11, c12)
        back = jnp.maximum(s - 2, 1)
        x_ref[back, :, most] = (x_in[back, :, most].astype(F32)
                                + jnp.where(s > 1, _cols(c21, c22), 0.0))
    else:
        (m1, m2), shared["out"] = _first_results(out, n_mem)
    return _cols(m1, m2, rest[:n_mem]), xn_next


def _pair_reduce(t, op):
    r = t[0:8]
    for i in range(8, t.shape[0], 8):
        r = op(r, t[i:i + 8])
    r = op(r, pltpu.roll(r, 4, 0))
    return op(r, pltpu.roll(r, 2, 0))


def _tile_rows(r, n):
    return jnp.concatenate([r] * (n // 8), axis=0)


def _feature_map(p):
    n = p.shape[0]
    e_pos = jnp.exp2(p - _tile_rows(_pair_reduce(p, jnp.maximum), n))
    e_neg = jnp.exp2(_tile_rows(_pair_reduce(p, jnp.minimum), n) - p)
    inv_pos = _recip(_pair_reduce(e_pos, jnp.add))
    inv_neg = _recip(_pair_reduce(e_neg, jnp.add))
    return jnp.concatenate(
        [e_pos * _tile_rows(inv_pos, n), e_neg * _tile_rows(inv_neg, n)], axis=0)


def _fold_span(b, blk):
    return b * blk // 128 * 128, -(-(b + 1) * blk // 128) * 128


def _expand_phi(wphi_ref, phi_ref):
    dh, _, heads = wphi_ref.shape
    d = dh * heads
    gr = 2 * dh
    c = _iota((dh, d), 1)
    c_feat = c - _div(c, dh) * dh
    spread = (_div(_iota((heads, d), 1), dh) == _iota((heads, d), 0)).astype(BF16)

    def gather(j, by_feat):
        for e in (j * (dh // 4) + i for i in range(dh // 4)):
            t = jnp.dot(wphi_ref[e], spread, preferred_element_type=F32)
            by_feat = jnp.where(c_feat == e, t, by_feat)
        return by_feat

    by_feat = lax.fori_loop(0, 4, gather, jnp.zeros((dh, d), F32)).astype(BF16)
    blk = F_PAIRS * gr
    r = _iota((blk, dh), 0)
    sel = (((r - _div(r, gr) * gr) >> 1) == _iota((blk, dh), 1)).astype(BF16)
    for b in range(d // blk):
        lo, hi = _fold_span(b, blk)
        r = _iota((blk, hi - lo), 0)
        head = 2 * (_div(r, gr) + b * F_PAIRS) + (r & 1)
        phi = jnp.dot(sel, by_feat[:, lo:hi], preferred_element_type=F32)
        phi_ref[b, :, 0:hi - lo] = _pack(
            jnp.where(_div(_iota((1, hi - lo), 1) + lo, dh) == head, phi, 0.0))


def _b_weights(wqkv_ref, phi_ref, wob_ref, bq_ref, bkv_ref, bo_ref):
    d = wqkv_ref.shape[0]
    blk = 2 * phi_ref.shape[1]
    half = bkv_ref.shape[1]
    bo_ref[...] = _pack(wob_ref[...])
    wv = wqkv_ref[:, 2 * d:3 * d].T
    for b in range(d // half):
        bkv_ref[b, half // 2:half, :] = _pack(wv[b * half:(b + 1) * half])
    for b in range(d // blk):
        lo, hi = _fold_span(b, blk)
        phi = _unpack(phi_ref[b, :, 0:hi - lo])
        wq = lax.dot_general(phi, wqkv_ref[:, lo:hi], NT, preferred_element_type=F32)
        wk = lax.dot_general(phi, wqkv_ref[:, d + lo:d + hi], NT, preferred_element_type=F32)
        bq_ref[b * blk // 2:(b + 1) * blk // 2, :] = _pack(wq * LOG2E)
        at = b * blk % half // 2
        bkv_ref[b * blk // half, at:at + blk // 2, :] = _pack(wk * LOG2E)


def _chunk_rows(ref, it, r0, n):
    seg = ref.shape[1]
    return pl.ds(it * (TB // seg) + r0 // seg, n // seg)


def _b_keys(it, carry, *, x_ref, xb_ref, bkv_ref, kv_ref, z_ref):
    n_blk, half, _ = bkv_ref.shape
    gr = half // K_PAIRS
    xb = xb_ref[_chunk_rows(xb_ref, it, 0, TB)].reshape(TB, -1)
    last = x_ref.shape[0] - 1 - jnp.minimum(it, 2)
    xb_ref[last] = _layernorm(x_ref[last]).astype(BF16)
    same_head = (_iota((gr, 2 * gr), 0) >= gr // 2) == ((_iota((gr, 2 * gr), 1) & 1) == 1)

    def accumulate(b, t):
        for i in range(K_PAIRS):
            g = b * K_PAIRS + i
            phi = _feature_map(t[i * gr:(i + 1) * gr])
            z_ref[g] = jnp.where(it > 0, z_ref[g], 0.0) + jnp.sum(phi, axis=1, keepdims=True)
            kv = lax.dot_general(t[half + i * gr:half + (i + 1) * gr], phi.astype(BF16), NT,
                                 preferred_element_type=F32)
            kv_ref[g] = jnp.where(it > 0, kv_ref[g], 0.0) + jnp.where(same_head, kv, 0.0)

    pending = None
    for b in range(n_blk):
        t = lax.dot_general(_unpack(bkv_ref[b]), xb, NT, preferred_element_type=F32)
        if pending is not None:
            accumulate(*pending)
        pending = (b, t)
    accumulate(*pending)
    return carry


def _b_queries(it, send, *, x_ref, xb_ref, y_ref, bq_ref, bo_ref, kv_ref, z_ref, ot_ref, on_ref):
    n_groups, gr, _ = kv_ref.shape
    blk = Q_PAIRS * gr
    sub = _iota((8, TB), 0)
    xb = xb_ref[_chunk_rows(xb_ref, it, 0, TB)].reshape(TB, -1)

    def attend(b, t):
        outs = []
        for i in range(Q_PAIRS):
            g = b * Q_PAIRS + i
            phi = _feature_map(t[i * gr:(i + 1) * gr])
            num = jnp.dot(kv_ref[g], phi.astype(BF16), preferred_element_type=F32)
            z = jnp.concatenate([z_ref[g]] * (TB // 128), axis=1)
            inv = _recip(_pair_reduce(phi * z, jnp.add) + 1e-6)
            other = pltpu.roll(inv, 1, 0)
            inv_a = jnp.where((sub & 1) == 0, inv, other)
            inv_b = jnp.where((sub & 1) == 0, other, inv)
            n = (gr - 8) // 16
            inv = jnp.concatenate(
                [inv_a] * n + [jnp.where(sub < 4, inv_a, inv_b)] + [inv_b] * n, axis=0)
            outs.append(num * inv)
        ot_ref[b * blk // 2:(b + 1) * blk // 2, :] = _pack(jnp.concatenate(outs, axis=0))

    n_blk = n_groups // Q_PAIRS
    proj = {}
    for b in range(n_blk + 1):
        if b < n_blk:
            proj[b] = lax.dot_general(_unpack(bq_ref[b * blk // 2:(b + 1) * blk // 2, :]), xb,
                                      NT, preferred_element_type=F32)
        if b > 0:
            attend(b - 1, proj[b - 1])
    on_ref[...] = _pack(_unpack(ot_ref[...]).T)
    r0 = 0
    for i, n in enumerate(O_ROWS):
        at = _chunk_rows(x_ref, it, r0, n)
        y = jnp.dot(_unpack(on_ref[r0 // 2:(r0 + n) // 2, :]), _unpack(bo_ref[...]),
                    preferred_element_type=F32)
        x = x_ref[at] + y.reshape((-1,) + x_ref.shape[1:])
        x_ref[at] = x
        y_ref[at] = x.astype(BF16)
        send(i)
        r0 += n


def _kernel(x_hbm, mem0_hbm, wq_hbm, wk_hbm, wv_hbm, wo_hbm, wqkvb_hbm, wphi_hbm, wob_hbm,
            out_hbm,
            x_ref, xb_ref, y_ref, xp_ref, stage_ref, pre_ref, ahead_ref,
            ws_ref, wp_ref, wos_ref, wop_ref, o_even_ref, o_odd_ref, near_ref,
            mem0_ref, wphi_ref, phi_ref, wqkvb_ref, wob_ref, bo_ref, bq_ref, bkv_ref,
            kv_ref, z_ref, ot_ref, on_ref,
            w_sem, in_sem, out_sem, *, dh):
    n_seg, seg, d = x_ref.shape
    n_pairs = wp_ref.shape[0]
    n_mem = mem0_ref.shape[0]
    pw = 2 * dh
    n_iter = n_seg * seg // TB

    def w_copies(p, j):
        src = (wq_hbm, wk_hbm, wv_hbm, wo_hbm)[j]
        if j < 2:
            return [pltpu.make_async_copy(src.at[p], stage_ref.at[p % RING, 3 * j:3 * j + 3],
                                          w_sem.at[p, j])]
        return [pltpu.make_async_copy(src.at[p, i], stage_ref.at[p % RING, 3 * j:3 * j + 3, i],
                                      w_sem.at[p, 2 * j - 2 + i]) for i in range(2)]

    def start_w(p, *slots):
        for j in slots:
            for copy in w_copies(p, j):
                copy.start()

    def wait_w(p, *slots):
        for j in slots:
            for copy in w_copies(p, j):
                copy.wait()

    def prepare_in(u, tiles, live=True, pace=lambda t, b: b):
        g, i = u // 2, u % 2
        for t in tiles:
            cols = pl.ds(pl.multiple_of(128 * t, 128), 128)
            blocks = [stage_ref[p % RING, t, :, :, pl.ds(pl.multiple_of(c + i * 128, 128), 128)]
                      .reshape(128, 128)
                      for c in (0, HALF) for p in (2 * g, jnp.where(live, 2 * g + 1, 0))]
            for n, r in enumerate(_strassen_weights(*(pace(t, b) for b in blocks))):
                ws_ref[g, n, pl.ds(pl.multiple_of(i * 64, 64), 64), cols] = _pack(r.T)
            wp_ref[u, :, cols] = _pack(stage_ref[u % RING, t, :, :, 2 * HALF:].reshape(128, -1).T)

    def wait_out(u):
        for i in range(2):
            pltpu.make_async_copy(stage_ref.at[0, 9:12, 0], stage_ref.at[0, 9:12, 0],
                                  w_sem.at[u // 2 * 2 + i, 4 + u % 2]).wait()

    def prepare_out(u, live=True, pace=lambda t, b: b):
        g, i = u // 2, u % 2
        for t in range(3):
            parts = [pace(3 * t + 1, stage_ref[p % RING, jnp.where(live, 9, 3) + t, i])
                     for p in (2 * g, jnp.where(live, 2 * g + 1, 0))]
            blocks = [part[:, c:c + HALF] for part in parts for c in (0, HALF)]
            for n, r in enumerate(_strassen_weights(*blocks)):
                wos_ref[g, n, t, i] = _pack(r)
            for n, part in enumerate(parts):
                wop_ref[2 * g + n, t, i] = _pack(part[:, 2 * HALF:])

    def out_copy(it, i):
        part = _chunk_rows(y_ref, it, sum(O_ROWS[:i]), O_ROWS[i])
        return pltpu.make_async_copy(y_ref.at[part], out_hbm.at[part], out_sem.at[0])

    def x_copy(part, rows, sem):
        return pltpu.make_async_copy(x_hbm.at[part, rows, :], y_ref.at[part, rows, :], sem)

    head, tail = slice(0, seg - PRE), slice(seg - PRE, seg)
    xt_copy = x_copy(slice(None), tail, in_sem.at[0])
    wqkvb_copy = pltpu.make_async_copy(wqkvb_hbm, wqkvb_ref, in_sem.at[1])
    wphi_copy = pltpu.make_async_copy(wphi_hbm, wphi_ref, in_sem.at[5])
    mem0_copy = pltpu.make_async_copy(mem0_hbm, mem0_ref, in_sem.at[4])
    wob_copy = pltpu.make_async_copy(wob_hbm, wob_ref, in_sem.at[2])

    wphi_copy.start()
    xt_copy.start()
    start_w(0, 0, 1, 2)
    wphi_copy.wait()
    _expand_phi(wphi_ref, phi_ref)
    xt_copy.wait()

    xp_ref[...] = _layernorm(y_ref[:, tail, :].astype(F32).reshape(n_seg * PRE, d)).astype(BF16)

    mem0_copy.start()
    start_w(1, 0, 1, 2)

    def pre_project(p, carry):
        @pl.when(p + 2 < n_pairs)
        def _():
            start_w(jnp.minimum(p + 2, n_pairs - 1), 0, 1, 2)

        part = pl.ds(p * (n_seg // n_pairs), n_seg // n_pairs)
        x_copy(part, head, in_sem.at[3]).start()
        start_w(p, 3)

        @pl.when(p >= WO_LAG)
        def _():
            wait_out(jnp.maximum(p - WO_LAG, 0))

        wait_w(p, 0, 1, 2)
        kv = lax.dot_general(xp_ref[...], stage_ref[p % RING, 3:9].reshape(-1, d), NT,
                             preferred_element_type=F32)
        pre_ref[p] = kv

        def pace(t, block):
            c, r = divmod(t * PACE, xp_ref.shape[0])
            early = kv[r:r + block.shape[0], 128 * c:128 * (c + 1)].astype(BF16)
            return jnp.where(p < 0, _cols(*[early] * (block.shape[1] // 128)), block)

        prepare_in(jnp.maximum(p - 1, 0), range(9), p >= 1, pace)
        prepare_out(jnp.maximum(p - WO_LAG, 0), p >= WO_LAG, pace)
        return carry

    lax.fori_loop(0, n_pairs, pre_project, 0)

    @pl.loop(0, 3)
    def _(j):
        prepare_in(n_pairs - 1, [3 * j + i for i in range(3)])

    @pl.loop(n_pairs - WO_LAG, n_pairs)
    def _(u):
        wait_out(u)
        prepare_out(u)

    x_copy(slice(None), head, in_sem.at[3]).wait()

    wqkvb_copy.start()
    wob_copy.start()
    mem0_copy.wait()
    x_ref[0] = y_ref[0].astype(F32)

    def layer_a(layer, x_in, pre):
        step = functools.partial(
            _a_step, layer=layer, dh=dh, x_in=x_in, x_ref=x_ref, xb_ref=xb_ref, ws_ref=ws_ref,
            wp_ref=wp_ref, wos_ref=wos_ref, wop_ref=wop_ref, pre_ref=pre, ahead_ref=ahead_ref,
            o_refs=(o_even_ref, o_odd_ref), near_ref=near_ref)
        xn = [_layernorm(x_in[i].astype(F32)) for i in range(3)]
        o_odd_ref[...] = jnp.zeros(o_odd_ref.shape, F32)
        cols, per = (slice(0, 3 * pw), 1) if pre is None else (slice(0, pw), 2)

        @pl.loop(0, n_pairs // 2 // per)
        def _(j):
            for g in (j * per + i for i in range(per)):
                for i, product in enumerate((_left_product, _right_product)):
                    ahead_ref[2 * g + i, :, cols] = product(
                        xn[0][:, :HALF], xn[0][:, HALF:2 * HALF],
                        lambda a, n: jnp.dot(a.astype(BF16), _unpack(ws_ref[g, n, :, cols]),
                                             preferred_element_type=F32))

        def two_steps(it, carry):
            mem, *xn = carry
            shared = {}
            for i in range(2):
                mem, xn_next = step(2 * it + i, mem, xn, shared)
                xn = xn[1:] + [xn_next]
            return (mem, *xn)

        lax.fori_loop(0, n_seg // 2, two_steps, (mem0_ref[...].astype(F32), *xn))

    def finish_a(layer):
        a = [_cols(*(o_odd_ref[n_mem:, (2 * g + i) * pw:(2 * g + i + 1) * pw]
                     for g in range(n_pairs // 2))) for i in range(2)]
        y = _cols(*(product(*a, lambda t, n: jnp.dot(
            t.astype(BF16), _unpack(wos_ref[:, n].reshape(-1, HALF)), preferred_element_type=F32))
            for product in (_left_product, _right_product)))
        at = (n_seg - 1, slice(None), slice(0, 2 * HALF))
        x_ref[at] = jnp.where(layer == 0, y_ref[at].astype(F32), x_ref[at]) + y

    b_keys = functools.partial(_b_keys, x_ref=x_ref, xb_ref=xb_ref, bkv_ref=bkv_ref,
                               kv_ref=kv_ref, z_ref=z_ref)
    b_queries = functools.partial(_b_queries, x_ref=x_ref, xb_ref=xb_ref, y_ref=y_ref,
                                  bq_ref=bq_ref, bo_ref=bo_ref, kv_ref=kv_ref, z_ref=z_ref,
                                  ot_ref=ot_ref, on_ref=on_ref)

    def layer_pair(layer, carry):
        @pl.when(layer == 0)
        def _():
            layer_a(0, y_ref, pre_ref)

        @pl.when(layer == 0)
        def _():
            wqkvb_copy.wait()
            wob_copy.wait()
            _b_weights(wqkvb_ref, phi_ref, wob_ref, bq_ref, bkv_ref, bo_ref)

        @pl.when(layer == 1)
        def _():
            layer_a(1, x_ref, None)

        finish_a(layer)

        lax.fori_loop(0, n_iter, b_keys, 0)

        def queries(it, carry):
            def send(i):
                @pl.when(layer == 1)
                def _():
                    out_copy(it, i).start()

            b_queries(it, send)
            return carry

        lax.fori_loop(0, n_iter, queries, 0)

        return carry

    lax.fori_loop(0, 2, layer_pair, 0)
    pltpu.make_async_copy(y_ref, out_hbm, out_sem.at[0]).wait()


@functools.partial(jax.jit, static_argnames=("A_seg_len",))
def pallas_interleave_layers__memory_aug_recurrent_mem_tr__linear_kernel_hedgehog__prompt_kernel(
    A_x, A_mem0, A_Wq, A_Wk, A_Wv, A_Wo, A_seg_len, B_x, B_wqkv, B_w_phi, B_wo,
):
    del B_x
    batch, s_len, d = A_x.shape
    _, heads, dh = A_Wq.shape
    n_mem = A_mem0.shape[1]
    seg = int(A_seg_len)
    b_heads, b_dh, _ = B_w_phi.shape
    rows = n_mem + seg
    n_pairs = heads // 2
    gr = 2 * b_dh
    half = K_PAIRS * gr
    n_seg = s_len // seg
    assert batch == 1 and dh == 192 and heads == 4 * O_SPLITS[0][-1] and d == 2 * HALF + 128
    assert n_mem % 8 == 0 and seg % 16 == 0 and 128 % seg == 0 and 2 * rows <= 128
    assert s_len % TB == 0 and s_len > 3 * TB == 3 * sum(O_ROWS) and n_seg % n_pairs == 0
    assert b_heads * b_dh == d and b_dh % 8 == 4 and d % half == 0

    def head_major(w):
        return w.transpose(1, 2, 0)

    hbm = pl.BlockSpec(memory_space=pltpu.HBM)
    out = pl.pallas_call(
        functools.partial(_kernel, dh=dh),
        out_shape=jax.ShapeDtypeStruct((n_seg, seg, d), A_x.dtype),
        in_specs=[hbm] * 9,
        out_specs=hbm,
        scratch_shapes=[
            pltpu.VMEM((n_seg, seg, d), F32),
            pltpu.VMEM((n_seg, seg, d), BF16),
            pltpu.VMEM((n_seg, seg, d), BF16),
            pltpu.VMEM((n_seg * PRE, d), BF16),
            pltpu.VMEM((RING, 12, 2, 64, d), BF16),
            pltpu.VMEM((n_pairs, n_seg * PRE, 4 * dh), F32),
            pltpu.VMEM((n_pairs, seg, 6 * dh), F32),
            pltpu.VMEM((n_pairs // 2, 7, HALF // 2, 6 * dh), jnp.uint32),
            pltpu.VMEM((n_pairs, d // 2 - HALF, 6 * dh), jnp.uint32),
            pltpu.VMEM((n_pairs // 2, 7, 3, 2, 32, HALF), jnp.uint32),
            pltpu.VMEM((n_pairs, 3, 2, 32, d - 2 * HALF), jnp.uint32),
            pltpu.VMEM((rows, heads * dh), F32),
            pltpu.VMEM((rows, heads * dh), F32),
            pltpu.VMEM((n_pairs, n_mem + 8, 4 * dh), F32),
            pltpu.VMEM((n_mem, d), BF16),
            pltpu.VMEM((b_dh, b_dh, b_heads), BF16),
            pltpu.VMEM((d // (F_PAIRS * gr), F_PAIRS * gr // 2, 256), jnp.uint32),
            pltpu.VMEM(B_wqkv.shape, BF16),
            pltpu.VMEM(B_wo.shape, BF16),
            pltpu.VMEM((d // 2, d), jnp.uint32),
            pltpu.VMEM((d // 2, d), jnp.uint32),
            pltpu.VMEM((d // half, half, d), jnp.uint32),
            pltpu.VMEM((b_heads // 2, gr, 2 * gr), F32),
            pltpu.VMEM((b_heads // 2, 2 * gr, 128), F32),
            pltpu.VMEM((d // 2, TB), jnp.uint32),
            pltpu.VMEM((TB // 2, d), jnp.uint32),
            pltpu.SemaphoreType.DMA((n_pairs, 6)),
            pltpu.SemaphoreType.DMA((6,)),
            pltpu.SemaphoreType.DMA((1,)),
        ],
        compiler_params=pltpu.CompilerParams(vmem_limit_bytes=124 * 1024 * 1024),
    )(
        A_x.reshape(n_seg, seg, d), A_mem0.reshape(n_mem, d),
        head_major(A_Wq).reshape(n_pairs, 3, 2, 64, d),
        head_major(A_Wk).reshape(n_pairs, 3, 2, 64, d),
        head_major(A_Wv).reshape(n_pairs, 2, 3, 64, d), A_Wo.reshape(n_pairs, 2, 3, 64, d),
        B_wqkv, B_w_phi.transpose(1, 2, 0), B_wo,
    )
    return out.reshape(batch, s_len, d)
```

```python
import functools
import math

import jax
import jax.numpy as jnp
from jax import lax
import jax.experimental.pallas as pl
import jax.experimental.pallas.tpu as pltpu

F32 = jnp.float32
BF16 = jnp.bfloat16
NT = (((1,), (1,)), ((), ()))
LOG2E = math.log2(math.e)
MASKED = -1e9

ISSUE = ("kqSVv", "qkVSv")
LAG_S = (2, 1)
LAG_PV = (2, 3)
O_SPLITS = ((0, 1, 2, 3, 4, 5, 6, 8), (0, 1, 2, 3, 4, 6, 8))
P_ORDER = ((((1, 3), (2, 4)), ((1, 0, 6), (5,))), (((1, 3), (4, 2)), ((1, 0, 6), (5,))))
O_ORDER = (((1, 3, 2, 4), (0, 6, 5, 1)), ((3, 2, 1, 4), (5, 6, 1, 0)))
VPU_DUE = 3
KEYS_AHEAD = (14, 9)
NORM_DUE = ((0, 2), (0, 1))
HALF = 256
PRE = 8
RING = 8
WO_LAG = 3
PACE = 256
TB = 512
K_PAIRS = 8
Q_PAIRS = 8
F_PAIRS = 2
O_ROWS = (128, 128, 128, 128)


def _iota(shape, axis):
    return lax.broadcasted_iota(jnp.int32, shape, axis)


def _div(v, d):
    return (v * ((1 << 18) // d + 1)) >> 18


def _pack(x):
    return pltpu.bitcast(x.astype(BF16), jnp.uint32)


def _unpack(x):
    return pltpu.bitcast(x, BF16)


def _recip(x):
    r = pl.reciprocal(x, approx=True)
    return r * (2.0 - x * r)


def _layernorm(x):
    m = jnp.mean(x, axis=-1, keepdims=True)
    c = x - m
    v = jnp.mean(c * c, axis=-1, keepdims=True)
    return c * lax.rsqrt(v + 1e-5)


def _rows(*parts):
    return jnp.concatenate(parts, axis=0)


def _cols(*parts):
    return jnp.concatenate(parts, axis=1)


def _strassen_weights(b11, b12, b21, b22):
    f11, f12, f21, f22 = (b.astype(F32) for b in (b11, b12, b21, b22))
    return [r.astype(BF16)
            for r in (f11 + f22, b11, f12 - f22, f21 - f11, b22, f11 + f12, f21 + f22)]


def _left_product(a1, a2, times):
    return times(a2, 3) + times(a1 + a2, 1)


def _right_product(a1, a2, times):
    return times(a1 + a2, 4) + times(a1, 2)


def _token_operands(a1, a2, b1, b2):
    low = b1 + b2
    n = low.shape[0] // 2
    return ({3: b2, 2: a1, 1: low[:n], 4: a1 + a2},
            {0: a1 + b2, 6: a2 - b2, 1: low[n:], 5: b1 - a1})


def _memory_operands(m1, m2):
    both = m1 + m2
    return {0: m2, 1: both, 2: m1, 3: m2, 4: both, 5: m1, 6: m2}


def _first_results(p, n):
    m1 = _rows(p[1][n:], jnp.zeros_like(p[1][n:]))
    return ((p[1][:n] + p[3][:n], p[2][:n] + p[4][:n]),
            (p[2][n:] + p[4][n:], p[3][n:] - p[4][n:], p[3][n:] + m1, p[2][n:] - m1))


def _second_left(p, n, c11, c21):
    m1 = _rows(jnp.zeros_like(p[1][n:]), p[1][n:])
    return p[1][:n] + p[6][:n] - p[0][:n], c11 + p[0][n:] + p[6][n:], c21 + m1


def _second_right(p, n, c22):
    m1 = _rows(jnp.zeros_like(p[1][n:]), p[1][n:])
    return p[5][:n] + p[0][:n] - p[1][:n], c22 + p[0][n:] + p[5][n:] - m1


def _a_step(s, mem, xn, shared, *, layer, dh, x_in, x_ref, xb_ref, ws_ref, wp_ref, wos_ref,
            wop_ref, pre_ref, ahead_ref, o_refs, near_ref):
    odd = bool(shared)
    n_mem, seg = mem.shape[0], xn[0].shape[0]
    n_seg = xb_ref.shape[0]
    rows = n_mem + seg
    pw = 2 * dh
    n_pairs = wp_ref.shape[0]
    o_ref = o_refs[odd]
    scale = dh ** -0.5

    def after(early, value):
        return value if early is None else jnp.where(s < 0, early[:, :value.shape[1]], value)

    def after_all(early, value):
        t = functools.reduce(jnp.maximum, [early[i:i + 8, j:j + 128]
                                           for i in range(0, early.shape[0], 8)
                                           for j in range(0, early.shape[1], 128)])
        return jnp.concatenate([after(t, value[0:8]), value[8:]], axis=0)

    def slow_norm(x):
        outs = [None, None]
        for i in range(0, seg, 8):
            outs.append(_layernorm(after(outs[-2], x[i:i + 8])))
        return jnp.concatenate(outs[2:], axis=0)

    xn_next = slow_norm(x_in[jnp.minimum(s + len(xn), n_seg - 1)].astype(F32))
    done = jnp.maximum(s - 3, 0)
    xb_done = slow_norm(x_ref[done])
    xb_ref[done] = xb_done.astype(BF16)

    h = _rows(mem, xn[0])

    first = _iota((rows, 128), 1) < 64
    zero = jnp.zeros((rows, 128), F32)

    def key_blocks(t):
        t0, t1, t2 = t[:, 0:128], t[:, 128:256], t[:, 256:384]
        top = jnp.concatenate([t0, jnp.where(first, t1, 0.0), zero], axis=1)
        bot = jnp.concatenate([zero, jnp.where(first, 0.0, t1), t2], axis=1)
        return jnp.concatenate([top, bot], axis=0).astype(BF16)

    def value_blocks(t):
        mine = jnp.concatenate([first] * 3, axis=1)
        return jnp.concatenate(
            [jnp.where(mine, t, 0.0), jnp.where(mine, 0.0, t)], axis=0).astype(BF16)

    near = n_mem + 8

    def far_rows(t):
        return _rows(t[:n_mem], t[near:])

    q, k, v, probs, near_done = {}, {}, {}, {}, {}

    def project_short(p, j):
        def dot(a, w):
            return jnp.dot(a.astype(BF16), _unpack(w), preferred_element_type=F32)

        cols, top = slice(j * pw, (j + 1) * pw), h[:rows - PRE]
        most = (_left_product, _right_product)[p % 2](
            top[:, :HALF], top[:, HALF:2 * HALF], lambda a, i: dot(a, ws_ref[p // 2, i, :, cols]))
        return _rows(dot(top[:, 2 * HALF:], wp_ref[p, :, cols]) + most,
                     pre_ref[p, pl.ds(pl.multiple_of(s * PRE, PRE), PRE), (j - 1) * pw:j * pw])

    if not odd:
        shared["in"] = _token_operands(*(t[:, c:c + HALF] for t in xn[1:3] for c in (0, HALF)))
    m_in = _memory_operands(mem[:, :HALF], mem[:, HALF:2 * HALF])
    lhs_in = {i: _rows(m_in[i], t) for i, t in shared["in"][odd].items()}
    products = {}

    def project_shared(p, j):
        g, right = divmod(p, 2)
        cols, prod = slice(j * pw, (j + 1) * pw), products.setdefault(j, {})
        for i in P_ORDER[layer][odd][right]:
            prod[i] = jnp.dot(lhs_in[i], _unpack(ws_ref[g, i, :, cols]),
                              preferred_element_type=F32)
        if not odd:
            tokens = ahead_ref[p, :, cols]
            if right:
                (_, m), shared[g, j] = _first_results(prod, n_mem)
            else:
                m = prod[1][:n_mem] + prod[3][:n_mem]
        elif right:
            tokens = shared[g, j][0]
            m, ahead_ref[p, :, cols] = _second_right(prod, n_mem, shared[g, j][3])
        else:
            m, tokens, ahead_ref[p, :, cols] = _second_left(prod, n_mem, *shared[g, j][1:3])
        return jnp.dot(h[:, 2 * HALF:], _unpack(wp_ref[p, :, cols]),
                       preferred_element_type=F32) + _rows(m, tokens)

    def scores(p):
        col = far_rows(_iota((rows, 2 * rows), 1))
        row = far_rows(_iota((rows, 2 * rows), 0))
        is_a = col < rows
        visible = (row < n_mem) | (row >= jnp.where(is_a, col, col - rows))
        sc = lax.dot_general(far_rows(q[p]), key_blocks(k[p]), NT, preferred_element_type=F32)
        sc = jnp.where(visible, sc * scale, MASKED)
        max_a = jnp.max(jnp.where(is_a, sc, -jnp.inf), axis=1, keepdims=True)
        max_b = jnp.max(jnp.where(is_a, -jnp.inf, sc), axis=1, keepdims=True)
        e = jnp.exp(sc - jnp.where(is_a, max_a, max_b))
        sum_a = jnp.sum(jnp.where(is_a, e, 0.0), axis=1, keepdims=True)
        sum_b = jnp.sum(jnp.where(is_a, 0.0, e), axis=1, keepdims=True)
        probs[p] = e * _recip(jnp.where(is_a, sum_a, sum_b))
        if p == NORM_DUE[layer][0]:
            probs[p] = after_all(xn_next, probs[p])
        if p == NORM_DUE[layer][1]:
            probs[p] = after_all(xb_done, probs[p])
        if p - VPU_DUE in near_done:
            probs[p] = after_all(near_done[p - VPU_DUE], probs[p])

    def values(p):
        o = jnp.dot(probs[p], value_blocks(v[p]), preferred_element_type=F32)
        o_ref[:n_mem, p * pw:(p + 1) * pw] = o[:n_mem]
        o_ref[near:, p * pw:(p + 1) * pw] = o[n_mem:]

    chain = [None, None]
    scored = [None] * KEYS_AHEAD[layer]

    def attend_near(p):
        def key_row(j, i):
            return jnp.broadcast_to(near_ref[p, j:j + 1, 128 * i:128 * (i + 1)], (8, 128))

        near_ref[p, :, 0:pw] = k[p][:near]
        near_ref[p, :, pw:2 * pw] = v[p][:near]
        half, sub = first[0:8], _iota((8, 128), 0)
        t = q[p][n_mem:near] * (scale * LOG2E)
        q0, q2 = t[:, 0:128], t[:, 256:384]
        q1a, q1b = jnp.where(half, t[:, 128:256], 0.0), jnp.where(half, 0.0, t[:, 128:256])
        for j in range(near):
            ready = after(scored[-KEYS_AHEAD[layer]], chain[0])
            k1 = after(ready, key_row(j, 1))
            dot_a = q0 * after(ready, key_row(j, 0)) + q1a * k1
            dot_b = q2 * after(dot_a, key_row(j, 2)) + q1b * k1
            t = jnp.where(half, jnp.sum(dot_a, axis=1, keepdims=True),
                          jnp.sum(dot_b, axis=1, keepdims=True))
            scored.append(t if j <= n_mem else jnp.where(sub >= j - n_mem, t, MASKED * LOG2E))
            chain[0] = dot_b
        sc = scored[-near:]
        top = functools.reduce(jnp.maximum, sc)
        for j in range(near):
            e = jnp.exp2(sc[j] - after(chain[1], top))
            weight = after(chain[1], e)
            terms = [weight * key_row(j, 3 + i) for i in range(3)]
            total = e if j == 0 else total + e
            acc = terms if j == 0 else [a + b for a, b in zip(acc, terms)]
            chain[1] = acc[2]
        inv = _recip(total)
        o_ref[n_mem:near, p * pw:(p + 1) * pw] = _cols(*(a * inv for a in acc))
        near_done[p] = acc[2]

    out = {}

    def project_out(g0, g1):
        def halves(ref, lo, hi):
            return [_cols(*(ref[lo:hi, (2 * g + i) * pw:(2 * g + i + 1) * pw]
                            for g in range(g0, g1))) for i in range(2)]

        if not odd:
            shared["out", g0] = _token_operands(*halves(o_refs[0], n_mem, rows),
                                                *halves(o_refs[1], n_mem, rows))
        m = _memory_operands(*halves(o_ref, 0, n_mem))
        for i in O_ORDER[layer][odd]:
            r = jnp.dot(_rows(m[i], shared["out", g0][odd][i]), _unpack(wos_ref[g0:g1, i].reshape(-1, HALF)),
                        preferred_element_type=F32)
            out[i] = r + out[i] if i in out else r

    lag_s, lag_v = LAG_S[layer], LAG_S[layer] + LAG_PV[layer]
    todo = list(zip(O_SPLITS[layer][:-1], O_SPLITS[layer][1:]))
    for t in range(n_pairs + lag_v):
        if t >= n_pairs:
            project_out(*todo.pop(0))
        for c in ISSUE[layer]:
            if c == "S" and 0 <= t - lag_s < n_pairs:
                scores(t - lag_s)
            elif c == "V" and 0 <= t - lag_v < n_pairs:
                values(t - lag_v)
            elif c in "qkv" and t < n_pairs:
                j = "qkv".index(c)
                (q, k, v)[j][t] = (project_short(t, j) if j and pre_ref is not None
                                   else project_shared(t, j))
        if t < n_pairs:
            attend_near(t)
    for part in todo:
        project_out(*part)
    rest = jnp.dot(o_ref[...], _unpack(wop_ref[...].reshape(-1, wop_ref.shape[-1])),
                   preferred_element_type=F32)

    most, tail = slice(0, 2 * HALF), slice(2 * HALF, None)
    x_ref[s, :, tail] = x_in[s, :, tail].astype(F32) + rest[n_mem:]
    if odd:
        c12, c11, c21, c22 = shared["out"]
        m1, c11, c21 = _second_left(out, n_mem, c11, c21)
        m2, c22 = _second_right(out, n_mem, c22)
        x_ref[s - 1, :, most] = x_in[s - 1, :, most].astype(F32) + _cols(c11, c12)
        back = jnp.maximum(s - 2, 1)
        x_ref[back, :, most] = (x_in[back, :, most].astype(F32)
                                + jnp.where(s > 1, _cols(c21, c22), 0.0))
    else:
        (m1, m2), shared["out"] = _first_results(out, n_mem)
    return _cols(m1, m2, rest[:n_mem]), xn_next


def _pair_reduce(t, op):
    r = t[0:8]
    for i in range(8, t.shape[0], 8):
        r = op(r, t[i:i + 8])
    r = op(r, pltpu.roll(r, 4, 0))
    return op(r, pltpu.roll(r, 2, 0))


def _tile_rows(r, n):
    return jnp.concatenate([r] * (n // 8), axis=0)


def _feature_map(p):
    n = p.shape[0]
    e_pos = jnp.exp2(p - _tile_rows(_pair_reduce(p, jnp.maximum), n))
    e_neg = jnp.exp2(_tile_rows(_pair_reduce(p, jnp.minimum), n) - p)
    inv_pos = _recip(_pair_reduce(e_pos, jnp.add))
    inv_neg = _recip(_pair_reduce(e_neg, jnp.add))
    return jnp.concatenate(
        [e_pos * _tile_rows(inv_pos, n), e_neg * _tile_rows(inv_neg, n)], axis=0)


def _fold_span(b, blk):
    return b * blk // 128 * 128, -(-(b + 1) * blk // 128) * 128


def _expand_phi(wphi_ref, phi_ref):
    dh, _, heads = wphi_ref.shape
    d = dh * heads
    gr = 2 * dh
    c = _iota((dh, d), 1)
    c_feat = c - _div(c, dh) * dh
    spread = (_div(_iota((heads, d), 1), dh) == _iota((heads, d), 0)).astype(BF16)

    def gather(j, by_feat):
        for e in (j * (dh // 4) + i for i in range(dh // 4)):
            t = jnp.dot(wphi_ref[e], spread, preferred_element_type=F32)
            by_feat = jnp.where(c_feat == e, t, by_feat)
        return by_feat

    by_feat = lax.fori_loop(0, 4, gather, jnp.zeros((dh, d), F32)).astype(BF16)
    blk = F_PAIRS * gr
    r = _iota((blk, dh), 0)
    sel = (((r - _div(r, gr) * gr) >> 1) == _iota((blk, dh), 1)).astype(BF16)
    for b in range(d // blk):
        lo, hi = _fold_span(b, blk)
        r = _iota((blk, hi - lo), 0)
        head = 2 * (_div(r, gr) + b * F_PAIRS) + (r & 1)
        phi = jnp.dot(sel, by_feat[:, lo:hi], preferred_element_type=F32)
        phi_ref[b, :, 0:hi - lo] = _pack(
            jnp.where(_div(_iota((1, hi - lo), 1) + lo, dh) == head, phi, 0.0))


def _b_weights(wqkv_ref, phi_ref, wob_ref, bq_ref, bkv_ref, bo_ref):
    d = wqkv_ref.shape[0]
    blk = 2 * phi_ref.shape[1]
    half = bkv_ref.shape[1]
    bo_ref[...] = _pack(wob_ref[...])
    wv = wqkv_ref[:, 2 * d:3 * d].T
    for b in range(d // half):
        bkv_ref[b, half // 2:half, :] = _pack(wv[b * half:(b + 1) * half])
    for b in range(d // blk):
        lo, hi = _fold_span(b, blk)
        phi = _unpack(phi_ref[b, :, 0:hi - lo])
        wq = lax.dot_general(phi, wqkv_ref[:, lo:hi], NT, preferred_element_type=F32)
        wk = lax.dot_general(phi, wqkv_ref[:, d + lo:d + hi], NT, preferred_element_type=F32)
        bq_ref[b * blk // 2:(b + 1) * blk // 2, :] = _pack(wq * LOG2E)
        at = b * blk % half // 2
        bkv_ref[b * blk // half, at:at + blk // 2, :] = _pack(wk * LOG2E)


def _chunk_rows(ref, it, r0, n):
    seg = ref.shape[1]
    return pl.ds(it * (TB // seg) + r0 // seg, n // seg)


def _b_keys(it, carry, *, x_ref, xb_ref, bkv_ref, kv_ref, z_ref):
    n_blk, half, _ = bkv_ref.shape
    gr = half // K_PAIRS
    xb = xb_ref[_chunk_rows(xb_ref, it, 0, TB)].reshape(TB, -1)
    last = x_ref.shape[0] - 1 - jnp.minimum(it, 2)
    xb_ref[last] = _layernorm(x_ref[last]).astype(BF16)
    same_head = (_iota((gr, 2 * gr), 0) >= gr // 2) == ((_iota((gr, 2 * gr), 1) & 1) == 1)

    def accumulate(b, t):
        for i in range(K_PAIRS):
            g = b * K_PAIRS + i
            phi = _feature_map(t[i * gr:(i + 1) * gr])
            z_ref[g] = jnp.where(it > 0, z_ref[g], 0.0) + jnp.sum(phi, axis=1, keepdims=True)
            kv = lax.dot_general(t[half + i * gr:half + (i + 1) * gr], phi.astype(BF16), NT,
                                 preferred_element_type=F32)
            kv_ref[g] = jnp.where(it > 0, kv_ref[g], 0.0) + jnp.where(same_head, kv, 0.0)

    pending = None
    for b in range(n_blk):
        t = lax.dot_general(_unpack(bkv_ref[b]), xb, NT, preferred_element_type=F32)
        if pending is not None:
            accumulate(*pending)
        pending = (b, t)
    accumulate(*pending)
    return carry


def _b_queries(it, send, *, x_ref, xb_ref, y_ref, bq_ref, bo_ref, kv_ref, z_ref, ot_ref, on_ref):
    n_groups, gr, _ = kv_ref.shape
    blk = Q_PAIRS * gr
    sub = _iota((8, TB), 0)
    xb = xb_ref[_chunk_rows(xb_ref, it, 0, TB)].reshape(TB, -1)

    def attend(b, t):
        outs = []
        for i in range(Q_PAIRS):
            g = b * Q_PAIRS + i
            phi = _feature_map(t[i * gr:(i + 1) * gr])
            num = jnp.dot(kv_ref[g], phi.astype(BF16), preferred_element_type=F32)
            z = jnp.concatenate([z_ref[g]] * (TB // 128), axis=1)
            inv = _recip(_pair_reduce(phi * z, jnp.add) + 1e-6)
            other = pltpu.roll(inv, 1, 0)
            inv_a = jnp.where((sub & 1) == 0, inv, other)
            inv_b = jnp.where((sub & 1) == 0, other, inv)
            n = (gr - 8) // 16
            inv = jnp.concatenate(
                [inv_a] * n + [jnp.where(sub < 4, inv_a, inv_b)] + [inv_b] * n, axis=0)
            outs.append(num * inv)
        ot_ref[b * blk // 2:(b + 1) * blk // 2, :] = _pack(jnp.concatenate(outs, axis=0))

    n_blk = n_groups // Q_PAIRS
    proj = {}
    for b in range(n_blk + 1):
        if b < n_blk:
            proj[b] = lax.dot_general(_unpack(bq_ref[b * blk // 2:(b + 1) * blk // 2, :]), xb,
                                      NT, preferred_element_type=F32)
        if b > 0:
            attend(b - 1, proj[b - 1])
    on_ref[...] = _pack(_unpack(ot_ref[...]).T)
    r0 = 0
    for i, n in enumerate(O_ROWS):
        at = _chunk_rows(x_ref, it, r0, n)
        y = jnp.dot(_unpack(on_ref[r0 // 2:(r0 + n) // 2, :]), _unpack(bo_ref[...]),
                    preferred_element_type=F32)
        x = x_ref[at] + y.reshape((-1,) + x_ref.shape[1:])
        x_ref[at] = x
        y_ref[at] = x.astype(BF16)
        send(i)
        r0 += n


def _kernel(x_hbm, mem0_hbm, wq_hbm, wk_hbm, wv_hbm, wo_hbm, wqkvb_hbm, wphi_hbm, wob_hbm,
            out_hbm,
            x_ref, xb_ref, y_ref, xp_ref, stage_ref, pre_ref, ahead_ref,
            ws_ref, wp_ref, wos_ref, wop_ref, o_even_ref, o_odd_ref, near_ref,
            mem0_ref, wphi_ref, phi_ref, wqkvb_ref, wob_ref, bo_ref, bq_ref, bkv_ref,
            kv_ref, z_ref, ot_ref, on_ref,
            w_sem, in_sem, out_sem, *, dh):
    n_seg, seg, d = x_ref.shape
    n_pairs = wp_ref.shape[0]
    n_mem = mem0_ref.shape[0]
    pw = 2 * dh
    n_iter = n_seg * seg // TB

    def w_copies(p, j):
        src = (wq_hbm, wk_hbm, wv_hbm, wo_hbm)[j]
        if j < 2:
            return [pltpu.make_async_copy(src.at[p], stage_ref.at[p % RING, 3 * j:3 * j + 3],
                                          w_sem.at[p, j])]
        return [pltpu.make_async_copy(src.at[p, i], stage_ref.at[p % RING, 3 * j:3 * j + 3, i],
                                      w_sem.at[p, 2 * j - 2 + i]) for i in range(2)]

    def start_w(p, *slots):
        for j in slots:
            for copy in w_copies(p, j):
                copy.start()

    def wait_w(p, *slots):
        for j in slots:
            for copy in w_copies(p, j):
                copy.wait()

    def prepare_in(u, tiles, live=True, pace=lambda t, b: b):
        g, i = u // 2, u % 2
        for t in tiles:
            cols = pl.ds(pl.multiple_of(128 * t, 128), 128)
            blocks = [stage_ref[p % RING, t, :, :, pl.ds(pl.multiple_of(c + i * 128, 128), 128)]
                      .reshape(128, 128)
                      for c in (0, HALF) for p in (2 * g, jnp.where(live, 2 * g + 1, 0))]
            for n, r in enumerate(_strassen_weights(*(pace(t, b) for b in blocks))):
                ws_ref[g, n, pl.ds(pl.multiple_of(i * 64, 64), 64), cols] = _pack(r.T)
            wp_ref[u, :, cols] = _pack(stage_ref[u % RING, t, :, :, 2 * HALF:].reshape(128, -1).T)

    def wait_out(u):
        for i in range(2):
            pltpu.make_async_copy(stage_ref.at[0, 9:12, 0], stage_ref.at[0, 9:12, 0],
                                  w_sem.at[u // 2 * 2 + i, 4 + u % 2]).wait()

    def prepare_out(u, live=True, pace=lambda t, b: b):
        g, i = u // 2, u % 2
        for t in range(3):
            parts = [pace(3 * t + 1, stage_ref[p % RING, jnp.where(live, 9, 3) + t, i])
                     for p in (2 * g, jnp.where(live, 2 * g + 1, 0))]
            blocks = [part[:, c:c + HALF] for part in parts for c in (0, HALF)]
            for n, r in enumerate(_strassen_weights(*blocks)):
                wos_ref[g, n, t, i] = _pack(r)
            for n, part in enumerate(parts):
                wop_ref[2 * g + n, t, i] = _pack(part[:, 2 * HALF:])

    def out_copy(it, i):
        part = _chunk_rows(y_ref, it, sum(O_ROWS[:i]), O_ROWS[i])
        return pltpu.make_async_copy(y_ref.at[part], out_hbm.at[part], out_sem.at[0])

    def x_copy(rows, sem):
        return pltpu.make_async_copy(x_hbm.at[:, rows, :], y_ref.at[:, rows, :], sem)

    head, tail = slice(0, seg - PRE), slice(seg - PRE, seg)
    xt_copy, xh_copy = x_copy(tail, in_sem.at[0]), x_copy(head, in_sem.at[3])
    wqkvb_copy = pltpu.make_async_copy(wqkvb_hbm, wqkvb_ref, in_sem.at[1])
    wphi_copy = pltpu.make_async_copy(wphi_hbm, wphi_ref, in_sem.at[5])
    mem0_copy = pltpu.make_async_copy(mem0_hbm, mem0_ref, in_sem.at[4])
    wob_copy = pltpu.make_async_copy(wob_hbm, wob_ref, in_sem.at[2])

    wphi_copy.start()
    xt_copy.start()
    start_w(0, 0, 1, 2)
    wphi_copy.wait()
    _expand_phi(wphi_ref, phi_ref)
    xt_copy.wait()

    xp_ref[...] = _layernorm(y_ref[:, tail, :].astype(F32).reshape(n_seg * PRE, d)).astype(BF16)

    mem0_copy.start()
    start_w(1, 0, 1, 2)

    def pre_project(p, carry):
        @pl.when(p + 2 < n_pairs)
        def _():
            start_w(jnp.minimum(p + 2, n_pairs - 1), 0, 1, 2)

        @pl.when(p + 2 == n_pairs)
        def _():
            xh_copy.start()

        start_w(p, 3)

        @pl.when(p >= WO_LAG)
        def _():
            wait_out(jnp.maximum(p - WO_LAG, 0))

        wait_w(p, 0, 1, 2)
        kv = lax.dot_general(xp_ref[...], stage_ref[p % RING, 3:9].reshape(-1, d), NT,
                             preferred_element_type=F32)
        pre_ref[p] = kv

        def pace(t, block):
            c, r = divmod(t * PACE, xp_ref.shape[0])
            early = kv[r:r + block.shape[0], 128 * c:128 * (c + 1)].astype(BF16)
            return jnp.where(p < 0, _cols(*[early] * (block.shape[1] // 128)), block)

        prepare_in(jnp.maximum(p - 1, 0), range(9), p >= 1, pace)
        prepare_out(jnp.maximum(p - WO_LAG, 0), p >= WO_LAG, pace)
        return carry

    lax.fori_loop(0, n_pairs, pre_project, 0)

    @pl.loop(0, 3)
    def _(j):
        prepare_in(n_pairs - 1, [3 * j + i for i in range(3)])

    @pl.loop(n_pairs - WO_LAG, n_pairs)
    def _(u):
        wait_out(u)
        prepare_out(u)

    xh_copy.wait()

    wqkvb_copy.start()
    wob_copy.start()
    mem0_copy.wait()
    x_ref[0] = y_ref[0].astype(F32)

    def layer_a(layer, x_in, pre):
        step = functools.partial(
            _a_step, layer=layer, dh=dh, x_in=x_in, x_ref=x_ref, xb_ref=xb_ref, ws_ref=ws_ref,
            wp_ref=wp_ref, wos_ref=wos_ref, wop_ref=wop_ref, pre_ref=pre, ahead_ref=ahead_ref,
            o_refs=(o_even_ref, o_odd_ref), near_ref=near_ref)
        xn = [_layernorm(x_in[i].astype(F32)) for i in range(3)]
        o_odd_ref[...] = jnp.zeros(o_odd_ref.shape, F32)
        cols, per = (slice(0, 3 * pw), 1) if pre is None else (slice(0, pw), 2)

        @pl.loop(0, n_pairs // 2 // per)
        def _(j):
            for g in (j * per + i for i in range(per)):
                for i, product in enumerate((_left_product, _right_product)):
                    ahead_ref[2 * g + i, :, cols] = product(
                        xn[0][:, :HALF], xn[0][:, HALF:2 * HALF],
                        lambda a, n: jnp.dot(a.astype(BF16), _unpack(ws_ref[g, n, :, cols]),
                                             preferred_element_type=F32))

        def two_steps(it, carry):
            mem, *xn = carry
            shared = {}
            for i in range(2):
                mem, xn_next = step(2 * it + i, mem, xn, shared)
                xn = xn[1:] + [xn_next]
            return (mem, *xn)

        lax.fori_loop(0, n_seg // 2, two_steps, (mem0_ref[...].astype(F32), *xn))

    def finish_a(layer):
        a = [_cols(*(o_odd_ref[n_mem:, (2 * g + i) * pw:(2 * g + i + 1) * pw]
                     for g in range(n_pairs // 2))) for i in range(2)]
        y = _cols(*(product(*a, lambda t, n: jnp.dot(
            t.astype(BF16), _unpack(wos_ref[:, n].reshape(-1, HALF)), preferred_element_type=F32))
            for product in (_left_product, _right_product)))
        at = (n_seg - 1, slice(None), slice(0, 2 * HALF))
        x_ref[at] = jnp.where(layer == 0, y_ref[at].astype(F32), x_ref[at]) + y

    b_keys = functools.partial(_b_keys, x_ref=x_ref, xb_ref=xb_ref, bkv_ref=bkv_ref,
                               kv_ref=kv_ref, z_ref=z_ref)
    b_queries = functools.partial(_b_queries, x_ref=x_ref, xb_ref=xb_ref, y_ref=y_ref,
                                  bq_ref=bq_ref, bo_ref=bo_ref, kv_ref=kv_ref, z_ref=z_ref,
                                  ot_ref=ot_ref, on_ref=on_ref)

    def layer_pair(layer, carry):
        @pl.when(layer == 0)
        def _():
            layer_a(0, y_ref, pre_ref)

        @pl.when(layer == 0)
        def _():
            wqkvb_copy.wait()
            wob_copy.wait()
            _b_weights(wqkvb_ref, phi_ref, wob_ref, bq_ref, bkv_ref, bo_ref)

        @pl.when(layer == 1)
        def _():
            layer_a(1, x_ref, None)

        finish_a(layer)

        lax.fori_loop(0, n_iter, b_keys, 0)

        def queries(it, carry):
            def send(i):
                @pl.when(layer == 1)
                def _():
                    out_copy(it, i).start()

            b_queries(it, send)
            return carry

        lax.fori_loop(0, n_iter, queries, 0)

        return carry

    lax.fori_loop(0, 2, layer_pair, 0)
    pltpu.make_async_copy(y_ref, out_hbm, out_sem.at[0]).wait()


@functools.partial(jax.jit, static_argnames=("A_seg_len",))
def pallas_interleave_layers__memory_aug_recurrent_mem_tr__linear_kernel_hedgehog__prompt_kernel(
    A_x, A_mem0, A_Wq, A_Wk, A_Wv, A_Wo, A_seg_len, B_x, B_wqkv, B_w_phi, B_wo,
):
    del B_x
    batch, s_len, d = A_x.shape
    _, heads, dh = A_Wq.shape
    n_mem = A_mem0.shape[1]
    seg = int(A_seg_len)
    b_heads, b_dh, _ = B_w_phi.shape
    rows = n_mem + seg
    n_pairs = heads // 2
    gr = 2 * b_dh
    half = K_PAIRS * gr
    n_seg = s_len // seg
    assert batch == 1 and dh == 192 and heads == 4 * O_SPLITS[0][-1] and d == 2 * HALF + 128
    assert n_mem % 8 == 0 and seg % 16 == 0 and 128 % seg == 0 and 2 * rows <= 128
    assert s_len % TB == 0 and s_len > 3 * TB == 3 * sum(O_ROWS) and n_seg % n_pairs == 0
    assert b_heads * b_dh == d and b_dh % 8 == 4 and d % half == 0

    def head_major(w):
        return w.transpose(1, 2, 0)

    hbm = pl.BlockSpec(memory_space=pltpu.HBM)
    out = pl.pallas_call(
        functools.partial(_kernel, dh=dh),
        out_shape=jax.ShapeDtypeStruct((n_seg, seg, d), A_x.dtype),
        in_specs=[hbm] * 9,
        out_specs=hbm,
        scratch_shapes=[
            pltpu.VMEM((n_seg, seg, d), F32),
            pltpu.VMEM((n_seg, seg, d), BF16),
            pltpu.VMEM((n_seg, seg, d), BF16),
            pltpu.VMEM((n_seg * PRE, d), BF16),
            pltpu.VMEM((RING, 12, 2, 64, d), BF16),
            pltpu.VMEM((n_pairs, n_seg * PRE, 4 * dh), F32),
            pltpu.VMEM((n_pairs, seg, 6 * dh), F32),
            pltpu.VMEM((n_pairs // 2, 7, HALF // 2, 6 * dh), jnp.uint32),
            pltpu.VMEM((n_pairs, d // 2 - HALF, 6 * dh), jnp.uint32),
            pltpu.VMEM((n_pairs // 2, 7, 3, 2, 32, HALF), jnp.uint32),
            pltpu.VMEM((n_pairs, 3, 2, 32, d - 2 * HALF), jnp.uint32),
            pltpu.VMEM((rows, heads * dh), F32),
            pltpu.VMEM((rows, heads * dh), F32),
            pltpu.VMEM((n_pairs, n_mem + 8, 4 * dh), F32),
            pltpu.VMEM((n_mem, d), BF16),
            pltpu.VMEM((b_dh, b_dh, b_heads), BF16),
            pltpu.VMEM((d // (F_PAIRS * gr), F_PAIRS * gr // 2, 256), jnp.uint32),
            pltpu.VMEM(B_wqkv.shape, BF16),
            pltpu.VMEM(B_wo.shape, BF16),
            pltpu.VMEM((d // 2, d), jnp.uint32),
            pltpu.VMEM((d // 2, d), jnp.uint32),
            pltpu.VMEM((d // half, half, d), jnp.uint32),
            pltpu.VMEM((b_heads // 2, gr, 2 * gr), F32),
            pltpu.VMEM((b_heads // 2, 2 * gr, 128), F32),
            pltpu.VMEM((d // 2, TB), jnp.uint32),
            pltpu.VMEM((TB // 2, d), jnp.uint32),
            pltpu.SemaphoreType.DMA((n_pairs, 6)),
            pltpu.SemaphoreType.DMA((6,)),
            pltpu.SemaphoreType.DMA((1,)),
        ],
        compiler_params=pltpu.CompilerParams(vmem_limit_bytes=124 * 1024 * 1024),
    )(
        A_x.reshape(n_seg, seg, d), A_mem0.reshape(n_mem, d),
        head_major(A_Wq).reshape(n_pairs, 3, 2, 64, d),
        head_major(A_Wk).reshape(n_pairs, 3, 2, 64, d),
        head_major(A_Wv).reshape(n_pairs, 2, 3, 64, d), A_Wo.reshape(n_pairs, 2, 3, 64, d),
        B_wqkv, B_w_phi.transpose(1, 2, 0), B_wo,
    )
    return out.reshape(batch, s_len, d)
```

```python
import functools
import math

import jax
import jax.numpy as jnp
from jax import lax
import jax.experimental.pallas as pl
import jax.experimental.pallas.tpu as pltpu

F32 = jnp.float32
BF16 = jnp.bfloat16
NT = (((1,), (1,)), ((), ()))
LOG2E = math.log2(math.e)
MASKED = -1e9

ISSUE = ("kqSVv", "qkVSv")
LAG_S = (2, 1)
LAG_PV = (2, 3)
O_SPLITS = ((0, 1, 2, 3, 4, 5, 6, 8), (0, 1, 2, 3, 4, 6, 8))
P_ORDER = ((((1, 3), (2, 4)), ((1, 0, 6), (5,))), (((1, 3), (4, 2)), ((1, 0, 6), (5,))))
O_ORDER = (((1, 3, 2, 4), (0, 6, 5, 1)), ((3, 2, 1, 4), (5, 6, 1, 0)))
VPU_DUE = 3
KEYS_AHEAD = (14, 9)
NORM_DUE = ((0, 2), (0, 1))
HALF = 256
PRE = 8
RING = 8
WO_LAG = 3
PACE = 256
TB = 512
K_PAIRS = 8
Q_PAIRS = 8
F_PAIRS = 2
O_ROWS = (128, 128, 128, 128)


def _iota(shape, axis):
    return lax.broadcasted_iota(jnp.int32, shape, axis)


def _div(v, d):
    return (v * ((1 << 18) // d + 1)) >> 18


def _pack(x):
    return pltpu.bitcast(x.astype(BF16), jnp.uint32)


def _unpack(x):
    return pltpu.bitcast(x, BF16)


def _recip(x):
    r = pl.reciprocal(x, approx=True)
    return r * (2.0 - x * r)


def _layernorm(x):
    m = jnp.mean(x, axis=-1, keepdims=True)
    c = x - m
    v = jnp.mean(c * c, axis=-1, keepdims=True)
    return c * lax.rsqrt(v + 1e-5)


def _rows(*parts):
    return jnp.concatenate(parts, axis=0)


def _cols(*parts):
    return jnp.concatenate(parts, axis=1)


def _strassen_weights(b11, b12, b21, b22):
    f11, f12, f21, f22 = (b.astype(F32) for b in (b11, b12, b21, b22))
    return [r.astype(BF16)
            for r in (f11 + f22, b11, f12 - f22, f21 - f11, b22, f11 + f12, f21 + f22)]


def _left_product(a1, a2, times):
    return times(a2, 3) + times(a1 + a2, 1)


def _right_product(a1, a2, times):
    return times(a1 + a2, 4) + times(a1, 2)


def _token_operands(a1, a2, b1, b2):
    low = b1 + b2
    n = low.shape[0] // 2
    return ({3: b2, 2: a1, 1: low[:n], 4: a1 + a2},
            {0: a1 + b2, 6: a2 - b2, 1: low[n:], 5: b1 - a1})


def _memory_operands(m1, m2):
    both = m1 + m2
    return {0: m2, 1: both, 2: m1, 3: m2, 4: both, 5: m1, 6: m2}


def _first_results(p, n):
    m1 = _rows(p[1][n:], jnp.zeros_like(p[1][n:]))
    return ((p[1][:n] + p[3][:n], p[2][:n] + p[4][:n]),
            (p[2][n:] + p[4][n:], p[3][n:] - p[4][n:], p[3][n:] + m1, p[2][n:] - m1))


def _second_left(p, n, c11, c21):
    m1 = _rows(jnp.zeros_like(p[1][n:]), p[1][n:])
    return p[1][:n] + p[6][:n] - p[0][:n], c11 + p[0][n:] + p[6][n:], c21 + m1


def _second_right(p, n, c22):
    m1 = _rows(jnp.zeros_like(p[1][n:]), p[1][n:])
    return p[5][:n] + p[0][:n] - p[1][:n], c22 + p[0][n:] + p[5][n:] - m1


def _a_step(s, mem, xn, shared, *, layer, dh, x_in, x_ref, xb_ref, ws_ref, wp_ref, wos_ref,
            wop_ref, pre_ref, ahead_ref, o_refs, near_ref):
    odd = bool(shared)
    n_mem, seg = mem.shape[0], xn[0].shape[0]
    n_seg = xb_ref.shape[0]
    rows = n_mem + seg
    pw = 2 * dh
    n_pairs = wp_ref.shape[0]
    o_ref = o_refs[odd]
    scale = dh ** -0.5

    def after(early, value):
        return value if early is None else jnp.where(s < 0, early[:, :value.shape[1]], value)

    def after_all(early, value):
        t = functools.reduce(jnp.maximum, [early[i:i + 8, j:j + 128]
                                           for i in range(0, early.shape[0], 8)
                                           for j in range(0, early.shape[1], 128)])
        return jnp.concatenate([after(t, value[0:8]), value[8:]], axis=0)

    def slow_norm(x):
        outs = [None, None]
        for i in range(0, seg, 8):
            outs.append(_layernorm(after(outs[-2], x[i:i + 8])))
        return jnp.concatenate(outs[2:], axis=0)

    xn_next = slow_norm(x_in[jnp.minimum(s + len(xn), n_seg - 1)].astype(F32))
    done = jnp.maximum(s - 3, 0)
    xb_done = slow_norm(x_ref[done])
    xb_ref[done] = xb_done.astype(BF16)

    h = _rows(mem, xn[0])

    first = _iota((rows, 128), 1) < 64
    zero = jnp.zeros((rows, 128), F32)

    def key_blocks(t):
        t0, t1, t2 = t[:, 0:128], t[:, 128:256], t[:, 256:384]
        top = jnp.concatenate([t0, jnp.where(first, t1, 0.0), zero], axis=1)
        bot = jnp.concatenate([zero, jnp.where(first, 0.0, t1), t2], axis=1)
        return jnp.concatenate([top, bot], axis=0).astype(BF16)

    def value_blocks(t):
        mine = jnp.concatenate([first] * 3, axis=1)
        return jnp.concatenate(
            [jnp.where(mine, t, 0.0), jnp.where(mine, 0.0, t)], axis=0).astype(BF16)

    near = n_mem + 8

    def far_rows(t):
        return _rows(t[:n_mem], t[near:])

    q, k, v, probs, near_done = {}, {}, {}, {}, {}

    def project_short(p, j):
        def dot(a, w):
            return jnp.dot(a.astype(BF16), _unpack(w), preferred_element_type=F32)

        cols, top = slice(j * pw, (j + 1) * pw), h[:rows - PRE]
        most = (_left_product, _right_product)[p % 2](
            top[:, :HALF], top[:, HALF:2 * HALF], lambda a, i: dot(a, ws_ref[p // 2, i, :, cols]))
        return _rows(dot(top[:, 2 * HALF:], wp_ref[p, :, cols]) + most,
                     pre_ref[p, pl.ds(pl.multiple_of(s * PRE, PRE), PRE), (j - 1) * pw:j * pw])

    if not odd:
        shared["in"] = _token_operands(*(t[:, c:c + HALF] for t in xn[1:3] for c in (0, HALF)))
    m_in = _memory_operands(mem[:, :HALF], mem[:, HALF:2 * HALF])
    lhs_in = {i: _rows(m_in[i], t) for i, t in shared["in"][odd].items()}
    products = {}

    def project_shared(p, j):
        g, right = divmod(p, 2)
        cols, prod = slice(j * pw, (j + 1) * pw), products.setdefault(j, {})
        for i in P_ORDER[layer][odd][right]:
            prod[i] = jnp.dot(lhs_in[i], _unpack(ws_ref[g, i, :, cols]),
                              preferred_element_type=F32)
        if not odd:
            tokens = ahead_ref[p, :, cols]
            if right:
                (_, m), shared[g, j] = _first_results(prod, n_mem)
            else:
                m = prod[1][:n_mem] + prod[3][:n_mem]
        elif right:
            tokens = shared[g, j][0]
            m, ahead_ref[p, :, cols] = _second_right(prod, n_mem, shared[g, j][3])
        else:
            m, tokens, ahead_ref[p, :, cols] = _second_left(prod, n_mem, *shared[g, j][1:3])
        return jnp.dot(h[:, 2 * HALF:], _unpack(wp_ref[p, :, cols]),
                       preferred_element_type=F32) + _rows(m, tokens)

    def scores(p):
        col = far_rows(_iota((rows, 2 * rows), 1))
        row = far_rows(_iota((rows, 2 * rows), 0))
        is_a = col < rows
        visible = (row < n_mem) | (row >= jnp.where(is_a, col, col - rows))
        sc = lax.dot_general(far_rows(q[p]), key_blocks(k[p]), NT, preferred_element_type=F32)
        sc = jnp.where(visible, sc * scale, MASKED)
        max_a = jnp.max(jnp.where(is_a, sc, -jnp.inf), axis=1, keepdims=True)
        max_b = jnp.max(jnp.where(is_a, -jnp.inf, sc), axis=1, keepdims=True)
        e = jnp.exp(sc - jnp.where(is_a, max_a, max_b))
        sum_a = jnp.sum(jnp.where(is_a, e, 0.0), axis=1, keepdims=True)
        sum_b = jnp.sum(jnp.where(is_a, 0.0, e), axis=1, keepdims=True)
        probs[p] = e * _recip(jnp.where(is_a, sum_a, sum_b))
        if p == NORM_DUE[layer][0]:
            probs[p] = after_all(xn_next, probs[p])
        if p == NORM_DUE[layer][1]:
            probs[p] = after_all(xb_done, probs[p])
        if p - VPU_DUE in near_done:
            probs[p] = after_all(near_done[p - VPU_DUE], probs[p])

    def values(p):
        o = jnp.dot(probs[p], value_blocks(v[p]), preferred_element_type=F32)
        o_ref[:n_mem, p * pw:(p + 1) * pw] = o[:n_mem]
        o_ref[near:, p * pw:(p + 1) * pw] = o[n_mem:]

    chain = [None, None]
    scored = [None] * KEYS_AHEAD[layer]

    def attend_near(p):
        def key_row(j, i):
            return jnp.broadcast_to(near_ref[p, j:j + 1, 128 * i:128 * (i + 1)], (8, 128))

        near_ref[p, :, 0:pw] = k[p][:near]
        near_ref[p, :, pw:2 * pw] = v[p][:near]
        half, sub = first[0:8], _iota((8, 128), 0)
        t = q[p][n_mem:near] * (scale * LOG2E)
        q0, q2 = t[:, 0:128], t[:, 256:384]
        q1a, q1b = jnp.where(half, t[:, 128:256], 0.0), jnp.where(half, 0.0, t[:, 128:256])
        for j in range(near):
            ready = after(scored[-KEYS_AHEAD[layer]], chain[0])
            k1 = after(ready, key_row(j, 1))
            dot_a = q0 * after(ready, key_row(j, 0)) + q1a * k1
            dot_b = q2 * after(dot_a, key_row(j, 2)) + q1b * k1
            t = jnp.where(half, jnp.sum(dot_a, axis=1, keepdims=True),
                          jnp.sum(dot_b, axis=1, keepdims=True))
            scored.append(t if j <= n_mem else jnp.where(sub >= j - n_mem, t, MASKED * LOG2E))
            chain[0] = dot_b
        sc = scored[-near:]
        top = functools.reduce(jnp.maximum, sc)
        for j in range(near):
            e = jnp.exp2(sc[j] - after(chain[1], top))
            weight = after(chain[1], e)
            terms = [weight * key_row(j, 3 + i) for i in range(3)]
            total = e if j == 0 else total + e
            acc = terms if j == 0 else [a + b for a, b in zip(acc, terms)]
            chain[1] = acc[2]
        inv = _recip(total)
        o_ref[n_mem:near, p * pw:(p + 1) * pw] = _cols(*(a * inv for a in acc))
        near_done[p] = acc[2]

    out = {}

    def project_out(g0, g1):
        def halves(ref, lo, hi):
            return [_cols(*(ref[lo:hi, (2 * g + i) * pw:(2 * g + i + 1) * pw]
                            for g in range(g0, g1))) for i in range(2)]

        if not odd:
            shared["out", g0] = _token_operands(*halves(o_refs[0], n_mem, rows),
                                                *halves(o_refs[1], n_mem, rows))
        m = _memory_operands(*halves(o_ref, 0, n_mem))
        for i in O_ORDER[layer][odd]:
            r = jnp.dot(_rows(m[i], shared["out", g0][odd][i]), _unpack(wos_ref[g0:g1, i].reshape(-1, HALF)),
                        preferred_element_type=F32)
            out[i] = r + out[i] if i in out else r

    lag_s, lag_v = LAG_S[layer], LAG_S[layer] + LAG_PV[layer]
    todo = list(zip(O_SPLITS[layer][:-1], O_SPLITS[layer][1:]))
    for t in range(n_pairs + lag_v):
        if t >= n_pairs:
            project_out(*todo.pop(0))
        for c in ISSUE[layer]:
            if c == "S" and 0 <= t - lag_s < n_pairs:
                scores(t - lag_s)
            elif c == "V" and 0 <= t - lag_v < n_pairs:
                values(t - lag_v)
            elif c in "qkv" and t < n_pairs:
                j = "qkv".index(c)
                (q, k, v)[j][t] = (project_short(t, j) if j and pre_ref is not None
                                   else project_shared(t, j))
        if t < n_pairs:
            attend_near(t)
    for part in todo:
        project_out(*part)
    rest = jnp.dot(o_ref[...], _unpack(wop_ref[...].reshape(-1, wop_ref.shape[-1])),
                   preferred_element_type=F32)

    most, tail = slice(0, 2 * HALF), slice(2 * HALF, None)
    x_ref[s, :, tail] = x_in[s, :, tail].astype(F32) + rest[n_mem:]
    if odd:
        c12, c11, c21, c22 = shared["out"]
        m1, c11, c21 = _second_left(out, n_mem, c11, c21)
        m2, c22 = _second_right(out, n_mem, c22)
        x_ref[s - 1, :, most] = x_in[s - 1, :, most].astype(F32) + _cols(c11, c12)
        back = jnp.maximum(s - 2, 1)
        x_ref[back, :, most] = (x_in[back, :, most].astype(F32)
                                + jnp.where(s > 1, _cols(c21, c22), 0.0))
    else:
        (m1, m2), shared["out"] = _first_results(out, n_mem)
    return _cols(m1, m2, rest[:n_mem]), xn_next


def _pair_reduce(t, op):
    r = t[0:8]
    for i in range(8, t.shape[0], 8):
        r = op(r, t[i:i + 8])
    r = op(r, pltpu.roll(r, 4, 0))
    return op(r, pltpu.roll(r, 2, 0))


def _tile_rows(r, n):
    return jnp.concatenate([r] * (n // 8), axis=0)


def _feature_map(p):
    n = p.shape[0]
    e_pos = jnp.exp2(p - _tile_rows(_pair_reduce(p, jnp.maximum), n))
    e_neg = jnp.exp2(_tile_rows(_pair_reduce(p, jnp.minimum), n) - p)
    inv_pos = _recip(_pair_reduce(e_pos, jnp.add))
    inv_neg = _recip(_pair_reduce(e_neg, jnp.add))
    return jnp.concatenate(
        [e_pos * _tile_rows(inv_pos, n), e_neg * _tile_rows(inv_neg, n)], axis=0)


def _fold_span(b, blk):
    return b * blk // 128 * 128, -(-(b + 1) * blk // 128) * 128


def _expand_phi(wphi_ref, phi_ref):
    dh, _, heads = wphi_ref.shape
    d = dh * heads
    gr = 2 * dh
    c = _iota((dh, d), 1)
    c_feat = c - _div(c, dh) * dh
    spread = (_div(_iota((heads, d), 1), dh) == _iota((heads, d), 0)).astype(BF16)

    def gather(j, by_feat):
        for e in (j * (dh // 4) + i for i in range(dh // 4)):
            t = jnp.dot(wphi_ref[e], spread, preferred_element_type=F32)
            by_feat = jnp.where(c_feat == e, t, by_feat)
        return by_feat

    by_feat = lax.fori_loop(0, 4, gather, jnp.zeros((dh, d), F32)).astype(BF16)
    blk = F_PAIRS * gr
    r = _iota((blk, dh), 0)
    sel = (((r - _div(r, gr) * gr) >> 1) == _iota((blk, dh), 1)).astype(BF16)
    for b in range(d // blk):
        lo, hi = _fold_span(b, blk)
        r = _iota((blk, hi - lo), 0)
        head = 2 * (_div(r, gr) + b * F_PAIRS) + (r & 1)
        phi = jnp.dot(sel, by_feat[:, lo:hi], preferred_element_type=F32)
        phi_ref[b, :, 0:hi - lo] = _pack(
            jnp.where(_div(_iota((1, hi - lo), 1) + lo, dh) == head, phi, 0.0))


def _b_weights(wqkv_ref, phi_ref, wob_ref, bq_ref, bkv_ref, bo_ref):
    d = wqkv_ref.shape[0]
    blk = 2 * phi_ref.shape[1]
    half = bkv_ref.shape[1]
    bo_ref[...] = _pack(wob_ref[...])
    wv = wqkv_ref[:, 2 * d:3 * d].T
    for b in range(d // half):
        bkv_ref[b, half // 2:half, :] = _pack(wv[b * half:(b + 1) * half])
    for b in range(d // blk):
        lo, hi = _fold_span(b, blk)
        phi = _unpack(phi_ref[b, :, 0:hi - lo])
        wq = lax.dot_general(phi, wqkv_ref[:, lo:hi], NT, preferred_element_type=F32)
        wk = lax.dot_general(phi, wqkv_ref[:, d + lo:d + hi], NT, preferred_element_type=F32)
        bq_ref[b * blk // 2:(b + 1) * blk // 2, :] = _pack(wq * LOG2E)
        at = b * blk % half // 2
        bkv_ref[b * blk // half, at:at + blk // 2, :] = _pack(wk * LOG2E)


def _chunk_rows(ref, it, r0, n):
    seg = ref.shape[1]
    return pl.ds(it * (TB // seg) + r0 // seg, n // seg)


def _b_keys(it, carry, *, x_ref, xb_ref, bkv_ref, kv_ref, z_ref):
    n_blk, half, _ = bkv_ref.shape
    gr = half // K_PAIRS
    xb = xb_ref[_chunk_rows(xb_ref, it, 0, TB)].reshape(TB, -1)
    last = x_ref.shape[0] - 1 - jnp.minimum(it, 2)
    xb_ref[last] = _layernorm(x_ref[last]).astype(BF16)
    same_head = (_iota((gr, 2 * gr), 0) >= gr // 2) == ((_iota((gr, 2 * gr), 1) & 1) == 1)

    def accumulate(b, t):
        for i in range(K_PAIRS):
            g = b * K_PAIRS + i
            phi = _feature_map(t[i * gr:(i + 1) * gr])
            z_ref[g] = jnp.where(it > 0, z_ref[g], 0.0) + jnp.sum(phi, axis=1, keepdims=True)
            kv = lax.dot_general(t[half + i * gr:half + (i + 1) * gr], phi.astype(BF16), NT,
                                 preferred_element_type=F32)
            kv_ref[g] = jnp.where(it > 0, kv_ref[g], 0.0) + jnp.where(same_head, kv, 0.0)

    pending = None
    for b in range(n_blk):
        t = lax.dot_general(_unpack(bkv_ref[b]), xb, NT, preferred_element_type=F32)
        if pending is not None:
            accumulate(*pending)
        pending = (b, t)
    accumulate(*pending)
    return carry


def _b_queries(it, send, *, x_ref, xb_ref, y_ref, bq_ref, bo_ref, kv_ref, z_ref, ot_ref, on_ref):
    n_groups, gr, _ = kv_ref.shape
    blk = Q_PAIRS * gr
    sub = _iota((8, TB), 0)
    xb = xb_ref[_chunk_rows(xb_ref, it, 0, TB)].reshape(TB, -1)

    def attend(b, t):
        outs = []
        for i in range(Q_PAIRS):
            g = b * Q_PAIRS + i
            phi = _feature_map(t[i * gr:(i + 1) * gr])
            num = jnp.dot(kv_ref[g], phi.astype(BF16), preferred_element_type=F32)
            z = jnp.concatenate([z_ref[g]] * (TB // 128), axis=1)
            inv = _recip(_pair_reduce(phi * z, jnp.add) + 1e-6)
            other = pltpu.roll(inv, 1, 0)
            inv_a = jnp.where((sub & 1) == 0, inv, other)
            inv_b = jnp.where((sub & 1) == 0, other, inv)
            n = (gr - 8) // 16
            inv = jnp.concatenate(
                [inv_a] * n + [jnp.where(sub < 4, inv_a, inv_b)] + [inv_b] * n, axis=0)
            outs.append(num * inv)
        ot_ref[b * blk // 2:(b + 1) * blk // 2, :] = _pack(jnp.concatenate(outs, axis=0))

    n_blk = n_groups // Q_PAIRS
    proj = {}
    for b in range(n_blk + 1):
        if b < n_blk:
            proj[b] = lax.dot_general(_unpack(bq_ref[b * blk // 2:(b + 1) * blk // 2, :]), xb,
                                      NT, preferred_element_type=F32)
        if b > 0:
            attend(b - 1, proj[b - 1])
    on_ref[...] = _pack(_unpack(ot_ref[...]).T)
    r0 = 0
    for i, n in enumerate(O_ROWS):
        at = _chunk_rows(x_ref, it, r0, n)
        y = jnp.dot(_unpack(on_ref[r0 // 2:(r0 + n) // 2, :]), _unpack(bo_ref[...]),
                    preferred_element_type=F32)
        x = x_ref[at] + y.reshape((-1,) + x_ref.shape[1:])
        x_ref[at] = x
        y_ref[at] = x.astype(BF16)
        send(i)
        r0 += n


def _kernel(x_hbm, mem0_hbm, wq_hbm, wk_hbm, wv_hbm, wo_hbm, wqkvb_hbm, wphi_hbm, wob_hbm,
            out_hbm,
            x_ref, xb_ref, y_ref, xp_ref, stage_ref, pre_ref, ahead_ref,
            ws_ref, wp_ref, wos_ref, wop_ref, o_even_ref, o_odd_ref, near_ref,
            mem0_ref, wphi_ref, phi_ref, wqkvb_ref, wob_ref, bo_ref, bq_ref, bkv_ref,
            kv_ref, z_ref, ot_ref, on_ref,
            w_sem, in_sem, out_sem, *, dh):
    n_seg, seg, d = x_ref.shape
    n_pairs = wp_ref.shape[0]
    n_mem = mem0_ref.shape[0]
    pw = 2 * dh
    n_iter = n_seg * seg // TB

    def head_copy(p, j, i):
        return pltpu.make_async_copy(
            (wv_hbm, wo_hbm)[j - 2].at[p, i], stage_ref.at[p % RING, 3 * j:3 * j + 3, i],
            w_sem.at[p, 2 * j - 2 + i])

    def w_copies(p, j):
        if j >= 2:
            return [head_copy(p, j, i) for i in range(2)]
        return [pltpu.make_async_copy(
            (wq_hbm, wk_hbm)[j].at[p], stage_ref.at[p % RING, 3 * j:3 * j + 3], w_sem.at[p, j])]

    def start_w(p, *slots):
        for j in slots:
            for copy in w_copies(p, j):
                copy.start()

    def wait_w(p, *slots):
        for j in slots:
            for copy in w_copies(p, j):
                copy.wait()

    def prepare_in(u, tiles, live=True, pace=lambda t, b: b):
        g, i = u // 2, u % 2
        for t in tiles:
            cols = pl.ds(pl.multiple_of(128 * t, 128), 128)
            blocks = [stage_ref[p % RING, t, :, :, pl.ds(pl.multiple_of(c + i * 128, 128), 128)]
                      .reshape(128, 128)
                      for c in (0, HALF) for p in (2 * g, jnp.where(live, 2 * g + 1, 0))]
            for n, r in enumerate(_strassen_weights(*(pace(t, b) for b in blocks))):
                ws_ref[g, n, pl.ds(pl.multiple_of(i * 64, 64), 64), cols] = _pack(r.T)
            wp_ref[u, :, cols] = _pack(stage_ref[u % RING, t, :, :, 2 * HALF:].reshape(128, -1).T)

    def wait_out(u):
        for p in (u // 2 * 2, u // 2 * 2 + 1):
            head_copy(p, 3, u % 2).wait()

    def prepare_out(u, live=True, pace=lambda t, b: b):
        g, i = u // 2, u % 2
        for t in range(3):
            parts = [pace(3 * t + 1, stage_ref[p % RING, jnp.where(live, 9, 3) + t, i])
                     for p in (2 * g, jnp.where(live, 2 * g + 1, 0))]
            blocks = [part[:, c:c + HALF] for part in parts for c in (0, HALF)]
            for n, r in enumerate(_strassen_weights(*blocks)):
                wos_ref[g, n, t, i] = _pack(r)
            for n, part in enumerate(parts):
                wop_ref[2 * g + n, t, i] = _pack(part[:, 2 * HALF:])

    def out_copy(it, i):
        part = _chunk_rows(y_ref, it, sum(O_ROWS[:i]), O_ROWS[i])
        return pltpu.make_async_copy(y_ref.at[part], out_hbm.at[part], out_sem.at[0])

    def x_copy(rows, sem):
        return pltpu.make_async_copy(x_hbm.at[:, rows, :], y_ref.at[:, rows, :], sem)

    head, tail = slice(0, seg - PRE), slice(seg - PRE, seg)
    xt_copy, xh_copy = x_copy(tail, in_sem.at[0]), x_copy(head, in_sem.at[3])
    wqkvb_copy = pltpu.make_async_copy(wqkvb_hbm, wqkvb_ref, in_sem.at[1])
    wphi_copy = pltpu.make_async_copy(wphi_hbm, wphi_ref, in_sem.at[5])
    mem0_copy = pltpu.make_async_copy(mem0_hbm, mem0_ref, in_sem.at[4])
    wob_copy = pltpu.make_async_copy(wob_hbm, wob_ref, in_sem.at[2])

    wphi_copy.start()
    xt_copy.start()
    start_w(0, 0, 1, 2)
    wphi_copy.wait()
    _expand_phi(wphi_ref, phi_ref)
    xt_copy.wait()

    xp_ref[...] = _layernorm(y_ref[:, tail, :].astype(F32).reshape(n_seg * PRE, d)).astype(BF16)

    mem0_copy.start()
    start_w(1, 0, 1, 2)

    def pre_project(p, carry):
        @pl.when(p + 2 < n_pairs)
        def _():
            start_w(jnp.minimum(p + 2, n_pairs - 1), 0, 1, 2)

        @pl.when(p + 2 == n_pairs)
        def _():
            xh_copy.start()

        start_w(p, 3)

        @pl.when(p >= WO_LAG)
        def _():
            wait_out(jnp.maximum(p - WO_LAG, 0))

        wait_w(p, 0, 1, 2)
        kv = lax.dot_general(xp_ref[...], stage_ref[p % RING, 3:9].reshape(-1, d), NT,
                             preferred_element_type=F32)
        pre_ref[p] = kv

        def pace(t, block):
            c, r = divmod(t * PACE, xp_ref.shape[0])
            early = kv[r:r + block.shape[0], 128 * c:128 * (c + 1)].astype(BF16)
            return jnp.where(p < 0, _cols(*[early] * (block.shape[1] // 128)), block)

        prepare_in(jnp.maximum(p - 1, 0), range(9), p >= 1, pace)
        prepare_out(jnp.maximum(p - WO_LAG, 0), p >= WO_LAG, pace)
        return carry

    lax.fori_loop(0, n_pairs, pre_project, 0)

    @pl.loop(0, 3)
    def _(j):
        prepare_in(n_pairs - 1, [3 * j + i for i in range(3)])

    @pl.loop(n_pairs - WO_LAG, n_pairs)
    def _(u):
        wait_out(u)
        prepare_out(u)

    xh_copy.wait()

    wqkvb_copy.start()
    wob_copy.start()
    mem0_copy.wait()
    x_ref[0] = y_ref[0].astype(F32)

    def layer_a(layer, x_in, pre):
        step = functools.partial(
            _a_step, layer=layer, dh=dh, x_in=x_in, x_ref=x_ref, xb_ref=xb_ref, ws_ref=ws_ref,
            wp_ref=wp_ref, wos_ref=wos_ref, wop_ref=wop_ref, pre_ref=pre, ahead_ref=ahead_ref,
            o_refs=(o_even_ref, o_odd_ref), near_ref=near_ref)
        xn = [_layernorm(x_in[i].astype(F32)) for i in range(3)]
        o_odd_ref[...] = jnp.zeros(o_odd_ref.shape, F32)
        cols, per = (slice(0, 3 * pw), 1) if pre is None else (slice(0, pw), 2)

        @pl.loop(0, n_pairs // 2 // per)
        def _(j):
            for g in (j * per + i for i in range(per)):
                for i, product in enumerate((_left_product, _right_product)):
                    ahead_ref[2 * g + i, :, cols] = product(
                        xn[0][:, :HALF], xn[0][:, HALF:2 * HALF],
                        lambda a, n: jnp.dot(a.astype(BF16), _unpack(ws_ref[g, n, :, cols]),
                                             preferred_element_type=F32))

        def two_steps(it, carry):
            mem, *xn = carry
            shared = {}
            for i in range(2):
                mem, xn_next = step(2 * it + i, mem, xn, shared)
                xn = xn[1:] + [xn_next]
            return (mem, *xn)

        lax.fori_loop(0, n_seg // 2, two_steps, (mem0_ref[...].astype(F32), *xn))

    def finish_a(layer):
        a = [_cols(*(o_odd_ref[n_mem:, (2 * g + i) * pw:(2 * g + i + 1) * pw]
                     for g in range(n_pairs // 2))) for i in range(2)]
        y = _cols(*(product(*a, lambda t, n: jnp.dot(
            t.astype(BF16), _unpack(wos_ref[:, n].reshape(-1, HALF)), preferred_element_type=F32))
            for product in (_left_product, _right_product)))
        at = (n_seg - 1, slice(None), slice(0, 2 * HALF))
        x_ref[at] = jnp.where(layer == 0, y_ref[at].astype(F32), x_ref[at]) + y

    b_keys = functools.partial(_b_keys, x_ref=x_ref, xb_ref=xb_ref, bkv_ref=bkv_ref,
                               kv_ref=kv_ref, z_ref=z_ref)
    b_queries = functools.partial(_b_queries, x_ref=x_ref, xb_ref=xb_ref, y_ref=y_ref,
                                  bq_ref=bq_ref, bo_ref=bo_ref, kv_ref=kv_ref, z_ref=z_ref,
                                  ot_ref=ot_ref, on_ref=on_ref)

    def layer_pair(layer, carry):
        @pl.when(layer == 0)
        def _():
            layer_a(0, y_ref, pre_ref)

        @pl.when(layer == 0)
        def _():
            wqkvb_copy.wait()
            wob_copy.wait()
            _b_weights(wqkvb_ref, phi_ref, wob_ref, bq_ref, bkv_ref, bo_ref)

        @pl.when(layer == 1)
        def _():
            layer_a(1, x_ref, None)

        finish_a(layer)

        lax.fori_loop(0, n_iter, b_keys, 0)

        def queries(it, carry):
            def send(i):
                @pl.when(layer == 1)
                def _():
                    out_copy(it, i).start()

            b_queries(it, send)
            return carry

        lax.fori_loop(0, n_iter, queries, 0)

        return carry

    lax.fori_loop(0, 2, layer_pair, 0)
    pltpu.make_async_copy(y_ref, out_hbm, out_sem.at[0]).wait()


@functools.partial(jax.jit, static_argnames=("A_seg_len",))
def pallas_interleave_layers__memory_aug_recurrent_mem_tr__linear_kernel_hedgehog__prompt_kernel(
    A_x, A_mem0, A_Wq, A_Wk, A_Wv, A_Wo, A_seg_len, B_x, B_wqkv, B_w_phi, B_wo,
):
    del B_x
    batch, s_len, d = A_x.shape
    _, heads, dh = A_Wq.shape
    n_mem = A_mem0.shape[1]
    seg = int(A_seg_len)
    b_heads, b_dh, _ = B_w_phi.shape
    rows = n_mem + seg
    n_pairs = heads // 2
    gr = 2 * b_dh
    half = K_PAIRS * gr
    n_seg = s_len // seg
    assert batch == 1 and dh == 192 and heads == 4 * O_SPLITS[0][-1] and d == 2 * HALF + 128
    assert n_mem % 8 == 0 and seg % 16 == 0 and 128 % seg == 0 and 2 * rows <= 128
    assert s_len % TB == 0 and s_len > 3 * TB == 3 * sum(O_ROWS) and n_seg % n_pairs == 0
    assert b_heads * b_dh == d and b_dh % 8 == 4 and d % half == 0

    def head_major(w):
        return w.transpose(1, 2, 0)

    hbm = pl.BlockSpec(memory_space=pltpu.HBM)
    out = pl.pallas_call(
        functools.partial(_kernel, dh=dh),
        out_shape=jax.ShapeDtypeStruct((n_seg, seg, d), A_x.dtype),
        in_specs=[hbm] * 9,
        out_specs=hbm,
        scratch_shapes=[
            pltpu.VMEM((n_seg, seg, d), F32),
            pltpu.VMEM((n_seg, seg, d), BF16),
            pltpu.VMEM((n_seg, seg, d), BF16),
            pltpu.VMEM((n_seg * PRE, d), BF16),
            pltpu.VMEM((RING, 12, 2, 64, d), BF16),
            pltpu.VMEM((n_pairs, n_seg * PRE, 4 * dh), F32),
            pltpu.VMEM((n_pairs, seg, 6 * dh), F32),
            pltpu.VMEM((n_pairs // 2, 7, HALF // 2, 6 * dh), jnp.uint32),
            pltpu.VMEM((n_pairs, d // 2 - HALF, 6 * dh), jnp.uint32),
            pltpu.VMEM((n_pairs // 2, 7, 3, 2, 32, HALF), jnp.uint32),
            pltpu.VMEM((n_pairs, 3, 2, 32, d - 2 * HALF), jnp.uint32),
            pltpu.VMEM((rows, heads * dh), F32),
            pltpu.VMEM((rows, heads * dh), F32),
            pltpu.VMEM((n_pairs, n_mem + 8, 4 * dh), F32),
            pltpu.VMEM((n_mem, d), BF16),
            pltpu.VMEM((b_dh, b_dh, b_heads), BF16),
            pltpu.VMEM((d // (F_PAIRS * gr), F_PAIRS * gr // 2, 256), jnp.uint32),
            pltpu.VMEM(B_wqkv.shape, BF16),
            pltpu.VMEM(B_wo.shape, BF16),
            pltpu.VMEM((d // 2, d), jnp.uint32),
            pltpu.VMEM((d // 2, d), jnp.uint32),
            pltpu.VMEM((d // half, half, d), jnp.uint32),
            pltpu.VMEM((b_heads // 2, gr, 2 * gr), F32),
            pltpu.VMEM((b_heads // 2, 2 * gr, 128), F32),
            pltpu.VMEM((d // 2, TB), jnp.uint32),
            pltpu.VMEM((TB // 2, d), jnp.uint32),
            pltpu.SemaphoreType.DMA((n_pairs, 6)),
            pltpu.SemaphoreType.DMA((6,)),
            pltpu.SemaphoreType.DMA((1,)),
        ],
        compiler_params=pltpu.CompilerParams(vmem_limit_bytes=124 * 1024 * 1024),
    )(
        A_x.reshape(n_seg, seg, d), A_mem0.reshape(n_mem, d),
        head_major(A_Wq).reshape(n_pairs, 3, 2, 64, d),
        head_major(A_Wk).reshape(n_pairs, 3, 2, 64, d),
        head_major(A_Wv).reshape(n_pairs, 2, 3, 64, d), A_Wo.reshape(n_pairs, 2, 3, 64, d),
        B_wqkv, B_w_phi.transpose(1, 2, 0), B_wo,
    )
    return out.reshape(batch, s_len, d)
```

```python
import functools
import math

import jax
import jax.numpy as jnp
from jax import lax
import jax.experimental.pallas as pl
import jax.experimental.pallas.tpu as pltpu

F32 = jnp.float32
BF16 = jnp.bfloat16
NT = (((1,), (1,)), ((), ()))
LOG2E = math.log2(math.e)
MASKED = -1e9

ISSUE = ("kqSVv", "qkVSv")
LAG_S = (2, 1)
LAG_PV = (2, 3)
O_SPLITS = ((0, 1, 2, 3, 4, 5, 6, 8), (0, 1, 2, 3, 4, 6, 8))
P_ORDER = ((((1, 3), (2, 4)), ((1, 0, 6), (5,))), (((1, 3), (4, 2)), ((1, 0, 6), (5,))))
O_ORDER = (((1, 3, 2, 4), (0, 6, 5, 1)), ((3, 2, 1, 4), (5, 6, 1, 0)))
VPU_DUE = 3
KEYS_AHEAD = (14, 9)
NORM_DUE = ((0, 2), (0, 1))
HALF = 256
PRE = 8
RING = 8
WO_LAG = 3
TB = 512
K_PAIRS = 8
Q_PAIRS = 8
F_PAIRS = 2
O_ROWS = (128, 128, 128, 128)


def _iota(shape, axis):
    return lax.broadcasted_iota(jnp.int32, shape, axis)


def _div(v, d):
    return (v * ((1 << 18) // d + 1)) >> 18


def _pack(x):
    return pltpu.bitcast(x.astype(BF16), jnp.uint32)


def _unpack(x):
    return pltpu.bitcast(x, BF16)


def _recip(x):
    r = pl.reciprocal(x, approx=True)
    return r * (2.0 - x * r)


def _layernorm(x):
    m = jnp.mean(x, axis=-1, keepdims=True)
    c = x - m
    v = jnp.mean(c * c, axis=-1, keepdims=True)
    return c * lax.rsqrt(v + 1e-5)


def _rows(*parts):
    return jnp.concatenate(parts, axis=0)


def _cols(*parts):
    return jnp.concatenate(parts, axis=1)


def _strassen_weights(b11, b12, b21, b22):
    f11, f12, f21, f22 = (b.astype(F32) for b in (b11, b12, b21, b22))
    return [r.astype(BF16)
            for r in (f11 + f22, b11, f12 - f22, f21 - f11, b22, f11 + f12, f21 + f22)]


def _balance(left, right):
    def exponent(t):
        bits = pltpu.bitcast(_pack(t) & 0x7F800000, F32)
        peak = jnp.max(jnp.max(bits, axis=1, keepdims=True), axis=0, keepdims=True)
        return pltpu.bitcast(jnp.broadcast_to(peak, (8, 128)), jnp.int32) >> 23

    left, right = exponent(left), exponent(right)
    shift = jnp.where(jnp.minimum(left, right) > 0, jnp.clip(left - right, -100, 100), 0)
    return [pltpu.bitcast((127 + e) << 23, F32) for e in (shift, -shift)]


def _left_product(a1, a2, times):
    return times(a2, 3) + times(a1 + a2, 1)


def _right_product(a1, a2, times):
    return times(a1 + a2, 4) + times(a1, 2)


def _token_operands(a1, a2, b1, b2):
    low = b1 + b2
    n = low.shape[0] // 2
    return ({3: b2, 2: a1, 1: low[:n], 4: a1 + a2},
            {0: a1 + b2, 6: a2 - b2, 1: low[n:], 5: b1 - a1})


def _memory_operands(m1, m2):
    both = m1 + m2
    return {0: m2, 1: both, 2: m1, 3: m2, 4: both, 5: m1, 6: m2}


def _first_results(p, n):
    m1 = _rows(p[1][n:], jnp.zeros_like(p[1][n:]))
    return ((p[1][:n] + p[3][:n], p[2][:n] + p[4][:n]),
            (p[2][n:] + p[4][n:], p[3][n:] - p[4][n:], p[3][n:] + m1, p[2][n:] - m1))


def _second_left(p, n, c11, c21):
    m1 = _rows(jnp.zeros_like(p[1][n:]), p[1][n:])
    return p[1][:n] + p[6][:n] - p[0][:n], c11 + p[0][n:] + p[6][n:], c21 + m1


def _second_right(p, n, c22):
    m1 = _rows(jnp.zeros_like(p[1][n:]), p[1][n:])
    return p[5][:n] + p[0][:n] - p[1][:n], c22 + p[0][n:] + p[5][n:] - m1


def _a_step(s, mem, xn, shared, *, layer, dh, x_in, x_ref, xb_ref, ws_ref, wp_ref, wos_ref,
            wop_ref, undo_ref, undo_v_ref, pre_ref, ahead_ref, o_refs, near_ref):
    odd = bool(shared)
    n_mem, seg = mem.shape[0], xn[0].shape[0]
    n_seg = xb_ref.shape[0]
    rows = n_mem + seg
    pw = 2 * dh
    n_pairs = wp_ref.shape[0]
    o_ref = o_refs[odd]
    scale = dh ** -0.5

    def after(early, value):
        return value if early is None else jnp.where(s < 0, early[:, :value.shape[1]], value)

    def after_all(early, value):
        t = functools.reduce(jnp.maximum, [early[i:i + 8, j:j + 128]
                                           for i in range(0, early.shape[0], 8)
                                           for j in range(0, early.shape[1], 128)])
        return jnp.concatenate([after(t, value[0:8]), value[8:]], axis=0)

    def slow_norm(x):
        outs = [None, None]
        for i in range(0, seg, 8):
            outs.append(_layernorm(after(outs[-2], x[i:i + 8])))
        return jnp.concatenate(outs[2:], axis=0)

    xn_next = slow_norm(x_in[jnp.minimum(s + len(xn), n_seg - 1)].astype(F32))
    done = jnp.maximum(s - 3, 0)
    xb_done = slow_norm(x_ref[done])
    xb_ref[done] = xb_done.astype(BF16)

    h = _rows(mem, xn[0])

    first = _iota((rows, 128), 1) < 64
    zero = jnp.zeros((rows, 128), F32)

    def key_blocks(t):
        t0, t1, t2 = t[:, 0:128], t[:, 128:256], t[:, 256:384]
        top = jnp.concatenate([t0, jnp.where(first, t1, 0.0), zero], axis=1)
        bot = jnp.concatenate([zero, jnp.where(first, 0.0, t1), t2], axis=1)
        return jnp.concatenate([top, bot], axis=0).astype(BF16)

    def value_blocks(t):
        mine = jnp.concatenate([first] * 3, axis=1)
        return jnp.concatenate(
            [jnp.where(mine, t, 0.0), jnp.where(mine, 0.0, t)], axis=0).astype(BF16)

    near = n_mem + 8

    def far_rows(t):
        return _rows(t[:n_mem], t[near:])

    q, k, v, probs, near_done = {}, {}, {}, {}, {}

    def project_short(p, j):
        def dot(a, w):
            return jnp.dot(a.astype(BF16), _unpack(w), preferred_element_type=F32)

        cols, top = slice(j * pw, (j + 1) * pw), h[:rows - PRE]
        most = (_left_product, _right_product)[p % 2](
            top[:, :HALF], top[:, HALF:2 * HALF], lambda a, i: dot(a, ws_ref[p // 2, i, :, cols]))
        if p % 2:
            most = most * _tile_rows(undo_ref[p // 2, :, cols], rows - PRE)
        return _rows(dot(top[:, 2 * HALF:], wp_ref[p, :, cols]) + most,
                     pre_ref[p, pl.ds(pl.multiple_of(s * PRE, PRE), PRE), (j - 1) * pw:j * pw])

    if not odd:
        shared["in"] = _token_operands(*(t[:, c:c + HALF] for t in xn[1:3] for c in (0, HALF)))
    m_in = _memory_operands(mem[:, :HALF], mem[:, HALF:2 * HALF])
    lhs_in = {i: _rows(m_in[i], t) for i, t in shared["in"][odd].items()}
    products = {}

    def project_shared(p, j):
        g, right = divmod(p, 2)
        cols, prod = slice(j * pw, (j + 1) * pw), products.setdefault(j, {})
        for i in P_ORDER[layer][odd][right]:
            prod[i] = jnp.dot(lhs_in[i], _unpack(ws_ref[g, i, :, cols]),
                              preferred_element_type=F32)
        if not odd:
            tokens = ahead_ref[p, :, cols]
            if right:
                (_, m), shared[g, j] = _first_results(prod, n_mem)
            else:
                m = prod[1][:n_mem] + prod[3][:n_mem]
        elif right:
            tokens = shared[g, j][0]
            m, ahead_ref[p, :, cols] = _second_right(prod, n_mem, shared[g, j][3])
        else:
            m, tokens, ahead_ref[p, :, cols] = _second_left(prod, n_mem, *shared[g, j][1:3])
        most = _rows(m, tokens)
        if right:
            most = most * _tile_rows(undo_ref[g, :, cols], rows)
        return jnp.dot(h[:, 2 * HALF:], _unpack(wp_ref[p, :, cols]),
                       preferred_element_type=F32) + most

    def scores(p):
        col = far_rows(_iota((rows, 2 * rows), 1))
        row = far_rows(_iota((rows, 2 * rows), 0))
        is_a = col < rows
        visible = (row < n_mem) | (row >= jnp.where(is_a, col, col - rows))
        sc = lax.dot_general(far_rows(q[p]), key_blocks(k[p]), NT, preferred_element_type=F32)
        sc = jnp.where(visible, sc * scale, MASKED)
        max_a = jnp.max(jnp.where(is_a, sc, -jnp.inf), axis=1, keepdims=True)
        max_b = jnp.max(jnp.where(is_a, -jnp.inf, sc), axis=1, keepdims=True)
        e = jnp.exp(sc - jnp.where(is_a, max_a, max_b))
        sum_a = jnp.sum(jnp.where(is_a, e, 0.0), axis=1, keepdims=True)
        sum_b = jnp.sum(jnp.where(is_a, 0.0, e), axis=1, keepdims=True)
        probs[p] = e * _recip(jnp.where(is_a, sum_a, sum_b))
        if p == NORM_DUE[layer][0]:
            probs[p] = after_all(xn_next, probs[p])
        if p == NORM_DUE[layer][1]:
            probs[p] = after_all(xb_done, probs[p])
        if p - VPU_DUE in near_done:
            probs[p] = after_all(near_done[p - VPU_DUE], probs[p])

    def values(p):
        o = jnp.dot(probs[p], value_blocks(v[p]), preferred_element_type=F32)
        o_ref[:n_mem, p * pw:(p + 1) * pw] = o[:n_mem]
        o_ref[near:, p * pw:(p + 1) * pw] = o[n_mem:]

    chain = [None, None]
    scored = [None] * KEYS_AHEAD[layer]

    def attend_near(p):
        def key_row(j, i):
            return jnp.broadcast_to(near_ref[p, j:j + 1, 128 * i:128 * (i + 1)], (8, 128))

        near_ref[p, :, 0:pw] = k[p][:near]
        near_ref[p, :, pw:2 * pw] = v[p][:near]
        half, sub = first[0:8], _iota((8, 128), 0)
        t = q[p][n_mem:near] * (scale * LOG2E)
        q0, q2 = t[:, 0:128], t[:, 256:384]
        q1a, q1b = jnp.where(half, t[:, 128:256], 0.0), jnp.where(half, 0.0, t[:, 128:256])
        for j in range(near):
            ready = after(scored[-KEYS_AHEAD[layer]], chain[0])
            k1 = after(ready, key_row(j, 1))
            dot_a = q0 * after(ready, key_row(j, 0)) + q1a * k1
            dot_b = q2 * after(dot_a, key_row(j, 2)) + q1b * k1
            t = jnp.where(half, jnp.sum(dot_a, axis=1, keepdims=True),
                          jnp.sum(dot_b, axis=1, keepdims=True))
            scored.append(t if j <= n_mem else jnp.where(sub >= j - n_mem, t, MASKED * LOG2E))
            chain[0] = dot_b
        sc = scored[-near:]
        top = functools.reduce(jnp.maximum, sc)
        for j in range(near):
            e = jnp.exp2(sc[j] - after(chain[1], top))
            weight = after(chain[1], e)
            terms = [weight * key_row(j, 3 + i) for i in range(3)]
            total = e if j == 0 else total + e
            acc = terms if j == 0 else [a + b for a, b in zip(acc, terms)]
            chain[1] = acc[2]
        inv = _recip(total)
        o_ref[n_mem:near, p * pw:(p + 1) * pw] = _cols(*(a * inv for a in acc))
        near_done[p] = acc[2]

    out = {}

    def project_out(g0, g1):
        def halves(ref, lo, hi):
            return [_cols(*(ref[lo:hi, (2 * g + i) * pw:(2 * g + i + 1) * pw]
                            for g in range(g0, g1))) for i in range(2)]

        if not odd:
            shared["out", g0] = _token_operands(*halves(o_refs[0], n_mem, rows),
                                                *halves(o_refs[1], n_mem, rows))
        m = _memory_operands(*halves(o_ref, 0, n_mem))
        for i in O_ORDER[layer][odd]:
            r = jnp.dot(_rows(m[i], shared["out", g0][odd][i]), _unpack(wos_ref[g0:g1, i].reshape(-1, HALF)),
                        preferred_element_type=F32)
            out[i] = r + out[i] if i in out else r

    lag_s, lag_v = LAG_S[layer], LAG_S[layer] + LAG_PV[layer]
    todo = list(zip(O_SPLITS[layer][:-1], O_SPLITS[layer][1:]))
    for t in range(n_pairs + lag_v):
        if t >= n_pairs:
            project_out(*todo.pop(0))
        for c in ISSUE[layer]:
            if c == "S" and 0 <= t - lag_s < n_pairs:
                scores(t - lag_s)
            elif c == "V" and 0 <= t - lag_v < n_pairs:
                values(t - lag_v)
            elif c in "qkv" and t < n_pairs:
                j = "qkv".index(c)
                (q, k, v)[j][t] = (project_short(t, j) if j and pre_ref is not None
                                   else project_shared(t, j))
                if c == "v" and t % 2:
                    undo = jnp.where(first[:8], undo_v_ref[t // 2, 0], undo_v_ref[t // 2, 1])
                    v[t] = v[t] * _cols(*[_tile_rows(undo, rows)] * 3)
        if t < n_pairs:
            attend_near(t)
    for part in todo:
        project_out(*part)
    rest = jnp.dot(o_ref[...], _unpack(wop_ref[...].reshape(-1, wop_ref.shape[-1])),
                   preferred_element_type=F32)

    most, tail = slice(0, 2 * HALF), slice(2 * HALF, None)
    x_ref[s, :, tail] = x_in[s, :, tail].astype(F32) + rest[n_mem:]
    if odd:
        c12, c11, c21, c22 = shared["out"]
        m1, c11, c21 = _second_left(out, n_mem, c11, c21)
        m2, c22 = _second_right(out, n_mem, c22)
        x_ref[s - 1, :, most] = x_in[s - 1, :, most].astype(F32) + _cols(c11, c12)
        back = jnp.maximum(s - 2, 1)
        x_ref[back, :, most] = (x_in[back, :, most].astype(F32)
                                + jnp.where(s > 1, _cols(c21, c22), 0.0))
    else:
        (m1, m2), shared["out"] = _first_results(out, n_mem)
    return _cols(m1, m2, rest[:n_mem]), xn_next


def _pair_reduce(t, op):
    r = t[0:8]
    for i in range(8, t.shape[0], 8):
        r = op(r, t[i:i + 8])
    r = op(r, pltpu.roll(r, 4, 0))
    return op(r, pltpu.roll(r, 2, 0))


def _tile_rows(r, n):
    return jnp.concatenate([r] * (n // 8), axis=0)


def _feature_map(p):
    n = p.shape[0]
    e_pos = jnp.exp2(p - _tile_rows(_pair_reduce(p, jnp.maximum), n))
    e_neg = jnp.exp2(_tile_rows(_pair_reduce(p, jnp.minimum), n) - p)
    inv_pos = _recip(_pair_reduce(e_pos, jnp.add))
    inv_neg = _recip(_pair_reduce(e_neg, jnp.add))
    return jnp.concatenate(
        [e_pos * _tile_rows(inv_pos, n), e_neg * _tile_rows(inv_neg, n)], axis=0)


def _fold_span(b, blk):
    return b * blk // 128 * 128, -(-(b + 1) * blk // 128) * 128


def _expand_phi(wphi_ref, phi_ref):
    dh, _, heads = wphi_ref.shape
    d = dh * heads
    gr = 2 * dh
    c = _iota((dh, d), 1)
    c_feat = c - _div(c, dh) * dh
    spread = (_div(_iota((heads, d), 1), dh) == _iota((heads, d), 0)).astype(BF16)

    def gather(j, by_feat):
        for e in (j * (dh // 4) + i for i in range(dh // 4)):
            t = jnp.dot(wphi_ref[e], spread, preferred_element_type=F32)
            by_feat = jnp.where(c_feat == e, t, by_feat)
        return by_feat

    by_feat = lax.fori_loop(0, 4, gather, jnp.zeros((dh, d), F32)).astype(BF16)
    blk = F_PAIRS * gr
    r = _iota((blk, dh), 0)
    sel = (((r - _div(r, gr) * gr) >> 1) == _iota((blk, dh), 1)).astype(BF16)
    for b in range(d // blk):
        lo, hi = _fold_span(b, blk)
        r = _iota((blk, hi - lo), 0)
        head = 2 * (_div(r, gr) + b * F_PAIRS) + (r & 1)
        phi = jnp.dot(sel, by_feat[:, lo:hi], preferred_element_type=F32)
        phi_ref[b, :, 0:hi - lo] = _pack(
            jnp.where(_div(_iota((1, hi - lo), 1) + lo, dh) == head, phi, 0.0))


def _b_weights(wqkv_ref, phi_ref, wob_ref, bq_ref, bkv_ref, bo_ref):
    d = wqkv_ref.shape[0]
    blk = 2 * phi_ref.shape[1]
    half = bkv_ref.shape[1]
    bo_ref[...] = _pack(wob_ref[...])
    wv = wqkv_ref[:, 2 * d:3 * d].T
    for b in range(d // half):
        bkv_ref[b, half // 2:half, :] = _pack(wv[b * half:(b + 1) * half])
    for b in range(d // blk):
        lo, hi = _fold_span(b, blk)
        phi = _unpack(phi_ref[b, :, 0:hi - lo])
        wq = lax.dot_general(phi, wqkv_ref[:, lo:hi], NT, preferred_element_type=F32)
        wk = lax.dot_general(phi, wqkv_ref[:, d + lo:d + hi], NT, preferred_element_type=F32)
        bq_ref[b * blk // 2:(b + 1) * blk // 2, :] = _pack(wq * LOG2E)
        at = b * blk % half // 2
        bkv_ref[b * blk // half, at:at + blk // 2, :] = _pack(wk * LOG2E)


def _chunk_rows(ref, it, r0, n):
    seg = ref.shape[1]
    return pl.ds(it * (TB // seg) + r0 // seg, n // seg)


def _b_keys(it, carry, *, x_ref, xb_ref, bkv_ref, kv_ref, z_ref):
    n_blk, half, _ = bkv_ref.shape
    gr = half // K_PAIRS
    xb = xb_ref[_chunk_rows(xb_ref, it, 0, TB)].reshape(TB, -1)
    last = x_ref.shape[0] - 1 - jnp.minimum(it, 2)
    xb_ref[last] = _layernorm(x_ref[last]).astype(BF16)
    same_head = (_iota((gr, 2 * gr), 0) >= gr // 2) == ((_iota((gr, 2 * gr), 1) & 1) == 1)

    def accumulate(b, t):
        for i in range(K_PAIRS):
            g = b * K_PAIRS + i
            phi = _feature_map(t[i * gr:(i + 1) * gr])
            z_ref[g] = jnp.where(it > 0, z_ref[g], 0.0) + jnp.sum(phi, axis=1, keepdims=True)
            kv = lax.dot_general(t[half + i * gr:half + (i + 1) * gr], phi.astype(BF16), NT,
                                 preferred_element_type=F32)
            kv_ref[g] = jnp.where(it > 0, kv_ref[g], 0.0) + jnp.where(same_head, kv, 0.0)

    pending = None
    for b in range(n_blk):
        t = lax.dot_general(_unpack(bkv_ref[b]), xb, NT, preferred_element_type=F32)
        if pending is not None:
            accumulate(*pending)
        pending = (b, t)
    accumulate(*pending)
    return carry


def _b_queries(it, send, *, x_ref, xb_ref, y_ref, bq_ref, bo_ref, kv_ref, z_ref, ot_ref, on_ref):
    n_groups, gr, _ = kv_ref.shape
    blk = Q_PAIRS * gr
    sub = _iota((8, TB), 0)
    xb = xb_ref[_chunk_rows(xb_ref, it, 0, TB)].reshape(TB, -1)

    def attend(b, t):
        outs = []
        for i in range(Q_PAIRS):
            g = b * Q_PAIRS + i
            phi = _feature_map(t[i * gr:(i + 1) * gr])
            num = jnp.dot(kv_ref[g], phi.astype(BF16), preferred_element_type=F32)
            z = jnp.concatenate([z_ref[g]] * (TB // 128), axis=1)
            inv = _recip(_pair_reduce(phi * z, jnp.add) + 1e-6)
            other = pltpu.roll(inv, 1, 0)
            inv_a = jnp.where((sub & 1) == 0, inv, other)
            inv_b = jnp.where((sub & 1) == 0, other, inv)
            n = (gr - 8) // 16
            inv = jnp.concatenate(
                [inv_a] * n + [jnp.where(sub < 4, inv_a, inv_b)] + [inv_b] * n, axis=0)
            outs.append(num * inv)
        ot_ref[b * blk // 2:(b + 1) * blk // 2, :] = _pack(jnp.concatenate(outs, axis=0))

    n_blk = n_groups // Q_PAIRS
    proj = {}
    for b in range(n_blk + 1):
        if b < n_blk:
            proj[b] = lax.dot_general(_unpack(bq_ref[b * blk // 2:(b + 1) * blk // 2, :]), xb,
                                      NT, preferred_element_type=F32)
        if b > 0:
            attend(b - 1, proj[b - 1])
    on_ref[...] = _pack(_unpack(ot_ref[...]).T)
    r0 = 0
    for i, n in enumerate(O_ROWS):
        at = _chunk_rows(x_ref, it, r0, n)
        y = jnp.dot(_unpack(on_ref[r0 // 2:(r0 + n) // 2, :]), _unpack(bo_ref[...]),
                    preferred_element_type=F32)
        x = x_ref[at] + y.reshape((-1,) + x_ref.shape[1:])
        x_ref[at] = x
        y_ref[at] = x.astype(BF16)
        send(i)
        r0 += n


def _kernel(x_hbm, mem0_hbm, wq_hbm, wk_hbm, wv_hbm, wo_hbm, wqkvb_hbm, wphi_hbm, wob_hbm,
            out_hbm,
            x_ref, xb_ref, y_ref, xp_ref, stage_ref, pre_ref, ahead_ref,
            ws_ref, wp_ref, wos_ref, wop_ref, scale_ref, undo_ref, undo_v_ref, o_even_ref, o_odd_ref, near_ref,
            mem0_ref, wphi_ref, phi_ref, wqkvb_ref, wob_ref, bo_ref, bq_ref, bkv_ref,
            kv_ref, z_ref, ot_ref, on_ref,
            w_sem, in_sem, out_sem, *, dh):
    n_seg, seg, d = x_ref.shape
    n_pairs = wp_ref.shape[0]
    n_mem = mem0_ref.shape[0]
    pw = 2 * dh
    n_iter = n_seg * seg // TB

    def head_copy(p, j, i):
        return pltpu.make_async_copy(
            (wv_hbm, wo_hbm)[j - 2].at[p, i], stage_ref.at[p % RING, 3 * j:3 * j + 3, i],
            w_sem.at[p, 2 * j - 2 + i])

    def w_copies(p, j):
        if j >= 2:
            return [head_copy(p, j, i) for i in range(2)]
        return [pltpu.make_async_copy(
            (wq_hbm, wk_hbm)[j].at[p], stage_ref.at[p % RING, 3 * j:3 * j + 3], w_sem.at[p, j])]

    def start_w(p, *slots):
        for j in slots:
            for copy in w_copies(p, j):
                copy.start()

    def wait_w(p, *slots):
        for j in slots:
            for copy in w_copies(p, j):
                copy.wait()

    def prepare_in(u, tiles, live=True, pace=None):
        g, i = u // 2, u % 2
        slots = [p % RING for p in (2 * g, jnp.where(live, 2 * g + 1, 0))]
        for j in range(3) if pace else ():
            factors = [_balance(*(stage_ref[p, 3 * j + 2 * n, n, :16, :2 * HALF] for p in slots))
                       for n in range(2)]
            for t in range(3):
                heads = [factors[n if j == 2 else (2 * t + n) // 3] for n in range(2)]
                undo_ref[g, :, pl.ds(128 * (3 * j + t), 128)] = jnp.where(
                    _iota((8, 128), 1) < 64, *(f[1] for f in heads))
                scale_ref[3 * j + t] = _rows(*(f[0] for f in heads))
        pace = pace or (lambda t, b: b)
        for t in tiles:
            cols = pl.ds(pl.multiple_of(128 * t, 128), 128)
            scale = _rows(*(_tile_rows(scale_ref[t, 8 * n:8 * n + 8, :], 64) for n in range(2)))
            b11, b12, b21, b22 = (
                pace(t, stage_ref[p, t, :, :, pl.ds(pl.multiple_of(c + i * 128, 128), 128)]
                     .reshape(128, 128)) for c in (0, HALF) for p in slots)
            for n, r in enumerate(_strassen_weights(b11, b12 * scale, b21, b22 * scale)):
                ws_ref[g, n, pl.ds(pl.multiple_of(i * 64, 64), 64), cols] = _pack(r.T)
            wp_ref[u, :, cols] = _pack(stage_ref[u % RING, t, :, :, 2 * HALF:].reshape(128, -1).T)

    def wait_out(u):
        for p in (u // 2 * 2, u // 2 * 2 + 1):
            head_copy(p, 3, u % 2).wait()

    def prepare_out(u, live=True, pace=lambda t, b: b):
        g, i = u // 2, u % 2
        slots = [p % RING for p in (2 * g, jnp.where(live, 2 * g + 1, 0))]
        base = jnp.where(live, 9, 3)
        scale, undo_v_ref[g, i] = _balance(*(stage_ref[p, base, i, :16] for p in slots))
        for t in range(3):
            parts = [pace(10 + 2 * t, stage_ref[p, base + t, i]) for p in slots]
            parts[1] = parts[1] * _cols(*[_tile_rows(scale, 64)] * (d // 128))
            blocks = [part[:, c:c + HALF] for part in parts for c in (0, HALF)]
            for n, r in enumerate(_strassen_weights(*blocks)):
                wos_ref[g, n, t, i] = _pack(r)
            for n, part in enumerate(parts):
                wop_ref[2 * g + n, t, i] = _pack(part[:, 2 * HALF:])

    def out_copy(it, i):
        part = _chunk_rows(y_ref, it, sum(O_ROWS[:i]), O_ROWS[i])
        return pltpu.make_async_copy(y_ref.at[part], out_hbm.at[part], out_sem.at[0])

    def x_copy(rows, sem):
        return pltpu.make_async_copy(x_hbm.at[:, rows, :], y_ref.at[:, rows, :], sem)

    head, tail = slice(0, seg - PRE), slice(seg - PRE, seg)
    xt_copy, xh_copy = x_copy(tail, in_sem.at[0]), x_copy(head, in_sem.at[3])
    wqkvb_copy = pltpu.make_async_copy(wqkvb_hbm, wqkvb_ref, in_sem.at[1])
    wphi_copy = pltpu.make_async_copy(wphi_hbm, wphi_ref, in_sem.at[5])
    mem0_copy = pltpu.make_async_copy(mem0_hbm, mem0_ref, in_sem.at[4])
    wob_copy = pltpu.make_async_copy(wob_hbm, wob_ref, in_sem.at[2])

    wphi_copy.start()
    xt_copy.start()
    start_w(0, 0, 1, 2)
    wphi_copy.wait()
    _expand_phi(wphi_ref, phi_ref)
    xt_copy.wait()

    xp_ref[...] = _layernorm(y_ref[:, tail, :].astype(F32).reshape(n_seg * PRE, d)).astype(BF16)

    mem0_copy.start()
    start_w(1, 0, 1, 2)

    def pre_project(p, carry):
        @pl.when(p + 2 < n_pairs)
        def _():
            start_w(jnp.minimum(p + 2, n_pairs - 1), 0, 1, 2)

        @pl.when(p + 2 == n_pairs)
        def _():
            xh_copy.start()

        start_w(p, 3)

        @pl.when(p >= WO_LAG)
        def _():
            wait_out(jnp.maximum(p - WO_LAG, 0))

        wait_w(p, 0, 1, 2)
        kv = lax.dot_general(xp_ref[...], stage_ref[p % RING, 3:9].reshape(-1, d), NT,
                             preferred_element_type=F32)
        pre_ref[p] = kv

        def pace(t, block):
            c, r = divmod(t * 128, xp_ref.shape[0])
            early = kv[r:r + block.shape[0], 128 * c:128 * (c + 1)].astype(BF16)
            return jnp.where(p < 0, _cols(*[early] * (block.shape[1] // 128)), block)

        prepare_out(jnp.maximum(p - WO_LAG, 0), p >= WO_LAG, pace)
        prepare_in(jnp.maximum(p - 1, 0), range(9), p >= 1, pace)
        return carry

    lax.fori_loop(0, n_pairs, pre_project, 0)

    @pl.loop(0, 3)
    def _(j):
        prepare_in(n_pairs - 1, [3 * j + i for i in range(3)])

    @pl.loop(n_pairs - WO_LAG, n_pairs)
    def _(u):
        wait_out(u)
        prepare_out(u)

    xh_copy.wait()

    wqkvb_copy.start()
    wob_copy.start()
    mem0_copy.wait()
    x_ref[0] = y_ref[0].astype(F32)

    def layer_a(layer, x_in, pre):
        step = functools.partial(
            _a_step, layer=layer, dh=dh, x_in=x_in, x_ref=x_ref, xb_ref=xb_ref, ws_ref=ws_ref,
            wp_ref=wp_ref, wos_ref=wos_ref, wop_ref=wop_ref, pre_ref=pre, ahead_ref=ahead_ref,
            undo_ref=undo_ref, undo_v_ref=undo_v_ref, o_refs=(o_even_ref, o_odd_ref),
            near_ref=near_ref)
        xn = [_layernorm(x_in[i].astype(F32)) for i in range(3)]
        o_odd_ref[...] = jnp.zeros(o_odd_ref.shape, F32)
        cols, per = (slice(0, 3 * pw), 1) if pre is None else (slice(0, pw), 2)

        @pl.loop(0, n_pairs // 2 // per)
        def _(j):
            for g in (j * per + i for i in range(per)):
                for i, product in enumerate((_left_product, _right_product)):
                    ahead_ref[2 * g + i, :, cols] = product(
                        xn[0][:, :HALF], xn[0][:, HALF:2 * HALF],
                        lambda a, n: jnp.dot(a.astype(BF16), _unpack(ws_ref[g, n, :, cols]),
                                             preferred_element_type=F32))

        def two_steps(it, carry):
            mem, *xn = carry
            shared = {}
            for i in range(2):
                mem, xn_next = step(2 * it + i, mem, xn, shared)
                xn = xn[1:] + [xn_next]
            return (mem, *xn)

        lax.fori_loop(0, n_seg // 2, two_steps, (mem0_ref[...].astype(F32), *xn))

    def finish_a(layer):
        a = [_cols(*(o_odd_ref[n_mem:, (2 * g + i) * pw:(2 * g + i + 1) * pw]
                     for g in range(n_pairs // 2))) for i in range(2)]
        y = _cols(*(product(*a, lambda t, n: jnp.dot(
            t.astype(BF16), _unpack(wos_ref[:, n].reshape(-1, HALF)), preferred_element_type=F32))
            for product in (_left_product, _right_product)))
        at = (n_seg - 1, slice(None), slice(0, 2 * HALF))
        x_ref[at] = jnp.where(layer == 0, y_ref[at].astype(F32), x_ref[at]) + y

    b_keys = functools.partial(_b_keys, x_ref=x_ref, xb_ref=xb_ref, bkv_ref=bkv_ref,
                               kv_ref=kv_ref, z_ref=z_ref)
    b_queries = functools.partial(_b_queries, x_ref=x_ref, xb_ref=xb_ref, y_ref=y_ref,
                                  bq_ref=bq_ref, bo_ref=bo_ref, kv_ref=kv_ref, z_ref=z_ref,
                                  ot_ref=ot_ref, on_ref=on_ref)

    def layer_pair(layer, carry):
        @pl.when(layer == 0)
        def _():
            layer_a(0, y_ref, pre_ref)

        @pl.when(layer == 0)
        def _():
            wqkvb_copy.wait()
            wob_copy.wait()
            _b_weights(wqkvb_ref, phi_ref, wob_ref, bq_ref, bkv_ref, bo_ref)

        @pl.when(layer == 1)
        def _():
            layer_a(1, x_ref, None)

        finish_a(layer)

        lax.fori_loop(0, n_iter, b_keys, 0)

        def queries(it, carry):
            def send(i):
                @pl.when(layer == 1)
                def _():
                    out_copy(it, i).start()

            b_queries(it, send)
            return carry

        lax.fori_loop(0, n_iter, queries, 0)

        return carry

    lax.fori_loop(0, 2, layer_pair, 0)
    pltpu.make_async_copy(y_ref, out_hbm, out_sem.at[0]).wait()


@functools.partial(jax.jit, static_argnames=("A_seg_len",))
def pallas_interleave_layers__memory_aug_recurrent_mem_tr__linear_kernel_hedgehog__prompt_kernel(
    A_x, A_mem0, A_Wq, A_Wk, A_Wv, A_Wo, A_seg_len, B_x, B_wqkv, B_w_phi, B_wo,
):
    del B_x
    batch, s_len, d = A_x.shape
    _, heads, dh = A_Wq.shape
    n_mem = A_mem0.shape[1]
    seg = int(A_seg_len)
    b_heads, b_dh, _ = B_w_phi.shape
    rows = n_mem + seg
    n_pairs = heads // 2
    gr = 2 * b_dh
    half = K_PAIRS * gr
    n_seg = s_len // seg
    assert batch == 1 and dh == 192 and heads == 4 * O_SPLITS[0][-1] and d == 2 * HALF + 128
    assert n_mem % 8 == 0 and seg % 16 == 0 and 128 % seg == 0 and 2 * rows <= 128
    assert s_len % TB == 0 and s_len > 3 * TB == 3 * sum(O_ROWS) and n_seg % n_pairs == 0
    assert b_heads * b_dh == d and b_dh % 8 == 4 and d % half == 0

    def head_major(w):
        return w.transpose(1, 2, 0)

    hbm = pl.BlockSpec(memory_space=pltpu.HBM)
    out = pl.pallas_call(
        functools.partial(_kernel, dh=dh),
        out_shape=jax.ShapeDtypeStruct((n_seg, seg, d), A_x.dtype),
        in_specs=[hbm] * 9,
        out_specs=hbm,
        scratch_shapes=[
            pltpu.VMEM((n_seg, seg, d), F32),
            pltpu.VMEM((n_seg, seg, d), BF16),
            pltpu.VMEM((n_seg, seg, d), BF16),
            pltpu.VMEM((n_seg * PRE, d), BF16),
            pltpu.VMEM((RING, 12, 2, 64, d), BF16),
            pltpu.VMEM((n_pairs, n_seg * PRE, 4 * dh), F32),
            pltpu.VMEM((n_pairs, seg, 6 * dh), F32),
            pltpu.VMEM((n_pairs // 2, 7, HALF // 2, 6 * dh), jnp.uint32),
            pltpu.VMEM((n_pairs, d // 2 - HALF, 6 * dh), jnp.uint32),
            pltpu.VMEM((n_pairs // 2, 7, 3, 2, 32, HALF), jnp.uint32),
            pltpu.VMEM((n_pairs, 3, 2, 32, d - 2 * HALF), jnp.uint32),
            pltpu.VMEM((9, 16, 128), F32),
            pltpu.VMEM((n_pairs // 2, 8, 6 * dh), F32),
            pltpu.VMEM((n_pairs // 2, 2, 8, 128), F32),
            pltpu.VMEM((rows, heads * dh), F32),
            pltpu.VMEM((rows, heads * dh), F32),
            pltpu.VMEM((n_pairs, n_mem + 8, 4 * dh), F32),
            pltpu.VMEM((n_mem, d), BF16),
            pltpu.VMEM((b_dh, b_dh, b_heads), BF16),
            pltpu.VMEM((d // (F_PAIRS * gr), F_PAIRS * gr // 2, 256), jnp.uint32),
            pltpu.VMEM(B_wqkv.shape, BF16),
            pltpu.VMEM(B_wo.shape, BF16),
            pltpu.VMEM((d // 2, d), jnp.uint32),
            pltpu.VMEM((d // 2, d), jnp.uint32),
            pltpu.VMEM((d // half, half, d), jnp.uint32),
            pltpu.VMEM((b_heads // 2, gr, 2 * gr), F32),
            pltpu.VMEM((b_heads // 2, 2 * gr, 128), F32),
            pltpu.VMEM((d // 2, TB), jnp.uint32),
            pltpu.VMEM((TB // 2, d), jnp.uint32),
            pltpu.SemaphoreType.DMA((n_pairs, 6)),
            pltpu.SemaphoreType.DMA((6,)),
            pltpu.SemaphoreType.DMA((1,)),
        ],
        compiler_params=pltpu.CompilerParams(vmem_limit_bytes=124 * 1024 * 1024),
    )(
        A_x.reshape(n_seg, seg, d), A_mem0.reshape(n_mem, d),
        head_major(A_Wq).reshape(n_pairs, 3, 2, 64, d),
        head_major(A_Wk).reshape(n_pairs, 3, 2, 64, d),
        head_major(A_Wv).reshape(n_pairs, 2, 3, 64, d), A_Wo.reshape(n_pairs, 2, 3, 64, d),
        B_wqkv, B_w_phi.transpose(1, 2, 0), B_wo,
    )
    return out.reshape(batch, s_len, d)
```

```python
import functools
import math

import jax
import jax.numpy as jnp
from jax import lax
import jax.experimental.pallas as pl
import jax.experimental.pallas.tpu as pltpu

F32 = jnp.float32
BF16 = jnp.bfloat16
NT = (((1,), (1,)), ((), ()))
LOG2E = math.log2(math.e)
MASKED = -1e9

ISSUE = ("kqSVv", "qkVSv")
LAG_S = 2
LAG_PV = 2
O_SPLITS = ((0, 1, 2, 3, 4, 5, 6, 8), (0, 1, 2, 3, 4, 6, 8))
P_ORDER = ((((1, 3), (2, 4)), ((1, 0, 6), (5,))), (((1, 3, 2), (4,)), ((1, 0, 6), (5,))))
O_ORDER = (((1, 3, 2, 4), (0, 6, 5, 1)), ((2, 3, 4, 1), (5, 6, 1, 0)))
VPU_DUE = 3
KEYS_AHEAD = (14, 9)
NORM_DUE = (0, 1)
HALF = 256
PRE = 8
RING = 8
WO_LAG = 3
TB = 512
K_PAIRS = 8
Q_PAIRS = 8
F_PAIRS = 2
O_ROWS = (128, 128, 128, 128)


def _iota(shape, axis):
    return lax.broadcasted_iota(jnp.int32, shape, axis)


def _div(v, d):
    return (v * ((1 << 18) // d + 1)) >> 18


def _pack(x):
    return pltpu.bitcast(x.astype(BF16), jnp.uint32)


def _unpack(x):
    return pltpu.bitcast(x, BF16)


def _recip(x):
    r = pl.reciprocal(x, approx=True)
    return r * (2.0 - x * r)


def _layernorm(x):
    m = jnp.mean(x, axis=-1, keepdims=True)
    c = x - m
    v = jnp.mean(c * c, axis=-1, keepdims=True)
    return c * lax.rsqrt(v + 1e-5)


def _rows(*parts):
    return jnp.concatenate(parts, axis=0)


def _cols(*parts):
    return jnp.concatenate(parts, axis=1)


def _strassen_weights(b11, b12, b21, b22):
    f11, f12, f21, f22 = (b.astype(F32) for b in (b11, b12, b21, b22))
    return [r.astype(BF16)
            for r in (f11 + f22, b11, f12 - f22, f21 - f11, b22, f11 + f12, f21 + f22)]


def _balance(left, right):
    def exponent(t):
        bits = pltpu.bitcast(_pack(t) & 0x7F800000, F32)
        peak = jnp.max(jnp.max(bits, axis=1, keepdims=True), axis=0, keepdims=True)
        return pltpu.bitcast(jnp.broadcast_to(peak, (8, 128)), jnp.int32) >> 23

    left, right = exponent(left), exponent(right)
    shift = jnp.where(jnp.minimum(left, right) > 0, jnp.clip(left - right, -100, 100), 0)
    return [pltpu.bitcast((127 + e) << 23, F32) for e in (shift, -shift)]


def _left_product(a1, a2, times):
    return times(a2, 3) + times(a1 + a2, 1)


def _right_product(a1, a2, times):
    return times(a1 + a2, 4) + times(a1, 2)


def _token_operands(a1, a2, b1, b2):
    low = b1 + b2
    n = low.shape[0] // 2
    return ({3: b2, 2: a1, 1: low[:n], 4: a1 + a2},
            {0: a1 + b2, 6: a2 - b2, 1: low[n:], 5: b1 - a1})


def _memory_operands(m1, m2):
    both = m1 + m2
    return {0: m2, 1: both, 2: m1, 3: m2, 4: both, 5: m1, 6: m2}


def _first_results(p, n):
    m1 = _rows(p[1][n:], jnp.zeros_like(p[1][n:]))
    return ((p[1][:n] + p[3][:n], p[2][:n] + p[4][:n]),
            (p[2][n:] + p[4][n:], p[3][n:] - p[4][n:], p[3][n:] + m1, p[2][n:] - m1))


def _second_left(p, n, c11, c21):
    m1 = _rows(jnp.zeros_like(p[1][n:]), p[1][n:])
    return p[1][:n] + p[6][:n] - p[0][:n], c11 + p[0][n:] + p[6][n:], c21 + m1


def _second_right(p, n, c22):
    m1 = _rows(jnp.zeros_like(p[1][n:]), p[1][n:])
    return p[5][:n] + p[0][:n] - p[1][:n], c22 + p[0][n:] + p[5][n:] - m1


def _a_step(s, mem, xn, shared, *, layer, dh, x_in, x_ref, xb_ref, ws_ref, wp_ref, wos_ref,
            wop_ref, undo_ref, undo_v_ref, pre_ref, ahead_ref, o_refs, near_ref):
    odd = bool(shared)
    n_mem, seg = mem.shape[0], xn[0].shape[0]
    n_seg = xb_ref.shape[0]
    rows = n_mem + seg
    pw = 2 * dh
    n_pairs = wp_ref.shape[0]
    o_ref = o_refs[odd]
    scale = dh ** -0.5

    def after(early, value):
        return value if early is None else jnp.where(s < 0, early[:, :value.shape[1]], value)

    def after_all(early, value):
        t = functools.reduce(jnp.maximum, [early[i:i + 8, j:j + 128]
                                           for i in range(0, early.shape[0], 8)
                                           for j in range(0, early.shape[1], 128)])
        return jnp.concatenate([after(t, value[0:8]), value[8:]], axis=0)

    def slow_norm(x):
        outs = [None, None]
        for i in range(0, seg, 8):
            outs.append(_layernorm(after(outs[-2], x[i:i + 8])))
        return jnp.concatenate(outs[2:], axis=0)

    xn_next = slow_norm(x_in[jnp.minimum(s + len(xn), n_seg - 1)].astype(F32))
    done = jnp.maximum(s - 3, 0)
    xb_done = slow_norm(x_ref[done])
    xb_ref[done] = xb_done.astype(BF16)

    h = _rows(mem, xn[0])

    first = _iota((rows, 128), 1) < 64
    zero = jnp.zeros((rows, 128), F32)

    def key_blocks(t):
        t0, t1, t2 = t[:, 0:128], t[:, 128:256], t[:, 256:384]
        top = jnp.concatenate([t0, jnp.where(first, t1, 0.0), zero], axis=1)
        bot = jnp.concatenate([zero, jnp.where(first, 0.0, t1), t2], axis=1)
        return jnp.concatenate([top, bot], axis=0).astype(BF16)

    def value_blocks(t):
        mine = jnp.concatenate([first] * 3, axis=1)
        return jnp.concatenate(
            [jnp.where(mine, t, 0.0), jnp.where(mine, 0.0, t)], axis=0).astype(BF16)

    near = n_mem + 8

    def far_rows(t):
        return _rows(t[:n_mem], t[near:])

    q, k, v, probs, near_done = {}, {}, {}, {}, {}

    def project_short(p, j):
        def dot(a, w):
            return jnp.dot(a.astype(BF16), _unpack(w), preferred_element_type=F32)

        cols, top = slice(j * pw, (j + 1) * pw), h[:rows - PRE]
        most = (_left_product, _right_product)[p % 2](
            top[:, :HALF], top[:, HALF:2 * HALF], lambda a, i: dot(a, ws_ref[p // 2, i, :, cols]))
        if p % 2:
            most = most * _tile_rows(undo_ref[p // 2, :, cols], rows - PRE)
        return _rows(dot(top[:, 2 * HALF:], wp_ref[p, :, cols]) + most,
                     pre_ref[p, pl.ds(pl.multiple_of(s * PRE, PRE), PRE), (j - 1) * pw:j * pw])

    if not odd:
        shared["in"] = _token_operands(*(t[:, c:c + HALF] for t in xn[1:3] for c in (0, HALF)))
    m_in = _memory_operands(mem[:, :HALF], mem[:, HALF:2 * HALF])
    lhs_in = {i: _rows(m_in[i], t) for i, t in shared["in"][odd].items()}
    products = {}

    def project_shared(p, j):
        g, right = divmod(p, 2)
        cols, prod = slice(j * pw, (j + 1) * pw), products.setdefault(j, {})
        for i in P_ORDER[layer][odd][right]:
            prod[i] = jnp.dot(lhs_in[i], _unpack(ws_ref[g, i, :, cols]),
                              preferred_element_type=F32)
        if not odd:
            tokens = ahead_ref[p, :, cols]
            if right:
                (_, m), shared[g, j] = _first_results(prod, n_mem)
            else:
                m = prod[1][:n_mem] + prod[3][:n_mem]
        elif right:
            tokens = shared[g, j][0]
            m, ahead_ref[p, :, cols] = _second_right(prod, n_mem, shared[g, j][3])
        else:
            m, tokens, ahead_ref[p, :, cols] = _second_left(prod, n_mem, *shared[g, j][1:3])
        most = _rows(m, tokens)
        if right:
            most = most * _tile_rows(undo_ref[g, :, cols], rows)
        return jnp.dot(h[:, 2 * HALF:], _unpack(wp_ref[p, :, cols]),
                       preferred_element_type=F32) + most

    def scores(p):
        col = far_rows(_iota((rows, 2 * rows), 1))
        row = far_rows(_iota((rows, 2 * rows), 0))
        is_a = col < rows
        visible = (row < n_mem) | (row >= jnp.where(is_a, col, col - rows))
        sc = lax.dot_general(far_rows(q[p]), key_blocks(k[p]), NT, preferred_element_type=F32)
        sc = jnp.where(visible, sc * scale, MASKED)
        max_a = jnp.max(jnp.where(is_a, sc, -jnp.inf), axis=1, keepdims=True)
        max_b = jnp.max(jnp.where(is_a, -jnp.inf, sc), axis=1, keepdims=True)
        e = jnp.exp(sc - jnp.where(is_a, max_a, max_b))
        sum_a = jnp.sum(jnp.where(is_a, e, 0.0), axis=1, keepdims=True)
        sum_b = jnp.sum(jnp.where(is_a, 0.0, e), axis=1, keepdims=True)
        probs[p] = e * _recip(jnp.where(is_a, sum_a, sum_b))
        if p == NORM_DUE[0]:
            probs[p] = after_all(xn_next, probs[p])
        if p == NORM_DUE[1]:
            probs[p] = after_all(xb_done, probs[p])
        if p - VPU_DUE in near_done:
            probs[p] = after_all(near_done[p - VPU_DUE], probs[p])

    def values(p):
        o = jnp.dot(probs[p], value_blocks(v[p]), preferred_element_type=F32)
        o_ref[:n_mem, p * pw:(p + 1) * pw] = o[:n_mem]
        o_ref[near:, p * pw:(p + 1) * pw] = o[n_mem:]

    chain = [None, None]
    scored = [None] * KEYS_AHEAD[layer]

    def attend_near(p):
        def key_row(j, i):
            return jnp.broadcast_to(near_ref[p, j:j + 1, 128 * i:128 * (i + 1)], (8, 128))

        near_ref[p, :, 0:pw] = k[p][:near]
        near_ref[p, :, pw:2 * pw] = v[p][:near]
        half, sub = first[0:8], _iota((8, 128), 0)
        t = q[p][n_mem:near] * (scale * LOG2E)
        q0, q2 = t[:, 0:128], t[:, 256:384]
        q1a, q1b = jnp.where(half, t[:, 128:256], 0.0), jnp.where(half, 0.0, t[:, 128:256])
        for j in range(near):
            ready = after(scored[-KEYS_AHEAD[layer]], chain[0])
            k1 = after(ready, key_row(j, 1))
            dot_a = q0 * after(ready, key_row(j, 0)) + q1a * k1
            dot_b = q2 * after(dot_a, key_row(j, 2)) + q1b * k1
            t = jnp.where(half, jnp.sum(dot_a, axis=1, keepdims=True),
                          jnp.sum(dot_b, axis=1, keepdims=True))
            scored.append(t if j <= n_mem else jnp.where(sub >= j - n_mem, t, MASKED * LOG2E))
            chain[0] = dot_b
        sc = scored[-near:]
        top = functools.reduce(jnp.maximum, sc)
        for j in range(near):
            e = jnp.exp2(sc[j] - after(chain[1], top))
            weight = after(chain[1], e)
            terms = [weight * key_row(j, 3 + i) for i in range(3)]
            total = e if j == 0 else total + e
            acc = terms if j == 0 else [a + b for a, b in zip(acc, terms)]
            chain[1] = acc[2]
        inv = _recip(total)
        o_ref[n_mem:near, p * pw:(p + 1) * pw] = _cols(*(a * inv for a in acc))
        near_done[p] = acc[2]

    out = {}

    def project_out(g0, g1):
        def halves(ref, lo, hi):
            return [_cols(*(ref[lo:hi, (2 * g + i) * pw:(2 * g + i + 1) * pw]
                            for g in range(g0, g1))) for i in range(2)]

        if not odd:
            shared["out", g0] = _token_operands(*halves(o_refs[0], n_mem, rows),
                                                *halves(o_refs[1], n_mem, rows))
        m = _memory_operands(*halves(o_ref, 0, n_mem))
        for i in O_ORDER[layer][odd]:
            r = jnp.dot(_rows(m[i], shared["out", g0][odd][i]), _unpack(wos_ref[g0:g1, i].reshape(-1, HALF)),
                        preferred_element_type=F32)
            out[i] = r + out[i] if i in out else r

    lag_s, lag_v = LAG_S, LAG_S + LAG_PV
    todo = list(zip(O_SPLITS[layer][:-1], O_SPLITS[layer][1:]))
    for t in range(n_pairs + lag_v):
        if t >= n_pairs:
            project_out(*todo.pop(0))
        for c in ISSUE[layer]:
            if c == "S" and 0 <= t - lag_s < n_pairs:
                scores(t - lag_s)
            elif c == "V" and 0 <= t - lag_v < n_pairs:
                values(t - lag_v)
            elif c in "qkv" and t < n_pairs:
                j = "qkv".index(c)
                (q, k, v)[j][t] = (project_short(t, j) if j and pre_ref is not None
                                   else project_shared(t, j))
                if c == "v" and t % 2:
                    undo = jnp.where(first[:8], undo_v_ref[t // 2, 0], undo_v_ref[t // 2, 1])
                    v[t] = v[t] * _cols(*[_tile_rows(undo, rows)] * 3)
        if t < n_pairs:
            attend_near(t)
    for part in todo:
        project_out(*part)
    rest = jnp.dot(o_ref[...], _unpack(wop_ref[...].reshape(-1, wop_ref.shape[-1])),
                   preferred_element_type=F32)

    most, tail = slice(0, 2 * HALF), slice(2 * HALF, None)
    x_ref[s, :, tail] = x_in[s, :, tail].astype(F32) + rest[n_mem:]
    if odd:
        c12, c11, c21, c22 = shared["out"]
        m1, c11, c21 = _second_left(out, n_mem, c11, c21)
        m2, c22 = _second_right(out, n_mem, c22)
        x_ref[s - 1, :, most] = x_in[s - 1, :, most].astype(F32) + _cols(c11, c12)
        back = jnp.maximum(s - 2, 1)
        x_ref[back, :, most] = (x_in[back, :, most].astype(F32)
                                + jnp.where(s > 1, _cols(c21, c22), 0.0))
    else:
        (m1, m2), shared["out"] = _first_results(out, n_mem)
    return _cols(m1, m2, rest[:n_mem]), xn_next


def _pair_reduce(t, op):
    r = t[0:8]
    for i in range(8, t.shape[0], 8):
        r = op(r, t[i:i + 8])
    r = op(r, pltpu.roll(r, 4, 0))
    return op(r, pltpu.roll(r, 2, 0))


def _tile_rows(r, n):
    return jnp.concatenate([r] * (n // 8), axis=0)


def _feature_map(p):
    n = p.shape[0]
    e_pos = jnp.exp2(p - _tile_rows(_pair_reduce(p, jnp.maximum), n))
    e_neg = jnp.exp2(_tile_rows(_pair_reduce(p, jnp.minimum), n) - p)
    inv_pos = _recip(_pair_reduce(e_pos, jnp.add))
    inv_neg = _recip(_pair_reduce(e_neg, jnp.add))
    return jnp.concatenate(
        [e_pos * _tile_rows(inv_pos, n), e_neg * _tile_rows(inv_neg, n)], axis=0)


def _fold_span(b, blk):
    return b * blk // 128 * 128, -(-(b + 1) * blk // 128) * 128


def _expand_phi(wphi_ref, phi_ref):
    dh, _, heads = wphi_ref.shape
    d = dh * heads
    gr = 2 * dh
    c = _iota((dh, d), 1)
    c_feat = c - _div(c, dh) * dh
    spread = (_div(_iota((heads, d), 1), dh) == _iota((heads, d), 0)).astype(BF16)

    def gather(j, by_feat):
        for e in (j * (dh // 4) + i for i in range(dh // 4)):
            t = jnp.dot(wphi_ref[e], spread, preferred_element_type=F32)
            by_feat = jnp.where(c_feat == e, t, by_feat)
        return by_feat

    by_feat = lax.fori_loop(0, 4, gather, jnp.zeros((dh, d), F32)).astype(BF16)
    blk = F_PAIRS * gr
    r = _iota((blk, dh), 0)
    sel = (((r - _div(r, gr) * gr) >> 1) == _iota((blk, dh), 1)).astype(BF16)
    for b in range(d // blk):
        lo, hi = _fold_span(b, blk)
        r = _iota((blk, hi - lo), 0)
        head = 2 * (_div(r, gr) + b * F_PAIRS) + (r & 1)
        phi = jnp.dot(sel, by_feat[:, lo:hi], preferred_element_type=F32)
        phi_ref[b, :, 0:hi - lo] = _pack(
            jnp.where(_div(_iota((1, hi - lo), 1) + lo, dh) == head, phi, 0.0))


def _b_weights(wqkv_ref, phi_ref, wob_ref, bq_ref, bkv_ref, bo_ref):
    d = wqkv_ref.shape[0]
    blk = 2 * phi_ref.shape[1]
    half = bkv_ref.shape[1]
    bo_ref[...] = _pack(wob_ref[...])
    wv = wqkv_ref[:, 2 * d:3 * d].T
    for b in range(d // half):
        bkv_ref[b, half // 2:half, :] = _pack(wv[b * half:(b + 1) * half])
    for b in range(d // blk):
        lo, hi = _fold_span(b, blk)
        phi = _unpack(phi_ref[b, :, 0:hi - lo])
        wq = lax.dot_general(phi, wqkv_ref[:, lo:hi], NT, preferred_element_type=F32)
        wk = lax.dot_general(phi, wqkv_ref[:, d + lo:d + hi], NT, preferred_element_type=F32)
        bq_ref[b * blk // 2:(b + 1) * blk // 2, :] = _pack(wq * LOG2E)
        at = b * blk % half // 2
        bkv_ref[b * blk // half, at:at + blk // 2, :] = _pack(wk * LOG2E)


def _chunk_rows(ref, it, r0, n):
    seg = ref.shape[1]
    return pl.ds(it * (TB // seg) + r0 // seg, n // seg)


def _b_keys(it, carry, *, x_ref, xb_ref, bkv_ref, kv_ref, z_ref):
    n_blk, half, _ = bkv_ref.shape
    gr = half // K_PAIRS
    xb = xb_ref[_chunk_rows(xb_ref, it, 0, TB)].reshape(TB, -1)
    last = x_ref.shape[0] - 1 - jnp.minimum(it, 2)
    xb_ref[last] = _layernorm(x_ref[last]).astype(BF16)
    same_head = (_iota((gr, 2 * gr), 0) >= gr // 2) == ((_iota((gr, 2 * gr), 1) & 1) == 1)

    def accumulate(b, t):
        for i in range(K_PAIRS):
            g = b * K_PAIRS + i
            phi = _feature_map(t[i * gr:(i + 1) * gr])
            z_ref[g] = jnp.where(it > 0, z_ref[g], 0.0) + jnp.sum(phi, axis=1, keepdims=True)
            kv = lax.dot_general(t[half + i * gr:half + (i + 1) * gr], phi.astype(BF16), NT,
                                 preferred_element_type=F32)
            kv_ref[g] = jnp.where(it > 0, kv_ref[g], 0.0) + jnp.where(same_head, kv, 0.0)

    pending = None
    for b in range(n_blk):
        t = lax.dot_general(_unpack(bkv_ref[b]), xb, NT, preferred_element_type=F32)
        if pending is not None:
            accumulate(*pending)
        pending = (b, t)
    accumulate(*pending)
    return carry


def _b_queries(it, send, *, x_ref, xb_ref, y_ref, bq_ref, bo_ref, kv_ref, z_ref, ot_ref, on_ref):
    n_groups, gr, _ = kv_ref.shape
    blk = Q_PAIRS * gr
    sub = _iota((8, TB), 0)
    xb = xb_ref[_chunk_rows(xb_ref, it, 0, TB)].reshape(TB, -1)

    def attend(b, t):
        outs = []
        for i in range(Q_PAIRS):
            g = b * Q_PAIRS + i
            phi = _feature_map(t[i * gr:(i + 1) * gr])
            num = jnp.dot(kv_ref[g], phi.astype(BF16), preferred_element_type=F32)
            z = jnp.concatenate([z_ref[g]] * (TB // 128), axis=1)
            inv = _recip(_pair_reduce(phi * z, jnp.add) + 1e-6)
            other = pltpu.roll(inv, 1, 0)
            inv_a = jnp.where((sub & 1) == 0, inv, other)
            inv_b = jnp.where((sub & 1) == 0, other, inv)
            n = (gr - 8) // 16
            inv = jnp.concatenate(
                [inv_a] * n + [jnp.where(sub < 4, inv_a, inv_b)] + [inv_b] * n, axis=0)
            outs.append(num * inv)
        ot_ref[b * blk // 2:(b + 1) * blk // 2, :] = _pack(jnp.concatenate(outs, axis=0))

    n_blk = n_groups // Q_PAIRS
    proj = {}
    for b in range(n_blk + 1):
        if b < n_blk:
            proj[b] = lax.dot_general(_unpack(bq_ref[b * blk // 2:(b + 1) * blk // 2, :]), xb,
                                      NT, preferred_element_type=F32)
        if b > 0:
            attend(b - 1, proj[b - 1])
    on_ref[...] = _pack(_unpack(ot_ref[...]).T)
    r0 = 0
    for i, n in enumerate(O_ROWS):
        at = _chunk_rows(x_ref, it, r0, n)
        y = jnp.dot(_unpack(on_ref[r0 // 2:(r0 + n) // 2, :]), _unpack(bo_ref[...]),
                    preferred_element_type=F32)
        x = x_ref[at] + y.reshape((-1,) + x_ref.shape[1:])
        x_ref[at] = x
        y_ref[at] = x.astype(BF16)
        send(i)
        r0 += n


def _kernel(x_hbm, mem0_hbm, wq_hbm, wk_hbm, wv_hbm, wo_hbm, wqkvb_hbm, wphi_hbm, wob_hbm,
            out_hbm,
            x_ref, xb_ref, y_ref, xp_ref, stage_ref, pre_ref, ahead_ref,
            ws_ref, wp_ref, wos_ref, wop_ref, scale_ref, undo_ref, undo_v_ref, o_even_ref, o_odd_ref, near_ref,
            mem0_ref, wphi_ref, phi_ref, wqkvb_ref, wob_ref, bo_ref, bq_ref, bkv_ref,
            kv_ref, z_ref, ot_ref, on_ref,
            w_sem, in_sem, out_sem, *, dh):
    n_seg, seg, d = x_ref.shape
    n_pairs = wp_ref.shape[0]
    n_mem = mem0_ref.shape[0]
    pw = 2 * dh
    n_iter = n_seg * seg // TB

    def head_copy(p, j, i):
        return pltpu.make_async_copy(
            (wv_hbm, wo_hbm)[j - 2].at[p, i], stage_ref.at[p % RING, 3 * j:3 * j + 3, i],
            w_sem.at[p, 2 * j - 2 + i])

    def w_copies(p, j):
        if j >= 2:
            return [head_copy(p, j, i) for i in range(2)]
        return [pltpu.make_async_copy(
            (wq_hbm, wk_hbm)[j].at[p], stage_ref.at[p % RING, 3 * j:3 * j + 3], w_sem.at[p, j])]

    def start_w(p, *slots):
        for j in slots:
            for copy in w_copies(p, j):
                copy.start()

    def wait_w(p, *slots):
        for j in slots:
            for copy in w_copies(p, j):
                copy.wait()

    def prepare_in(u, tiles, live=True, pace=None):
        g, i = u // 2, u % 2
        slots = [p % RING for p in (2 * g, jnp.where(live, 2 * g + 1, 0))]
        for j in range(3) if pace else ():
            factors = [_balance(*(stage_ref[p, 3 * j + 2 * n, n, :16, :2 * HALF] for p in slots))
                       for n in range(2)]
            for t in range(3):
                heads = [factors[n if j == 2 else (2 * t + n) // 3] for n in range(2)]
                undo_ref[g, :, pl.ds(128 * (3 * j + t), 128)] = jnp.where(
                    _iota((8, 128), 1) < 64, *(f[1] for f in heads))
                scale_ref[3 * j + t] = _rows(*(f[0] for f in heads))
        pace = pace or (lambda t, b: b)
        for t in tiles:
            cols = pl.ds(pl.multiple_of(128 * t, 128), 128)
            scale = _rows(*(_tile_rows(scale_ref[t, 8 * n:8 * n + 8, :], 64) for n in range(2)))
            b11, b12, b21, b22 = (
                pace(t, stage_ref[p, t, :, :, pl.ds(pl.multiple_of(c + i * 128, 128), 128)]
                     .reshape(128, 128)) for c in (0, HALF) for p in slots)
            for n, r in enumerate(_strassen_weights(b11, b12 * scale, b21, b22 * scale)):
                ws_ref[g, n, pl.ds(pl.multiple_of(i * 64, 64), 64), cols] = _pack(r.T)
            wp_ref[u, :, cols] = _pack(stage_ref[u % RING, t, :, :, 2 * HALF:].reshape(128, -1).T)

    def wait_out(u):
        for p in (u // 2 * 2, u // 2 * 2 + 1):
            head_copy(p, 3, u % 2).wait()

    def prepare_out(u, live=True, pace=lambda t, b: b):
        g, i = u // 2, u % 2
        slots = [p % RING for p in (2 * g, jnp.where(live, 2 * g + 1, 0))]
        base = jnp.where(live, 9, 3)
        scale, undo_v_ref[g, i] = _balance(*(stage_ref[p, base, i, :16] for p in slots))
        for t in range(3):
            parts = [pace(10 + 2 * t, stage_ref[p, base + t, i]) for p in slots]
            parts[1] = parts[1] * _cols(*[_tile_rows(scale, 64)] * (d // 128))
            blocks = [part[:, c:c + HALF] for part in parts for c in (0, HALF)]
            for n, r in enumerate(_strassen_weights(*blocks)):
                wos_ref[g, n, t, i] = _pack(r)
            for n, part in enumerate(parts):
                wop_ref[2 * g + n, t, i] = _pack(part[:, 2 * HALF:])

    def out_copy(it, i):
        part = _chunk_rows(y_ref, it, sum(O_ROWS[:i]), O_ROWS[i])
        return pltpu.make_async_copy(y_ref.at[part], out_hbm.at[part], out_sem.at[0])

    def x_copy(rows, sem):
        return pltpu.make_async_copy(x_hbm.at[:, rows, :], y_ref.at[:, rows, :], sem)

    head, tail = slice(0, seg - PRE), slice(seg - PRE, seg)
    xt_copy, xh_copy = x_copy(tail, in_sem.at[0]), x_copy(head, in_sem.at[3])
    wqkvb_copy = pltpu.make_async_copy(wqkvb_hbm, wqkvb_ref, in_sem.at[1])
    wphi_copy = pltpu.make_async_copy(wphi_hbm, wphi_ref, in_sem.at[5])
    mem0_copy = pltpu.make_async_copy(mem0_hbm, mem0_ref, in_sem.at[4])
    wob_copy = pltpu.make_async_copy(wob_hbm, wob_ref, in_sem.at[2])

    wphi_copy.start()
    xt_copy.start()
    start_w(0, 0, 1, 2)
    wphi_copy.wait()
    _expand_phi(wphi_ref, phi_ref)
    xt_copy.wait()

    xp_ref[...] = _layernorm(y_ref[:, tail, :].astype(F32).reshape(n_seg * PRE, d)).astype(BF16)

    mem0_copy.start()
    start_w(1, 0, 1, 2)

    def pre_project(p, carry):
        @pl.when(p + 2 < n_pairs)
        def _():
            start_w(jnp.minimum(p + 2, n_pairs - 1), 0, 1, 2)

        @pl.when(p + 2 == n_pairs)
        def _():
            xh_copy.start()

        start_w(p, 3)

        @pl.when(p >= WO_LAG)
        def _():
            wait_out(jnp.maximum(p - WO_LAG, 0))

        wait_w(p, 0, 1, 2)
        kv = lax.dot_general(xp_ref[...], stage_ref[p % RING, 3:9].reshape(-1, d), NT,
                             preferred_element_type=F32)
        pre_ref[p] = kv

        def pace(t, block):
            c, r = divmod(t * 128, xp_ref.shape[0])
            early = kv[r:r + block.shape[0], 128 * c:128 * (c + 1)].astype(BF16)
            return jnp.where(p < 0, _cols(*[early] * (block.shape[1] // 128)), block)

        prepare_out(jnp.maximum(p - WO_LAG, 0), p >= WO_LAG, pace)
        prepare_in(jnp.maximum(p - 1, 0), range(9), p >= 1, pace)
        return carry

    lax.fori_loop(0, n_pairs, pre_project, 0)

    @pl.loop(0, 3)
    def _(j):
        prepare_in(n_pairs - 1, [3 * j + i for i in range(3)])

    @pl.loop(n_pairs - WO_LAG, n_pairs)
    def _(u):
        wait_out(u)
        prepare_out(u)

    xh_copy.wait()

    wqkvb_copy.start()
    wob_copy.start()
    mem0_copy.wait()
    x_ref[0] = y_ref[0].astype(F32)

    def layer_a(layer, x_in, pre):
        step = functools.partial(
            _a_step, layer=layer, dh=dh, x_in=x_in, x_ref=x_ref, xb_ref=xb_ref, ws_ref=ws_ref,
            wp_ref=wp_ref, wos_ref=wos_ref, wop_ref=wop_ref, pre_ref=pre, ahead_ref=ahead_ref,
            undo_ref=undo_ref, undo_v_ref=undo_v_ref, o_refs=(o_even_ref, o_odd_ref),
            near_ref=near_ref)
        xn = [_layernorm(x_in[i].astype(F32)) for i in range(3)]
        o_odd_ref[...] = jnp.zeros(o_odd_ref.shape, F32)
        cols, per = (slice(0, 3 * pw), 1) if pre is None else (slice(0, pw), 2)

        @pl.loop(0, n_pairs // 2 // per)
        def _(j):
            for g in (j * per + i for i in range(per)):
                for i, product in enumerate((_left_product, _right_product)):
                    ahead_ref[2 * g + i, :, cols] = product(
                        xn[0][:, :HALF], xn[0][:, HALF:2 * HALF],
                        lambda a, n: jnp.dot(a.astype(BF16), _unpack(ws_ref[g, n, :, cols]),
                                             preferred_element_type=F32))

        def two_steps(it, carry):
            mem, *xn = carry
            shared = {}
            for i in range(2):
                mem, xn_next = step(2 * it + i, mem, xn, shared)
                xn = xn[1:] + [xn_next]
            return (mem, *xn)

        lax.fori_loop(0, n_seg // 2, two_steps, (mem0_ref[...].astype(F32), *xn))

    def finish_a(layer):
        a = [_cols(*(o_odd_ref[n_mem:, (2 * g + i) * pw:(2 * g + i + 1) * pw]
                     for g in range(n_pairs // 2))) for i in range(2)]
        y = _cols(*(product(*a, lambda t, n: jnp.dot(
            t.astype(BF16), _unpack(wos_ref[:, n].reshape(-1, HALF)), preferred_element_type=F32))
            for product in (_left_product, _right_product)))
        at = (n_seg - 1, slice(None), slice(0, 2 * HALF))
        x_ref[at] = jnp.where(layer == 0, y_ref[at].astype(F32), x_ref[at]) + y

    b_keys = functools.partial(_b_keys, x_ref=x_ref, xb_ref=xb_ref, bkv_ref=bkv_ref,
                               kv_ref=kv_ref, z_ref=z_ref)
    b_queries = functools.partial(_b_queries, x_ref=x_ref, xb_ref=xb_ref, y_ref=y_ref,
                                  bq_ref=bq_ref, bo_ref=bo_ref, kv_ref=kv_ref, z_ref=z_ref,
                                  ot_ref=ot_ref, on_ref=on_ref)

    def layer_pair(layer, carry):
        @pl.when(layer == 0)
        def _():
            layer_a(0, y_ref, pre_ref)

        @pl.when(layer == 0)
        def _():
            wqkvb_copy.wait()
            wob_copy.wait()
            _b_weights(wqkvb_ref, phi_ref, wob_ref, bq_ref, bkv_ref, bo_ref)

        @pl.when(layer == 1)
        def _():
            layer_a(1, x_ref, None)

        finish_a(layer)

        lax.fori_loop(0, n_iter, b_keys, 0)

        def queries(it, carry):
            def send(i):
                @pl.when(layer == 1)
                def _():
                    out_copy(it, i).start()

            b_queries(it, send)
            return carry

        lax.fori_loop(0, n_iter, queries, 0)

        return carry

    lax.fori_loop(0, 2, layer_pair, 0)
    pltpu.make_async_copy(y_ref, out_hbm, out_sem.at[0]).wait()


@functools.partial(jax.jit, static_argnames=("A_seg_len",))
def pallas_interleave_layers__memory_aug_recurrent_mem_tr__linear_kernel_hedgehog__prompt_kernel(
    A_x, A_mem0, A_Wq, A_Wk, A_Wv, A_Wo, A_seg_len, B_x, B_wqkv, B_w_phi, B_wo,
):
    del B_x
    batch, s_len, d = A_x.shape
    _, heads, dh = A_Wq.shape
    n_mem = A_mem0.shape[1]
    seg = int(A_seg_len)
    b_heads, b_dh, _ = B_w_phi.shape
    rows = n_mem + seg
    n_pairs = heads // 2
    gr = 2 * b_dh
    half = K_PAIRS * gr
    n_seg = s_len // seg
    assert batch == 1 and dh == 192 and heads == 4 * O_SPLITS[0][-1] and d == 2 * HALF + 128
    assert n_mem % 8 == 0 and seg % 16 == 0 and 128 % seg == 0 and 2 * rows <= 128
    assert s_len % TB == 0 and s_len > 3 * TB == 3 * sum(O_ROWS) and n_seg % n_pairs == 0
    assert b_heads * b_dh == d and b_dh % 8 == 4 and d % half == 0

    def head_major(w):
        return w.transpose(1, 2, 0)

    hbm = pl.BlockSpec(memory_space=pltpu.HBM)
    out = pl.pallas_call(
        functools.partial(_kernel, dh=dh),
        out_shape=jax.ShapeDtypeStruct((n_seg, seg, d), A_x.dtype),
        in_specs=[hbm] * 9,
        out_specs=hbm,
        scratch_shapes=[
            pltpu.VMEM((n_seg, seg, d), F32),
            pltpu.VMEM((n_seg, seg, d), BF16),
            pltpu.VMEM((n_seg, seg, d), BF16),
            pltpu.VMEM((n_seg * PRE, d), BF16),
            pltpu.VMEM((RING, 12, 2, 64, d), BF16),
            pltpu.VMEM((n_pairs, n_seg * PRE, 4 * dh), F32),
            pltpu.VMEM((n_pairs, seg, 6 * dh), F32),
            pltpu.VMEM((n_pairs // 2, 7, HALF // 2, 6 * dh), jnp.uint32),
            pltpu.VMEM((n_pairs, d // 2 - HALF, 6 * dh), jnp.uint32),
            pltpu.VMEM((n_pairs // 2, 7, 3, 2, 32, HALF), jnp.uint32),
            pltpu.VMEM((n_pairs, 3, 2, 32, d - 2 * HALF), jnp.uint32),
            pltpu.VMEM((9, 16, 128), F32),
            pltpu.VMEM((n_pairs // 2, 8, 6 * dh), F32),
            pltpu.VMEM((n_pairs // 2, 2, 8, 128), F32),
            pltpu.VMEM((rows, heads * dh), F32),
            pltpu.VMEM((rows, heads * dh), F32),
            pltpu.VMEM((n_pairs, n_mem + 8, 4 * dh), F32),
            pltpu.VMEM((n_mem, d), BF16),
            pltpu.VMEM((b_dh, b_dh, b_heads), BF16),
            pltpu.VMEM((d // (F_PAIRS * gr), F_PAIRS * gr // 2, 256), jnp.uint32),
            pltpu.VMEM(B_wqkv.shape, BF16),
            pltpu.VMEM(B_wo.shape, BF16),
            pltpu.VMEM((d // 2, d), jnp.uint32),
            pltpu.VMEM((d // 2, d), jnp.uint32),
            pltpu.VMEM((d // half, half, d), jnp.uint32),
            pltpu.VMEM((b_heads // 2, gr, 2 * gr), F32),
            pltpu.VMEM((b_heads // 2, 2 * gr, 128), F32),
            pltpu.VMEM((d // 2, TB), jnp.uint32),
            pltpu.VMEM((TB // 2, d), jnp.uint32),
            pltpu.SemaphoreType.DMA((n_pairs, 6)),
            pltpu.SemaphoreType.DMA((6,)),
            pltpu.SemaphoreType.DMA((1,)),
        ],
        compiler_params=pltpu.CompilerParams(vmem_limit_bytes=124 * 1024 * 1024),
    )(
        A_x.reshape(n_seg, seg, d), A_mem0.reshape(n_mem, d),
        head_major(A_Wq).reshape(n_pairs, 3, 2, 64, d),
        head_major(A_Wk).reshape(n_pairs, 3, 2, 64, d),
        head_major(A_Wv).reshape(n_pairs, 2, 3, 64, d), A_Wo.reshape(n_pairs, 2, 3, 64, d),
        B_wqkv, B_w_phi.transpose(1, 2, 0), B_wo,
    )
    return out.reshape(batch, s_len, d)
```

```python
import functools
import math

import jax
import jax.numpy as jnp
from jax import lax
import jax.experimental.pallas as pl
import jax.experimental.pallas.tpu as pltpu

F32 = jnp.float32
BF16 = jnp.bfloat16
NT = (((1,), (1,)), ((), ()))
LOG2E = math.log2(math.e)
MASKED = -1e9

ISSUE = ("kqSVv", "qkVSv")
LAG_S = 2
LAG_PV = 2
O_SPLITS = ((0, 1, 2, 3, 4, 5, 6, 8), (0, 1, 2, 3, 4, 6, 8))
P_ORDER = ((((1, 3), (2, 4)), ((1, 0, 6), (5,))), (((1, 3, 2), (4,)), ((1, 0, 6), (5,))))
O_ORDER = (((1, 3, 2, 4), (0, 6, 5, 1)), ((2, 3, 4, 1), (5, 6, 1, 0)))
VPU_DUE = 3
KEYS_AHEAD = (14, 9)
NORM_DUE = (0, 1)
HALF = 256
PRE = 8
RING = 8
WO_LAG = 3
TB = 512
K_PAIRS = 8
Q_PAIRS = 8
F_PAIRS = 2
O_ROWS = (128, 128, 128, 128)


def _iota(shape, axis):
    return lax.broadcasted_iota(jnp.int32, shape, axis)


def _div(v, d):
    return (v * ((1 << 18) // d + 1)) >> 18


def _pack(x):
    return pltpu.bitcast(x.astype(BF16), jnp.uint32)


def _unpack(x):
    return pltpu.bitcast(x, BF16)


def _recip(x):
    r = pl.reciprocal(x, approx=True)
    return r * (2.0 - x * r)


def _layernorm(x):
    m = jnp.mean(x, axis=-1, keepdims=True)
    c = x - m
    v = jnp.mean(c * c, axis=-1, keepdims=True)
    return c * lax.rsqrt(v + 1e-5)


def _rows(*parts):
    return jnp.concatenate(parts, axis=0)


def _cols(*parts):
    return jnp.concatenate(parts, axis=1)


def _strassen_weights(b11, b12, b21, b22):
    f11, f12, f21, f22 = (b.astype(F32) for b in (b11, b12, b21, b22))
    return [r.astype(BF16)
            for r in (f11 + f22, b11, f12 - f22, f21 - f11, b22, f11 + f12, f21 + f22)]


def _balance(left, right):
    def exponent(t):
        bits = pltpu.bitcast(_pack(t) & 0x7F800000, F32)
        peak = jnp.max(jnp.max(bits, axis=1, keepdims=True), axis=0, keepdims=True)
        return pltpu.bitcast(jnp.broadcast_to(peak, (8, 128)), jnp.int32) >> 23

    left, right = exponent(left), exponent(right)
    shift = jnp.where(jnp.minimum(left, right) > 0, jnp.clip(left - right, -100, 100), 0)
    return [pltpu.bitcast((127 + e) << 23, F32) for e in (shift, -shift)]


def _left_product(a1, a2, times):
    return times(a2, 3) + times(a1 + a2, 1)


def _right_product(a1, a2, times):
    return times(a1 + a2, 4) + times(a1, 2)


def _token_operands(a1, a2, b1, b2):
    low = b1 + b2
    n = low.shape[0] // 2
    return ({3: b2, 2: a1, 1: low[:n], 4: a1 + a2},
            {0: a1 + b2, 6: a2 - b2, 1: low[n:], 5: b1 - a1})


def _memory_operands(m1, m2):
    both = m1 + m2
    return {0: m2, 1: both, 2: m1, 3: m2, 4: both, 5: m1, 6: m2}


def _first_results(p, n):
    low = _rows(p[1][n:], jnp.zeros_like(p[1][n:]))
    return ((p[1][:n] + p[3][:n], p[2][:n] + p[4][:n]),
            (p[2][n:] + p[4][n:], p[3][n:] - p[4][n:], p[3][n:] + low, p[2][n:] - low))


def _second_left(p, n, c11, c21):
    low = _rows(jnp.zeros_like(p[1][n:]), p[1][n:])
    return p[1][:n] + p[6][:n] - p[0][:n], c11 + p[0][n:] + p[6][n:], c21 + low


def _second_right(p, n, c22):
    low = _rows(jnp.zeros_like(p[1][n:]), p[1][n:])
    return p[5][:n] + p[0][:n] - p[1][:n], c22 + p[0][n:] + p[5][n:] - low


def _a_step(s, mem, xn, shared, *, layer, dh, x_in, x_ref, xb_ref, ws_ref, wp_ref, wos_ref,
            wop_ref, undo_ref, undo_v_ref, pre_ref, ahead_ref, o_refs, near_ref):
    odd = bool(shared)
    n_mem, seg = mem.shape[0], xn[0].shape[0]
    n_seg = xb_ref.shape[0]
    rows = n_mem + seg
    pw = 2 * dh
    n_pairs = wp_ref.shape[0]
    o_ref = o_refs[odd]
    scale = dh ** -0.5

    def after(early, value):
        return value if early is None else jnp.where(s < 0, early[:, :value.shape[1]], value)

    def after_all(early, value):
        t = functools.reduce(jnp.maximum, [early[i:i + 8, j:j + 128]
                                           for i in range(0, early.shape[0], 8)
                                           for j in range(0, early.shape[1], 128)])
        return jnp.concatenate([after(t, value[0:8]), value[8:]], axis=0)

    def slow_norm(x):
        outs = [None, None]
        for i in range(0, seg, 8):
            outs.append(_layernorm(after(outs[-2], x[i:i + 8])))
        return jnp.concatenate(outs[2:], axis=0)

    xn_next = slow_norm(x_in[jnp.minimum(s + len(xn), n_seg - 1)].astype(F32))
    done = jnp.maximum(s - 3, 0)
    xb_done = slow_norm(x_ref[done])
    xb_ref[done] = xb_done.astype(BF16)

    h = _rows(mem, xn[0])

    first = _iota((rows, 128), 1) < 64
    zero = jnp.zeros((rows, 128), F32)

    def key_blocks(t):
        t0, t1, t2 = t[:, 0:128], t[:, 128:256], t[:, 256:384]
        top = jnp.concatenate([t0, jnp.where(first, t1, 0.0), zero], axis=1)
        bot = jnp.concatenate([zero, jnp.where(first, 0.0, t1), t2], axis=1)
        return jnp.concatenate([top, bot], axis=0).astype(BF16)

    def value_blocks(t):
        mine = jnp.concatenate([first] * 3, axis=1)
        return jnp.concatenate(
            [jnp.where(mine, t, 0.0), jnp.where(mine, 0.0, t)], axis=0).astype(BF16)

    near = n_mem + 8

    def far_rows(t):
        return _rows(t[:n_mem], t[near:])

    q, k, v, probs, near_done = {}, {}, {}, {}, {}

    def project_short(p, j):
        def dot(a, w):
            return jnp.dot(a.astype(BF16), _unpack(w), preferred_element_type=F32)

        cols, top = slice(j * pw, (j + 1) * pw), h[:rows - PRE]
        most = (_left_product, _right_product)[p % 2](
            top[:, :HALF], top[:, HALF:2 * HALF], lambda a, i: dot(a, ws_ref[p // 2, i, :, cols]))
        if p % 2:
            most = most * _tile_rows(undo_ref[p // 2, :, cols], rows - PRE)
        return _rows(dot(top[:, 2 * HALF:], wp_ref[p, :, cols]) + most,
                     pre_ref[p, pl.ds(pl.multiple_of(s * PRE, PRE), PRE), (j - 1) * pw:j * pw])

    if not odd:
        shared["in"] = _token_operands(*(t[:, c:c + HALF] for t in xn[1:3] for c in (0, HALF)))
    m_in = _memory_operands(mem[:, :HALF], mem[:, HALF:2 * HALF])
    lhs_in = {i: _rows(m_in[i], t) for i, t in shared["in"][odd].items()}
    products = {}

    def project_shared(p, j):
        g, right = divmod(p, 2)
        cols, prod = slice(j * pw, (j + 1) * pw), products.setdefault(j, {})
        for i in P_ORDER[layer][odd][right]:
            prod[i] = jnp.dot(lhs_in[i], _unpack(ws_ref[g, i, :, cols]),
                              preferred_element_type=F32)
        if not odd:
            tokens = ahead_ref[p, :, cols]
            if right:
                (_, m), shared[g, j] = _first_results(prod, n_mem)
            else:
                m = prod[1][:n_mem] + prod[3][:n_mem]
        elif right:
            tokens = shared[g, j][0]
            m, ahead_ref[p, :, cols] = _second_right(prod, n_mem, shared[g, j][3])
        else:
            m, tokens, ahead_ref[p, :, cols] = _second_left(prod, n_mem, *shared[g, j][1:3])
        most = _rows(m, tokens)
        if right:
            most = most * _tile_rows(undo_ref[g, :, cols], rows)
        return jnp.dot(h[:, 2 * HALF:], _unpack(wp_ref[p, :, cols]),
                       preferred_element_type=F32) + most

    def scores(p):
        col = far_rows(_iota((rows, 2 * rows), 1))
        row = far_rows(_iota((rows, 2 * rows), 0))
        is_a = col < rows
        visible = (row < n_mem) | (row >= jnp.where(is_a, col, col - rows))
        sc = lax.dot_general(far_rows(q[p]), key_blocks(k[p]), NT, preferred_element_type=F32)
        sc = jnp.where(visible, sc * scale, MASKED)
        max_a = jnp.max(jnp.where(is_a, sc, -jnp.inf), axis=1, keepdims=True)
        max_b = jnp.max(jnp.where(is_a, -jnp.inf, sc), axis=1, keepdims=True)
        e = jnp.exp(sc - jnp.where(is_a, max_a, max_b))
        sum_a = jnp.sum(jnp.where(is_a, e, 0.0), axis=1, keepdims=True)
        sum_b = jnp.sum(jnp.where(is_a, 0.0, e), axis=1, keepdims=True)
        probs[p] = e * _recip(jnp.where(is_a, sum_a, sum_b))
        if p == NORM_DUE[0]:
            probs[p] = after_all(xn_next, probs[p])
        if p == NORM_DUE[1]:
            probs[p] = after_all(xb_done, probs[p])
        if p - VPU_DUE in near_done:
            probs[p] = after_all(near_done[p - VPU_DUE], probs[p])

    def values(p):
        o = jnp.dot(probs[p], value_blocks(v[p]), preferred_element_type=F32)
        o_ref[:n_mem, p * pw:(p + 1) * pw] = o[:n_mem]
        o_ref[near:, p * pw:(p + 1) * pw] = o[n_mem:]

    chain = [None, None]
    scored = [None] * KEYS_AHEAD[layer]

    def attend_near(p):
        def key_row(j, i):
            return jnp.broadcast_to(near_ref[p, j:j + 1, 128 * i:128 * (i + 1)], (8, 128))

        near_ref[p, :, 0:pw] = k[p][:near]
        near_ref[p, :, pw:2 * pw] = v[p][:near]
        half, sub = first[0:8], _iota((8, 128), 0)
        t = q[p][n_mem:near] * (scale * LOG2E)
        q0, q2 = t[:, 0:128], t[:, 256:384]
        q1a, q1b = jnp.where(half, t[:, 128:256], 0.0), jnp.where(half, 0.0, t[:, 128:256])
        for j in range(near):
            ready = after(scored[-KEYS_AHEAD[layer]], chain[0])
            k1 = after(ready, key_row(j, 1))
            dot_a = q0 * after(ready, key_row(j, 0)) + q1a * k1
            dot_b = q2 * after(dot_a, key_row(j, 2)) + q1b * k1
            t = jnp.where(half, jnp.sum(dot_a, axis=1, keepdims=True),
                          jnp.sum(dot_b, axis=1, keepdims=True))
            scored.append(t if j <= n_mem else jnp.where(sub >= j - n_mem, t, MASKED * LOG2E))
            chain[0] = dot_b
        sc = scored[-near:]
        top = functools.reduce(jnp.maximum, sc)
        for j in range(near):
            e = jnp.exp2(sc[j] - after(chain[1], top))
            weight = after(chain[1], e)
            terms = [weight * key_row(j, 3 + i) for i in range(3)]
            total = e if j == 0 else total + e
            acc = terms if j == 0 else [a + b for a, b in zip(acc, terms)]
            chain[1] = acc[2]
        inv = _recip(total)
        o_ref[n_mem:near, p * pw:(p + 1) * pw] = _cols(*(a * inv for a in acc))
        near_done[p] = acc[2]

    out = {}

    def project_out(g0, g1):
        def halves(ref, lo, hi):
            return [_cols(*(ref[lo:hi, (2 * g + i) * pw:(2 * g + i + 1) * pw]
                            for g in range(g0, g1))) for i in range(2)]

        if not odd:
            shared["out", g0] = _token_operands(*halves(o_refs[0], n_mem, rows),
                                                *halves(o_refs[1], n_mem, rows))
        m = _memory_operands(*halves(o_ref, 0, n_mem))
        for i in O_ORDER[layer][odd]:
            r = jnp.dot(_rows(m[i], shared["out", g0][odd][i]),
                        _unpack(wos_ref[g0:g1, i].reshape(-1, HALF)), preferred_element_type=F32)
            out[i] = r + out[i] if i in out else r

    lag_s, lag_v = LAG_S, LAG_S + LAG_PV
    todo = list(zip(O_SPLITS[layer][:-1], O_SPLITS[layer][1:]))
    for t in range(n_pairs + lag_v):
        if t >= n_pairs:
            project_out(*todo.pop(0))
        for c in ISSUE[layer]:
            if c == "S" and 0 <= t - lag_s < n_pairs:
                scores(t - lag_s)
            elif c == "V" and 0 <= t - lag_v < n_pairs:
                values(t - lag_v)
            elif c in "qkv" and t < n_pairs:
                j = "qkv".index(c)
                (q, k, v)[j][t] = (project_short(t, j) if j and pre_ref is not None
                                   else project_shared(t, j))
                if c == "v" and t % 2:
                    undo = jnp.where(first[:8], undo_v_ref[t // 2, 0], undo_v_ref[t // 2, 1])
                    v[t] = v[t] * _cols(*[_tile_rows(undo, rows)] * 3)
        if t < n_pairs:
            attend_near(t)
    for part in todo:
        project_out(*part)
    rest = jnp.dot(o_ref[...], _unpack(wop_ref[...].reshape(-1, wop_ref.shape[-1])),
                   preferred_element_type=F32)

    most, tail = slice(0, 2 * HALF), slice(2 * HALF, None)
    x_ref[s, :, tail] = x_in[s, :, tail].astype(F32) + rest[n_mem:]
    if odd:
        c12, c11, c21, c22 = shared["out"]
        m1, c11, c21 = _second_left(out, n_mem, c11, c21)
        m2, c22 = _second_right(out, n_mem, c22)
        x_ref[s - 1, :, most] = x_in[s - 1, :, most].astype(F32) + _cols(c11, c12)
        back = jnp.maximum(s - 2, 1)
        x_ref[back, :, most] = (x_in[back, :, most].astype(F32)
                                + jnp.where(s > 1, _cols(c21, c22), 0.0))
    else:
        (m1, m2), shared["out"] = _first_results(out, n_mem)
    return _cols(m1, m2, rest[:n_mem]), xn_next


def _pair_reduce(t, op):
    r = t[0:8]
    for i in range(8, t.shape[0], 8):
        r = op(r, t[i:i + 8])
    r = op(r, pltpu.roll(r, 4, 0))
    return op(r, pltpu.roll(r, 2, 0))


def _tile_rows(r, n):
    return jnp.concatenate([r] * (n // 8), axis=0)


def _feature_map(p):
    n = p.shape[0]
    e_pos = jnp.exp2(p - _tile_rows(_pair_reduce(p, jnp.maximum), n))
    e_neg = jnp.exp2(_tile_rows(_pair_reduce(p, jnp.minimum), n) - p)
    inv_pos = _recip(_pair_reduce(e_pos, jnp.add))
    inv_neg = _recip(_pair_reduce(e_neg, jnp.add))
    return jnp.concatenate(
        [e_pos * _tile_rows(inv_pos, n), e_neg * _tile_rows(inv_neg, n)], axis=0)


def _fold_span(b, blk):
    return b * blk // 128 * 128, -(-(b + 1) * blk // 128) * 128


def _expand_phi(wphi_ref, phi_ref):
    dh, _, heads = wphi_ref.shape
    d = dh * heads
    gr = 2 * dh
    c = _iota((dh, d), 1)
    c_feat = c - _div(c, dh) * dh
    spread = (_div(_iota((heads, d), 1), dh) == _iota((heads, d), 0)).astype(BF16)

    def gather(j, by_feat):
        for e in (j * (dh // 4) + i for i in range(dh // 4)):
            t = jnp.dot(wphi_ref[e], spread, preferred_element_type=F32)
            by_feat = jnp.where(c_feat == e, t, by_feat)
        return by_feat

    by_feat = lax.fori_loop(0, 4, gather, jnp.zeros((dh, d), F32)).astype(BF16)
    blk = F_PAIRS * gr
    r = _iota((blk, dh), 0)
    sel = (((r - _div(r, gr) * gr) >> 1) == _iota((blk, dh), 1)).astype(BF16)
    for b in range(d // blk):
        lo, hi = _fold_span(b, blk)
        r = _iota((blk, hi - lo), 0)
        head = 2 * (_div(r, gr) + b * F_PAIRS) + (r & 1)
        phi = jnp.dot(sel, by_feat[:, lo:hi], preferred_element_type=F32)
        phi_ref[b, :, 0:hi - lo] = _pack(
            jnp.where(_div(_iota((1, hi - lo), 1) + lo, dh) == head, phi, 0.0))


def _b_weights(wqkv_ref, phi_ref, wob_ref, bq_ref, bkv_ref, bo_ref):
    d = wqkv_ref.shape[0]
    blk = 2 * phi_ref.shape[1]
    half = bkv_ref.shape[1]
    bo_ref[...] = _pack(wob_ref[...])
    wv = wqkv_ref[:, 2 * d:3 * d].T
    for b in range(d // half):
        bkv_ref[b, half // 2:half, :] = _pack(wv[b * half:(b + 1) * half])
    for b in range(d // blk):
        lo, hi = _fold_span(b, blk)
        phi = _unpack(phi_ref[b, :, 0:hi - lo])
        wq = lax.dot_general(phi, wqkv_ref[:, lo:hi], NT, preferred_element_type=F32)
        wk = lax.dot_general(phi, wqkv_ref[:, d + lo:d + hi], NT, preferred_element_type=F32)
        bq_ref[b * blk // 2:(b + 1) * blk // 2, :] = _pack(wq * LOG2E)
        at = b * blk % half // 2
        bkv_ref[b * blk // half, at:at + blk // 2, :] = _pack(wk * LOG2E)


def _chunk_rows(ref, it, r0, n):
    seg = ref.shape[1]
    return pl.ds(it * (TB // seg) + r0 // seg, n // seg)


def _b_keys(it, carry, *, x_ref, xb_ref, bkv_ref, kv_ref, z_ref):
    n_blk, half, _ = bkv_ref.shape
    gr = half // K_PAIRS
    xb = xb_ref[_chunk_rows(xb_ref, it, 0, TB)].reshape(TB, -1)
    last = x_ref.shape[0] - 1 - jnp.minimum(it, 2)
    xb_ref[last] = _layernorm(x_ref[last]).astype(BF16)
    same_head = (_iota((gr, 2 * gr), 0) >= gr // 2) == ((_iota((gr, 2 * gr), 1) & 1) == 1)

    def accumulate(b, t):
        for i in range(K_PAIRS):
            g = b * K_PAIRS + i
            phi = _feature_map(t[i * gr:(i + 1) * gr])
            z_ref[g] = jnp.where(it > 0, z_ref[g], 0.0) + jnp.sum(phi, axis=1, keepdims=True)
            kv = lax.dot_general(t[half + i * gr:half + (i + 1) * gr], phi.astype(BF16), NT,
                                 preferred_element_type=F32)
            kv_ref[g] = jnp.where(it > 0, kv_ref[g], 0.0) + jnp.where(same_head, kv, 0.0)

    pending = None
    for b in range(n_blk):
        t = lax.dot_general(_unpack(bkv_ref[b]), xb, NT, preferred_element_type=F32)
        if pending is not None:
            accumulate(*pending)
        pending = (b, t)
    accumulate(*pending)
    return carry


def _b_queries(it, send, *, x_ref, xb_ref, y_ref, bq_ref, bo_ref, kv_ref, z_ref, ot_ref, on_ref):
    n_groups, gr, _ = kv_ref.shape
    blk = Q_PAIRS * gr
    sub = _iota((8, TB), 0)
    xb = xb_ref[_chunk_rows(xb_ref, it, 0, TB)].reshape(TB, -1)

    def attend(b, t):
        outs = []
        for i in range(Q_PAIRS):
            g = b * Q_PAIRS + i
            phi = _feature_map(t[i * gr:(i + 1) * gr])
            num = jnp.dot(kv_ref[g], phi.astype(BF16), preferred_element_type=F32)
            z = jnp.concatenate([z_ref[g]] * (TB // 128), axis=1)
            inv = _recip(_pair_reduce(phi * z, jnp.add) + 1e-6)
            other = pltpu.roll(inv, 1, 0)
            inv_a = jnp.where((sub & 1) == 0, inv, other)
            inv_b = jnp.where((sub & 1) == 0, other, inv)
            n = (gr - 8) // 16
            inv = jnp.concatenate(
                [inv_a] * n + [jnp.where(sub < 4, inv_a, inv_b)] + [inv_b] * n, axis=0)
            outs.append(num * inv)
        ot_ref[b * blk // 2:(b + 1) * blk // 2, :] = _pack(jnp.concatenate(outs, axis=0))

    n_blk = n_groups // Q_PAIRS
    proj = {}
    for b in range(n_blk + 1):
        if b < n_blk:
            proj[b] = lax.dot_general(_unpack(bq_ref[b * blk // 2:(b + 1) * blk // 2, :]), xb,
                                      NT, preferred_element_type=F32)
        if b > 0:
            attend(b - 1, proj[b - 1])
    on_ref[...] = _pack(_unpack(ot_ref[...]).T)
    r0 = 0
    for i, n in enumerate(O_ROWS):
        at = _chunk_rows(x_ref, it, r0, n)
        y = jnp.dot(_unpack(on_ref[r0 // 2:(r0 + n) // 2, :]), _unpack(bo_ref[...]),
                    preferred_element_type=F32)
        x = x_ref[at] + y.reshape((-1,) + x_ref.shape[1:])
        x_ref[at] = x
        y_ref[at] = x.astype(BF16)
        send(i)
        r0 += n


def _kernel(x_hbm, mem0_hbm, wq_hbm, wk_hbm, wv_hbm, wo_hbm, wqkvb_hbm, wphi_hbm, wob_hbm,
            out_hbm,
            x_ref, xb_ref, y_ref, xp_ref, stage_ref, pre_ref, ahead_ref,
            ws_ref, wp_ref, wos_ref, wop_ref, scale_ref, undo_ref, undo_v_ref,
            o_even_ref, o_odd_ref, near_ref,
            mem0_ref, wphi_ref, phi_ref, wqkvb_ref, wob_ref, bo_ref, bq_ref, bkv_ref,
            kv_ref, z_ref, ot_ref, on_ref,
            w_sem, in_sem, out_sem, *, dh):
    n_seg, seg, d = x_ref.shape
    n_pairs = wp_ref.shape[0]
    n_mem = mem0_ref.shape[0]
    pw = 2 * dh
    n_iter = n_seg * seg // TB

    def head_copy(p, j, i):
        return pltpu.make_async_copy(
            (wv_hbm, wo_hbm)[j - 2].at[p, i], stage_ref.at[p % RING, 3 * j:3 * j + 3, i],
            w_sem.at[p, 2 * j - 2 + i])

    def w_copies(p, j):
        if j >= 2:
            return [head_copy(p, j, i) for i in range(2)]
        return [pltpu.make_async_copy(
            (wq_hbm, wk_hbm)[j].at[p], stage_ref.at[p % RING, 3 * j:3 * j + 3], w_sem.at[p, j])]

    def start_w(p, *slots):
        for j in slots:
            for copy in w_copies(p, j):
                copy.start()

    def wait_w(p, *slots):
        for j in slots:
            for copy in w_copies(p, j):
                copy.wait()

    def prepare_in(u, tiles, live=True, pace=None):
        g, i = u // 2, u % 2
        slots = [p % RING for p in (2 * g, jnp.where(live, 2 * g + 1, 0))]
        for j in range(3) if pace else ():
            factors = [_balance(*(stage_ref[p, 3 * j + 2 * n, n, :16, :2 * HALF] for p in slots))
                       for n in range(2)]
            for t in range(3):
                heads = [factors[n if j == 2 else (2 * t + n) // 3] for n in range(2)]
                undo_ref[g, :, pl.ds(128 * (3 * j + t), 128)] = jnp.where(
                    _iota((8, 128), 1) < 64, *(f[1] for f in heads))
                scale_ref[3 * j + t] = _rows(*(f[0] for f in heads))
        pace = pace or (lambda t, b: b)
        for t in tiles:
            cols = pl.ds(pl.multiple_of(128 * t, 128), 128)
            scale = _rows(*(_tile_rows(scale_ref[t, 8 * n:8 * n + 8, :], 64) for n in range(2)))
            b11, b12, b21, b22 = (
                pace(t, stage_ref[p, t, :, :, pl.ds(pl.multiple_of(c + i * 128, 128), 128)]
                     .reshape(128, 128)) for c in (0, HALF) for p in slots)
            for n, r in enumerate(_strassen_weights(b11, b12 * scale, b21, b22 * scale)):
                ws_ref[g, n, pl.ds(pl.multiple_of(i * 64, 64), 64), cols] = _pack(r.T)
            wp_ref[u, :, cols] = _pack(stage_ref[u % RING, t, :, :, 2 * HALF:].reshape(128, -1).T)

    def wait_out(u):
        for p in (u // 2 * 2, u // 2 * 2 + 1):
            head_copy(p, 3, u % 2).wait()

    def prepare_out(u, live=True, pace=lambda t, b: b):
        g, i = u // 2, u % 2
        slots = [p % RING for p in (2 * g, jnp.where(live, 2 * g + 1, 0))]
        base = jnp.where(live, 9, 3)
        scale, undo_v_ref[g, i] = _balance(*(stage_ref[p, base, i, :16] for p in slots))
        for t in range(3):
            parts = [pace(10 + 2 * t, stage_ref[p, base + t, i]) for p in slots]
            parts[1] = parts[1] * _cols(*[_tile_rows(scale, 64)] * (d // 128))
            blocks = [part[:, c:c + HALF] for part in parts for c in (0, HALF)]
            for n, r in enumerate(_strassen_weights(*blocks)):
                wos_ref[g, n, t, i] = _pack(r)
            for n, part in enumerate(parts):
                wop_ref[2 * g + n, t, i] = _pack(part[:, 2 * HALF:])

    def out_copy(it, i):
        part = _chunk_rows(y_ref, it, sum(O_ROWS[:i]), O_ROWS[i])
        return pltpu.make_async_copy(y_ref.at[part], out_hbm.at[part], out_sem.at[0])

    def x_copy(rows, sem):
        return pltpu.make_async_copy(x_hbm.at[:, rows, :], y_ref.at[:, rows, :], sem)

    head, tail = slice(0, seg - PRE), slice(seg - PRE, seg)
    xt_copy, xh_copy = x_copy(tail, in_sem.at[0]), x_copy(head, in_sem.at[3])
    wqkvb_copy = pltpu.make_async_copy(wqkvb_hbm, wqkvb_ref, in_sem.at[1])
    wphi_copy = pltpu.make_async_copy(wphi_hbm, wphi_ref, in_sem.at[5])
    mem0_copy = pltpu.make_async_copy(mem0_hbm, mem0_ref, in_sem.at[4])
    wob_copy = pltpu.make_async_copy(wob_hbm, wob_ref, in_sem.at[2])

    wphi_copy.start()
    xt_copy.start()
    start_w(0, 0, 1, 2)
    wphi_copy.wait()
    _expand_phi(wphi_ref, phi_ref)
    xt_copy.wait()

    xp_ref[...] = _layernorm(y_ref[:, tail, :].astype(F32).reshape(n_seg * PRE, d)).astype(BF16)

    mem0_copy.start()
    start_w(1, 0, 1, 2)

    def pre_project(p, carry):
        @pl.when(p + 2 < n_pairs)
        def _():
            start_w(jnp.minimum(p + 2, n_pairs - 1), 0, 1, 2)

        @pl.when(p + 2 == n_pairs)
        def _():
            xh_copy.start()

        start_w(p, 3)

        @pl.when(p >= WO_LAG)
        def _():
            wait_out(jnp.maximum(p - WO_LAG, 0))

        wait_w(p, 0, 1, 2)
        kv = lax.dot_general(xp_ref[...], stage_ref[p % RING, 3:9].reshape(-1, d), NT,
                             preferred_element_type=F32)
        pre_ref[p] = kv

        def pace(t, block):
            c, r = divmod(t * 128, xp_ref.shape[0])
            early = kv[r:r + block.shape[0], 128 * c:128 * (c + 1)].astype(BF16)
            return jnp.where(p < 0, _cols(*[early] * (block.shape[1] // 128)), block)

        prepare_out(jnp.maximum(p - WO_LAG, 0), p >= WO_LAG, pace)
        prepare_in(jnp.maximum(p - 1, 0), range(9), p >= 1, pace)
        return carry

    lax.fori_loop(0, n_pairs, pre_project, 0)

    @pl.loop(0, 3)
    def _(j):
        prepare_in(n_pairs - 1, [3 * j + i for i in range(3)])

    @pl.loop(n_pairs - WO_LAG, n_pairs)
    def _(u):
        wait_out(u)
        prepare_out(u)

    xh_copy.wait()

    wqkvb_copy.start()
    wob_copy.start()
    mem0_copy.wait()
    x_ref[0] = y_ref[0].astype(F32)

    def layer_a(layer, x_in, pre):
        step = functools.partial(
            _a_step, layer=layer, dh=dh, x_in=x_in, x_ref=x_ref, xb_ref=xb_ref, ws_ref=ws_ref,
            wp_ref=wp_ref, wos_ref=wos_ref, wop_ref=wop_ref, pre_ref=pre, ahead_ref=ahead_ref,
            undo_ref=undo_ref, undo_v_ref=undo_v_ref, o_refs=(o_even_ref, o_odd_ref),
            near_ref=near_ref)
        xn = [_layernorm(x_in[i].astype(F32)) for i in range(3)]
        o_odd_ref[...] = jnp.zeros(o_odd_ref.shape, F32)
        cols, per = (slice(0, 3 * pw), 1) if pre is None else (slice(0, pw), 2)

        @pl.loop(0, n_pairs // 2 // per)
        def _(j):
            for g in (j * per + i for i in range(per)):
                for i, product in enumerate((_left_product, _right_product)):
                    ahead_ref[2 * g + i, :, cols] = product(
                        xn[0][:, :HALF], xn[0][:, HALF:2 * HALF],
                        lambda a, n: jnp.dot(a.astype(BF16), _unpack(ws_ref[g, n, :, cols]),
                                             preferred_element_type=F32))

        def two_steps(it, carry):
            mem, *xn = carry
            shared = {}
            for i in range(2):
                mem, xn_next = step(2 * it + i, mem, xn, shared)
                xn = xn[1:] + [xn_next]
            return (mem, *xn)

        lax.fori_loop(0, n_seg // 2, two_steps, (mem0_ref[...].astype(F32), *xn))

    def finish_a(layer):
        a = [_cols(*(o_odd_ref[n_mem:, (2 * g + i) * pw:(2 * g + i + 1) * pw]
                     for g in range(n_pairs // 2))) for i in range(2)]
        y = _cols(*(product(*a, lambda t, n: jnp.dot(
            t.astype(BF16), _unpack(wos_ref[:, n].reshape(-1, HALF)), preferred_element_type=F32))
            for product in (_left_product, _right_product)))
        at = (n_seg - 1, slice(None), slice(0, 2 * HALF))
        x_ref[at] = jnp.where(layer == 0, y_ref[at].astype(F32), x_ref[at]) + y

    b_keys = functools.partial(_b_keys, x_ref=x_ref, xb_ref=xb_ref, bkv_ref=bkv_ref,
                               kv_ref=kv_ref, z_ref=z_ref)
    b_queries = functools.partial(_b_queries, x_ref=x_ref, xb_ref=xb_ref, y_ref=y_ref,
                                  bq_ref=bq_ref, bo_ref=bo_ref, kv_ref=kv_ref, z_ref=z_ref,
                                  ot_ref=ot_ref, on_ref=on_ref)

    def layer_pair(layer, carry):
        @pl.when(layer == 0)
        def _():
            layer_a(0, y_ref, pre_ref)

        @pl.when(layer == 0)
        def _():
            wqkvb_copy.wait()
            wob_copy.wait()
            _b_weights(wqkvb_ref, phi_ref, wob_ref, bq_ref, bkv_ref, bo_ref)

        @pl.when(layer == 1)
        def _():
            layer_a(1, x_ref, None)

        finish_a(layer)

        lax.fori_loop(0, n_iter, b_keys, 0)

        def queries(it, carry):
            def send(i):
                @pl.when(layer == 1)
                def _():
                    out_copy(it, i).start()

            b_queries(it, send)
            return carry

        lax.fori_loop(0, n_iter, queries, 0)

        return carry

    lax.fori_loop(0, 2, layer_pair, 0)
    pltpu.make_async_copy(y_ref, out_hbm, out_sem.at[0]).wait()


@functools.partial(jax.jit, static_argnames=("A_seg_len",))
def pallas_interleave_layers__memory_aug_recurrent_mem_tr__linear_kernel_hedgehog__prompt_kernel(
    A_x, A_mem0, A_Wq, A_Wk, A_Wv, A_Wo, A_seg_len, B_x, B_wqkv, B_w_phi, B_wo,
):
    del B_x
    batch, s_len, d = A_x.shape
    _, heads, dh = A_Wq.shape
    n_mem = A_mem0.shape[1]
    seg = int(A_seg_len)
    b_heads, b_dh, _ = B_w_phi.shape
    rows = n_mem + seg
    n_pairs = heads // 2
    gr = 2 * b_dh
    half = K_PAIRS * gr
    n_seg = s_len // seg
    assert batch == 1 and dh == 192 and heads == 4 * O_SPLITS[0][-1] and d == 2 * HALF + 128
    assert n_mem % 8 == 0 and seg % 16 == 0 and 128 % seg == 0 and 2 * rows <= 128
    assert s_len % TB == 0 and s_len > 3 * TB == 3 * sum(O_ROWS) and n_seg % n_pairs == 0
    assert b_heads * b_dh == d and b_dh % 8 == 4 and d % half == 0

    def head_major(w):
        return w.transpose(1, 2, 0)

    hbm = pl.BlockSpec(memory_space=pltpu.HBM)
    out = pl.pallas_call(
        functools.partial(_kernel, dh=dh),
        out_shape=jax.ShapeDtypeStruct((n_seg, seg, d), A_x.dtype),
        in_specs=[hbm] * 9,
        out_specs=hbm,
        scratch_shapes=[
            pltpu.VMEM((n_seg, seg, d), F32),
            pltpu.VMEM((n_seg, seg, d), BF16),
            pltpu.VMEM((n_seg, seg, d), BF16),
            pltpu.VMEM((n_seg * PRE, d), BF16),
            pltpu.VMEM((RING, 12, 2, 64, d), BF16),
            pltpu.VMEM((n_pairs, n_seg * PRE, 4 * dh), F32),
            pltpu.VMEM((n_pairs, seg, 6 * dh), F32),
            pltpu.VMEM((n_pairs // 2, 7, HALF // 2, 6 * dh), jnp.uint32),
            pltpu.VMEM((n_pairs, d // 2 - HALF, 6 * dh), jnp.uint32),
            pltpu.VMEM((n_pairs // 2, 7, 3, 2, 32, HALF), jnp.uint32),
            pltpu.VMEM((n_pairs, 3, 2, 32, d - 2 * HALF), jnp.uint32),
            pltpu.VMEM((9, 16, 128), F32),
            pltpu.VMEM((n_pairs // 2, 8, 6 * dh), F32),
            pltpu.VMEM((n_pairs // 2, 2, 8, 128), F32),
            pltpu.VMEM((rows, heads * dh), F32),
            pltpu.VMEM((rows, heads * dh), F32),
            pltpu.VMEM((n_pairs, n_mem + 8, 4 * dh), F32),
            pltpu.VMEM((n_mem, d), BF16),
            pltpu.VMEM((b_dh, b_dh, b_heads), BF16),
            pltpu.VMEM((d // (F_PAIRS * gr), F_PAIRS * gr // 2, 256), jnp.uint32),
            pltpu.VMEM(B_wqkv.shape, BF16),
            pltpu.VMEM(B_wo.shape, BF16),
            pltpu.VMEM((d // 2, d), jnp.uint32),
            pltpu.VMEM((d // 2, d), jnp.uint32),
            pltpu.VMEM((d // half, half, d), jnp.uint32),
            pltpu.VMEM((b_heads // 2, gr, 2 * gr), F32),
            pltpu.VMEM((b_heads // 2, 2 * gr, 128), F32),
            pltpu.VMEM((d // 2, TB), jnp.uint32),
            pltpu.VMEM((TB // 2, d), jnp.uint32),
            pltpu.SemaphoreType.DMA((n_pairs, 6)),
            pltpu.SemaphoreType.DMA((6,)),
            pltpu.SemaphoreType.DMA((1,)),
        ],
        compiler_params=pltpu.CompilerParams(vmem_limit_bytes=124 * 1024 * 1024),
    )(
        A_x.reshape(n_seg, seg, d), A_mem0.reshape(n_mem, d),
        head_major(A_Wq).reshape(n_pairs, 3, 2, 64, d),
        head_major(A_Wk).reshape(n_pairs, 3, 2, 64, d),
        head_major(A_Wv).reshape(n_pairs, 2, 3, 64, d), A_Wo.reshape(n_pairs, 2, 3, 64, d),
        B_wqkv, B_w_phi.transpose(1, 2, 0), B_wo,
    )
    return out.reshape(batch, s_len, d)
```
